```python
import jax
import jax.numpy as jnp

def _softmax(x, axis=-1):
    return jax.nn.softmax(x, axis=axis)
def _gelu(x):
    return jax.nn.gelu(x, approximate=True)
def _silu(x):
    return jax.nn.silu(x)
def _sigmoid(x):
    return jax.nn.sigmoid(x)
def _layernorm(x, axis=-1, eps=1e-5):
    m = jnp.mean(x, axis=axis, keepdims=True)
    v = jnp.var(x, axis=axis, keepdims=True)
    return (x - m) / jnp.sqrt(v + eps)
def _scatter_add(tgt, idx, src, axis=0):
    return tgt.at[idx].add(src)
def _segment_sum(src, seg, n):
    return jax.ops.segment_sum(src, seg, n)
class _Rng:
    def __init__(self, key):
        self._k = key
    def _next(self):
        self._k, sub = jax.random.split(self._k)
        return sub
    def normal(self, shape):
        return jax.random.normal(self._next(), shape, dtype=jnp.bfloat16)
    def randint(self, lo, hi, shape):
        return jax.random.randint(self._next(), shape, lo, hi, dtype=jnp.int32)
    def uniform(self, shape, lo=0.0, hi=1.0):
        return jax.random.uniform(self._next(), shape, jnp.bfloat16, lo, hi)
    def permutation(self, n):
        return jax.random.permutation(self._next(), n)


kernel_name = 'sequential_preLN__linear_attn_block__moe_arch_mod__prompt'

def setup_inputs():
    _rng = _Rng(jax.random.key(int.from_bytes(__import__("os").urandom(4), "little")))
    _w = (lambda a: (lambda t: t.astype(jnp.bfloat16) if jnp.issubdtype(t.dtype, jnp.floating) else t)(jnp.asarray(a)))
    def _A_setup():
        B, S, D = 1, 2048, 1024
        return {
            "x": _w((lambda *s: _rng.normal(s) * 0.05)(B, S, D)),
            "wqkv": _w((lambda *s: _rng.normal(s) * 0.05)(D, 3 * D)),
            "wo": _w((lambda *s: _rng.normal(s) * 0.05)(D, D)),
        }
    _A_in = _A_setup()

    def _B_setup():
        B, S, D, F, C = 1, 2048, 1024, 3584, 2
        return {
            "x": _w((lambda *s: _rng.normal(s) * 0.05)(B, S, D)),
            "w_r": _w((lambda *s: _rng.normal(s) * 0.05)(D)),
            "w_gate": _w((lambda *s: _rng.normal(s) * 0.05)(D, F)),
            "w_up": _w((lambda *s: _rng.normal(s) * 0.05)(D, F)),
            "w_down": _w((lambda *s: _rng.normal(s) * 0.05)(F, D)),
        }
    _B_in = _B_setup()

    return {
        "A_x": _A_in["x"],
        "A_wqkv": _A_in["wqkv"],
        "A_wo": _A_in["wo"],
        "B_x": _B_in["x"],
        "B_w_r": _B_in["w_r"],
        "B_w_gate": _B_in["w_gate"],
        "B_w_up": _B_in["w_up"],
        "B_w_down": _B_in["w_down"],
    }

def reference(A_x, A_wqkv, A_wo, B_x, B_w_r, B_w_gate, B_w_up, B_w_down):
    def _A_ref(x, wqkv, wo):
        B, S, D = x.shape
        H = 32; Dh = D // H
        qkv = (lambda x, *d: x.transpose(*d))((x @ wqkv).reshape(B, S, 3, H, Dh), 2, 0, 3, 1, 4)
        q, k, v = qkv[0], qkv[1], qkv[2]
        phi = lambda t: jnp.where(t > 0, t + 1, jnp.exp(t)) + 1e-6
        pq, pk = phi(q), phi(k)
        kv = jnp.einsum("bhsd,bhse->bhde", pk, v)
        z = jnp.einsum("bhsd->bhd", pk)
        num = jnp.einsum("bhqd,bhde->bhqe", pq, kv)
        den = jnp.einsum("bhqd,bhd->bhq", pq, z)[..., None] + 1e-6
        o = num / den
        return (lambda x, *d: x.transpose(*d))(o, 0, 2, 1, 3).reshape(B, S, D) @ wo

    def _B_ref(x, w_r, w_gate, w_up, w_down):
        B, S, D = x.shape
        C = 2
        r = x @ w_r
        idx = jnp.argsort(-r, axis=-1)[:, :C]
        idx_e = jnp.repeat(idx.reshape(B, C, 1), D, axis=2)
        x_sel = jnp.take_along_axis(x, idx_e, axis=1)
        g = _silu(x_sel @ w_gate)
        u = x_sel @ w_up
        y = (g * u) @ w_down
        r_sel = _sigmoid(jnp.take_along_axis(r, idx, axis=1))
        y = y * r_sel.reshape(B, C, 1)
        b_off = (jnp.arange(B) * S).reshape(B, 1)
        flat_idx = (idx + b_off).reshape(B * C)
        zero = (x * 0.0).reshape(B * S, D)
        upd = _scatter_add(zero, flat_idx, y.reshape(B * C, D), axis=0)
        return x + upd.reshape(B, S, D)

    x = A_x
    h = x + _A_ref(_layernorm(x, axis=-1), A_wqkv, A_wo)
    h2 = h + _B_ref(_layernorm(h, axis=-1), B_w_r, B_w_gate, B_w_up, B_w_down)
    return h2
```

```python
import functools
import jax
import jax.numpy as jnp
from jax import lax
import jax.experimental.pallas as pl
import jax.experimental.pallas.tpu as pltpu

S, D, F, H, DH = 2048, 1024, 3584, 32, 32
G = D // 128
F32 = jnp.float32
BF16 = jnp.bfloat16


def _rb(x):
    return x.astype(BF16).astype(F32)


def _ln_stats(xf):
    mu = jnp.sum(xf, axis=-1, keepdims=True) * (1.0 / D)
    xc = xf - mu
    var = jnp.sum(xc * xc, axis=-1, keepdims=True) * (1.0 / D)
    sd = _rb(jnp.sqrt(_rb(_rb(var) + 1e-5)))
    return _rb(mu), 1.0 / sd


def _phi(t):
    return jnp.where(t > 0, t + 1.0, jnp.exp(t)) + 1e-6


def make_kernel(T1=256, T2=256, NW=6):
    WC = 3 * D // NW

    def kernel(x_hbm, wqkv_hbm, wo_hbm, wr_ref, wg_hbm, wu_hbm, wd_hbm, out_hbm,
               x_v, wqkv_v, wo_v, wg_v, wu_v, wd_v, pq_v, kv_v, z_v, m_v, zb_v,
               out_v, hn_v, r_v, sem_x, sem_w, sem_o, sem_m):
        n1 = S // T1
        n2 = S // T2

        def x_copy(i):
            return pltpu.make_async_copy(x_hbm.at[pl.ds(i * T1, T1)], x_v.at[pl.ds(i * T1, T1)], sem_x.at[i])

        def w_copy(j):
            return pltpu.make_async_copy(wqkv_hbm.at[:, pl.ds(j * WC, WC)], wqkv_v.at[:, pl.ds(j * WC, WC)], sem_w.at[j])

        wo_copy = pltpu.make_async_copy(wo_hbm, wo_v, sem_m.at[0])
        wg_copy = pltpu.make_async_copy(wg_hbm, wg_v, sem_m.at[1])
        wu_copy = pltpu.make_async_copy(wu_hbm, wu_v, sem_m.at[2])
        wd_copy = pltpu.make_async_copy(wd_hbm, wd_v, sem_m.at[3])

        def out_copy(i):
            return pltpu.make_async_copy(out_v.at[pl.ds(i * T2, T2)], out_hbm.at[pl.ds(i * T2, T2)], sem_o.at[i])

        order = list(range(NW // 3, NW)) + list(range(NW // 3))
        x_copy(0).start()
        for j in order:
            w_copy(j).start()
        for i in range(1, n1):
            x_copy(i).start()
        wo_copy.start()

        kv_v[...] = jnp.zeros_like(kv_v)
        z_v[...] = jnp.zeros_like(z_v)

        def p1_tile(i, first):
            r0 = pl.multiple_of(i * T1, T1)
            x_copy(i).wait()
            xf = x_v[pl.ds(r0, T1), :].astype(F32)
            mu, rs = _ln_stats(xf)
            xn = ((xf - mu) * rs).astype(BF16)

            def proj(c0):
                outs = []
                for j in range(c0 // WC, (c0 + D) // WC):
                    if first:
                        w_copy(j).wait()
                    outs.append(jnp.dot(xn, wqkv_v[:, j * WC:(j + 1) * WC], preferred_element_type=F32))
                return jnp.concatenate(outs, axis=1) if len(outs) > 1 else outs[0]

            pk = _phi(proj(D)).astype(BF16)
            v = proj(2 * D).astype(BF16)
            for g in range(G):
                kv_v[g] += lax.dot_general(pk[:, g * 128:(g + 1) * 128], v[:, g * 128:(g + 1) * 128],
                                           (((0,), (0,)), ((), ())), preferred_element_type=F32)
            z_v[...] += jnp.sum(pk.astype(F32).reshape(T1 // 8, 8, D), axis=0)
            pq_v[pl.ds(r0, T1), :] = _phi(proj(0)).astype(BF16)

        p1_tile(0, True)
        wg_copy.start()
        wu_copy.start()
        wd_copy.start()

        def p1_body(i, c):
            p1_tile(i, False)
            return c
        lax.fori_loop(1, n1, p1_body, 0)

        wo_copy.wait()
        row = lax.broadcasted_iota(jnp.int32, (128, 128), 0) // DH
        col = lax.broadcasted_iota(jnp.int32, (128, 128), 1) // DH
        same = row == col
        z = _rb(jnp.sum(z_v[...], axis=0, keepdims=True))
        for g in range(G):
            kvg = jnp.where(same, kv_v[g], 0.0).astype(BF16)
            m_v[g * 128:(g + 1) * 128, :] = jnp.dot(kvg, wo_v[g * 128:(g + 1) * 128, :], preferred_element_type=F32).astype(BF16)
            zcol = jnp.broadcast_to(z[:, g * 128:(g + 1) * 128], (128, 128)).T
            zb_v[g] = jnp.where(same, zcol, 0.0).astype(BF16)

        wr = wr_ref[...].astype(F32)

        def p2_body(i, c):
            r0 = pl.multiple_of(i * T2, T2)
            pq = pq_v[pl.ds(r0, T2), :]
            os = []
            for g in range(G):
                pqg = pq[:, g * 128:(g + 1) * 128]
                den = jnp.dot(pqg, zb_v[g], preferred_element_type=F32) + 1e-6
                os.append((pqg.astype(F32) / den).astype(BF16))
            o = jnp.concatenate(os, axis=1)
            attn = jnp.dot(o, m_v[...], preferred_element_type=F32)
            h = _rb(x_v[pl.ds(r0, T2), :].astype(F32) + _rb(attn))
            mu, rs = _ln_stats(h)
            hnb = ((h - mu) * rs).astype(BF16)
            hn = hnb.astype(F32)
            hn_v[pl.ds(r0, T2), :] = hnb
            out_v[pl.ds(r0, T2), :] = (h + hn).astype(BF16)
            r_v[pl.ds(r0, T2), :] = _rb(jnp.sum(hn * wr, axis=-1, keepdims=True))
            out_copy(i).start()
            return c
        lax.fori_loop(0, n2, p2_body, 0)

        r = r_v[...]
        idx = lax.broadcasted_iota(jnp.int32, (S, 1), 0)
        m1 = jnp.max(r)
        i1 = jnp.min(jnp.where(r == m1, idx, S))
        r2 = jnp.where(idx == i1, -jnp.inf, r)
        m2 = jnp.max(r2)
        i2 = jnp.min(jnp.where(r2 == m2, idx, S))
        i1 = jnp.clip(i1, 0, S - 1)
        i2 = jnp.clip(i2, 0, S - 1)
        g1 = pl.multiple_of((i1 // 16) * 16, 16)
        g2 = pl.multiple_of((i2 // 16) * 16, 16)
        rows = lax.broadcasted_iota(jnp.int32, (16, D), 0)
        sel1 = rows == (i1 - g1)
        sel2 = rows == (i2 - g2)
        x1 = jnp.sum(jnp.where(sel1, hn_v[pl.ds(g1, 16), :].astype(F32), 0.0), axis=0, keepdims=True)
        x2 = jnp.sum(jnp.where(sel2, hn_v[pl.ds(g2, 16), :].astype(F32), 0.0), axis=0, keepdims=True)
        xs = jnp.where(rows == 0, x1, x2).astype(BF16)

        wg_copy.wait()
        wu_copy.wait()
        wd_copy.wait()
        gt = _rb(jnp.dot(xs, wg_v[...], preferred_element_type=F32))
        gt = _rb(gt * jax.nn.sigmoid(gt))
        ut = _rb(jnp.dot(xs, wu_v[...], preferred_element_type=F32))
        a = (gt * ut).astype(BF16)
        y = _rb(jnp.dot(a, wd_v[...], preferred_element_type=F32))
        rsel = jnp.where(rows[:, 0:1] == 0, m1, m2)
        y = _rb(y * _rb(jax.nn.sigmoid(rsel)))
        y1 = y[0:1, :]
        y2 = y[1:2, :]

        for i in range(n2):
            out_copy(i).wait()
        o1 = out_v[pl.ds(g1, 16), :].astype(F32)
        out_v[pl.ds(g1, 16), :] = jnp.where(sel1, o1 + y1, o1).astype(BF16)
        o2 = out_v[pl.ds(g2, 16), :].astype(F32)
        out_v[pl.ds(g2, 16), :] = jnp.where(sel2, o2 + y2, o2).astype(BF16)
        c1 = pltpu.make_async_copy(out_v.at[pl.ds(g1, 16)], out_hbm.at[pl.ds(g1, 16)], sem_o.at[0])
        c2 = pltpu.make_async_copy(out_v.at[pl.ds(g2, 16)], out_hbm.at[pl.ds(g2, 16)], sem_o.at[1])
        c1.start()

        @pl.when(g1 != g2)
        def _():
            c2.start()
            c2.wait()
        c1.wait()

    scratch = [
        pltpu.VMEM((S, D), BF16),
        pltpu.VMEM((D, 3 * D), BF16),
        pltpu.VMEM((D, D), BF16),
        pltpu.VMEM((D, F), BF16),
        pltpu.VMEM((D, F), BF16),
        pltpu.VMEM((F, D), BF16),
        pltpu.VMEM((S, D), BF16),
        pltpu.VMEM((G, 128, 128), F32),
        pltpu.VMEM((8, D), F32),
        pltpu.VMEM((D, D), BF16),
        pltpu.VMEM((G, 128, 128), BF16),
        pltpu.VMEM((S, D), BF16),
        pltpu.VMEM((S, D), BF16),
        pltpu.VMEM((S, 1), F32),
        pltpu.SemaphoreType.DMA((S // T1,)),
        pltpu.SemaphoreType.DMA((NW,)),
        pltpu.SemaphoreType.DMA((max(S // T2, 2),)),
        pltpu.SemaphoreType.DMA((4,)),
    ]

    @jax.jit
    def f(A_x, A_wqkv, A_wo, B_x, B_w_r, B_w_gate, B_w_up, B_w_down):
        any_spec = pl.BlockSpec(memory_space=pl.ANY)
        out = pl.pallas_call(
            kernel,
            out_shape=jax.ShapeDtypeStruct((S, D), BF16),
            in_specs=[any_spec, any_spec, any_spec, pl.BlockSpec(memory_space=pltpu.VMEM), any_spec, any_spec, any_spec],
            out_specs=any_spec,
            scratch_shapes=scratch,
            compiler_params=pltpu.CompilerParams(vmem_limit_bytes=100 * 1024 * 1024),
        )(A_x.reshape(S, D), A_wqkv, A_wo, B_w_r.reshape(1, D), B_w_gate, B_w_up, B_w_down)
        return out.reshape(1, S, D)
    return f


_impl = make_kernel()


@jax.jit
def pallas_sequential_preLN__linear_attn_block__moe_arch_mod__prompt_kernel(
    A_x: jax.Array,
    A_wqkv: jax.Array,
    A_wo: jax.Array,
    B_x: jax.Array,
    B_w_r: jax.Array,
    B_w_gate: jax.Array,
    B_w_up: jax.Array,
    B_w_down: jax.Array,
):
    return _impl(A_x, A_wqkv, A_wo, B_x, B_w_r, B_w_gate, B_w_up, B_w_down)
```

```python
import contextlib

import jax
import jax.numpy as jnp
from jax import lax
import jax.experimental.pallas as pl
import jax.experimental.pallas.tpu as pltpu

S, D, F, H, DH = 2048, 1024, 3584, 32, 32
G = D // 128
F32 = jnp.float32
BF16 = jnp.bfloat16
I32 = jnp.int32
U32 = jnp.uint32
PAD = 128


def _rb(x):
    return x.astype(BF16).astype(F32)


def _pace(dep, n, lo=0.0, hi=1.0):
    nrg, nch = dep.shape[0] // 8, dep.shape[1] // 128
    parts = []
    for p in range(n):
        pos = int((lo + (hi - lo) * p / n) * nch * nrg)
        c, rg = pos // nrg, pos % nrg
        parts.append(dep[rg * 8:(rg + 1) * 8, c * 128:(c + 1) * 128])
    bits = pltpu.bitcast(jnp.concatenate(parts, axis=0), U32)
    return lax.shift_right_logical(lax.shift_right_logical(bits, U32(31)), U32(1))


def _tie(x, zero):
    return pltpu.bitcast(pltpu.bitcast(x, U32) | zero, F32)


def _lanes(x, n):
    return jnp.concatenate([x] * n, axis=1) if n > 1 else x


def _ln_stats(xf, zero=None):
    t = xf.shape[0]
    mu = jnp.broadcast_to(jnp.sum(xf, axis=-1, keepdims=True) * (1.0 / D), (t, 128))
    if zero is not None:
        mu = _tie(mu, zero)
    xc = xf - _lanes(mu, G)
    var = jnp.broadcast_to(jnp.sum(xc * xc, axis=-1, keepdims=True) * (1.0 / D), (t, 128))
    sd = _rb(jnp.sqrt(_rb(_rb(var) + 1e-5)))
    return _rb(mu), 1.0 / sd


def _phi(t):
    return jnp.where(t > 0, t + 1.0, jnp.exp(t)) + 1e-6


def _recip(d):
    r = pl.reciprocal(d, approx=True)
    return r * (2.0 - d * r)


def _dot(a, b):
    return jnp.dot(a, b, preferred_element_type=F32)


def _dot_tn(a, b):
    return lax.dot_general(a, b, (((0,), (0,)), ((), ())), preferred_element_type=F32)


def _pk(x):
    return pltpu.bitcast(x, U32)


def _unpk(x):
    return pltpu.bitcast(x, BF16)


def make_kernel(P2T="256,256,256,256,256,256,256,128,128", FC=512, CHI=75, scopes=0):
    T1 = 512
    p2_tiles = [int(t) for t in P2T.split(",")]
    assert sum(p2_tiles) == S
    p2_off = [sum(p2_tiles[:i]) for i in range(len(p2_tiles))]
    n1 = S // T1
    n2 = len(p2_tiles)
    HT = T1 // 2
    KC, QC, VC = 0, D, 2 * D
    wch = [(D, KC, 256), (D + 256, KC + 256, 256), (D + 512, KC + 512, 512), (0, QC, D), (2 * D, VC, D)]
    SX0A, SX0B = 0, 1
    SW = 2
    SX = SW + len(wch)
    SWO = SX + n1 - 1
    SWG, SWU, SWD, SWR = SWO + 1, SWO + 2, SWO + 3, SWO + 4
    SO = SWR + 1
    NSEM = SO + n2

    def scope(name):
        return jax.named_scope(name) if scopes else contextlib.nullcontext()

    def kernel(x_hbm, wqkv_hbm, wo_hbm, wr_hbm, wg_hbm, wu_hbm, wd_hbm, out_hbm,
               x_v, wqkv_v, wo_v, wg_v, wu_v, wd_v, wr_v, xn_v, mu_v, rs_v, pqt_v, g_v, z_v, cs_v,
               m_v, out_v, hn_v, sems):

        def rows_copy(r0, n, s):
            return pltpu.make_async_copy(x_hbm.at[pl.ds(r0, n)], x_v.at[pl.ds(r0, n), pl.ds(0, D)], sems.at[s])

        x0a = rows_copy(0, HT, SX0A)
        x0b = rows_copy(HT, HT, SX0B)
        xcp = [rows_copy(i * T1, T1, SX + i - 1) for i in range(1, n1)]
        wcp = [pltpu.make_async_copy(wqkv_hbm.at[:, pl.ds(c0, n)], wqkv_v.at[:, pl.ds(d0, n)], sems.at[SW + j])
               for j, (c0, d0, n) in enumerate(wch)]
        wo_copy = pltpu.make_async_copy(wo_hbm, wo_v.at[:, pl.ds(0, D)], sems.at[SWO])
        wg_copy = pltpu.make_async_copy(wg_hbm, wg_v, sems.at[SWG])
        wu_copy = pltpu.make_async_copy(wu_hbm, wu_v, sems.at[SWU])
        wd_copy = pltpu.make_async_copy(wd_hbm, wd_v.at[:, pl.ds(0, D)], sems.at[SWD])
        wr_copy = pltpu.make_async_copy(wr_hbm, wr_v, sems.at[SWR])

        def out_copy(i):
            return pltpu.make_async_copy(out_v.at[pl.ds(p2_off[i], p2_tiles[i])],
                                         out_hbm.at[pl.ds(p2_off[i], p2_tiles[i])], sems.at[SO + i])

        for c in [x0a, wcp[0], x0b] + wcp[1:4] + xcp + [wcp[4], wr_copy, wo_copy, wg_copy, wu_copy, wd_copy]:
            c.start()

        def colsum(c0, n):
            w = wqkv_v[:, c0:c0 + n].astype(F32)
            cs_v[:, c0:c0 + n] = jnp.sum(w, axis=0, keepdims=True)

        def raw(xb, c0, n):
            return _dot(xb, wqkv_v[:, c0:c0 + n])

        def fix(acc, mu, rs, c0, n):
            k = n // 128
            return (acc - _lanes(mu, k) * cs_v[:, c0:c0 + n]) * _lanes(rs, k)

        def prep(r0, t, zero=None):
            xf = x_v[pl.ds(r0, t), 0:D].astype(F32)
            mu, rs = _ln_stats(xf, zero)
            mu_v[pl.ds(r0, t), :] = mu
            rs_v[pl.ds(r0, t), :] = rs
            xn = ((xf - _lanes(mu, G)) * _lanes(rs, G)).astype(BF16)
            h0 = r0 // 2 if isinstance(r0, int) else pl.multiple_of(r0 // 2, 8)
            xn_v[pl.ds(h0, t // 2), :] = _pk(xn)
            return mu, rs

        def g_update(pk, r0, first):
            h0 = r0 // 2 if isinstance(r0, int) else pl.multiple_of(r0 // 2, 8)
            upd = _dot_tn(pk, _unpk(xn_v[pl.ds(h0, T1 // 2), :]))
            zs = jnp.sum(pk.astype(F32).reshape(T1 // 8, 8, D), axis=0)
            if first:
                g_v[...] = upd
                z_v[...] = zs
            else:
                g_v[...] += upd
                z_v[...] += zs

        def q_part(i, r0, mu, rs, nxt):
            acc = raw(x_v[pl.ds(r0, T1), 0:D], QC, D)
            pq = _phi(fix(acc, mu, rs, QC, D)).astype(BF16)
            pqt_v[i] = _pk(pq.T)
            if nxt:
                prep(r0 + T1, T1, _pace(acc, T1 // 8, 0.0, 0.9))
            return acc

        with scope("p1_first"):
            x0a.wait()
            mua, rsa = prep(0, HT)
            wcp[0].wait()
            colsum(*wch[0][1:])
            pka = _phi(fix(raw(x_v[0:HT, 0:D], *wch[0][1:]), mua, rsa, *wch[0][1:])).astype(BF16)
            x0b.wait()
            mub, rsb = prep(HT, HT)
            pkb = _phi(fix(raw(x_v[HT:T1, 0:D], *wch[0][1:]), mub, rsb, *wch[0][1:])).astype(BF16)
            mu = jnp.concatenate([mua, mub], axis=0)
            rs = jnp.concatenate([rsa, rsb], axis=0)
            pks = [jnp.concatenate([pka, pkb], axis=0)]
            for j in (1, 2):
                wcp[j].wait()
                colsum(*wch[j][1:])
                pks.append(_phi(fix(raw(x_v[0:T1, 0:D], *wch[j][1:]), mu, rs, *wch[j][1:])).astype(BF16))
            g_update(jnp.concatenate(pks, axis=1), 0, True)
            wcp[3].wait()
            for c in xcp:
                c.wait()
            colsum(*wch[3][1:])
            q_part(0, 0, mu, rs, True)

        def p1_kg(r0):
            mu = mu_v[pl.ds(r0, T1), :]
            rs = rs_v[pl.ds(r0, T1), :]
            pk = _phi(fix(raw(x_v[pl.ds(r0, T1), 0:D], KC, D), mu, rs, KC, D)).astype(BF16)
            g_update(pk, r0, False)
            return mu, rs

        def p1_body(i, c):
            r0 = pl.multiple_of(i * T1, T1)
            mu, rs = p1_kg(r0)
            q_part(i, r0, mu, rs, True)
            return c

        with scope("p1_loop"):
            lax.fori_loop(1, n1 - 1, p1_body, 0)

        sc = scope("p2")
        sc.__enter__()
        wcp[4].wait()
        wr_copy.wait()
        wo_copy.wait()
        wg_copy.wait()
        wu_copy.wait()
        wd_copy.wait()

        rl = (n1 - 1) * T1
        mu, rs = p1_kg(rl)

        z = _rb(jnp.sum(z_v[...], axis=0, keepdims=True))
        zc = jnp.concatenate(
            [jnp.broadcast_to(z[:, g * 128:(g + 1) * 128], (128, 128)).T for g in range(G)], axis=0)
        wr = wr_v[...].astype(F32).reshape(1, D)

        def stage_a(i, zero=None):
            r0, t = p2_off[i], p2_tiles[i]
            k = t // 128
            pqt = _unpk(pqt_v[r0 // T1, :, r0 % T1:r0 % T1 + t]).astype(F32)
            zz = zc
            if zero is not None:
                n = zero.shape[0] // 8
                zz = _tie(zc, jnp.concatenate(
                    [z8 for z8 in jnp.split(zero, n, axis=0) for _ in range(D // 8 // n)], axis=0))
            w = (pqt * _lanes(zz, k)).reshape(H, DH // 8, 8, t)
            den = jnp.sum(jnp.sum(w, axis=1), axis=1, keepdims=True) + 1e-6
            o = pqt.reshape(H, DH, t) * _recip(den)
            return o.reshape(D, t).astype(BF16)

        def stage_c(i, attn, top, dep=None):
            r0, t = p2_off[i], p2_tiles[i]
            h = _rb(x_v[r0:r0 + t, 0:D].astype(F32) + attn)
            mu, rs = _ln_stats(h, None if dep is None else _pace(dep, t // 8, 0.0, CHI / 100))
            hnb = ((h - _lanes(mu, G)) * _lanes(rs, G)).astype(BF16)
            hn = hnb.astype(F32)
            hn_v[r0:r0 + t, :] = hnb
            out_v[r0:r0 + t, :] = (h + hn).astype(BF16)
            out_copy(i).start()
            r = _rb(jnp.sum(hn * wr, axis=-1, keepdims=True))
            bits = pltpu.bitcast(jnp.where(r == 0.0, 0.0, r), I32)
            mono = jnp.where(bits < 0, bits ^ 0x7FFF0000, bits)
            idx = lax.broadcasted_iota(I32, (t, 1), 0) + r0
            key = mono | (0xFFFF - idx)
            done = pltpu.bitcast(jnp.broadcast_to(key, (t, 128)), U32)
            done = lax.shift_right_logical(lax.shift_right_logical(done, U32(31)), U32(1))
            key = key.reshape(t // 8, 8, 1)
            n = t // 16
            k1 = jnp.maximum(key[:n], key[n:])
            k2 = jnp.minimum(key[:n], key[n:])
            while n > 1:
                n //= 2
                a1, b1, a2, b2 = k1[:n], k1[n:], k2[:n], k2[n:]
                k1 = jnp.maximum(a1, b1)
                k2 = jnp.maximum(jnp.minimum(a1, b1), jnp.maximum(a2, b2))
            k1, k2 = k1[0], k2[0]
            if top is None:
                return (k1, k2), done
            t1, t2 = top
            return (jnp.maximum(t1, k1), jnp.maximum(jnp.minimum(t1, k1), jnp.maximum(t2, k2))), done

        accq = q_part(n1 - 1, rl, mu, rs, False)
        o_next = stage_a(0, _pace(accq, H, 0.0, 0.8))

        row = lax.broadcasted_iota(I32, (128, 128), 0) // DH
        col = lax.broadcasted_iota(I32, (128, 128), 1) // DH
        same = row == col
        kvs = []
        for g in range(G):
            gg = g_v[g * 128:(g + 1) * 128, :].astype(BF16)
            kvs.append(jnp.where(same, _dot(gg, wqkv_v[:, VC + g * 128:VC + (g + 1) * 128]), 0.0).astype(BF16))
        for g in range(G):
            m_v[g * 64:(g + 1) * 64, :] = _pk(_dot(kvs[g], wo_v[g * 128:(g + 1) * 128, 0:D]).astype(BF16))

        top = None
        attn_prev = None
        for i in range(n2):
            o_cur = o_next
            attn = _dot_tn(o_cur, _unpk(m_v[...]))
            if i > 0:
                top, done = stage_c(i - 1, attn_prev, top, attn)
            else:
                done = _pace(attn, H, 0.0, 0.8)
            if i + 1 < n2:
                o_next = stage_a(i + 1, done)
            attn_prev = attn
        top, _ = stage_c(n2 - 1, attn_prev, top)
        sc.__exit__(None, None, None)

        sc = scope("tail")
        sc.__enter__()
        t1, t2 = top
        k1 = jnp.max(t1, axis=0, keepdims=True)
        k2 = jnp.max(jnp.where(t1 == k1, t2, t1), axis=0, keepdims=True)
        i1 = jnp.clip(0xFFFF - (k1[0, 0] & 0xFFFF), 0, S - 1)
        i2 = jnp.clip(0xFFFF - (k2[0, 0] & 0xFFFF), 0, S - 1)
        g1 = pl.multiple_of((i1 // 16) * 16, 16)
        g2 = pl.multiple_of((i2 // 16) * 16, 16)
        rows = lax.broadcasted_iota(I32, (16, D), 0)
        sel1 = rows == (i1 - g1)
        sel2 = rows == (i2 - g2)
        x1 = jnp.sum(jnp.where(sel1, hn_v[pl.ds(g1, 16), :].astype(F32), 0.0), axis=0, keepdims=True)
        x2 = jnp.sum(jnp.where(sel2, hn_v[pl.ds(g2, 16), :].astype(F32), 0.0), axis=0, keepdims=True)
        xs = jnp.where(rows == 0, x1, x2).astype(BF16)

        nfc = F // FC
        y = None
        a_prev = None
        for c in range(nfc + 1):
            if c < nfc:
                gt = _rb(_dot(xs, wg_v[:, c * FC:(c + 1) * FC]))
                ut = _rb(_dot(xs, wu_v[:, c * FC:(c + 1) * FC]))
            if c > 0:
                part = _dot(a_prev, wd_v[(c - 1) * FC:c * FC, 0:D])
                y = part if y is None else y + part
            if c < nfc:
                gt = _rb(gt * _recip(1.0 + jnp.exp(-gt)))
                a_prev = (gt * ut).astype(BF16)
        ksel = jnp.where(rows[:, 0:1] == 0, k1, k2) & jnp.int32(-65536)
        rsel = pltpu.bitcast(jnp.where(ksel < 0, ksel ^ 0x7FFF0000, ksel), F32)
        y = _rb(_rb(y) * _rb(jax.nn.sigmoid(rsel)))
        y1 = y[0:1, :]
        y2 = y[1:2, :]

        for i in range(n2):
            out_copy(i).wait()
        o1 = out_v[pl.ds(g1, 16), :].astype(F32)
        out_v[pl.ds(g1, 16), :] = jnp.where(sel1, o1 + y1, o1).astype(BF16)
        o2 = out_v[pl.ds(g2, 16), :].astype(F32)
        out_v[pl.ds(g2, 16), :] = jnp.where(sel2, o2 + y2, o2).astype(BF16)
        c1 = pltpu.make_async_copy(out_v.at[pl.ds(g1, 16)], out_hbm.at[pl.ds(g1, 16)], sems.at[SO])
        c2 = pltpu.make_async_copy(out_v.at[pl.ds(g2, 16)], out_hbm.at[pl.ds(g2, 16)], sems.at[SO + 1])
        c1.start()

        @pl.when(g1 != g2)
        def _():
            c2.start()
            c2.wait()
        c1.wait()
        sc.__exit__(None, None, None)

    scratch = [
        pltpu.VMEM((S, D + PAD), BF16),
        pltpu.VMEM((D, 3 * D + PAD), BF16),
        pltpu.VMEM((D, D + PAD), BF16),
        pltpu.VMEM((D, F), BF16),
        pltpu.VMEM((D, F), BF16),
        pltpu.VMEM((F, D + PAD), BF16),
        pltpu.VMEM((D,), BF16),
        pltpu.VMEM((S // 2, D), U32),
        pltpu.VMEM((S, 128), F32),
        pltpu.VMEM((S, 128), F32),
        pltpu.VMEM((n1, D // 2, T1), U32),
        pltpu.VMEM((D, D), F32),
        pltpu.VMEM((8, D), F32),
        pltpu.VMEM((1, 2 * D), F32),
        pltpu.VMEM((D // 2, D), U32),
        pltpu.VMEM((S, D), BF16),
        pltpu.VMEM((S, D), BF16),
        pltpu.SemaphoreType.DMA((NSEM,)),
    ]

    @jax.jit
    def f(A_x, A_wqkv, A_wo, B_x, B_w_r, B_w_gate, B_w_up, B_w_down):
        any_spec = pl.BlockSpec(memory_space=pl.ANY)
        out = pl.pallas_call(
            kernel,
            out_shape=jax.ShapeDtypeStruct((S, D), BF16),
            in_specs=[any_spec] * 7,
            out_specs=any_spec,
            scratch_shapes=scratch,
            compiler_params=pltpu.CompilerParams(vmem_limit_bytes=100 * 1024 * 1024),
        )(A_x.reshape(S, D), A_wqkv, A_wo, B_w_r, B_w_gate, B_w_up, B_w_down)
        return out.reshape(1, S, D)
    return f


_impl = make_kernel()


@jax.jit
def pallas_sequential_preLN__linear_attn_block__moe_arch_mod__prompt_kernel(
    A_x: jax.Array,
    A_wqkv: jax.Array,
    A_wo: jax.Array,
    B_x: jax.Array,
    B_w_r: jax.Array,
    B_w_gate: jax.Array,
    B_w_up: jax.Array,
    B_w_down: jax.Array,
):
    return _impl(A_x, A_wqkv, A_wo, B_x, B_w_r, B_w_gate, B_w_up, B_w_down)
```

```python
import contextlib

import jax
import jax.numpy as jnp
from jax import lax
import jax.experimental.pallas as pl
import jax.experimental.pallas.tpu as pltpu

S, D, F, H, DH = 2048, 1024, 3584, 32, 32
G = D // 128
F32 = jnp.float32
BF16 = jnp.bfloat16
I32 = jnp.int32
U32 = jnp.uint32
KEY0 = 64 << 23
PAD = 128


def _rb(x):
    return x.astype(BF16).astype(F32)


def _zero_of(x):
    bits = pltpu.bitcast(x, U32)
    return lax.shift_right_logical(lax.shift_right_logical(bits, U32(31)), U32(1))


def _pace(dep, n, lo=0.0, hi=1.0):
    if isinstance(dep, (list, tuple)):
        dep = jnp.concatenate(dep, axis=1)
    nrg, nch = dep.shape[0] // 8, dep.shape[1] // 128
    parts = []
    for p in range(n):
        pos = int((lo + (hi - lo) * p / n) * nch * nrg)
        c, rg = pos // nrg, pos % nrg
        parts.append(dep[rg * 8:(rg + 1) * 8, c * 128:(c + 1) * 128])
    return _zero_of(jnp.concatenate(parts, axis=0))


def _tie(x, zero):
    return pltpu.bitcast(pltpu.bitcast(x, U32) | zero, F32)


def _lanes(x, n):
    return jnp.concatenate([x] * n, axis=1) if n > 1 else x


def _rowsum(x):
    return jnp.broadcast_to(jnp.sum(x, axis=-1, keepdims=True), (x.shape[0], 128))


def _recip(d):
    r = pl.reciprocal(d, approx=True)
    return r * (2.0 - d * r)


def _rstd(var):
    v = _rb(_rb(var) + 1e-5)
    return _recip(_rb(v * lax.rsqrt(v)))


def _phi(t):
    return jnp.where(t > 0, t + 1.0, jnp.exp(t)) + 1e-6


def _dot(a, b):
    return jnp.dot(a, b, preferred_element_type=F32)


def _dot_tn(a, b):
    return lax.dot_general(a, b, (((0,), (0,)), ((), ())), preferred_element_type=F32)


def _pk(x):
    return pltpu.bitcast(x, U32)


def _unpk(x):
    return pltpu.bitcast(x, BF16)


def make_kernel(P2T="256,256,256,256,256,256,256,192,64", FC=512, CHI=80, late=0, NB=128, NAG=4, scopes=0):
    T1 = 512
    p2_tiles = [int(t) for t in P2T.split(",")]
    assert sum(p2_tiles) == S
    p2_off = [sum(p2_tiles[:i]) for i in range(len(p2_tiles))]
    n1 = S // T1
    n2 = len(p2_tiles)
    HT = T1 // 2
    KC, QC, VC = 0, D, 2 * D
    wch = [(D, KC, 256), (D + 256, KC + 256, 256), (D + 512, KC + 512, 512), (0, QC, D), (2 * D, VC, D)]
    SX0A, SX0B = 0, 1
    SW = 2
    SX = SW + len(wch)
    SWO = SX + n1 - 1
    SWG, SWU, SWD, SWR = SWO + 1, SWO + 2, SWO + 3, SWO + 4
    SO = SWR + 1
    NSEM = SO + n2

    def scope(name):
        return jax.named_scope(name) if scopes else contextlib.nullcontext()

    def kernel(x_hbm, wqkv_hbm, wo_hbm, wr_hbm, wg_hbm, wu_hbm, wd_hbm, out_hbm,
               x_v, wqkv_v, wo_v, wg_v, wu_v, wd_v, wr_v, xn_v, mu_v, rs_v, pqt_v, g_v, z_v, cs_v,
               m_v, out_v, h_v, sems):

        def rows_copy(r0, n, s):
            return pltpu.make_async_copy(x_hbm.at[pl.ds(r0, n)], x_v.at[pl.ds(r0, n), pl.ds(0, D)], sems.at[s])

        x0a = rows_copy(0, HT, SX0A)
        x0b = rows_copy(HT, HT, SX0B)
        xcp = [rows_copy(i * T1, T1, SX + i - 1) for i in range(1, n1)]
        wcp = [pltpu.make_async_copy(wqkv_hbm.at[:, pl.ds(c0, n)], wqkv_v.at[:, pl.ds(d0, n)], sems.at[SW + j])
               for j, (c0, d0, n) in enumerate(wch)]
        wo_copy = pltpu.make_async_copy(wo_hbm, wo_v.at[:, pl.ds(0, D)], sems.at[SWO])
        wg_copy = pltpu.make_async_copy(wg_hbm, wg_v, sems.at[SWG])
        wu_copy = pltpu.make_async_copy(wu_hbm, wu_v, sems.at[SWU])
        wd_copy = pltpu.make_async_copy(wd_hbm, wd_v.at[:, pl.ds(0, D)], sems.at[SWD])
        wr_copy = pltpu.make_async_copy(wr_hbm, wr_v, sems.at[SWR])

        def out_copy(i):
            return pltpu.make_async_copy(out_v.at[pl.ds(p2_off[i], p2_tiles[i])],
                                         out_hbm.at[pl.ds(p2_off[i], p2_tiles[i])], sems.at[SO + i])

        for c in [x0a, wcp[0], x0b] + wcp[1:4] + xcp + [wcp[4], wr_copy, wo_copy] + ([] if late else [wg_copy, wu_copy, wd_copy]):
            c.start()

        def raw(r0, t, c0, n, first=False):
            xb = x_v[r0:r0 + t, 0:D]
            if not first:
                return _dot(xb, wqkv_v[:, c0:c0 + n])
            acc = _dot(jnp.concatenate([jnp.ones((16, D), BF16), xb], axis=0), wqkv_v[:, c0:c0 + n])
            cs_v[:, c0:c0 + n] = acc[0:8]
            return acc[16:]

        def feat(acc, r0, c0):
            t, n = acc.shape
            k = n // 128
            mu = _lanes(mu_v[r0:r0 + t, :], k).reshape(t // 8, 8, n)
            rs = _lanes(rs_v[r0:r0 + t, :], k)
            y = (acc.reshape(t // 8, 8, n) - mu * cs_v[:, c0:c0 + n]).reshape(t, n) * rs
            return _phi(y).astype(BF16)

        def prep(r0, t, zero=None):
            xf = x_v[r0:r0 + t, 0:D].astype(F32)
            if zero is not None:
                xf = jnp.concatenate([_tie(xf[:, 0:128], zero), xf[:, 128:]], axis=1)
            mu = _rowsum(xf) * (1.0 / D)
            mur = _rb(mu)
            mu_v[r0:r0 + t, :] = mur
            xc = x_v[r0:r0 + t, 0:D].astype(F32) - _lanes(mu, G)
            rs = _rstd(_rowsum(xc * xc) * (1.0 / D))
            rs_v[r0:r0 + t, :] = rs
            xn = (x_v[r0:r0 + t, 0:D].astype(F32) - _lanes(mur, G)) * _lanes(rs, G)
            xn_v[r0 // 2:(r0 + t) // 2, :] = _pk(xn.astype(BF16))

        def g_update(pk, i):
            upd = _dot_tn(pk, _unpk(xn_v[i * T1 // 2:(i + 1) * T1 // 2, :]))
            zs = jnp.sum(pk.astype(F32).reshape(T1 // 8, 8, D), axis=0)
            if i == 0:
                g_v[...] = upd
                z_v[...] = zs
            else:
                g_v[...] += upd
                z_v[...] += zs
            return upd

        def q_part(i):
            acc = raw(i * T1, T1, QC, D, i == 0)
            pqt_v[i] = _pk(feat(acc, i * T1, QC).T)
            return acc

        def k_part(i):
            return feat(raw(i * T1, T1, KC, D), i * T1, KC)

        with scope("p1_first"):
            x0a.wait()
            prep(0, HT)
            wcp[0].wait()
            pka = feat(raw(0, HT, KC, 256, True), 0, KC)
            x0b.wait()
            prep(HT, HT)
            pkb = feat(raw(HT, HT, KC, 256), HT, KC)
            pks = [jnp.concatenate([pka, pkb], axis=0)]
            for j in (1, 2):
                wcp[j].wait()
                _, c0, n = wch[j]
                pks.append(feat(raw(0, T1, c0, n, True), 0, c0))
            g_update(jnp.concatenate(pks, axis=1), 0)

        with scope("p1_mid"):
            wcp[3].wait()
            for c in xcp:
                c.wait()
            prep(T1, T1, _pace(q_part(0), T1 // 8, 0.0, 0.9))
            for i in range(1, n1 - 1):
                pk = k_part(i)
                q_part(i)
                prep((i + 1) * T1, T1, _pace(g_update(pk, i), T1 // 8, 0.0, 0.9))

        sc = scope("p2")
        sc.__enter__()
        wcp[4].wait()
        wr_copy.wait()
        wo_copy.wait()
        if late:
            for c in (wg_copy, wu_copy, wd_copy):
                c.start()
        else:
            for c in (wg_copy, wu_copy, wd_copy):
                c.wait()

        g_last = g_update(k_part(n1 - 1), n1 - 1)

        z = _rb(jnp.sum(z_v[...], axis=0, keepdims=True))
        zc = jnp.concatenate(
            [jnp.broadcast_to(z[:, g * 128:(g + 1) * 128], (128, 128)).T for g in range(G)], axis=0)
        wr = wr_v[...].astype(F32).reshape(1, D)
        wr_sum = _rowsum(wr)

        def stage_a(r0, t, zero):
            k = t // 128
            pqt = _unpk(pqt_v[r0 // T1, :, r0 % T1:r0 % T1 + t]).astype(F32)
            z4 = zc.reshape(H, DH // 8, 8, 128)
            z0 = _tie(z4[:, 0].reshape(H * 8, 128), zero).reshape(H, 1, 8, 128)
            zz = jnp.concatenate([z0, z4[:, 1:]], axis=1).reshape(D, 128)
            w = (pqt * _lanes(zz, k)).reshape(H, DH // 8, 8, t)
            den = jnp.sum(jnp.sum(w, axis=1), axis=1, keepdims=True) + 1e-6
            o = pqt.reshape(H, DH, t) * _recip(den)
            return _pk(o.reshape(D, t).astype(BF16).T)

        def stage_b(i, gate):
            r0, t = p2_off[i], p2_tiles[i]
            ou = jnp.concatenate(os, axis=0)[r0 // 2:(r0 + t) // 2, :]
            if gate is not None:
                ou = jnp.concatenate(
                    [jnp.concatenate([ou[0:8, 0:128] | gate, ou[0:8, 128:]], axis=1), ou[8:]], axis=0)
            o = _unpk(ou)
            deps = []
            for c in range(0, D, NB):
                lo = _dot(o[:, 0:D // 2], _unpk(m_v[0:D // 4, c:c + NB]))
                attn = lo + _dot(o[:, D // 2:], _unpk(m_v[D // 4:, c:c + NB]))
                h_v[r0:r0 + t, c:c + NB] = x_v[r0:r0 + t, c:c + NB].astype(F32) + attn
                deps += [lo, attn]
            return deps, _rowsum(h_v[r0:r0 + t, :]) * (1.0 / D)

        def keys_of(r, idx):
            bits = pltpu.bitcast(jnp.where(r == 0.0, 0.0, r), I32)
            hi = lax.shift_right_logical(bits, 16)
            mono = jnp.where(bits < 0, 0xFFFF - hi, hi | 0x8000)
            return pltpu.bitcast((mono << 11) + (KEY0 + S - 1 - idx), F32)

        def merge(top, k1, k2):
            if top is None:
                return k1, k2
            t1, t2 = top
            return jnp.maximum(t1, k1), jnp.maximum(jnp.minimum(t1, k1), jnp.maximum(t2, k2))

        def write_out(i, mur, rs):
            r0, t = p2_off[i], p2_tiles[i]
            out_v[r0:r0 + t, :] = (h_v[r0:r0 + t, :] * _lanes(1.0 + rs, G) - _lanes(mur * rs, G)).astype(BF16)
            back = out_v[r0:r0 + t, D - 128:D].astype(F32)
            out_copy(i).start()
            return back

        def stage_c(i, mu, dep=None):
            r0, t = p2_off[i], p2_tiles[i]
            if dep is not None:
                mu = _tie(mu, _pace(dep, t // 8, 0.0, CHI / 100))
            d = h_v[r0:r0 + t, :] - _lanes(mu, G)
            rs = _rstd(_rowsum(d * d) * (1.0 / D))
            mur = _rb(mu)
            r = _rb((_rowsum(d * wr) + (mu - mur) * wr_sum) * rs)
            mu_v[r0:r0 + t, :] = mur
            rs_v[r0:r0 + t, :] = rs
            return r, mur, rs

        lane = lax.broadcasted_iota(I32, (8, 128), 1)
        sub = lax.broadcasted_iota(I32, (8, 128), 0)

        def compact(i, r):
            r0, t = p2_off[i], p2_tiles[i]
            parts = [r[p * 8:(p + 1) * 8] for p in range(t // 8)]
            acc = parts[0]
            for p in range(1, t // 8):
                acc = jnp.where(lane == p, parts[p], acc)
            key = keys_of(acc, r0 + lane * 8 + sub)
            return jnp.where(lane < t // 8, key, 0.0)

        def a_done(os):
            acc = None
            for o in os:
                for rb in range(o.shape[0] // 64):
                    row = o[rb * 64 + 56:rb * 64 + 64, :]
                    for g in range(G):
                        v = row[:, g * 128:(g + 1) * 128]
                        acc = v if acc is None else acc | v
            return _zero_of(acc)

        ta = 256
        na = S // ta
        nearly = (S - T1) // ta
        pz = _pace(g_last, NAG * H, 0.0, 1.0)
        os = [stage_a(j * ta, ta, pz[j * H * 8:(j + 1) * H * 8]) for j in range(NAG)]
        accq = q_part(n1 - 1)
        if nearly > NAG:
            pz = _pace(accq, (nearly - NAG) * H, 0.0, 0.9)
            os += [stage_a(j * ta, ta, pz[(j - NAG) * H * 8:(j - NAG + 1) * H * 8]) for j in range(NAG, nearly)]

        row = lax.broadcasted_iota(I32, (128, 128), 0) // DH
        col = lax.broadcasted_iota(I32, (128, 128), 1) // DH
        same = row == col
        kvs = []
        for g in range(G):
            gg = g_v[g * 128:(g + 1) * 128, :]
            if g == 0:
                gg = jnp.concatenate([jnp.concatenate(
                    [_tie(gg[0:8, 0:128], a_done(os)), gg[0:8, 128:]], axis=1), gg[8:]], axis=0)
            kv = _dot(gg.astype(BF16), wqkv_v[:, VC + g * 128:VC + (g + 1) * 128])
            kvs.append(jnp.where(same, kv, 0.0).astype(BF16))
        for g in range(G):
            m_v[g * 64:(g + 1) * 64, :] = _pk(_dot(kvs[g], wo_v[g * 128:(g + 1) * 128, 0:D]).astype(BF16))

        top = None
        mu_prev = None
        gate = None
        for i in range(n2):
            deps, mu = stage_b(i, gate)
            if i == 0:
                pz = _pace(deps, (na - nearly) * H, 0.0, 0.8)
                late_os = [stage_a(j * ta, ta, pz[(j - nearly) * H * 8:(j - nearly + 1) * H * 8])
                           for j in range(nearly, na)]
                os += late_os
                gate = a_done(late_os)
            else:
                r, mur, rs = stage_c(i - 1, mu_prev, deps)
                back = write_out(i - 1, mur, rs)
                key = compact(i - 1, r)
                top = merge(top, key, jnp.zeros_like(key))
                gate = _zero_of(key + jnp.sum(back.reshape(-1, 8, 128), axis=0))
            mu_prev = mu
        t1, t2 = top
        b1 = jnp.max(jnp.max(t1, axis=0, keepdims=True), axis=1, keepdims=True)
        rest = jnp.where(t1 == b1, t2, t1)
        b2 = jnp.max(jnp.max(rest, axis=0, keepdims=True), axis=1, keepdims=True)
        r, mur_l, rs_l = stage_c(n2 - 1, mu_prev)
        tl = p2_tiles[-1]
        key = keys_of(r, lax.broadcasted_iota(I32, (tl, 128), 0) + p2_off[-1]).reshape(tl // 8, 8, 128)
        n = tl // 16
        k1 = jnp.maximum(key[:n], key[n:])
        k2 = jnp.minimum(key[:n], key[n:])
        while n > 1:
            n //= 2
            k1, k2 = merge((k1[:n], k2[:n]), k1[n:], k2[n:])
        top = merge((k1[0], k2[0]), jnp.where(sub == 0, b1, 0.0), jnp.where(sub == 0, b2, 0.0))
        sc.__exit__(None, None, None)

        sc = scope("tail")
        sc.__enter__()
        if late:
            for c in (wg_copy, wu_copy, wd_copy):
                c.wait()
        t1, t2 = top
        k1 = jnp.max(t1, axis=0, keepdims=True)
        k2 = jnp.max(jnp.where(t1 == k1, t2, t1), axis=0, keepdims=True)
        k1 = pltpu.bitcast(k1, I32)
        k2 = pltpu.bitcast(k2, I32)
        i1 = S - 1 - (k1[0, 0] & (S - 1))
        i2 = S - 1 - (k2[0, 0] & (S - 1))
        first = lax.broadcasted_iota(I32, (16, 128), 0) == 0

        def pick(ref, k):
            a = ref[pl.ds(i1, 1), :]
            b = ref[pl.ds(i2, 1), :]
            return jnp.where(_lanes(first, k), a, b)

        hs = pick(h_v, G)
        xs = ((hs - _lanes(pick(mu_v, 1), G)) * _lanes(pick(rs_v, 1), G)).astype(BF16)

        nfc = F // FC
        y = None
        a_prev = None
        for c in range(nfc + 1):
            if c < nfc:
                gt = _rb(_dot(xs, wg_v[:, c * FC:(c + 1) * FC]))
                ut = _rb(_dot(xs, wu_v[:, c * FC:(c + 1) * FC]))
            if c > 0:
                part = _dot(a_prev, wd_v[(c - 1) * FC:c * FC, 0:D])
                y = part if y is None else y + part
            if c == 1:
                write_out(n2 - 1, _tie(mur_l, jnp.concatenate([_zero_of(gt[0:8, 0:128])] * (tl // 8), axis=0)), rs_l)
            if c < nfc:
                gt = _rb(gt * _recip(1.0 + jnp.exp(-gt)))
                a_prev = (gt * ut).astype(BF16)
        mono = lax.shift_right_logical(jnp.where(first, k1, k2) - KEY0, 11)
        rsel = pltpu.bitcast(jnp.where(mono < 0x8000, 0xFFFF - mono, mono & 0x7FFF) << 16, F32)
        y = _rb(_rb(y) * _lanes(_rb(jax.nn.sigmoid(rsel)), G))
        new = hs + _rb(xs.astype(F32) + y)

        for i in range(n2):
            out_copy(i).wait()
        g1 = pl.multiple_of((i1 // 16) * 16, 16)
        g2 = pl.multiple_of((i2 // 16) * 16, 16)
        rows = lax.broadcasted_iota(I32, (16, D), 0)
        o1 = out_v[pl.ds(g1, 16), :].astype(F32)
        out_v[pl.ds(g1, 16), :] = jnp.where(rows == i1 - g1, new[0:1], o1).astype(BF16)
        o2 = out_v[pl.ds(g2, 16), :].astype(F32)
        out_v[pl.ds(g2, 16), :] = jnp.where(rows == i2 - g2, new[1:2], o2).astype(BF16)
        c1 = pltpu.make_async_copy(out_v.at[pl.ds(g1, 16)], out_hbm.at[pl.ds(g1, 16)], sems.at[SO])
        c2 = pltpu.make_async_copy(out_v.at[pl.ds(g2, 16)], out_hbm.at[pl.ds(g2, 16)], sems.at[SO + 1])
        c1.start()

        @pl.when(g1 != g2)
        def _():
            c2.start()
            c2.wait()
        c1.wait()
        sc.__exit__(None, None, None)

    scratch = [
        pltpu.VMEM((S, D + PAD), BF16),
        pltpu.VMEM((D, 3 * D + PAD), BF16),
        pltpu.VMEM((D, D + PAD), BF16),
        pltpu.VMEM((D, F), BF16),
        pltpu.VMEM((D, F), BF16),
        pltpu.VMEM((F, D + PAD), BF16),
        pltpu.VMEM((D,), BF16),
        pltpu.VMEM((S // 2, D), U32),
        pltpu.VMEM((S, 128), F32),
        pltpu.VMEM((S, 128), F32),
        pltpu.VMEM((n1, D // 2, T1), U32),
        pltpu.VMEM((D, D), F32),
        pltpu.VMEM((8, D), F32),
        pltpu.VMEM((8, 2 * D), F32),
        pltpu.VMEM((D // 2, D), U32),
        pltpu.VMEM((S, D), BF16),
        pltpu.VMEM((S, D), F32),
        pltpu.SemaphoreType.DMA((NSEM,)),
    ]

    @jax.jit
    def f(A_x, A_wqkv, A_wo, B_x, B_w_r, B_w_gate, B_w_up, B_w_down):
        any_spec = pl.BlockSpec(memory_space=pl.ANY)
        out = pl.pallas_call(
            kernel,
            out_shape=jax.ShapeDtypeStruct((S, D), BF16),
            in_specs=[any_spec] * 7,
            out_specs=any_spec,
            scratch_shapes=scratch,
            compiler_params=pltpu.CompilerParams(vmem_limit_bytes=100 * 1024 * 1024),
        )(A_x.reshape(S, D), A_wqkv, A_wo, B_w_r, B_w_gate, B_w_up, B_w_down)
        return out.reshape(1, S, D)
    return f


_impl = make_kernel()


@jax.jit
def pallas_sequential_preLN__linear_attn_block__moe_arch_mod__prompt_kernel(
    A_x: jax.Array,
    A_wqkv: jax.Array,
    A_wo: jax.Array,
    B_x: jax.Array,
    B_w_r: jax.Array,
    B_w_gate: jax.Array,
    B_w_up: jax.Array,
    B_w_down: jax.Array,
):
    return _impl(A_x, A_wqkv, A_wo, B_x, B_w_r, B_w_gate, B_w_up, B_w_down)
```

```python
import contextlib

import jax
import jax.numpy as jnp
from jax import lax
import jax.experimental.pallas as pl
import jax.experimental.pallas.tpu as pltpu

S, D, F, H, DH = 2048, 1024, 3584, 32, 32
G = D // 128
F32 = jnp.float32
BF16 = jnp.bfloat16
I32 = jnp.int32
U32 = jnp.uint32
KEY0 = 64 << 23
PAD = 128


def _rb(x):
    return x.astype(BF16).astype(F32)


def _zero_of(x):
    bits = pltpu.bitcast(x, U32)
    return lax.shift_right_logical(lax.shift_right_logical(bits, U32(31)), U32(1))


def _pace(dep, n, lo=0.0, hi=1.0):
    if isinstance(dep, (list, tuple)):
        dep = jnp.concatenate(dep, axis=1)
    nrg, nch = dep.shape[0] // 8, dep.shape[1] // 128
    parts = []
    for p in range(n):
        pos = int((lo + (hi - lo) * p / n) * nch * nrg)
        c, rg = pos // nrg, pos % nrg
        parts.append(dep[rg * 8:(rg + 1) * 8, c * 128:(c + 1) * 128])
    return _zero_of(jnp.concatenate(parts, axis=0))


def _tie(x, zero):
    return pltpu.bitcast(pltpu.bitcast(x, U32) | zero, F32)


def _lanes(x, n):
    return jnp.concatenate([x] * n, axis=1) if n > 1 else x


def _rowsum(x):
    return jnp.broadcast_to(jnp.sum(x, axis=-1, keepdims=True), (x.shape[0], 128))


def _recip(d):
    r = pl.reciprocal(d, approx=True)
    return r * (2.0 - d * r)


def _rstd(var):
    v = _rb(_rb(var) + 1e-5)
    return _recip(_rb(v * lax.rsqrt(v)))


def _phi(t):
    return jnp.where(t > 0, t + 1.0, jnp.exp(t)) + 1e-6


def _dot(a, b):
    return jnp.dot(a, b, preferred_element_type=F32)


def _dot_tn(a, b):
    return lax.dot_general(a, b, (((0,), (0,)), ((), ())), preferred_element_type=F32)


def _pk(x):
    return pltpu.bitcast(x, U32)


def _unpk(x):
    return pltpu.bitcast(x, BF16)


def _gate(xu, zero):
    if zero is None:
        return xu
    top = jnp.concatenate([xu[0:8, 0:128] | zero, xu[0:8, 128:]], axis=1)
    return jnp.concatenate([top, xu[8:]], axis=0)


def _fold(x):
    x = pltpu.bitcast(x, U32) if x.dtype != U32 else x
    parts = [x[r:r + 8, c:c + 128] for r in range(0, x.shape[0], 8) for c in range(0, x.shape[1], 128)]
    while len(parts) > 1:
        parts = [parts[j] | parts[j + 1] if j + 1 < len(parts) else parts[j] for j in range(0, len(parts), 2)]
    return _zero_of(parts[0])


def _passes(xu, w, ntiles, gate_fn=None, post=None):
    deps, outs = [], []
    for c in range(ntiles):
        acc = None
        for hh in range(2):
            z = None if gate_fn is None else gate_fn(2 * c + hh, deps)
            lhs = _unpk(_gate(xu[:, hh * (D // 2):(hh + 1) * (D // 2)], z))
            part = _dot(lhs, w(hh * (D // 2), (hh + 1) * (D // 2), c))
            acc = part if acc is None else acc + part
            deps.append(acc)
        outs.append(acc if post is None else post(c, acc))
    return outs, deps


def make_kernel(P2T="256,256,256,256,256,256,256,128,64,64", FC=512, CHI=80, KCH="256,256,512", XP="128,128,256", PHI=85, NAG=4, CLAST=50, CGATE=13, SLAG=4, LAT=560, PRI="p0", PT=0, scopes=0):
    T1 = 512
    p2_tiles = [int(t) for t in P2T.split(",")]
    assert sum(p2_tiles) == S
    p2_off = [sum(p2_tiles[:i]) for i in range(len(p2_tiles))]
    n1 = S // T1
    n2 = len(p2_tiles)
    HT = T1 // 2
    KC, QC, VC = 0, D, 2 * D
    kch = [int(t) for t in KCH.split(",")]
    NKC = len(kch)
    wch = [(D + sum(kch[:j]), KC + sum(kch[:j]), kch[j]) for j in range(NKC)] + [(0, QC, D), (2 * D, VC, D)]
    xp = [int(t) for t in XP.split(",")]
    assert sum(xp) == T1 and len(xp) == NKC
    SW = len(xp)
    SX = SW + len(wch)
    SWO = SX + n1 - 1
    SWG, SWU, SWD, SWR = SWO + 1, SWO + 2, SWO + 3, SWO + 4
    SO = SWR + 1
    NSEM = SO + 3

    def scope(name):
        return jax.named_scope(name) if scopes else contextlib.nullcontext()

    def kernel(x_hbm, wqkv_hbm, wo_hbm, wr_hbm, wg_hbm, wu_hbm, wd_hbm, out_hbm,
               x_v, wqkv_v, wo_v, wg_v, wu_v, wd_v, wr_v, xn_v, mu_v, rs_v, pqt_v, g_v, z_v,
               m_v, out_v, h_v, fix_v, sems):

        def rows_copy(r0, n, s):
            return pltpu.make_async_copy(x_hbm.at[pl.ds(r0, n)], x_v.at[pl.ds(r0, n), pl.ds(0, D)], sems.at[s])

        x0 = [rows_copy(sum(xp[:j]), xp[j], j) for j in range(NKC)]
        xcp = [rows_copy(i * T1, T1, SX + i - 1) for i in range(1, n1)]
        wcp = [pltpu.make_async_copy(wqkv_hbm.at[:, pl.ds(c0, n)], wqkv_v.at[:, pl.ds(d0, n)], sems.at[SW + j])
               for j, (c0, d0, n) in enumerate(wch)]
        wo_copy = pltpu.make_async_copy(wo_hbm, wo_v.at[:, pl.ds(0, D)], sems.at[SWO])
        wg_copy = pltpu.make_async_copy(wg_hbm, wg_v, sems.at[SWG])
        wu_copy = pltpu.make_async_copy(wu_hbm, wu_v, sems.at[SWU])
        wd_copy = pltpu.make_async_copy(wd_hbm, wd_v.at[:, pl.ds(0, D)], sems.at[SWD])
        wr_copy = pltpu.make_async_copy(wr_hbm, wr_v, sems.at[SWR])

        def out_copy(i):
            return pltpu.make_async_copy(out_v.at[pl.ds(p2_off[i], p2_tiles[i])],
                                         out_hbm.at[pl.ds(p2_off[i], p2_tiles[i])], sems.at[SO])

        order = [c for j in range(NKC) for c in (x0[j], wcp[j])] + [wcp[NKC]] + xcp + [wcp[NKC + 1], wr_copy, wo_copy, wg_copy, wu_copy, wd_copy]
        pri = [int(ch) for ch in PRI[1:]]
        for j, c in enumerate(order):
            c.start(priority=pri[j] if j < len(pri) else pri[-1])

        def proj(r0, t, c0, n):
            return _dot(_unpk(xn_v[r0 // 2:(r0 + t) // 2, :]), wqkv_v[:, c0:c0 + n])

        def feat(y):
            return _phi(y).astype(BF16)

        def prep(r0, t, zero=None):
            xf = x_v[r0:r0 + t, 0:D].astype(F32)
            if zero is not None:
                xf = jnp.concatenate([_tie(xf[:, 0:128], zero), xf[:, 128:]], axis=1)
            mu = _rowsum(xf) * (1.0 / D)
            mur = _rb(mu)
            mu_v[r0:r0 + t, :] = mur
            xc = x_v[r0:r0 + t, 0:D].astype(F32) - _lanes(mu, G)
            rs = _rstd(_rowsum(xc * xc) * (1.0 / D))
            rs_v[r0:r0 + t, :] = rs
            xn = (x_v[r0:r0 + t, 0:D].astype(F32) - _lanes(mur, G)) * _lanes(rs, G)
            xu = _pk(xn.astype(BF16))
            xn_v[r0 // 2:(r0 + t) // 2, :] = xu
            return xu

        def g_piece(pk, r0, c0, pkt=None):
            t, n = pk.shape
            upd = _dot(pk.T if pkt is None else pkt, _unpk(xn_v[r0 // 2:(r0 + t) // 2, :]))
            zs = jnp.sum(pk.astype(F32).reshape(t // 8, 8, n), axis=0)
            if r0 == 0:
                g_v[c0:c0 + n, :] = upd
                z_v[:, c0:c0 + n] = zs
            else:
                g_v[c0:c0 + n, :] += upd
                z_v[:, c0:c0 + n] += zs
            return upd

        def g_update(pk, i):
            return g_piece(pk, i * T1, 0)

        def q_part(i):
            acc = proj(i * T1, T1, QC, D)
            pqt_v[i] = _pk(feat(acc).T)
            return acc

        def k_part(i):
            return feat(proj(i * T1, T1, KC, D))

        def wait(c, name):
            with scope(name):
                c.wait()

        pending = None
        rows = cols = 0
        for j in range(NKC):
            wait(x0[j], "w_x%d" % j)
            if pending is not None:
                g_piece(*pending)
                pending = None
            prep(rows, xp[j])
            if cols:
                pending = (feat(proj(rows, xp[j], KC, cols)), rows, 0)
            rows += xp[j]
            wait(wcp[j], "w_c%d" % j)
            pk = feat(proj(0, rows, KC + cols, kch[j]))
            if pending is not None:
                g_piece(*pending)
            pending = (pk, 0, cols, pk.T if j >= PT else None)
            cols += kch[j]
        g_piece(*pending)

        with scope("p1_mid"):
            wcp[NKC].wait()
            for c in xcp:
                c.wait()
            prep(T1, T1, _pace(q_part(0), T1 // 8, 0.0, PHI / 100))
            for i in range(1, n1 - 1):
                pk = k_part(i)
                q_part(i)
                prep((i + 1) * T1, T1, _pace(g_update(pk, i), T1 // 8, 0.0, PHI / 100))

        sc = scope("p2")
        sc.__enter__()
        wcp[NKC + 1].wait()
        wr_copy.wait()
        wo_copy.wait()
        for c in (wg_copy, wu_copy, wd_copy):
            c.wait()

        g_last = g_update(k_part(n1 - 1), n1 - 1)

        z = _rb(jnp.sum(z_v[...], axis=0, keepdims=True))
        zc = jnp.concatenate(
            [jnp.broadcast_to(z[:, g * 128:(g + 1) * 128], (128, 128)).T for g in range(G)], axis=0)
        wr = wr_v[...].astype(F32).reshape(1, D)
        wr_sum = _rowsum(wr)

        def stage_a(r0, t, zero):
            k = t // 128
            pqt = _unpk(pqt_v[r0 // T1, :, r0 % T1:r0 % T1 + t]).astype(F32)
            z4 = zc.reshape(H, DH // 8, 8, 128)
            z0 = _tie(z4[:, 0].reshape(H * 8, 128), zero).reshape(H, 1, 8, 128)
            zz = jnp.concatenate([z0, z4[:, 1:]], axis=1).reshape(D, 128)
            w = (pqt * _lanes(zz, k)).reshape(H, DH // 8, 8, t)
            den = jnp.sum(jnp.sum(w, axis=1), axis=1, keepdims=True) + 1e-6
            o = pqt.reshape(H, DH, t) * _recip(den)
            return _pk(o.reshape(D, t).astype(BF16).T)

        def m_tile(a, b, c):
            return _unpk(m_v[a // 2:b // 2, c * 128:(c + 1) * 128])

        def stage_b(i, gate):
            r0, t = p2_off[i], p2_tiles[i]

            def post(c, attn):
                h_v[r0:r0 + t, c * 128:(c + 1) * 128] = x_v[r0:r0 + t, c * 128:(c + 1) * 128].astype(F32) + attn

            _, deps = _passes(jnp.concatenate(os, axis=0)[r0 // 2:(r0 + t) // 2, :], m_tile, G,
                              lambda p, deps: gate if p == 0 else None, post)
            return deps, _rowsum(h_v[r0:r0 + t, :]) * (1.0 / D)

        def keys_of(r, idx):
            bits = pltpu.bitcast(jnp.where(r == 0.0, 0.0, r), I32)
            hi = lax.shift_right_logical(bits, 16)
            mono = jnp.where(bits < 0, 0xFFFF - hi, hi | 0x8000)
            return pltpu.bitcast((mono << 11) + (KEY0 + S - 1 - idx), F32)

        def merge(top, k1, k2):
            if top is None:
                return k1, k2
            t1, t2 = top
            return jnp.maximum(t1, k1), jnp.maximum(jnp.minimum(t1, k1), jnp.maximum(t2, k2))

        def write_out(i, mur, rs):
            r0, t = p2_off[i], p2_tiles[i]
            out_v[r0:r0 + t, :] = (h_v[r0:r0 + t, :] * _lanes(1.0 + rs, G) - _lanes(mur * rs, G)).astype(BF16)
            back = out_v[r0:r0 + t, D - 128:D].astype(F32)
            out_copy(i).start()
            return back

        def stage_c(i, mu, dep, hi=CHI / 100):
            r0, t = p2_off[i], p2_tiles[i]
            mu = _tie(mu, _pace(dep, t // 8, 0.0, hi))
            d = h_v[r0:r0 + t, :] - _lanes(mu, G)
            rs = _rstd(_rowsum(d * d) * (1.0 / D))
            mur = _rb(mu)
            r = _rb((_rowsum(d * wr) + (mu - mur) * wr_sum) * rs)
            mu_v[r0:r0 + t, :] = mur
            rs_v[r0:r0 + t, :] = rs
            return r, mur, rs

        lane = lax.broadcasted_iota(I32, (8, 128), 1)
        sub = lax.broadcasted_iota(I32, (8, 128), 0)

        def compact(i, r):
            r0, t = p2_off[i], p2_tiles[i]
            parts = [r[p * 8:(p + 1) * 8] for p in range(t // 8)]
            acc = parts[0]
            for p in range(1, t // 8):
                acc = jnp.where(lane == p, parts[p], acc)
            key = keys_of(acc, r0 + lane * 8 + sub)
            return jnp.where(lane < t // 8, key, 0.0)

        def a_done(os):
            acc = None
            for o in os:
                for rb in range(o.shape[0] // 64):
                    row = o[rb * 64 + 56:rb * 64 + 64, :]
                    for g in range(G):
                        v = row[:, g * 128:(g + 1) * 128]
                        acc = v if acc is None else acc | v
            return _zero_of(acc)

        ta = 256
        na = S // ta
        nearly = (S - T1) // ta
        pz = _pace(g_last, NAG * H, 0.0, 1.0)
        os = [stage_a(j * ta, ta, pz[j * H * 8:(j + 1) * H * 8]) for j in range(NAG)]
        accq = q_part(n1 - 1)
        if nearly > NAG:
            pz = _pace(accq, (nearly - NAG) * H, 0.0, 0.9)
            os += [stage_a(j * ta, ta, pz[(j - NAG) * H * 8:(j - NAG + 1) * H * 8]) for j in range(NAG, nearly)]

        row = lax.broadcasted_iota(I32, (128, 128), 0) // DH
        col = lax.broadcasted_iota(I32, (128, 128), 1) // DH
        same = row == col
        kvs = []
        for g in range(G):
            gg = g_v[g * 128:(g + 1) * 128, :]
            if g == 0:
                gg = jnp.concatenate([jnp.concatenate(
                    [_tie(gg[0:8, 0:128], a_done(os)), gg[0:8, 128:]], axis=1), gg[8:]], axis=0)
            kv = _dot(gg.astype(BF16), wqkv_v[:, VC + g * 128:VC + (g + 1) * 128])
            kvs.append(jnp.where(same, kv, 0.0).astype(BF16))
        for g in range(G):
            m_v[g * 64:(g + 1) * 64, :] = _pk(_dot(kvs[g], wo_v[g * 128:(g + 1) * 128, 0:D]).astype(BF16))

        def tree(i, r):
            t = p2_tiles[i]
            key = keys_of(r, lax.broadcasted_iota(I32, (t, 128), 0) + p2_off[i])
            level = [(key[p * 8:(p + 1) * 8], None) for p in range(t // 8)]
            while len(level) > 1:
                nxt = []
                for p in range(0, len(level) - 1, 2):
                    (a1, a2), (b1, b2) = level[p], level[p + 1]
                    lo = jnp.minimum(a1, b1)
                    for e in (a2, b2):
                        lo = lo if e is None else jnp.maximum(lo, e)
                    nxt.append((jnp.maximum(a1, b1), lo))
                if len(level) % 2:
                    nxt.append(level[-1])
                level = nxt
            return level[0]

        def stage_last(gate, mu_prev, top):
            i = n2 - 1
            r0, t = p2_off[i], p2_tiles[i]
            st = {}

            def post(c, attn):
                h = x_v[r0:r0 + t, c * 128:(c + 1) * 128].astype(F32) + attn
                h_v[r0:r0 + t, c * 128:(c + 1) * 128] = h
                if c == 0:
                    st["shift"] = jnp.broadcast_to(h[:, 0:1], (t, 128))
                d = h - st["shift"]
                new = (d, d * d, d * wr[:, c * 128:(c + 1) * 128])
                st[c] = new if c == 0 else tuple(a + b for a, b in zip(st[c - 1], new))

            def gate_fn(p, deps):
                if p == 0:
                    return gate
                z = None
                if p % 2 == 1 and p // 2 - SLAG >= 0:
                    z = _fold(jnp.concatenate(st[p // 2 - SLAG], axis=1))
                if p == CGATE:
                    r, st["mur_p"], st["rs_p"] = stage_c(i - 1, mu_prev, deps, CLAST / 100)
                    st["top"] = merge(top, *tree(i - 1, r))
                    zz = _zero_of(st["top"][0] + st["top"][1])
                    z = zz if z is None else z | zz
                return z

            _passes(jnp.concatenate(os, axis=0)[r0 // 2:(r0 + t) // 2, :], m_tile, G, gate_fn, post)
            s1, s2, s3 = st[G - 1]
            shift = st["shift"]
            m1 = _rowsum(s1) * (1.0 / D)
            var = jnp.maximum(_rowsum(s2) * (1.0 / D) - m1 * m1, 0.0)
            rs = _rstd(var)
            mur = _rb(shift + m1)
            r = _rb((_rowsum(s3) + (shift - mur) * wr_sum) * rs)
            mu_v[r0:r0 + t, :] = mur
            rs_v[r0:r0 + t, :] = rs
            return merge(st["top"], *tree(i, r)), st["mur_p"], st["rs_p"], mur, rs

        top = None
        mu_prev = None
        gate = None
        for i in range(n2 - 1):
            deps, mu = stage_b(i, gate)
            if i == 0:
                pz = _pace(deps, (na - nearly) * H, 0.0, 0.8)
                late_os = [stage_a(j * ta, ta, pz[(j - nearly) * H * 8:(j - nearly + 1) * H * 8])
                           for j in range(nearly, na)]
                os += late_os
                gate = a_done(late_os)
            else:
                r, mur, rs = stage_c(i - 1, mu_prev, deps, min(CHI / 100, 1 - LAT / (16 * p2_tiles[i])))
                back = write_out(i - 1, mur, rs)
                key = compact(i - 1, r)
                top = merge(top, key, jnp.zeros_like(key))
                gate = _zero_of(key + jnp.sum(back.reshape(-1, 8, 128), axis=0))
                if i == n2 - 2:
                    t1, t2 = top
                    b1 = jnp.max(jnp.max(t1, axis=0, keepdims=True), axis=1, keepdims=True)
                    rest = jnp.where(t1 == b1, t2, t1)
                    b2 = jnp.max(jnp.max(rest, axis=0, keepdims=True), axis=1, keepdims=True)
                    top = (jnp.where(sub == 0, b1, 0.0), jnp.where(sub == 0, b2, 0.0))
            mu_prev = mu
        top, mur_p, rs_p, mur_l, rs_l = stage_last(gate, mu_prev, top)
        sc.__exit__(None, None, None)

        sc = scope("tail")
        sc.__enter__()
        t1, t2 = top
        k1 = jnp.max(t1, axis=0, keepdims=True)
        k2 = jnp.max(jnp.where(t1 == k1, t2, t1), axis=0, keepdims=True)
        k1 = pltpu.bitcast(k1, I32)
        k2 = pltpu.bitcast(k2, I32)
        i1 = S - 1 - (k1[0, 0] & (S - 1))
        i2 = S - 1 - (k2[0, 0] & (S - 1))
        first = lax.broadcasted_iota(I32, (16, 128), 0) == 0

        def pick(ref, k):
            a = ref[pl.ds(i1, 1), :]
            b = ref[pl.ds(i2, 1), :]
            return jnp.where(_lanes(first, k), a, b)

        hs = pick(h_v, G)
        xs = ((hs - _lanes(pick(mu_v, 1), G)) * _lanes(pick(rs_v, 1), G)).astype(BF16)

        nfc = F // FC
        xu = _pk(xs)
        y = None
        a_prev = None
        gate = None
        for c in range(nfc + 1):
            if c < nfc:
                xc = _unpk(jnp.concatenate([xu[:, 0:128] | gate, xu[:, 128:]], axis=1)) if c == 3 else xs
                gt = _rb(_dot(xc, wg_v[:, c * FC:(c + 1) * FC]))
                ut = _rb(_dot(xc, wu_v[:, c * FC:(c + 1) * FC]))
            if c > 0:
                part = _dot(a_prev, wd_v[(c - 1) * FC:c * FC, 0:D])
                y = part if y is None else y + part
            if c in (0, 1):
                j, m_, r_ = (n2 - 2, mur_p, rs_p) if c == 0 else (n2 - 1, mur_l, rs_l)
                back = write_out(j, _tie(m_, _pace(gt[0:8], p2_tiles[j] // 8)), r_)
                gate = _fold(back) if gate is None else gate | _fold(back)
                if c == 1:
                    out_v[S:S + 16, 0:128] = gt[:, 0:128].astype(BF16)
                    gate = gate | _fold(out_v[S:S + 16, 0:128].astype(F32))
            if c < nfc:
                gt = _rb(gt * _recip(1.0 + jnp.exp(-gt)))
                a_prev = (gt * ut).astype(BF16)
        mono = lax.shift_right_logical(jnp.where(first, k1, k2) - KEY0, 11)
        rsel = pltpu.bitcast(jnp.where(mono < 0x8000, 0xFFFF - mono, mono & 0x7FFF) << 16, F32)
        y = _rb(_rb(y) * _lanes(_rb(jax.nn.sigmoid(rsel)), G))
        new = hs + _rb(xs.astype(F32) + y)

        g1 = pl.multiple_of(lax.shift_right_logical(i1, 4) * 16, 16)
        g2 = pl.multiple_of(lax.shift_right_logical(i2, 4) * 16, 16)
        rows = lax.broadcasted_iota(I32, (16, D), 0)
        for j, g in enumerate((g1, g2)):
            old = out_v[pl.ds(g, 16), :].astype(F32)
            fix_v[j] = jnp.where(rows == i1 - g, new[0:1], jnp.where(rows == i2 - g, new[1:2], old)).astype(BF16)
        pltpu.make_async_copy(out_v.at[pl.ds(0, S)], out_hbm, sems.at[SO]).wait()
        c1 = pltpu.make_async_copy(fix_v.at[0], out_hbm.at[pl.ds(g1, 16)], sems.at[SO + 1])
        c2 = pltpu.make_async_copy(fix_v.at[1], out_hbm.at[pl.ds(g2, 16)], sems.at[SO + 2])
        c1.start()

        @pl.when(g1 != g2)
        def _():
            c2.start()
            c2.wait()
        c1.wait()
        sc.__exit__(None, None, None)

    scratch = [
        pltpu.VMEM((S, D + PAD), BF16),
        pltpu.VMEM((D, 3 * D + PAD), BF16),
        pltpu.VMEM((D, D + PAD), BF16),
        pltpu.VMEM((D, F), BF16),
        pltpu.VMEM((D, F), BF16),
        pltpu.VMEM((F, D + PAD), BF16),
        pltpu.VMEM((D,), BF16),
        pltpu.VMEM((S // 2, D), U32),
        pltpu.VMEM((S, 128), F32),
        pltpu.VMEM((S, 128), F32),
        pltpu.VMEM((n1, D // 2, T1), U32),
        pltpu.VMEM((D, D), F32),
        pltpu.VMEM((8, D), F32),
        pltpu.VMEM((D // 2, D), U32),
        pltpu.VMEM((S + 16, D), BF16),
        pltpu.VMEM((S, D), F32),
        pltpu.VMEM((2, 16, D), BF16),
        pltpu.SemaphoreType.DMA((NSEM,)),
    ]

    @jax.jit
    def f(A_x, A_wqkv, A_wo, B_x, B_w_r, B_w_gate, B_w_up, B_w_down):
        any_spec = pl.BlockSpec(memory_space=pl.ANY)
        out = pl.pallas_call(
            kernel,
            out_shape=jax.ShapeDtypeStruct((S, D), BF16),
            in_specs=[any_spec] * 7,
            out_specs=any_spec,
            scratch_shapes=scratch,
            compiler_params=pltpu.CompilerParams(vmem_limit_bytes=100 * 1024 * 1024, disable_bounds_checks=True),
        )(A_x.reshape(S, D), A_wqkv, A_wo, B_w_r, B_w_gate, B_w_up, B_w_down)
        return out.reshape(1, S, D)
    return f


_impl = make_kernel(PT=1)


@jax.jit
def pallas_sequential_preLN__linear_attn_block__moe_arch_mod__prompt_kernel(
    A_x: jax.Array,
    A_wqkv: jax.Array,
    A_wo: jax.Array,
    B_x: jax.Array,
    B_w_r: jax.Array,
    B_w_gate: jax.Array,
    B_w_up: jax.Array,
    B_w_down: jax.Array,
):
    return _impl(A_x, A_wqkv, A_wo, B_x, B_w_r, B_w_gate, B_w_up, B_w_down)
```

```python
import contextlib

import jax
import jax.numpy as jnp
from jax import lax
import jax.experimental.pallas as pl
import jax.experimental.pallas.tpu as pltpu

S, D, F, H, DH = 2048, 1024, 3584, 32, 32
G = D // 128
F32 = jnp.float32
BF16 = jnp.bfloat16
I32 = jnp.int32
U32 = jnp.uint32
KEY0 = 64 << 23
PAD = 128


def _rb(x):
    return x.astype(BF16).astype(F32)


def _zero_of(x):
    bits = pltpu.bitcast(x, U32)
    return lax.shift_right_logical(lax.shift_right_logical(bits, U32(31)), U32(1))


def _pace(dep, n, lo=0.0, hi=1.0):
    if isinstance(dep, (list, tuple)):
        dep = jnp.concatenate(dep, axis=1)
    nrg, nch = dep.shape[0] // 8, dep.shape[1] // 128
    parts = []
    for p in range(n):
        pos = int((lo + (hi - lo) * p / n) * nch * nrg)
        c, rg = pos // nrg, pos % nrg
        parts.append(dep[rg * 8:(rg + 1) * 8, c * 128:(c + 1) * 128])
    return _zero_of(jnp.concatenate(parts, axis=0))


def _tie(x, zero):
    return pltpu.bitcast(pltpu.bitcast(x, U32) | zero, F32)


def _lanes(x, n):
    return jnp.concatenate([x] * n, axis=1) if n > 1 else x


def _rowsum(x):
    return jnp.broadcast_to(jnp.sum(x, axis=-1, keepdims=True), (x.shape[0], 128))


def _recip(d):
    r = pl.reciprocal(d, approx=True)
    return r * (2.0 - d * r)


def _rstd(var):
    v = _rb(_rb(var) + 1e-5)
    return _recip(_rb(v * lax.rsqrt(v)))


def _phi(t):
    return jnp.where(t > 0, t + 1.0, jnp.exp(t)) + 1e-6


def _dot(a, b):
    return jnp.dot(a, b, preferred_element_type=F32)


def _dot_tn(a, b):
    return lax.dot_general(a, b, (((0,), (0,)), ((), ())), preferred_element_type=F32)


def _pk(x):
    return pltpu.bitcast(x, U32)


def _unpk(x):
    return pltpu.bitcast(x, BF16)


def _gate(xu, zero):
    if zero is None:
        return xu
    top = jnp.concatenate([xu[0:8, 0:128] | zero, xu[0:8, 128:]], axis=1)
    return jnp.concatenate([top, xu[8:]], axis=0)


def _fold(x):
    x = pltpu.bitcast(x, U32) if x.dtype != U32 else x
    parts = [x[r:r + 8, c:c + 128] for r in range(0, x.shape[0], 8) for c in range(0, x.shape[1], 128)]
    while len(parts) > 1:
        parts = [parts[j] | parts[j + 1] if j + 1 < len(parts) else parts[j] for j in range(0, len(parts), 2)]
    return _zero_of(parts[0])


def _passes(xu, w, ntiles, gate_fn=None, post=None):
    deps, outs = [], []
    for c in range(ntiles):
        acc = None
        for hh in range(2):
            z = None if gate_fn is None else gate_fn(2 * c + hh, deps)
            lhs = _unpk(_gate(xu[:, hh * (D // 2):(hh + 1) * (D // 2)], z))
            part = _dot(lhs, w(hh * (D // 2), (hh + 1) * (D // 2), c))
            acc = part if acc is None else acc + part
            deps.append(acc)
        outs.append(acc if post is None else post(c, acc))
    return outs, deps


def make_kernel(P2T="256,256,256,256,256,256,256,128,64,64", FC=512, CHI=80, KCH="256,256,512", XP="128,128,256", PHI=85, NAG=4, CLAST=50, CGATE=13, SLAG=4, LAT=560, PRI="p0", PT=1, FC0=512, scopes=0):
    T1 = 512
    p2_tiles = [int(t) for t in P2T.split(",")]
    assert sum(p2_tiles) == S
    p2_off = [sum(p2_tiles[:i]) for i in range(len(p2_tiles))]
    n1 = S // T1
    n2 = len(p2_tiles)
    HT = T1 // 2
    KC, QC, VC = 0, D, 2 * D
    kch = [int(t) for t in KCH.split(",")]
    NKC = len(kch)
    wch = [(D + sum(kch[:j]), KC + sum(kch[:j]), kch[j]) for j in range(NKC)] + [(0, QC, D), (2 * D, VC, D)]
    xp = [int(t) for t in XP.split(",")]
    assert sum(xp) == T1 and len(xp) == NKC
    SW = len(xp)
    SX = SW + len(wch)
    SWO = SX + n1 - 1
    SWG, SWU, SWD, SWR = SWO + 1, SWO + 2, SWO + 3, SWO + 4
    SO = SWR + 1
    NSEM = SO + 3

    def scope(name):
        return jax.named_scope(name) if scopes else contextlib.nullcontext()

    def kernel(x_hbm, wqkv_hbm, wo_hbm, wr_hbm, wg_hbm, wu_hbm, wd_hbm, out_hbm,
               x_v, wqkv_v, wo_v, wg_v, wu_v, wd_v, wr_v, xn_v, mu_v, rs_v, pqt_v, g_v, z_v,
               m_v, out_v, h_v, fix_v, sems):

        def rows_copy(r0, n, s):
            return pltpu.make_async_copy(x_hbm.at[pl.ds(r0, n)], x_v.at[pl.ds(r0, n), pl.ds(0, D)], sems.at[s])

        x0 = [rows_copy(sum(xp[:j]), xp[j], j) for j in range(NKC)]
        xcp = [rows_copy(i * T1, T1, SX + i - 1) for i in range(1, n1)]
        wcp = [pltpu.make_async_copy(wqkv_hbm.at[:, pl.ds(c0, n)], wqkv_v.at[:, pl.ds(d0, n)], sems.at[SW + j])
               for j, (c0, d0, n) in enumerate(wch)]
        wo_copy = pltpu.make_async_copy(wo_hbm, wo_v.at[:, pl.ds(0, D)], sems.at[SWO])
        wg_copy = pltpu.make_async_copy(wg_hbm, wg_v, sems.at[SWG])
        wu_copy = pltpu.make_async_copy(wu_hbm, wu_v, sems.at[SWU])
        wd_copy = pltpu.make_async_copy(wd_hbm, wd_v.at[:, pl.ds(0, D)], sems.at[SWD])
        wr_copy = pltpu.make_async_copy(wr_hbm, wr_v, sems.at[SWR])

        def out_copy(i):
            return pltpu.make_async_copy(out_v.at[pl.ds(p2_off[i], p2_tiles[i])],
                                         out_hbm.at[pl.ds(p2_off[i], p2_tiles[i])], sems.at[SO])

        order = [c for j in range(NKC) for c in (x0[j], wcp[j])] + [wcp[NKC]] + xcp + [wcp[NKC + 1], wr_copy, wo_copy, wg_copy, wu_copy, wd_copy]
        pri = [int(ch) for ch in PRI[1:]]
        for j, c in enumerate(order):
            c.start(priority=pri[j] if j < len(pri) else pri[-1])

        def proj(r0, t, c0, n):
            return _dot(_unpk(xn_v[r0 // 2:(r0 + t) // 2, :]), wqkv_v[:, c0:c0 + n])

        def feat(y):
            return _phi(y).astype(BF16)

        def prep(r0, t, zero=None):
            xf = x_v[r0:r0 + t, 0:D].astype(F32)
            if zero is not None:
                xf = jnp.concatenate([_tie(xf[:, 0:128], zero), xf[:, 128:]], axis=1)
            mu = _rowsum(xf) * (1.0 / D)
            mur = _rb(mu)
            mu_v[r0:r0 + t, :] = mur
            xc = x_v[r0:r0 + t, 0:D].astype(F32) - _lanes(mu, G)
            rs = _rstd(_rowsum(xc * xc) * (1.0 / D))
            rs_v[r0:r0 + t, :] = rs
            xn = (x_v[r0:r0 + t, 0:D].astype(F32) - _lanes(mur, G)) * _lanes(rs, G)
            xu = _pk(xn.astype(BF16))
            xn_v[r0 // 2:(r0 + t) // 2, :] = xu
            return xu

        def g_piece(pk, r0, c0, pkt=None):
            t, n = pk.shape
            upd = _dot(pk.T if pkt is None else pkt, _unpk(xn_v[r0 // 2:(r0 + t) // 2, :]))
            zs = jnp.sum(pk.astype(F32).reshape(t // 8, 8, n), axis=0)
            if r0 == 0:
                g_v[c0:c0 + n, :] = upd
                z_v[:, c0:c0 + n] = zs
            else:
                g_v[c0:c0 + n, :] += upd
                z_v[:, c0:c0 + n] += zs
            return upd

        def g_update(pk, i):
            return g_piece(pk, i * T1, 0)

        def q_part(i):
            acc = proj(i * T1, T1, QC, D)
            pqt_v[i] = _pk(feat(acc).T)
            return acc

        def k_part(i):
            return feat(proj(i * T1, T1, KC, D))

        def wait(c, name):
            with scope(name):
                c.wait()

        pending = None
        rows = cols = 0
        for j in range(NKC):
            wait(x0[j], "w_x%d" % j)
            if pending is not None:
                g_piece(*pending)
                pending = None
            prep(rows, xp[j])
            if cols:
                pending = (feat(proj(rows, xp[j], KC, cols)), rows, 0)
            rows += xp[j]
            wait(wcp[j], "w_c%d" % j)
            pk = feat(proj(0, rows, KC + cols, kch[j]))
            if pending is not None:
                g_piece(*pending)
            pending = (pk, 0, cols, pk.T if j >= PT else None)
            cols += kch[j]
        g_piece(*pending)

        with scope("p1_mid"):
            wcp[NKC].wait()
            for c in xcp:
                c.wait()
            prep(T1, T1, _pace(q_part(0), T1 // 8, 0.0, PHI / 100))
            for i in range(1, n1 - 1):
                pk = k_part(i)
                q_part(i)
                prep((i + 1) * T1, T1, _pace(g_update(pk, i), T1 // 8, 0.0, PHI / 100))

        sc = scope("p2")
        sc.__enter__()
        wcp[NKC + 1].wait()
        wr_copy.wait()
        wo_copy.wait()
        for c in (wg_copy, wu_copy, wd_copy):
            c.wait()

        g_last = g_update(k_part(n1 - 1), n1 - 1)

        z = _rb(jnp.sum(z_v[...], axis=0, keepdims=True))
        zc = jnp.concatenate(
            [jnp.broadcast_to(z[:, g * 128:(g + 1) * 128], (128, 128)).T for g in range(G)], axis=0)
        wr = wr_v[...].astype(F32).reshape(1, D)
        wr_sum = _rowsum(wr)

        def stage_a(r0, t, zero):
            k = t // 128
            pqt = _unpk(pqt_v[r0 // T1, :, r0 % T1:r0 % T1 + t]).astype(F32)
            z4 = zc.reshape(H, DH // 8, 8, 128)
            z0 = _tie(z4[:, 0].reshape(H * 8, 128), zero).reshape(H, 1, 8, 128)
            zz = jnp.concatenate([z0, z4[:, 1:]], axis=1).reshape(D, 128)
            w = (pqt * _lanes(zz, k)).reshape(H, DH // 8, 8, t)
            den = jnp.sum(jnp.sum(w, axis=1), axis=1, keepdims=True) + 1e-6
            o = pqt.reshape(H, DH, t) * _recip(den)
            return _pk(o.reshape(D, t).astype(BF16).T)

        def m_tile(a, b, c):
            return _unpk(m_v[a // 2:b // 2, c * 128:(c + 1) * 128])

        def stage_b(i, gate):
            r0, t = p2_off[i], p2_tiles[i]

            def post(c, attn):
                h_v[r0:r0 + t, c * 128:(c + 1) * 128] = x_v[r0:r0 + t, c * 128:(c + 1) * 128].astype(F32) + attn

            _, deps = _passes(jnp.concatenate(os, axis=0)[r0 // 2:(r0 + t) // 2, :], m_tile, G,
                              lambda p, deps: gate if p == 0 else None, post)
            return deps, _rowsum(h_v[r0:r0 + t, :]) * (1.0 / D)

        def keys_of(r, idx):
            bits = pltpu.bitcast(jnp.where(r == 0.0, 0.0, r), I32)
            hi = lax.shift_right_logical(bits, 16)
            mono = jnp.where(bits < 0, 0xFFFF - hi, hi | 0x8000)
            return pltpu.bitcast((mono << 11) + (KEY0 + S - 1 - idx), F32)

        def merge(top, k1, k2):
            if top is None:
                return k1, k2
            t1, t2 = top
            return jnp.maximum(t1, k1), jnp.maximum(jnp.minimum(t1, k1), jnp.maximum(t2, k2))

        def write_out(i, mur, rs):
            r0, t = p2_off[i], p2_tiles[i]
            out_v[r0:r0 + t, :] = (h_v[r0:r0 + t, :] * _lanes(1.0 + rs, G) - _lanes(mur * rs, G)).astype(BF16)
            back = out_v[r0:r0 + t, D - 128:D].astype(F32)
            out_copy(i).start()
            return back

        def stage_c(i, mu, dep, hi=CHI / 100):
            r0, t = p2_off[i], p2_tiles[i]
            mu = _tie(mu, _pace(dep, t // 8, 0.0, hi))
            d = h_v[r0:r0 + t, :] - _lanes(mu, G)
            rs = _rstd(_rowsum(d * d) * (1.0 / D))
            mur = _rb(mu)
            r = _rb((_rowsum(d * wr) + (mu - mur) * wr_sum) * rs)
            mu_v[r0:r0 + t, :] = mur
            rs_v[r0:r0 + t, :] = rs
            return r, mur, rs

        lane = lax.broadcasted_iota(I32, (8, 128), 1)
        sub = lax.broadcasted_iota(I32, (8, 128), 0)

        def compact(i, r):
            r0, t = p2_off[i], p2_tiles[i]
            parts = [r[p * 8:(p + 1) * 8] for p in range(t // 8)]
            acc = parts[0]
            for p in range(1, t // 8):
                acc = jnp.where(lane == p, parts[p], acc)
            key = keys_of(acc, r0 + lane * 8 + sub)
            return jnp.where(lane < t // 8, key, 0.0)

        def a_done(os):
            acc = None
            for o in os:
                for rb in range(o.shape[0] // 64):
                    row = o[rb * 64 + 56:rb * 64 + 64, :]
                    for g in range(G):
                        v = row[:, g * 128:(g + 1) * 128]
                        acc = v if acc is None else acc | v
            return _zero_of(acc)

        ta = 256
        na = S // ta
        nearly = (S - T1) // ta
        pz = _pace(g_last, NAG * H, 0.0, 1.0)
        os = [stage_a(j * ta, ta, pz[j * H * 8:(j + 1) * H * 8]) for j in range(NAG)]
        accq = q_part(n1 - 1)
        if nearly > NAG:
            pz = _pace(accq, (nearly - NAG) * H, 0.0, 0.9)
            os += [stage_a(j * ta, ta, pz[(j - NAG) * H * 8:(j - NAG + 1) * H * 8]) for j in range(NAG, nearly)]

        row = lax.broadcasted_iota(I32, (128, 128), 0) // DH
        col = lax.broadcasted_iota(I32, (128, 128), 1) // DH
        same = row == col
        kvs = []
        for g in range(G):
            gg = g_v[g * 128:(g + 1) * 128, :]
            if g == 0:
                gg = jnp.concatenate([jnp.concatenate(
                    [_tie(gg[0:8, 0:128], a_done(os)), gg[0:8, 128:]], axis=1), gg[8:]], axis=0)
            kv = _dot(gg.astype(BF16), wqkv_v[:, VC + g * 128:VC + (g + 1) * 128])
            kvs.append(jnp.where(same, kv, 0.0).astype(BF16))
        for g in range(G):
            m_v[g * 64:(g + 1) * 64, :] = _pk(_dot(kvs[g], wo_v[g * 128:(g + 1) * 128, 0:D]).astype(BF16))

        def tree(i, r):
            t = p2_tiles[i]
            key = keys_of(r, lax.broadcasted_iota(I32, (t, 128), 0) + p2_off[i])
            level = [(key[p * 8:(p + 1) * 8], None) for p in range(t // 8)]
            while len(level) > 1:
                nxt = []
                for p in range(0, len(level) - 1, 2):
                    (a1, a2), (b1, b2) = level[p], level[p + 1]
                    lo = jnp.minimum(a1, b1)
                    for e in (a2, b2):
                        lo = lo if e is None else jnp.maximum(lo, e)
                    nxt.append((jnp.maximum(a1, b1), lo))
                if len(level) % 2:
                    nxt.append(level[-1])
                level = nxt
            return level[0]

        first = lax.broadcasted_iota(I32, (16, 128), 0) == 0

        def select(top):
            t1, t2 = top
            k1 = jnp.max(t1, axis=0, keepdims=True)
            k2 = jnp.max(jnp.where(t1 == k1, t2, t1), axis=0, keepdims=True)
            k1 = pltpu.bitcast(k1, I32)
            k2 = pltpu.bitcast(k2, I32)
            i1 = S - 1 - (k1[0, 0] & (S - 1))
            i2 = S - 1 - (k2[0, 0] & (S - 1))

            def pick(ref, k):
                return jnp.where(_lanes(first, k), ref[pl.ds(i1, 1), :], ref[pl.ds(i2, 1), :])

            hs = pick(h_v, G)
            xs = ((hs - _lanes(pick(mu_v, 1), G)) * _lanes(pick(rs_v, 1), G)).astype(BF16)
            return k1, k2, i1, i2, hs, xs

        def gate_up(xs, c0, n):
            return _rb(_dot(xs, wg_v[:, c0:c0 + n])), _rb(_dot(xs, wu_v[:, c0:c0 + n]))

        def act(gt, ut):
            return (_rb(gt * jax.nn.sigmoid(gt)) * ut).astype(BF16)

        def stage_last(gate, mu_prev, top):
            i = n2 - 1
            r0, t = p2_off[i], p2_tiles[i]
            st = {}

            def post(c, attn):
                h = x_v[r0:r0 + t, c * 128:(c + 1) * 128].astype(F32) + attn
                h_v[r0:r0 + t, c * 128:(c + 1) * 128] = h
                if c == 0:
                    st["shift"] = jnp.broadcast_to(h[:, 0:1], (t, 128))
                d = h - st["shift"]
                new = (d, d * d, d * wr[:, c * 128:(c + 1) * 128])
                st[c] = new if c == 0 else tuple(a + b for a, b in zip(st[c - 1], new))

            def gate_fn(p, deps):
                if p == 0:
                    return gate
                z = None
                if p % 2 == 1 and p // 2 - SLAG >= 0:
                    z = _fold(jnp.concatenate(st[p // 2 - SLAG], axis=1))
                if p == CGATE:
                    r, st["mur_p"], st["rs_p"] = stage_c(i - 1, mu_prev, deps, CLAST / 100)
                    st["top"] = merge(top, *tree(i - 1, r))
                    st["guess"] = select(st["top"])
                    zz = _zero_of(st["top"][0] + st["top"][1])
                    z = zz if z is None else z | zz
                return z

            _passes(jnp.concatenate(os, axis=0)[r0 // 2:(r0 + t) // 2, :], m_tile, G, gate_fn, post)
            st["a0"] = act(*gate_up(st["guess"][5], 0, FC0))
            s1, s2, s3 = st[G - 1]
            shift = st["shift"]
            m1 = _rowsum(s1) * (1.0 / D)
            var = jnp.maximum(_rowsum(s2) * (1.0 / D) - m1 * m1, 0.0)
            rs = _rstd(var)
            mur = _rb(shift + m1)
            r = _rb((_rowsum(s3) + (shift - mur) * wr_sum) * rs)
            mu_v[r0:r0 + t, :] = mur
            rs_v[r0:r0 + t, :] = rs
            return merge(st["top"], *tree(i, r)), st["mur_p"], st["rs_p"], mur, rs, st["guess"], st["a0"]

        top = None
        mu_prev = None
        gate = None
        for i in range(n2 - 1):
            deps, mu = stage_b(i, gate)
            if i == 0:
                pz = _pace(deps, (na - nearly) * H, 0.0, 0.8)
                late_os = [stage_a(j * ta, ta, pz[(j - nearly) * H * 8:(j - nearly + 1) * H * 8])
                           for j in range(nearly, na)]
                os += late_os
                gate = a_done(late_os)
            else:
                r, mur, rs = stage_c(i - 1, mu_prev, deps, min(CHI / 100, 1 - LAT / (16 * p2_tiles[i])))
                back = write_out(i - 1, mur, rs)
                key = compact(i - 1, r)
                top = merge(top, key, jnp.zeros_like(key))
                gate = _zero_of(key + jnp.sum(back.reshape(-1, 8, 128), axis=0))
                if i == n2 - 2:
                    t1, t2 = top
                    b1 = jnp.max(jnp.max(t1, axis=0, keepdims=True), axis=1, keepdims=True)
                    rest = jnp.where(t1 == b1, t2, t1)
                    b2 = jnp.max(jnp.max(rest, axis=0, keepdims=True), axis=1, keepdims=True)
                    top = (jnp.where(sub == 0, b1, 0.0), jnp.where(sub == 0, b2, 0.0))
            mu_prev = mu
        top, mur_p, rs_p, mur_l, rs_l, guess, a0 = stage_last(gate, mu_prev, top)
        sc.__exit__(None, None, None)

        sc = scope("tail")
        sc.__enter__()
        k1, k2, i1, i2, hs, xs = select(top)
        chunks = [(c0, min(FC, F - c0)) for c0 in range(FC0, F, FC)]
        xu = _pk(xs)
        y = None
        prev = None
        gate = None
        for c, ch in enumerate(chunks + [None]):
            if ch is not None:
                xc = _unpk(jnp.concatenate([xu[:, 0:128] | gate, xu[:, 128:]], axis=1)) if c == 3 else xs
                gt, ut = gate_up(xc, *ch)
            if c == 0:
                y0 = _dot(a0, wd_v[0:FC0, 0:D])
            if prev is not None:
                part = _dot(a_prev, wd_v[prev[0]:prev[0] + prev[1], 0:D])
                y = part if y is None else y + part
            if c in (0, 1):
                j, m_, r_ = (n2 - 2, mur_p, rs_p) if c == 0 else (n2 - 1, mur_l, rs_l)
                back = write_out(j, _tie(m_, _pace(gt[0:8], p2_tiles[j] // 8)), r_)
                gate = _fold(back) if gate is None else gate | _fold(back)
                if c == 1:
                    out_v[S:S + 16, 0:128] = gt[:, 0:128].astype(BF16)
                    gate = gate | _fold(out_v[S:S + 16, 0:128].astype(F32))
            if ch is not None:
                a_prev = act(gt, ut)
            prev = ch
        mono = lax.shift_right_logical(jnp.where(first, k1, k2) - KEY0, 11)
        rsel = pltpu.bitcast(jnp.where(mono < 0x8000, 0xFFFF - mono, mono & 0x7FFF) << 16, F32)
        gain = _lanes(_rb(jax.nn.sigmoid(rsel)), G)
        g1 = pl.multiple_of(lax.shift_right_logical(i1, 4) * 16, 16)
        g2 = pl.multiple_of(lax.shift_right_logical(i2, 4) * 16, 16)
        rows = lax.broadcasted_iota(I32, (16, D), 0)

        def finish(y):
            new = hs + _rb(xs.astype(F32) + _rb(_rb(y) * gain))
            for j, g in enumerate((g1, g2)):
                old = out_v[pl.ds(g, 16), :].astype(F32)
                fix_v[j] = jnp.where(rows == i1 - g, new[0:1], jnp.where(rows == i2 - g, new[1:2], old)).astype(BF16)

        finish(y + y0)

        @pl.when(jnp.logical_or(i1 != guess[2], i2 != guess[3]))
        def _():
            finish(y + _dot(act(*gate_up(xs, 0, FC0)), wd_v[0:FC0, 0:D]))

        pltpu.make_async_copy(out_v.at[pl.ds(0, S)], out_hbm, sems.at[SO]).wait()
        c1 = pltpu.make_async_copy(fix_v.at[0], out_hbm.at[pl.ds(g1, 16)], sems.at[SO + 1])
        c2 = pltpu.make_async_copy(fix_v.at[1], out_hbm.at[pl.ds(g2, 16)], sems.at[SO + 2])
        c1.start()

        @pl.when(g1 != g2)
        def _():
            c2.start()
            c2.wait()
        c1.wait()
        sc.__exit__(None, None, None)

    scratch = [
        pltpu.VMEM((S, D + PAD), BF16),
        pltpu.VMEM((D, 3 * D + PAD), BF16),
        pltpu.VMEM((D, D + PAD), BF16),
        pltpu.VMEM((D, F), BF16),
        pltpu.VMEM((D, F), BF16),
        pltpu.VMEM((F, D + PAD), BF16),
        pltpu.VMEM((D,), BF16),
        pltpu.VMEM((S // 2, D), U32),
        pltpu.VMEM((S, 128), F32),
        pltpu.VMEM((S, 128), F32),
        pltpu.VMEM((n1, D // 2, T1), U32),
        pltpu.VMEM((D, D), F32),
        pltpu.VMEM((8, D), F32),
        pltpu.VMEM((D // 2, D), U32),
        pltpu.VMEM((S + 16, D), BF16),
        pltpu.VMEM((S, D), F32),
        pltpu.VMEM((2, 16, D), BF16),
        pltpu.SemaphoreType.DMA((NSEM,)),
    ]

    @jax.jit
    def f(A_x, A_wqkv, A_wo, B_x, B_w_r, B_w_gate, B_w_up, B_w_down):
        any_spec = pl.BlockSpec(memory_space=pl.ANY)
        out = pl.pallas_call(
            kernel,
            out_shape=jax.ShapeDtypeStruct((S, D), BF16),
            in_specs=[any_spec] * 7,
            out_specs=any_spec,
            scratch_shapes=scratch,
            compiler_params=pltpu.CompilerParams(vmem_limit_bytes=100 * 1024 * 1024, disable_bounds_checks=True),
        )(A_x.reshape(S, D), A_wqkv, A_wo, B_w_r, B_w_gate, B_w_up, B_w_down)
        return out.reshape(1, S, D)
    return f


_impl = make_kernel()


@jax.jit
def pallas_sequential_preLN__linear_attn_block__moe_arch_mod__prompt_kernel(
    A_x: jax.Array,
    A_wqkv: jax.Array,
    A_wo: jax.Array,
    B_x: jax.Array,
    B_w_r: jax.Array,
    B_w_gate: jax.Array,
    B_w_up: jax.Array,
    B_w_down: jax.Array,
):
    return _impl(A_x, A_wqkv, A_wo, B_x, B_w_r, B_w_gate, B_w_up, B_w_down)
```

```python
import contextlib

import jax
import jax.numpy as jnp
from jax import lax
import jax.experimental.pallas as pl
import jax.experimental.pallas.tpu as pltpu

S, D, F, H, DH = 2048, 1024, 3584, 32, 32
G = D // 128
F32 = jnp.float32
BF16 = jnp.bfloat16
I32 = jnp.int32
U32 = jnp.uint32
KEY0 = 64 << 23
PAD = 128


def _rb(x):
    return x.astype(BF16).astype(F32)


def _zero_of(x):
    bits = pltpu.bitcast(x, U32)
    return lax.shift_right_logical(lax.shift_right_logical(bits, U32(31)), U32(1))


def _pace(dep, n, lo=0.0, hi=1.0):
    if isinstance(dep, (list, tuple)):
        dep = jnp.concatenate(dep, axis=1)
    nrg, nch = dep.shape[0] // 8, dep.shape[1] // 128
    parts = []
    for p in range(n):
        pos = int((lo + (hi - lo) * p / n) * nch * nrg)
        c, rg = pos // nrg, pos % nrg
        parts.append(dep[rg * 8:(rg + 1) * 8, c * 128:(c + 1) * 128])
    return _zero_of(jnp.concatenate(parts, axis=0))


def _tie(x, zero):
    return pltpu.bitcast(pltpu.bitcast(x, U32) | zero, F32)


def _lanes(x, n):
    return jnp.concatenate([x] * n, axis=1) if n > 1 else x


def _rowsum(x):
    return jnp.broadcast_to(jnp.sum(x, axis=-1, keepdims=True), (x.shape[0], 128))


def _recip(d):
    r = pl.reciprocal(d, approx=True)
    return r * (2.0 - d * r)


def _rstd(var):
    v = _rb(_rb(var) + 1e-5)
    return _recip(_rb(v * lax.rsqrt(v)))


def _phi(t):
    return jnp.where(t > 0, t + 1.0, jnp.exp(t)) + 1e-6


def _dot(a, b):
    return jnp.dot(a, b, preferred_element_type=F32)


def _dot_tn(a, b):
    return lax.dot_general(a, b, (((0,), (0,)), ((), ())), preferred_element_type=F32)


def _pk(x):
    return pltpu.bitcast(x, U32)


def _unpk(x):
    return pltpu.bitcast(x, BF16)


def _gate(xu, zero):
    if zero is None:
        return xu
    top = jnp.concatenate([xu[0:8, 0:128] | zero, xu[0:8, 128:]], axis=1)
    return jnp.concatenate([top, xu[8:]], axis=0)


def _fold(x):
    x = pltpu.bitcast(x, U32) if x.dtype != U32 else x
    parts = [x[r:r + 8, c:c + 128] for r in range(0, x.shape[0], 8) for c in range(0, x.shape[1], 128)]
    while len(parts) > 1:
        parts = [parts[j] | parts[j + 1] if j + 1 < len(parts) else parts[j] for j in range(0, len(parts), 2)]
    return _zero_of(parts[0])


def _passes(xu, w, ntiles, gate_fn=None, post=None):
    deps, outs = [], []
    for c in range(ntiles):
        acc = None
        for hh in range(2):
            z = None if gate_fn is None else gate_fn(2 * c + hh, deps)
            lhs = _unpk(_gate(xu[:, hh * (D // 2):(hh + 1) * (D // 2)], z))
            part = _dot(lhs, w(hh * (D // 2), (hh + 1) * (D // 2), c))
            acc = part if acc is None else acc + part
            deps.append(acc)
        outs.append(acc if post is None else post(c, acc))
    return outs, deps


def make_kernel(P2T="256,256,256,256,256,256,256,128,64,64", FC=512, CHI=80, KCH="256,256,512", XP="128,128,256", PHI=85, NAG=4, CLAST=50, CGATE=13, SLAG=4, LAT=560, PRI="p0", PT=1, FC0=512, FV=768, VHI=95, VLEAD=512, XLEAD=16, WOC=1, scopes=0):
    T1 = 512
    p2_tiles = [int(t) for t in P2T.split(",")]
    assert sum(p2_tiles) == S
    p2_off = [sum(p2_tiles[:i]) for i in range(len(p2_tiles))]
    n1 = S // T1
    FM = F - FV
    n2 = len(p2_tiles)
    HT = T1 // 2
    KC, QC, VC = 0, D, 2 * D
    kch = [int(t) for t in KCH.split(",")]
    NKC = len(kch)
    wch = [(D + sum(kch[:j]), KC + sum(kch[:j]), kch[j]) for j in range(NKC)] + [(0, QC, D), (2 * D, VC, D)]
    xp = [int(t) for t in XP.split(",")]
    assert sum(xp) == T1 and len(xp) == NKC
    SW = len(xp)
    SX = SW + len(wch)
    SWO = SX + n1 - 1
    SWG, SWU, SWD, SWR = SWO + 1, SWO + 2, SWO + 3, SWO + 4
    SO = SWR + 1
    NSEM = SO + 3

    def scope(name):
        return jax.named_scope(name) if scopes else contextlib.nullcontext()

    def kernel(x_hbm, wqkv_hbm, wo_hbm, wr_hbm, wg_hbm, wu_hbm, wd_hbm, out_hbm,
               x_v, wqkv_v, wo_v, wg_v, wu_v, wd_v, wr_v, mu_v, rs_v,
               out_v, h_v, fix_v, wg_p, wu_p, wd_p, sems):

        xn_rows = {}
        pqt = {}
        g_acc = {}
        z_acc = {}
        m_rows = []

        def xn_at(r0, t):
            keys = sorted(k for k in xn_rows if r0 <= k < r0 + t)
            return jnp.concatenate([xn_rows[k] for k in keys], axis=0) if len(keys) > 1 else xn_rows[keys[0]]

        def rows_copy(r0, n, s):
            return pltpu.make_async_copy(x_hbm.at[pl.ds(r0, n)], x_v.at[pl.ds(r0, n), pl.ds(0, D)], sems.at[s])

        x0 = [rows_copy(sum(xp[:j]), xp[j], j) for j in range(NKC)]
        xcp = [rows_copy(i * T1, T1, SX + i - 1) for i in range(1, n1)]
        wcp = [pltpu.make_async_copy(wqkv_hbm.at[:, pl.ds(c0, n)], wqkv_v.at[:, pl.ds(d0, n)], sems.at[SW + j])
               for j, (c0, d0, n) in enumerate(wch)]
        wo_copy = pltpu.make_async_copy(wo_hbm, wo_v.at[:, pl.ds(0, D)], sems.at[SWO])
        wg_copy = pltpu.make_async_copy(wg_hbm, wg_v, sems.at[SWG])
        wu_copy = pltpu.make_async_copy(wu_hbm, wu_v, sems.at[SWU])
        wd_copy = pltpu.make_async_copy(wd_hbm, wd_v.at[:, pl.ds(0, D)], sems.at[SWD])
        wr_copy = pltpu.make_async_copy(wr_hbm, wr_v, sems.at[SWR])

        def out_copy(i):
            return pltpu.make_async_copy(out_v.at[pl.ds(p2_off[i], p2_tiles[i])],
                                         out_hbm.at[pl.ds(p2_off[i], p2_tiles[i])], sems.at[SO])

        order = [c for j in range(NKC) for c in (x0[j], wcp[j])] + [wcp[NKC]] + xcp + [wcp[NKC + 1], wr_copy, wo_copy, wg_copy, wu_copy, wd_copy]
        pri = [int(ch) for ch in PRI[1:]]
        for j, c in enumerate(order):
            c.start(priority=pri[j] if j < len(pri) else pri[-1])

        def proj(r0, t, c0, n):
            return _dot(_unpk(xn_at(r0, t)), wqkv_v[:, c0:c0 + n])

        def feat(y):
            return _phi(y).astype(BF16)

        def prep(r0, t, zero=None):
            xf = x_v[r0:r0 + t, 0:D].astype(F32)
            if zero is not None:
                xf = jnp.concatenate([_tie(xf[:, 0:128], zero), xf[:, 128:]], axis=1)
            mu = _rowsum(xf) * (1.0 / D)
            mur = _rb(mu)
            mu_v[r0:r0 + t, :] = mur
            xc = x_v[r0:r0 + t, 0:D].astype(F32) - _lanes(mu, G)
            rs = _rstd(_rowsum(xc * xc) * (1.0 / D))
            rs_v[r0:r0 + t, :] = rs
            xn = (x_v[r0:r0 + t, 0:D].astype(F32) - _lanes(mur, G)) * _lanes(rs, G)
            xu = _pk(xn.astype(BF16))
            xn_rows[r0] = xu
            return xu

        def g_piece(pk, r0, c0, pkt=None):
            t, n = pk.shape
            upd = _dot(pk.T if pkt is None else pkt, _unpk(xn_at(r0, t)))
            zs = jnp.sum(pk.astype(F32).reshape(t // 8, 8, n), axis=0)
            for c in range(0, n, 128):
                b = (c0 + c) // 128
                g_acc[b] = upd[c:c + 128] if r0 == 0 else g_acc[b] + upd[c:c + 128]
                z_acc[b] = zs[:, c:c + 128] if r0 == 0 else z_acc[b] + zs[:, c:c + 128]
            return upd

        def g_update(pk, i):
            return g_piece(pk, i * T1, 0)

        def q_part(i, gate=None):
            acc = _dot(_unpk(_gate(xn_at(i * T1, T1), gate)), wqkv_v[:, QC:QC + D])
            pqt[i] = _pk(feat(acc).T)
            return acc

        def k_part(i):
            return feat(proj(i * T1, T1, KC, D))

        def wait(c, name):
            with scope(name):
                c.wait()

        pending = None
        rows = cols = 0
        for j in range(NKC):
            wait(x0[j], "w_x%d" % j)
            if pending is not None:
                g_piece(*pending)
                pending = None
            prep(rows, xp[j])
            if cols:
                pending = (feat(proj(rows, xp[j], KC, cols)), rows, 0)
            rows += xp[j]
            wait(wcp[j], "w_c%d" % j)
            pk = feat(proj(0, rows, KC + cols, kch[j]))
            if pending is not None:
                g_piece(*pending)
            pending = (pk, 0, cols, pk.T if j >= PT else None)
            cols += kch[j]
        g_piece(*pending)

        with scope("p1_mid"):
            wcp[NKC].wait()
            for c in xcp:
                c.wait()
            prep(T1, T1, _pace(q_part(0), T1 // 8, 0.0, PHI / 100))
            for i in range(1, n1 - 1):
                pk = k_part(i)
                q_part(i)
                prep((i + 1) * T1, T1, _pace(g_update(pk, i), T1 // 8, 0.0, PHI / 100))

        sc = scope("p2")
        sc.__enter__()
        wcp[NKC + 1].wait()
        wr_copy.wait()
        wo_copy.wait()
        for c in (wg_copy, wu_copy, wd_copy):
            c.wait()

        jobs = ([(src, dst, r, c, min(D, FM - c)) for src, dst in ((wg_v, wg_p), (wu_v, wu_p))
                 for r in range(0, D, 16) for c in range(0, FM, D)]
                + [(wd_v, wd_p, r, 0, D) for r in range(0, F, 16)])
        hosts = [2, 2, 2] + [1] * (n2 - 3)
        dyn0 = pltpu.bitcast(_zero_of(rs_v[0:8, :]), I32)[0, 0]

        def retile(h, deps):
            mine = jobs[len(jobs) * sum(hosts[:h]) // sum(hosts):len(jobs) * sum(hosts[:h + 1]) // sum(hosts)]
            pz = _pace(deps, len(mine), 0.0, 0.85)
            for k, (src, dst, r, c, n) in enumerate(mine):
                dst[r // 2:r // 2 + 8, c:c + n] = _pk(src[r:r + 16, c:c + n]) | _lanes(pz[k * 8:(k + 1) * 8], n // 128)
            done = None
            for dst in (wg_p, wu_p, wd_p):
                if any(j[1] is dst for j in mine):
                    r = max(j[2] for j in mine if j[1] is dst) // 2
                    c = min(j[3] for j in mine if j[1] is dst and j[2] // 2 == r)
                    v = dst[pl.ds(pl.multiple_of(r + dyn0, 8), 8), c:c + 128]
                    done = v if done is None else done | v
            return _zero_of(done)

        acck = proj((n1 - 1) * T1, T1, KC, D)
        pk = _unpk(_gate(_pk(feat(acck)), retile(0, acck)))
        g_last = g_update(pk, n1 - 1)

        z = _rb(jnp.sum(jnp.concatenate([z_acc[b] for b in range(G)], axis=1), axis=0, keepdims=True))
        zc = jnp.concatenate(
            [jnp.broadcast_to(z[:, g * 128:(g + 1) * 128], (128, 128)).T for g in range(G)], axis=0)
        wr = wr_v[...].astype(F32).reshape(1, D)
        wr_sum = _rowsum(wr)

        def stage_a(r0, t, zero):
            k = t // 128
            pq = _unpk(pqt[r0 // T1][:, r0 % T1:r0 % T1 + t]).astype(F32)
            z4 = zc.reshape(H, DH // 8, 8, 128)
            z0 = _tie(z4[:, 0].reshape(H * 8, 128), zero).reshape(H, 1, 8, 128)
            zz = jnp.concatenate([z0, z4[:, 1:]], axis=1).reshape(D, 128)
            w = (pq * _lanes(zz, k)).reshape(H, DH // 8, 8, t)
            den = jnp.sum(jnp.sum(w, axis=1), axis=1, keepdims=True) + 1e-6
            o = pq.reshape(H, DH, t) * _recip(den)
            return _pk(o.reshape(D, t).astype(BF16).T)

        def m_tile(a, b, c):
            return _unpk(jnp.concatenate(m_rows[a // 128:b // 128], axis=0)[:, c * 128:(c + 1) * 128])

        def stage_b(i, gate):
            r0, t = p2_off[i], p2_tiles[i]

            def post(c, attn):
                h_v[r0:r0 + t, c * 128:(c + 1) * 128] = x_v[r0:r0 + t, c * 128:(c + 1) * 128].astype(F32) + attn

            _, deps = _passes(jnp.concatenate(os, axis=0)[r0 // 2:(r0 + t) // 2, :], m_tile, G,
                              lambda p, deps: gate if p == 0 else None, post)
            return deps, _rowsum(h_v[r0:r0 + t, :]) * (1.0 / D)

        def keys_of(r, idx):
            bits = pltpu.bitcast(jnp.where(r == 0.0, 0.0, r), I32)
            hi = lax.shift_right_logical(bits, 16)
            mono = jnp.where(bits < 0, 0xFFFF - hi, hi | 0x8000)
            return pltpu.bitcast((mono << 11) + (KEY0 + S - 1 - idx), F32)

        def merge(top, k1, k2):
            if top is None:
                return k1, k2
            t1, t2 = top
            return jnp.maximum(t1, k1), jnp.maximum(jnp.minimum(t1, k1), jnp.maximum(t2, k2))

        def write_out(i, mur, rs):
            r0, t = p2_off[i], p2_tiles[i]
            out_v[r0:r0 + t, :] = (h_v[r0:r0 + t, :] * _lanes(1.0 + rs, G) - _lanes(mur * rs, G)).astype(BF16)
            back = out_v[r0:r0 + t, D - 128:D].astype(F32)
            out_copy(i).start()
            return back

        def stage_c(i, mu, dep, hi=CHI / 100):
            r0, t = p2_off[i], p2_tiles[i]
            mu = _tie(mu, _pace(dep, t // 8, 0.0, hi))
            d = h_v[r0:r0 + t, :] - _lanes(mu, G)
            rs = _rstd(_rowsum(d * d) * (1.0 / D))
            mur = _rb(mu)
            r = _rb((_rowsum(d * wr) + (mu - mur) * wr_sum) * rs)
            mu_v[r0:r0 + t, :] = mur
            rs_v[r0:r0 + t, :] = rs
            return r, mur, rs

        lane = lax.broadcasted_iota(I32, (8, 128), 1)
        sub = lax.broadcasted_iota(I32, (8, 128), 0)

        def compact(i, r):
            r0, t = p2_off[i], p2_tiles[i]
            parts = [r[p * 8:(p + 1) * 8] for p in range(t // 8)]
            acc = parts[0]
            for p in range(1, t // 8):
                acc = jnp.where(lane == p, parts[p], acc)
            key = keys_of(acc, r0 + lane * 8 + sub)
            return jnp.where(lane < t // 8, key, 0.0)

        def a_done(os):
            acc = None
            for o in os:
                for rb in range(o.shape[0] // 64):
                    row = o[rb * 64 + 56:rb * 64 + 64, :]
                    for g in range(G):
                        v = row[:, g * 128:(g + 1) * 128]
                        acc = v if acc is None else acc | v
            return _zero_of(acc)

        ta = 256
        na = S // ta
        nearly = (S - T1) // ta
        pz = _pace(g_last, NAG * H, 0.0, 1.0)
        os = [stage_a(j * ta, ta, pz[j * H * 8:(j + 1) * H * 8]) for j in range(NAG)]
        accq = q_part(n1 - 1, retile(1, g_last))
        if nearly > NAG:
            pz = _pace(accq, (nearly - NAG) * H, 0.0, 0.9)
            os += [stage_a(j * ta, ta, pz[(j - NAG) * H * 8:(j - NAG + 1) * H * 8]) for j in range(NAG, nearly)]

        row = lax.broadcasted_iota(I32, (128, 128), 0) // DH
        col = lax.broadcasted_iota(I32, (128, 128), 1) // DH
        same = row == col
        kvs = []
        for g in range(G):
            gg = g_acc[g]
            if g == 0:
                gg = jnp.concatenate([jnp.concatenate(
                    [_tie(gg[0:8, 0:128], a_done(os) | retile(2, accq)), gg[0:8, 128:]], axis=1), gg[8:]], axis=0)
            kv = _dot(gg.astype(BF16), wqkv_v[:, VC + g * 128:VC + (g + 1) * 128])
            kvs.append(jnp.where(same, kv, 0.0).astype(BF16))
        for g in range(G):
            m_rows.append(_pk(_dot(kvs[g], wo_v[g * 128:(g + 1) * 128, 0:D]).astype(BF16)))

        def tree(i, r):
            t = p2_tiles[i]
            key = keys_of(r, lax.broadcasted_iota(I32, (t, 128), 0) + p2_off[i])
            level = [(key[p * 8:(p + 1) * 8], None) for p in range(t // 8)]
            while len(level) > 1:
                nxt = []
                for p in range(0, len(level) - 1, 2):
                    (a1, a2), (b1, b2) = level[p], level[p + 1]
                    lo = jnp.minimum(a1, b1)
                    for e in (a2, b2):
                        lo = lo if e is None else jnp.maximum(lo, e)
                    nxt.append((jnp.maximum(a1, b1), lo))
                if len(level) % 2:
                    nxt.append(level[-1])
                level = nxt
            return level[0]

        first = lax.broadcasted_iota(I32, (16, 128), 0) == 0

        def select(top):
            t1, t2 = top
            k1 = jnp.max(t1, axis=0, keepdims=True)
            k2 = jnp.max(jnp.where(t1 == k1, t2, t1), axis=0, keepdims=True)
            k1 = pltpu.bitcast(k1, I32)
            k2 = pltpu.bitcast(k2, I32)
            i1 = S - 1 - (k1[0, 0] & (S - 1))
            i2 = S - 1 - (k2[0, 0] & (S - 1))

            def pick(ref, k):
                return jnp.where(_lanes(first, k), ref[pl.ds(i1, 1), :], ref[pl.ds(i2, 1), :])

            hs = pick(h_v, G)
            xs = ((hs - _lanes(pick(mu_v, 1), G)) * _lanes(pick(rs_v, 1), G)).astype(BF16)
            return k1, k2, i1, i2, hs, xs

        ticks = []

        def gate_up(xs, c0, n):
            gt = _dot(xs, _unpk(wg_p[:, c0:c0 + n]))
            ut = _dot(xs, _unpk(wu_p[:, c0:c0 + n]))
            ticks.extend((v[0:8, c:c + 128], 64) for v in (gt, ut) for c in range(0, n, 128))
            return _rb(gt[0:8]), _rb(ut[0:8])

        def down(a, c0):
            y = _dot(a, _unpk(wd_p[c0 // 2:(c0 + a.shape[1]) // 2, 0:D]))
            ticks.extend((y[0:8, c:c + 128], a.shape[1] // 16) for c in range(0, D, 128))
            return y

        def vpu_acts(xg, zeros):
            nd = D // 8
            xb = {}
            acts = []
            for j in range(FV // 256):
                c0 = FM + j * 256
                acc = {}
                for d in range(nd):
                    zero = zeros[j * nd + d]
                    if j == 0 and d % 16 == 0:
                        g = d // 16
                        zg = zeros[max(0, d - XLEAD)]
                        for t in range(2):
                            row = _tie(jnp.broadcast_to(xg[t:t + 1, g * 128:(g + 1) * 128], (8, 128)), zg)
                            blk = jnp.concatenate([row] * 16, axis=0).T
                            for e in range(16):
                                xb[t, d + e] = blk[e * 8:(e + 1) * 8]
                    xt = [_lanes(_tie(xb[t, d], zero), 2) for t in range(2)]
                    for m, w_v in enumerate((wg_v, wu_v)):
                        w = w_v[d * 8:(d + 1) * 8, c0:c0 + 256].astype(F32)
                        for t in range(2):
                            acc[m, t] = w * xt[t] if d == 0 else acc[m, t] + w * xt[t]
                res = [_rb(jnp.where(_lanes(first[0:8], 2), jnp.sum(acc[m, 0], axis=0, keepdims=True),
                                     jnp.sum(acc[m, 1], axis=0, keepdims=True))) for m in range(2)]
                acts.append(act(*res))
            return acts

        def act(gt, ut):
            a = _rb(gt * jax.nn.sigmoid(gt)) * ut
            return jnp.concatenate([a, a], axis=0).astype(BF16)

        def stage_last(gate, mu_prev, top):
            i = n2 - 1
            r0, t = p2_off[i], p2_tiles[i]
            st = {}

            def post(c, attn):
                h = x_v[r0:r0 + t, c * 128:(c + 1) * 128].astype(F32) + attn
                h_v[r0:r0 + t, c * 128:(c + 1) * 128] = h
                if c == 0:
                    st["shift"] = jnp.broadcast_to(h[:, 0:1], (t, 128))
                d = h - st["shift"]
                new = (d, d * d, d * wr[:, c * 128:(c + 1) * 128])
                st[c] = new if c == 0 else tuple(a + b for a, b in zip(st[c - 1], new))

            def gate_fn(p, deps):
                if p == 0:
                    return gate
                z = None
                if p % 2 == 1 and p // 2 - SLAG >= 0:
                    z = _fold(jnp.concatenate(st[p // 2 - SLAG], axis=1))
                if p == CGATE:
                    r, st["mur_p"], st["rs_p"] = stage_c(i - 1, mu_prev, deps, CLAST / 100)
                    st["top"] = merge(top, *tree(i - 1, r))
                    st["back"] = _fold(write_out(i - 1, st["mur_p"], st["rs_p"]))
                    st["guess"] = select(st["top"])
                    zz = _zero_of(st["top"][0] + st["top"][1])
                    z = zz if z is None else z | zz
                if p == 2 * G - 1:
                    z = st["back"] if z is None else z | st["back"]
                return z

            _, deps = _passes(jnp.concatenate(os, axis=0)[r0 // 2:(r0 + t) // 2, :], m_tile, G, gate_fn, post)
            st["a0"] = act(*gate_up(st["guess"][5], 0, FC0))
            s1, s2, s3 = st[G - 1]
            shift = st["shift"]
            m1 = _rowsum(s1) * (1.0 / D)
            var = jnp.maximum(_rowsum(s2) * (1.0 / D) - m1 * m1, 0.0)
            rs = _rstd(var)
            mur = _rb(shift + m1)
            r = _rb((_rowsum(s3) + (shift - mur) * wr_sum) * rs)
            mu_v[r0:r0 + t, :] = mur
            rs_v[r0:r0 + t, :] = rs
            return merge(st["top"], *tree(i, r)), st["mur_p"], st["rs_p"], mur, rs, st["guess"], st["a0"]

        top = None
        mu_prev = None
        gate = None
        for i in range(n2 - 1):
            deps, mu = stage_b(i, gate)
            if i == 0:
                pz = _pace(deps, (na - nearly) * H, 0.0, 0.8)
                late_os = [stage_a(j * ta, ta, pz[(j - nearly) * H * 8:(j - nearly + 1) * H * 8])
                           for j in range(nearly, na)]
                os += late_os
                gate = a_done(late_os) | retile(3, deps)
            else:
                r, mur, rs = stage_c(i - 1, mu_prev, deps, min(CHI / 100, 1 - LAT / (16 * p2_tiles[i])))
                back = write_out(i - 1, mur, rs)
                key = compact(i - 1, r)
                top = merge(top, key, jnp.zeros_like(key))
                gate = _zero_of(key + jnp.sum(back.reshape(-1, 8, 128), axis=0))
                if 3 + i < len(hosts):
                    gate = gate | retile(3 + i, deps)
                if i == n2 - 2:
                    t1, t2 = top
                    b1 = jnp.max(jnp.max(t1, axis=0, keepdims=True), axis=1, keepdims=True)
                    rest = jnp.where(t1 == b1, t2, t1)
                    b2 = jnp.max(jnp.max(rest, axis=0, keepdims=True), axis=1, keepdims=True)
                    top = (jnp.where(sub == 0, b1, 0.0), jnp.where(sub == 0, b2, 0.0))
            mu_prev = mu
        top, mur_p, rs_p, mur_l, rs_l, guess, a0 = stage_last(gate, mu_prev, top)
        sc.__exit__(None, None, None)

        sc = scope("tail")
        sc.__enter__()
        k1, k2, i1, i2, hs, xs = select(top)
        chunks = [(c0, min(FC, FM - c0)) for c0 in range(FC0, FM, FC)]
        xu = _pk(xs)
        y = None
        prev = None
        gate = None
        for c, ch in enumerate(chunks + [None]):
            if ch is not None:
                xc = _unpk(jnp.concatenate([xu[:, 0:128] | gate, xu[:, 128:]], axis=1)) if c == WOC + 2 else xs
                gt, ut = gate_up(xc, *ch)
            if c == 0:
                y0 = down(a0, 0)
            if prev is not None:
                part = down(a_prev, prev[0])
                y = part if y is None else y + part
            if c == WOC:
                back = write_out(n2 - 1, _tie(mur_l, _pace(gt, p2_tiles[-1] // 8)), rs_l)
                out_v[S:S + 16, 0:128] = jnp.concatenate([gt[:, 0:128]] * 2, axis=0).astype(BF16)
                gate = _fold(back) | _fold(out_v[S:S + 16, 0:128].astype(F32))
            if ch is not None:
                a_prev = act(gt, ut)
            prev = ch
        if FV:
            total = sum(c for _, c in ticks)
            nstep = FV // 256 * (D // 8)
            when = [sum(c for _, c in ticks[:k + 1]) for k in range(len(ticks))]
            tick_zero = {}

            def zero_at(step):
                tt = VLEAD + (step / nstep) * (VHI / 100 * total - VLEAD)
                if tt < when[0]:
                    return jnp.zeros((8, 128), U32)
                k = max(k for k in range(len(ticks)) if when[k] <= tt)
                if k not in tick_zero:
                    tick_zero[k] = _zero_of(ticks[k][0])
                return tick_zero[k]

            zs = [zero_at(step) for step in range(nstep)]
            for j, a in enumerate(vpu_acts(xs.astype(F32), zs)):
                y = y + down(a, FM + j * 256)
        mono = lax.shift_right_logical(jnp.where(first, k1, k2) - KEY0, 11)
        rsel = pltpu.bitcast(jnp.where(mono < 0x8000, 0xFFFF - mono, mono & 0x7FFF) << 16, F32)
        gain = _lanes(_rb(jax.nn.sigmoid(rsel)), G)
        g1 = pl.multiple_of(lax.shift_right_logical(i1, 4) * 16, 16)
        g2 = pl.multiple_of(lax.shift_right_logical(i2, 4) * 16, 16)
        rows = lax.broadcasted_iota(I32, (16, D), 0)

        def finish(y):
            new = hs + _rb(xs.astype(F32) + _rb(_rb(y) * gain))
            for j, g in enumerate((g1, g2)):
                old = out_v[pl.ds(g, 16), :].astype(F32)
                fix_v[j] = jnp.where(rows == i1 - g, new[0:1], jnp.where(rows == i2 - g, new[1:2], old)).astype(BF16)

        finish(y + y0)

        @pl.when(jnp.logical_or(i1 != guess[2], i2 != guess[3]))
        def _():
            finish(y + down(act(*gate_up(xs, 0, FC0)), 0))

        pltpu.make_async_copy(out_v.at[pl.ds(0, S)], out_hbm, sems.at[SO]).wait()
        c1 = pltpu.make_async_copy(fix_v.at[0], out_hbm.at[pl.ds(g1, 16)], sems.at[SO + 1])
        c2 = pltpu.make_async_copy(fix_v.at[1], out_hbm.at[pl.ds(g2, 16)], sems.at[SO + 2])
        c1.start()

        @pl.when(g1 != g2)
        def _():
            c2.start()
            c2.wait()
        c1.wait()
        sc.__exit__(None, None, None)

    scratch = [
        pltpu.VMEM((S, D + PAD), BF16),
        pltpu.VMEM((D, 3 * D + PAD), BF16),
        pltpu.VMEM((D, D + PAD), BF16),
        pltpu.VMEM((D, F), BF16),
        pltpu.VMEM((D, F), BF16),
        pltpu.VMEM((F, D + PAD), BF16),
        pltpu.VMEM((D,), BF16),
        pltpu.VMEM((S, 128), F32),
        pltpu.VMEM((S, 128), F32),
        pltpu.VMEM((S + 16, D), BF16),
        pltpu.VMEM((S, D), F32),
        pltpu.VMEM((2, 16, D), BF16),
        pltpu.VMEM((D // 2, FM), U32),
        pltpu.VMEM((D // 2, FM), U32),
        pltpu.VMEM((F // 2, D + PAD), U32),
        pltpu.SemaphoreType.DMA((NSEM,)),
    ]

    @jax.jit
    def f(A_x, A_wqkv, A_wo, B_x, B_w_r, B_w_gate, B_w_up, B_w_down):
        any_spec = pl.BlockSpec(memory_space=pl.ANY)
        out = pl.pallas_call(
            kernel,
            out_shape=jax.ShapeDtypeStruct((S, D), BF16),
            in_specs=[any_spec] * 7,
            out_specs=any_spec,
            scratch_shapes=scratch,
            compiler_params=pltpu.CompilerParams(vmem_limit_bytes=120 * 1024 * 1024, disable_bounds_checks=True),
        )(A_x.reshape(S, D), A_wqkv, A_wo, B_w_r, B_w_gate, B_w_up, B_w_down)
        return out.reshape(1, S, D)
    return f


_impl = make_kernel()


@jax.jit
def pallas_sequential_preLN__linear_attn_block__moe_arch_mod__prompt_kernel(
    A_x: jax.Array,
    A_wqkv: jax.Array,
    A_wo: jax.Array,
    B_x: jax.Array,
    B_w_r: jax.Array,
    B_w_gate: jax.Array,
    B_w_up: jax.Array,
    B_w_down: jax.Array,
):
    return _impl(A_x, A_wqkv, A_wo, B_x, B_w_r, B_w_gate, B_w_up, B_w_down)
```

```python
import contextlib

import jax
import jax.numpy as jnp
from jax import lax
import jax.experimental.pallas as pl
import jax.experimental.pallas.tpu as pltpu

S, D, F, H, DH = 2048, 1024, 3584, 32, 32
G = D // 128
F32 = jnp.float32
BF16 = jnp.bfloat16
I32 = jnp.int32
U32 = jnp.uint32
KEY0 = 64 << 23
PAD = 128


def _rb(x):
    return x.astype(BF16).astype(F32)


def _zero_of(x):
    bits = pltpu.bitcast(x, U32)
    return lax.shift_right_logical(lax.shift_right_logical(bits, U32(31)), U32(1))


def _pace(dep, n, lo=0.0, hi=1.0):
    if isinstance(dep, (list, tuple)):
        dep = jnp.concatenate(dep, axis=1)
    nrg, nch = dep.shape[0] // 8, dep.shape[1] // 128
    parts = []
    for p in range(n):
        pos = int((lo + (hi - lo) * p / n) * nch * nrg)
        c, rg = pos // nrg, pos % nrg
        parts.append(dep[rg * 8:(rg + 1) * 8, c * 128:(c + 1) * 128])
    return _zero_of(jnp.concatenate(parts, axis=0))


def _tie(x, zero):
    return pltpu.bitcast(pltpu.bitcast(x, U32) | zero, F32)


def _lanes(x, n):
    return jnp.concatenate([x] * n, axis=1) if n > 1 else x


def _rowsum(x):
    return jnp.broadcast_to(jnp.sum(x, axis=-1, keepdims=True), (x.shape[0], 128))


def _recip(d):
    r = pl.reciprocal(d, approx=True)
    return r * (2.0 - d * r)


def _rstd(var):
    v = _rb(_rb(var) + 1e-5)
    return _recip(_rb(v * lax.rsqrt(v)))


def _phi(t):
    return jnp.where(t > 0, t + 1.0, jnp.exp(t)) + 1e-6


def _dot(a, b):
    return jnp.dot(a, b, preferred_element_type=F32)


def _dot_tn(a, b):
    return lax.dot_general(a, b, (((0,), (0,)), ((), ())), preferred_element_type=F32)


def _pk(x):
    return pltpu.bitcast(x, U32)


def _unpk(x):
    return pltpu.bitcast(x, BF16)


def _gate(xu, zero):
    if zero is None:
        return xu
    top = jnp.concatenate([xu[0:8, 0:128] | zero, xu[0:8, 128:]], axis=1)
    return jnp.concatenate([top, xu[8:]], axis=0)


def _fold(x):
    x = pltpu.bitcast(x, U32) if x.dtype != U32 else x
    parts = [x[r:r + 8, c:c + 128] for r in range(0, x.shape[0], 8) for c in range(0, x.shape[1], 128)]
    while len(parts) > 1:
        parts = [parts[j] | parts[j + 1] if j + 1 < len(parts) else parts[j] for j in range(0, len(parts), 2)]
    return _zero_of(parts[0])


def _passes(xu, w, ntiles, gate_fn=None, post=None):
    deps, outs = [], []
    for c in range(ntiles):
        acc = None
        for hh in range(2):
            z = None if gate_fn is None else gate_fn(2 * c + hh, deps)
            lhs = _unpk(_gate(xu[:, hh * (D // 2):(hh + 1) * (D // 2)], z))
            part = _dot(lhs, w(hh * (D // 2), (hh + 1) * (D // 2), c))
            acc = part if acc is None else acc + part
            deps.append(acc)
        outs.append(acc if post is None else post(c, acc))
    return outs, deps


def make_kernel(P2T="256,256,256,256,256,256,256,128,64,64", FC=512, CHI=80, P1T="1024,512,512", QE=128, KCH="128,128,256,512", SHI=90, SLAST=40, XLO=30, XHI=95, FLO=60, FHI=92, GHI=70, GB=256, PHI=85, NAG=4, CLAST=50, CGATE=13, SLAG=4, LAT=560, PRI="p0", FC0=512, FV=768, VHI=95, VLEAD=512, XLEAD=16, WOC=1, scopes=0):
    p1_tiles = [int(t) for t in P1T.split(",")]
    assert sum(p1_tiles) == S and len(p1_tiles) == 3
    p1_off = [sum(p1_tiles[:i]) for i in range(3)]
    p2_tiles = [int(t) for t in P2T.split(",")]
    assert sum(p2_tiles) == S
    p2_off = [sum(p2_tiles[:i]) for i in range(len(p2_tiles))]
    FM = F - FV
    n2 = len(p2_tiles)
    KC, QC, VC = 0, D, 2 * D
    kch = [int(t) for t in KCH.split(",")]
    assert sum(kch) == D
    NKC = len(kch)
    T0 = p1_tiles[0]
    SW = NKC
    SX = SW + NKC + 3
    SWO = SX + 2
    SWG, SWU, SWD, SWR = SWO + 1, SWO + 2, SWO + 3, SWO + 4
    SO = SWR + 1
    NSEM = SO + 3

    def scope(name):
        return jax.named_scope(name) if scopes else contextlib.nullcontext()

    def kernel(x_hbm, wqkv_hbm, wo_hbm, wr_hbm, wg_hbm, wu_hbm, wd_hbm, out_hbm,
               x_v, wqkv_v, wo_v, wg_v, wu_v, wd_v, wr_v, mu_v, rs_v,
               out_v, h_v, fix_v, wg_p, wu_p, wd_p, sems):

        xn_rows = {}
        pqt = []
        g_acc = {}
        z_acc = {}
        m_rows = []

        def xn_at(r0, t):
            keys = sorted(k for k in xn_rows if r0 <= k < r0 + t)
            return jnp.concatenate([xn_rows[k] for k in keys], axis=0) if len(keys) > 1 else xn_rows[keys[0]]

        def rows_copy(r0, n, s):
            return pltpu.make_async_copy(x_hbm.at[pl.ds(r0, n)], x_v.at[pl.ds(r0, n), pl.ds(0, D)], sems.at[s])

        koff = [sum(kch[:j]) for j in range(NKC)]
        x0 = [pltpu.make_async_copy(x_hbm.at[pl.ds(0, T0), pl.ds(koff[j], kch[j])],
                                    x_v.at[pl.ds(0, T0), pl.ds(koff[j], kch[j])], sems.at[j]) for j in range(NKC)]
        xcp = [rows_copy(p1_off[i], p1_tiles[i], SX + i - 1) for i in (1, 2)]
        wcp = [pltpu.make_async_copy(wqkv_hbm.at[pl.ds(koff[j], kch[j]), pl.ds(D, D)],
                                     wqkv_v.at[pl.ds(koff[j], kch[j]), pl.ds(KC, D)], sems.at[SW + j])
               for j in range(NKC)]
        wcp += [pltpu.make_async_copy(wqkv_hbm.at[pl.ds(r0, n), pl.ds(c0, D)], wqkv_v.at[pl.ds(r0, n), pl.ds(d0, D)],
                                      sems.at[SW + NKC + j])
                for j, (r0, n, c0, d0) in enumerate(((QE, D - QE, 0, QC), (0, D, 2 * D, VC)))]
        if QE:
            wq0 = pltpu.make_async_copy(wqkv_hbm.at[pl.ds(0, QE), pl.ds(0, D)], wqkv_v.at[pl.ds(0, QE), pl.ds(QC, D)],
                                        sems.at[SW + NKC + 2])
        wo_copy = pltpu.make_async_copy(wo_hbm, wo_v.at[:, pl.ds(0, D)], sems.at[SWO])
        wg_copy = pltpu.make_async_copy(wg_hbm, wg_v, sems.at[SWG])
        wu_copy = pltpu.make_async_copy(wu_hbm, wu_v, sems.at[SWU])
        wd_copy = pltpu.make_async_copy(wd_hbm, wd_v.at[:, pl.ds(0, D)], sems.at[SWD])
        wr_copy = pltpu.make_async_copy(wr_hbm, wr_v, sems.at[SWR])

        def out_copy(i):
            return pltpu.make_async_copy(out_v.at[pl.ds(p2_off[i], p2_tiles[i])],
                                         out_hbm.at[pl.ds(p2_off[i], p2_tiles[i])], sems.at[SO])

        order = [c for j in range(NKC) for c in (x0[j], wcp[j]) + ((wq0,) if QE and j == 1 else ())] + [wcp[NKC]] + xcp + [wcp[NKC + 1], wr_copy, wo_copy, wg_copy, wu_copy, wd_copy]
        pri = [int(ch) for ch in PRI[1:]]
        for j, c in enumerate(order):
            c.start(priority=pri[j] if j < len(pri) else pri[-1])

        def proj(r0, t, c0, n):
            return _dot(_unpk(xn_at(r0, t)), wqkv_v[:, c0:c0 + n])

        def feat(y):
            return _phi(y).astype(BF16)

        def prep(r0, t, zero=None):
            xf = x_v[r0:r0 + t, 0:D].astype(F32)
            if zero is not None:
                xf = jnp.concatenate([_tie(xf[:, 0:128], zero), xf[:, 128:]], axis=1)
            mu = _rowsum(xf) * (1.0 / D)
            mur = _rb(mu)
            mu_v[r0:r0 + t, :] = mur
            xc = x_v[r0:r0 + t, 0:D].astype(F32) - _lanes(mu, G)
            rs = _rstd(_rowsum(xc * xc) * (1.0 / D))
            rs_v[r0:r0 + t, :] = rs
            xn = (x_v[r0:r0 + t, 0:D].astype(F32) - _lanes(mur, G)) * _lanes(rs, G)
            xu = _pk(xn.astype(BF16))
            xn_rows[r0] = xu
            return xu

        def g_piece(pk, r0, c0, pkt=None):
            t, n = pk.shape
            upd = _dot(pk.T if pkt is None else pkt, _unpk(xn_at(r0, t)))
            zs = jnp.sum(pk.astype(F32).reshape(t // 8, 8, n), axis=0)
            for c in range(0, n, 128):
                b = (c0 + c) // 128
                g_acc[b] = upd[c:c + 128] if r0 == 0 else g_acc[b] + upd[c:c + 128]
                z_acc[b] = zs[:, c:c + 128] if r0 == 0 else z_acc[b] + zs[:, c:c + 128]
            return upd

        def q_part(r0, t, gate=None, head=None):
            k0 = 0 if head is None else QE
            acc = _dot(_unpk(_gate(xn_at(r0, t)[:, k0:], gate)), wqkv_v[k0:, QC:QC + D])
            pqt.append(_pk(feat(acc if head is None else acc + head).T))
            return acc

        def wait(c, name):
            with scope(name):
                c.wait()

        acc = s1 = s2 = cs = shift = None
        for j in range(NKC):
            wait(x0[j], "w_x%d" % j)
            wait(wcp[j], "w_c%d" % j)
            if QE and j == 1:
                wait(wq0, "w_q0")
            c0, n = koff[j], kch[j]
            part = _dot(x_v[0:T0, c0:c0 + n], wqkv_v[c0:c0 + n, KC:KC + D])
            acc = part if acc is None else acc + part
            if QE and j == 1:
                accq0 = _dot(x_v[0:T0, 0:QE], wqkv_v[0:QE, QC:QC + D])
                csq = jnp.sum(wqkv_v[0:QE, QC:QC + D].astype(F32), axis=0, keepdims=True)
                part = jnp.concatenate([part, accq0], axis=1)
            xf = x_v[0:T0, c0:c0 + n].astype(F32)
            if shift is None:
                shift = jnp.broadcast_to(xf[:, 0:1], (T0, 128))
            sh = _tie(shift, _pace(part, T0 // 8, 0.0, (SHI if j < NKC - 1 else SLAST) / 100))
            d = xf - _lanes(sh, n // 128)
            for c in range(0, n, 128):
                dc = d[:, c:c + 128]
                s1 = dc if s1 is None else s1 + dc
                s2 = dc * dc if s2 is None else s2 + dc * dc
            w = jnp.sum(wqkv_v[c0:c0 + n, KC:KC + D].astype(F32).reshape(n // 8, 8, D), axis=0)
            cs = w if cs is None else cs + w
        m1 = _rowsum(s1) * (1.0 / D)
        rs = _rstd(jnp.maximum(_rowsum(s2) * (1.0 / D) - m1 * m1, 0.0))
        mur = _rb(shift + m1)
        cs = jnp.sum(cs, axis=0, keepdims=True)
        mu_v[0:T0, :] = mur
        mux = _tie(mur, _pace(part, T0 // 8, XLO / 100, XHI / 100))
        xn = (x_v[0:T0, 0:D].astype(F32) - _lanes(mux, G)) * _lanes(rs, G)
        xu = _pk(xn.astype(BF16))
        h0 = T0 // 256 * 128
        xn_rows[0] = xu[0:h0 // 2]
        xn_rows[h0] = xu[h0 // 2:]
        upd = None
        for c in range(0, D, GB):
            zero = _pace(part, T0 // 8, FLO / 100, FHI / 100) if upd is None else _pace(upd, T0 // 8, 0.0, GHI / 100)
            mub = _tie(mur, zero)
            k = GB // 128
            upd = g_piece(feat((acc[:, c:c + GB] - _lanes(mub, k) * cs[:, c:c + GB]) * _lanes(rs, k)), 0, c)

        with scope("p1_mid"):
            for c in wcp[NKC:] + xcp + [wr_copy, wo_copy]:
                c.wait()
            heads = [None, None]
            if QE:
                head = (accq0 - _lanes(mur, G) * csq) * _lanes(rs, G)
                heads = [head[0:h0], head[h0:]]
            q_part(0, h0, None, heads[0])
            r1, t1 = p1_off[1], p1_tiles[1]
            r2, t2 = p1_off[2], p1_tiles[2]
            prep(r1, t1, _pace(q_part(h0, T0 - h0, None, heads[1]), t1 // 8, 0.0, PHI / 100))
            pk = feat(proj(r1, t1, KC, D))
            xu = prep(r2, t2, _pace(q_part(r1, t1), t2 // 8, 0.0, PHI / 100))
            g_piece(_unpk(_gate(_pk(pk), _fold(xu[:, D - 128:D]))), r1, 0)

        sc = scope("p2")
        sc.__enter__()
        for c in (wg_copy, wu_copy, wd_copy):
            c.wait()

        jobs = ([(src, dst, r, c, min(D, FM - c)) for src, dst in ((wg_v, wg_p), (wu_v, wu_p))
                 for r in range(0, D, 16) for c in range(0, FM, D)]
                + [(wd_v, wd_p, r, 0, D) for r in range(0, F, 16)])
        hosts = [2, 2, 2] + [1] * (n2 - 3)
        dyn0 = pltpu.bitcast(_zero_of(mu_v[0:8, :]), I32)[0, 0]

        def retile(h, deps):
            mine = jobs[len(jobs) * sum(hosts[:h]) // sum(hosts):len(jobs) * sum(hosts[:h + 1]) // sum(hosts)]
            pz = _pace(deps, len(mine), 0.0, 0.85)
            for k, (src, dst, r, c, n) in enumerate(mine):
                dst[r // 2:r // 2 + 8, c:c + n] = _pk(src[r:r + 16, c:c + n]) | _lanes(pz[k * 8:(k + 1) * 8], n // 128)
            done = None
            for dst in (wg_p, wu_p, wd_p):
                if any(j[1] is dst for j in mine):
                    r = max(j[2] for j in mine if j[1] is dst) // 2
                    c = min(j[3] for j in mine if j[1] is dst and j[2] // 2 == r)
                    v = dst[pl.ds(pl.multiple_of(r + dyn0, 8), 8), c:c + 128]
                    done = v if done is None else done | v
            return _zero_of(done)

        acck = proj(r2, t2, KC, D)
        pk = _unpk(_gate(_pk(feat(acck)), retile(0, acck)))
        g_last = g_piece(pk, r2, 0)

        z = _rb(jnp.sum(jnp.concatenate([z_acc[b] for b in range(G)], axis=1), axis=0, keepdims=True))
        zc = jnp.concatenate(
            [jnp.broadcast_to(z[:, g * 128:(g + 1) * 128], (128, 128)).T for g in range(G)], axis=0)
        wr = wr_v[...].astype(F32).reshape(1, D)
        wr_sum = _rowsum(wr)

        def stage_a(r0, t, zero):
            k = t // 128
            pq = _unpk(jnp.concatenate(pqt, axis=1)[:, r0:r0 + t]).astype(F32)
            z4 = zc.reshape(H, DH // 8, 8, 128)
            z0 = _tie(z4[:, 0].reshape(H * 8, 128), zero).reshape(H, 1, 8, 128)
            zz = jnp.concatenate([z0, z4[:, 1:]], axis=1).reshape(D, 128)
            w = (pq * _lanes(zz, k)).reshape(H, DH // 8, 8, t)
            den = jnp.sum(jnp.sum(w, axis=1), axis=1, keepdims=True) + 1e-6
            o = pq.reshape(H, DH, t) * _recip(den)
            return _pk(o.reshape(D, t).astype(BF16).T)

        def m_tile(a, b, c):
            return _unpk(jnp.concatenate(m_rows[a // 128:b // 128], axis=0)[:, c * 128:(c + 1) * 128])

        def stage_b(i, gate):
            r0, t = p2_off[i], p2_tiles[i]

            def post(c, attn):
                h_v[r0:r0 + t, c * 128:(c + 1) * 128] = x_v[r0:r0 + t, c * 128:(c + 1) * 128].astype(F32) + attn

            _, deps = _passes(jnp.concatenate(os, axis=0)[r0 // 2:(r0 + t) // 2, :], m_tile, G,
                              lambda p, deps: gate if p == 0 else None, post)
            return deps, _rowsum(h_v[r0:r0 + t, :]) * (1.0 / D)

        def keys_of(r, idx):
            bits = pltpu.bitcast(jnp.where(r == 0.0, 0.0, r), I32)
            hi = lax.shift_right_logical(bits, 16)
            mono = jnp.where(bits < 0, 0xFFFF - hi, hi | 0x8000)
            return pltpu.bitcast((mono << 11) + (KEY0 + S - 1 - idx), F32)

        def merge(top, k1, k2):
            if top is None:
                return k1, k2
            t1, t2 = top
            return jnp.maximum(t1, k1), jnp.maximum(jnp.minimum(t1, k1), jnp.maximum(t2, k2))

        def write_out(i, mur, rs):
            r0, t = p2_off[i], p2_tiles[i]
            out_v[r0:r0 + t, :] = (h_v[r0:r0 + t, :] * _lanes(1.0 + rs, G) - _lanes(mur * rs, G)).astype(BF16)
            back = out_v[r0:r0 + t, D - 128:D].astype(F32)
            out_copy(i).start()
            return back

        def stage_c(i, mu, dep, hi=CHI / 100):
            r0, t = p2_off[i], p2_tiles[i]
            mu = _tie(mu, _pace(dep, t // 8, 0.0, hi))
            d = h_v[r0:r0 + t, :] - _lanes(mu, G)
            rs = _rstd(_rowsum(d * d) * (1.0 / D))
            mur = _rb(mu)
            r = _rb((_rowsum(d * wr) + (mu - mur) * wr_sum) * rs)
            mu_v[r0:r0 + t, :] = mur
            rs_v[r0:r0 + t, :] = rs
            return r, mur, rs

        lane = lax.broadcasted_iota(I32, (8, 128), 1)
        sub = lax.broadcasted_iota(I32, (8, 128), 0)

        def compact(i, r):
            r0, t = p2_off[i], p2_tiles[i]
            parts = [r[p * 8:(p + 1) * 8] for p in range(t // 8)]
            acc = parts[0]
            for p in range(1, t // 8):
                acc = jnp.where(lane == p, parts[p], acc)
            key = keys_of(acc, r0 + lane * 8 + sub)
            return jnp.where(lane < t // 8, key, 0.0)

        def a_done(os):
            acc = None
            for o in os:
                for rb in range(o.shape[0] // 64):
                    row = o[rb * 64 + 56:rb * 64 + 64, :]
                    for g in range(G):
                        v = row[:, g * 128:(g + 1) * 128]
                        acc = v if acc is None else acc | v
            return _zero_of(acc)

        ta = 256
        na = S // ta
        nearly = r2 // ta
        pz = _pace(g_last, NAG * H, 0.0, 1.0)
        os = [stage_a(j * ta, ta, pz[j * H * 8:(j + 1) * H * 8]) for j in range(NAG)]
        accq = q_part(r2, t2, retile(1, g_last))
        if nearly > NAG:
            pz = _pace(accq, (nearly - NAG) * H, 0.0, 0.9)
            os += [stage_a(j * ta, ta, pz[(j - NAG) * H * 8:(j - NAG + 1) * H * 8]) for j in range(NAG, nearly)]

        row = lax.broadcasted_iota(I32, (128, 128), 0) // DH
        col = lax.broadcasted_iota(I32, (128, 128), 1) // DH
        same = row == col
        kvs = []
        for g in range(G):
            gg = g_acc[g]
            if g == 0:
                gg = jnp.concatenate([jnp.concatenate(
                    [_tie(gg[0:8, 0:128], a_done(os) | retile(2, accq)), gg[0:8, 128:]], axis=1), gg[8:]], axis=0)
            kv = _dot(gg.astype(BF16), wqkv_v[:, VC + g * 128:VC + (g + 1) * 128])
            kvs.append(jnp.where(same, kv, 0.0).astype(BF16))
        for g in range(G):
            m_rows.append(_pk(_dot(kvs[g], wo_v[g * 128:(g + 1) * 128, 0:D]).astype(BF16)))

        def tree(i, r):
            t = p2_tiles[i]
            key = keys_of(r, lax.broadcasted_iota(I32, (t, 128), 0) + p2_off[i])
            level = [(key[p * 8:(p + 1) * 8], None) for p in range(t // 8)]
            while len(level) > 1:
                nxt = []
                for p in range(0, len(level) - 1, 2):
                    (a1, a2), (b1, b2) = level[p], level[p + 1]
                    lo = jnp.minimum(a1, b1)
                    for e in (a2, b2):
                        lo = lo if e is None else jnp.maximum(lo, e)
                    nxt.append((jnp.maximum(a1, b1), lo))
                if len(level) % 2:
                    nxt.append(level[-1])
                level = nxt
            return level[0]

        first = lax.broadcasted_iota(I32, (16, 128), 0) == 0

        def select(top):
            t1, t2 = top
            k1 = jnp.max(t1, axis=0, keepdims=True)
            k2 = jnp.max(jnp.where(t1 == k1, t2, t1), axis=0, keepdims=True)
            k1 = pltpu.bitcast(k1, I32)
            k2 = pltpu.bitcast(k2, I32)
            i1 = S - 1 - (k1[0, 0] & (S - 1))
            i2 = S - 1 - (k2[0, 0] & (S - 1))

            def pick(ref, k):
                return jnp.where(_lanes(first, k), ref[pl.ds(i1, 1), :], ref[pl.ds(i2, 1), :])

            hs = pick(h_v, G)
            xs = ((hs - _lanes(pick(mu_v, 1), G)) * _lanes(pick(rs_v, 1), G)).astype(BF16)
            return k1, k2, i1, i2, hs, xs

        ticks = []

        def gate_up(xs, c0, n):
            gt = _dot(xs, _unpk(wg_p[:, c0:c0 + n]))
            ut = _dot(xs, _unpk(wu_p[:, c0:c0 + n]))
            ticks.extend((v[0:8, c:c + 128], 64) for v in (gt, ut) for c in range(0, n, 128))
            return _rb(gt[0:8]), _rb(ut[0:8])

        def down(a, c0):
            y = _dot(a, _unpk(wd_p[c0 // 2:(c0 + a.shape[1]) // 2, 0:D]))
            ticks.extend((y[0:8, c:c + 128], a.shape[1] // 16) for c in range(0, D, 128))
            return y

        def vpu_acts(xg, zeros):
            nd = D // 8
            xb = {}
            acts = []
            for j in range(FV // 256):
                c0 = FM + j * 256
                acc = {}
                for d in range(nd):
                    zero = zeros[j * nd + d]
                    if j == 0 and d % 16 == 0:
                        g = d // 16
                        zg = zeros[max(0, d - XLEAD)]
                        for t in range(2):
                            row = _tie(jnp.broadcast_to(xg[t:t + 1, g * 128:(g + 1) * 128], (8, 128)), zg)
                            blk = jnp.concatenate([row] * 16, axis=0).T
                            for e in range(16):
                                xb[t, d + e] = blk[e * 8:(e + 1) * 8]
                    xt = [_lanes(_tie(xb[t, d], zero), 2) for t in range(2)]
                    for m, w_v in enumerate((wg_v, wu_v)):
                        w = w_v[d * 8:(d + 1) * 8, c0:c0 + 256].astype(F32)
                        for t in range(2):
                            acc[m, t] = w * xt[t] if d == 0 else acc[m, t] + w * xt[t]
                res = [_rb(jnp.where(_lanes(first[0:8], 2), jnp.sum(acc[m, 0], axis=0, keepdims=True),
                                     jnp.sum(acc[m, 1], axis=0, keepdims=True))) for m in range(2)]
                acts.append(act(*res))
            return acts

        def act(gt, ut):
            a = _rb(gt * jax.nn.sigmoid(gt)) * ut
            return jnp.concatenate([a, a], axis=0).astype(BF16)

        def stage_last(gate, mu_prev, top):
            i = n2 - 1
            r0, t = p2_off[i], p2_tiles[i]
            st = {}

            def post(c, attn):
                h = x_v[r0:r0 + t, c * 128:(c + 1) * 128].astype(F32) + attn
                h_v[r0:r0 + t, c * 128:(c + 1) * 128] = h
                if c == 0:
                    st["shift"] = jnp.broadcast_to(h[:, 0:1], (t, 128))
                d = h - st["shift"]
                new = (d, d * d, d * wr[:, c * 128:(c + 1) * 128])
                st[c] = new if c == 0 else tuple(a + b for a, b in zip(st[c - 1], new))

            def gate_fn(p, deps):
                if p == 0:
                    return gate
                z = None
                if p % 2 == 1 and p // 2 - SLAG >= 0:
                    z = _fold(jnp.concatenate(st[p // 2 - SLAG], axis=1))
                if p == CGATE:
                    r, st["mur_p"], st["rs_p"] = stage_c(i - 1, mu_prev, deps, CLAST / 100)
                    st["top"] = merge(top, *tree(i - 1, r))
                    st["back"] = _fold(write_out(i - 1, st["mur_p"], st["rs_p"]))
                    st["guess"] = select(st["top"])
                    zz = _zero_of(st["top"][0] + st["top"][1])
                    z = zz if z is None else z | zz
                if p == 2 * G - 1:
                    z = st["back"] if z is None else z | st["back"]
                return z

            _, deps = _passes(jnp.concatenate(os, axis=0)[r0 // 2:(r0 + t) // 2, :], m_tile, G, gate_fn, post)
            st["a0"] = act(*gate_up(st["guess"][5], 0, FC0))
            s1, s2, s3 = st[G - 1]
            shift = st["shift"]
            m1 = _rowsum(s1) * (1.0 / D)
            var = jnp.maximum(_rowsum(s2) * (1.0 / D) - m1 * m1, 0.0)
            rs = _rstd(var)
            mur = _rb(shift + m1)
            r = _rb((_rowsum(s3) + (shift - mur) * wr_sum) * rs)
            mu_v[r0:r0 + t, :] = mur
            rs_v[r0:r0 + t, :] = rs
            return merge(st["top"], *tree(i, r)), st["mur_p"], st["rs_p"], mur, rs, st["guess"], st["a0"]

        top = None
        mu_prev = None
        gate = None
        for i in range(n2 - 1):
            deps, mu = stage_b(i, gate)
            if i == 0:
                pz = _pace(deps, (na - nearly) * H, 0.0, 0.8)
                late_os = [stage_a(j * ta, ta, pz[(j - nearly) * H * 8:(j - nearly + 1) * H * 8])
                           for j in range(nearly, na)]
                os += late_os
                gate = a_done(late_os) | retile(3, deps)
            else:
                r, mur, rs = stage_c(i - 1, mu_prev, deps, min(CHI / 100, 1 - LAT / (16 * p2_tiles[i])))
                back = write_out(i - 1, mur, rs)
                key = compact(i - 1, r)
                top = merge(top, key, jnp.zeros_like(key))
                gate = _zero_of(key + jnp.sum(back.reshape(-1, 8, 128), axis=0))
                if 3 + i < len(hosts):
                    gate = gate | retile(3 + i, deps)
                if i == n2 - 2:
                    t1, t2 = top
                    b1 = jnp.max(jnp.max(t1, axis=0, keepdims=True), axis=1, keepdims=True)
                    rest = jnp.where(t1 == b1, t2, t1)
                    b2 = jnp.max(jnp.max(rest, axis=0, keepdims=True), axis=1, keepdims=True)
                    top = (jnp.where(sub == 0, b1, 0.0), jnp.where(sub == 0, b2, 0.0))
            mu_prev = mu
        top, mur_p, rs_p, mur_l, rs_l, guess, a0 = stage_last(gate, mu_prev, top)
        sc.__exit__(None, None, None)

        sc = scope("tail")
        sc.__enter__()
        k1, k2, i1, i2, hs, xs = select(top)
        chunks = [(c0, min(FC, FM - c0)) for c0 in range(FC0, FM, FC)]
        xu = _pk(xs)
        y = None
        prev = None
        gate = None
        for c, ch in enumerate(chunks + [None]):
            if ch is not None:
                xc = _unpk(jnp.concatenate([xu[:, 0:128] | gate, xu[:, 128:]], axis=1)) if c == WOC + 2 else xs
                gt, ut = gate_up(xc, *ch)
            if c == 0:
                y0 = down(a0, 0)
            if prev is not None:
                part = down(a_prev, prev[0])
                y = part if y is None else y + part
            if c == WOC:
                back = write_out(n2 - 1, _tie(mur_l, _pace(gt, p2_tiles[-1] // 8)), rs_l)
                out_v[S:S + 16, 0:128] = jnp.concatenate([gt[:, 0:128]] * 2, axis=0).astype(BF16)
                gate = _fold(back) | _fold(out_v[S:S + 16, 0:128].astype(F32))
            if ch is not None:
                a_prev = act(gt, ut)
            prev = ch
        if FV:
            total = sum(c for _, c in ticks)
            nstep = FV // 256 * (D // 8)
            when = [sum(c for _, c in ticks[:k + 1]) for k in range(len(ticks))]
            tick_zero = {}

            def zero_at(step):
                tt = VLEAD + (step / nstep) * (VHI / 100 * total - VLEAD)
                if tt < when[0]:
                    return jnp.zeros((8, 128), U32)
                k = max(k for k in range(len(ticks)) if when[k] <= tt)
                if k not in tick_zero:
                    tick_zero[k] = _zero_of(ticks[k][0])
                return tick_zero[k]

            zs = [zero_at(step) for step in range(nstep)]
            for j, a in enumerate(vpu_acts(xs.astype(F32), zs)):
                y = y + down(a, FM + j * 256)
        mono = lax.shift_right_logical(jnp.where(first, k1, k2) - KEY0, 11)
        rsel = pltpu.bitcast(jnp.where(mono < 0x8000, 0xFFFF - mono, mono & 0x7FFF) << 16, F32)
        gain = _lanes(_rb(jax.nn.sigmoid(rsel)), G)
        g1 = pl.multiple_of(lax.shift_right_logical(i1, 4) * 16, 16)
        g2 = pl.multiple_of(lax.shift_right_logical(i2, 4) * 16, 16)
        rows = lax.broadcasted_iota(I32, (16, D), 0)

        def finish(y):
            new = hs + _rb(xs.astype(F32) + _rb(_rb(y) * gain))
            for j, g in enumerate((g1, g2)):
                old = out_v[pl.ds(g, 16), :].astype(F32)
                fix_v[j] = jnp.where(rows == i1 - g, new[0:1], jnp.where(rows == i2 - g, new[1:2], old)).astype(BF16)

        finish(y + y0)

        @pl.when(jnp.logical_or(i1 != guess[2], i2 != guess[3]))
        def _():
            finish(y + down(act(*gate_up(xs, 0, FC0)), 0))

        pltpu.make_async_copy(out_v.at[pl.ds(0, S)], out_hbm, sems.at[SO]).wait()
        c1 = pltpu.make_async_copy(fix_v.at[0], out_hbm.at[pl.ds(g1, 16)], sems.at[SO + 1])
        c2 = pltpu.make_async_copy(fix_v.at[1], out_hbm.at[pl.ds(g2, 16)], sems.at[SO + 2])
        c1.start()

        @pl.when(g1 != g2)
        def _():
            c2.start()
            c2.wait()
        c1.wait()
        sc.__exit__(None, None, None)

    scratch = [
        pltpu.VMEM((S, D + PAD), BF16),
        pltpu.VMEM((D, 3 * D + PAD), BF16),
        pltpu.VMEM((D, D + PAD), BF16),
        pltpu.VMEM((D, F), BF16),
        pltpu.VMEM((D, F), BF16),
        pltpu.VMEM((F, D + PAD), BF16),
        pltpu.VMEM((D,), BF16),
        pltpu.VMEM((S, 128), F32),
        pltpu.VMEM((S, 128), F32),
        pltpu.VMEM((S + 16, D), BF16),
        pltpu.VMEM((S, D), F32),
        pltpu.VMEM((2, 16, D), BF16),
        pltpu.VMEM((D // 2, FM), U32),
        pltpu.VMEM((D // 2, FM), U32),
        pltpu.VMEM((F // 2, D + PAD), U32),
        pltpu.SemaphoreType.DMA((NSEM,)),
    ]

    @jax.jit
    def f(A_x, A_wqkv, A_wo, B_x, B_w_r, B_w_gate, B_w_up, B_w_down):
        any_spec = pl.BlockSpec(memory_space=pl.ANY)
        out = pl.pallas_call(
            kernel,
            out_shape=jax.ShapeDtypeStruct((S, D), BF16),
            in_specs=[any_spec] * 7,
            out_specs=any_spec,
            scratch_shapes=scratch,
            compiler_params=pltpu.CompilerParams(vmem_limit_bytes=120 * 1024 * 1024, disable_bounds_checks=True),
        )(A_x.reshape(S, D), A_wqkv, A_wo, B_w_r, B_w_gate, B_w_up, B_w_down)
        return out.reshape(1, S, D)
    return f


_impl = make_kernel()


@jax.jit
def pallas_sequential_preLN__linear_attn_block__moe_arch_mod__prompt_kernel(
    A_x: jax.Array,
    A_wqkv: jax.Array,
    A_wo: jax.Array,
    B_x: jax.Array,
    B_w_r: jax.Array,
    B_w_gate: jax.Array,
    B_w_up: jax.Array,
    B_w_down: jax.Array,
):
    return _impl(A_x, A_wqkv, A_wo, B_x, B_w_r, B_w_gate, B_w_up, B_w_down)
```

```python
import contextlib

import jax
import jax.numpy as jnp
from jax import lax
import jax.experimental.pallas as pl
import jax.experimental.pallas.tpu as pltpu

S, D, F, H, DH = 2048, 1024, 3584, 32, 32
G = D // 128
F32 = jnp.float32
BF16 = jnp.bfloat16
I32 = jnp.int32
U32 = jnp.uint32
KEY0 = 64 << 23
PAD = 128


def _rb(x):
    return x.astype(BF16).astype(F32)


def _zero_of(x):
    bits = pltpu.bitcast(x, U32)
    return lax.shift_right_logical(lax.shift_right_logical(bits, U32(31)), U32(1))


def _pace(dep, n, lo=0.0, hi=1.0):
    if isinstance(dep, (list, tuple)):
        dep = jnp.concatenate(dep, axis=1)
    nrg, nch = dep.shape[0] // 8, dep.shape[1] // 128
    parts = []
    for p in range(n):
        pos = int((lo + (hi - lo) * p / n) * nch * nrg)
        c, rg = pos // nrg, pos % nrg
        parts.append(dep[rg * 8:(rg + 1) * 8, c * 128:(c + 1) * 128])
    return _zero_of(jnp.concatenate(parts, axis=0))


def _tie(x, zero):
    return pltpu.bitcast(pltpu.bitcast(x, U32) | zero, F32)


def _lanes(x, n):
    return jnp.concatenate([x] * n, axis=1) if n > 1 else x


def _rowsum(x):
    return jnp.broadcast_to(jnp.sum(x, axis=-1, keepdims=True), (x.shape[0], 128))


def _recip(d):
    r = pl.reciprocal(d, approx=True)
    return r * (2.0 - d * r)


def _rstd(var):
    v = _rb(_rb(var) + 1e-5)
    return _recip(_rb(v * lax.rsqrt(v)))


def _phi(t):
    return jnp.where(t > 0, t + 1.0, jnp.exp(t)) + 1e-6


def _dot(a, b):
    return jnp.dot(a, b, preferred_element_type=F32)


def _dot_tn(a, b):
    return lax.dot_general(a, b, (((0,), (0,)), ((), ())), preferred_element_type=F32)


def _pk(x):
    return pltpu.bitcast(x, U32)


def _unpk(x):
    return pltpu.bitcast(x, BF16)


def _gate(xu, zero):
    if zero is None:
        return xu
    top = jnp.concatenate([xu[0:8, 0:128] | zero, xu[0:8, 128:]], axis=1)
    return jnp.concatenate([top, xu[8:]], axis=0)


def _fold(x):
    x = pltpu.bitcast(x, U32) if x.dtype != U32 else x
    parts = [x[r:r + 8, c:c + 128] for r in range(0, x.shape[0], 8) for c in range(0, x.shape[1], 128)]
    while len(parts) > 1:
        parts = [parts[j] | parts[j + 1] if j + 1 < len(parts) else parts[j] for j in range(0, len(parts), 2)]
    return _zero_of(parts[0])


def _passes(xu, w, ntiles, gate_fn=None, post=None):
    deps, outs = [], []
    for c in range(ntiles):
        acc = None
        for hh in range(2):
            z = None if gate_fn is None else gate_fn(2 * c + hh, deps)
            lhs = _unpk(_gate(xu[:, hh * (D // 2):(hh + 1) * (D // 2)], z))
            part = _dot(lhs, w(hh * (D // 2), (hh + 1) * (D // 2), c))
            acc = part if acc is None else acc + part
            deps.append(acc)
        outs.append(acc if post is None else post(c, acc))
    return outs, deps


def make_kernel(P2T="256,256,256,256,256,256,256,128,64,64", FC=512, CHI=80, P1T="1024,512,512", QE=128, KCH="128,128,256,512", SHI=90, SLAST=40, XLO=30, XHI=95, FLO=60, FHI=92, GHI=70, GB=256, PHI=90, NAG=4, CLAST=50, CGATE=13, SLAG=4, LAT=560, PRI="p0", FC0=512, FV=768, VHI=95, VLEAD=512, XLEAD=16, WOC=1, TIE=4, JUNK=1280, scopes=0):
    p1_tiles = [int(t) for t in P1T.split(",")]
    assert sum(p1_tiles) == S and len(p1_tiles) == 3
    p1_off = [sum(p1_tiles[:i]) for i in range(3)]
    p2_tiles = [int(t) for t in P2T.split(",")]
    assert sum(p2_tiles) == S
    p2_off = [sum(p2_tiles[:i]) for i in range(len(p2_tiles))]
    FM = F - FV
    n2 = len(p2_tiles)
    KC, QC, VC = 0, D, 2 * D
    kch = [int(t) for t in KCH.split(",")]
    assert sum(kch) == D
    NKC = len(kch)
    T0 = p1_tiles[0]
    SW = NKC
    SX = SW + NKC + 3
    SWO = SX + 2
    SWG, SWU, SWD, SWR = SWO + 1, SWO + 2, SWO + 3, SWO + 4
    SO = SWR + 1
    NSEM = SO + 3

    def scope(name):
        return jax.named_scope(name) if scopes else contextlib.nullcontext()

    def kernel(x_hbm, wqkv_hbm, wo_hbm, wr_hbm, wg_hbm, wu_hbm, wd_hbm, out_hbm,
               x_v, wqkv_v, wo_v, wg_v, wu_v, wd_v, wr_v, mu_v, rs_v,
               out_v, h_v, fix_v, wg_p, wu_p, wd_p, sems):

        xn_rows = {}
        pqt = []
        g_acc = {}
        z_acc = {}
        m_rows = []

        def xn_at(r0, t):
            keys = sorted(k for k in xn_rows if r0 <= k < r0 + t)
            return jnp.concatenate([xn_rows[k] for k in keys], axis=0) if len(keys) > 1 else xn_rows[keys[0]]

        def rows_copy(r0, n, s):
            return pltpu.make_async_copy(x_hbm.at[pl.ds(r0, n)], x_v.at[pl.ds(r0, n), pl.ds(0, D)], sems.at[s])

        koff = [sum(kch[:j]) for j in range(NKC)]
        x0 = [pltpu.make_async_copy(x_hbm.at[pl.ds(0, T0), pl.ds(koff[j], kch[j])],
                                    x_v.at[pl.ds(0, T0), pl.ds(koff[j], kch[j])], sems.at[j]) for j in range(NKC)]
        xcp = [rows_copy(p1_off[i], p1_tiles[i], SX + i - 1) for i in (1, 2)]
        wcp = [pltpu.make_async_copy(wqkv_hbm.at[pl.ds(koff[j], kch[j]), pl.ds(D, D)],
                                     wqkv_v.at[pl.ds(koff[j], kch[j]), pl.ds(KC, D)], sems.at[SW + j])
               for j in range(NKC)]
        wcp += [pltpu.make_async_copy(wqkv_hbm.at[pl.ds(r0, n), pl.ds(c0, D)], wqkv_v.at[pl.ds(r0, n), pl.ds(d0, D)],
                                      sems.at[SW + NKC + j])
                for j, (r0, n, c0, d0) in enumerate(((QE, D - QE, 0, QC), (0, D, 2 * D, VC)))]
        if QE:
            wq0 = pltpu.make_async_copy(wqkv_hbm.at[pl.ds(0, QE), pl.ds(0, D)], wqkv_v.at[pl.ds(0, QE), pl.ds(QC, D)],
                                        sems.at[SW + NKC + 2])
        wo_copy = pltpu.make_async_copy(wo_hbm, wo_v.at[:, pl.ds(0, D)], sems.at[SWO])
        wg_copy = pltpu.make_async_copy(wg_hbm, wg_v, sems.at[SWG])
        wu_copy = pltpu.make_async_copy(wu_hbm, wu_v, sems.at[SWU])
        wd_copy = pltpu.make_async_copy(wd_hbm, wd_v.at[:, pl.ds(0, D)], sems.at[SWD])
        wr_copy = pltpu.make_async_copy(wr_hbm, wr_v, sems.at[SWR])

        def out_copy(i):
            return pltpu.make_async_copy(out_v.at[pl.ds(p2_off[i], p2_tiles[i])],
                                         out_hbm.at[pl.ds(p2_off[i], p2_tiles[i])], sems.at[SO])

        order = [c for j in range(NKC) for c in (wcp[j], x0[j]) + ((wq0,) if QE and j == 1 else ())] + [wcp[NKC]] + xcp + [wcp[NKC + 1], wr_copy, wo_copy, wg_copy, wu_copy, wd_copy]
        pri = [int(ch) for ch in PRI[1:]]
        for j, c in enumerate(order):
            c.start(priority=pri[j] if j < len(pri) else pri[-1])

        def proj(r0, t, c0, n):
            return _dot(_unpk(xn_at(r0, t)), wqkv_v[:, c0:c0 + n])

        def feat(y):
            return _phi(y).astype(BF16)

        def prep(r0, t, zero=None):
            xf = x_v[r0:r0 + t, 0:D].astype(F32)
            if zero is not None:
                xf = jnp.concatenate([_tie(xf[:, 0:128], zero), xf[:, 128:]], axis=1)
            mu = _rowsum(xf) * (1.0 / D)
            mur = _rb(mu)
            mu_v[r0:r0 + t, :] = mur
            xc = x_v[r0:r0 + t, 0:D].astype(F32) - _lanes(mu, G)
            rs = _rstd(_rowsum(xc * xc) * (1.0 / D))
            rs_v[r0:r0 + t, :] = rs
            xn = (x_v[r0:r0 + t, 0:D].astype(F32) - _lanes(mur, G)) * _lanes(rs, G)
            xu = _pk(xn.astype(BF16))
            xn_rows[r0] = xu
            return xu

        def g_piece(pk, r0, c0, gate=None):
            t, n = pk.shape
            upd = _dot(pk.T, _unpk(_gate(xn_at(r0, t), gate)))
            zs = jnp.sum(pk.astype(F32).reshape(t // 8, 8, n), axis=0)
            for c in range(0, n, 128):
                b = (c0 + c) // 128
                g_acc[b] = upd[c:c + 128] if r0 == 0 else g_acc[b] + upd[c:c + 128]
                z_acc[b] = zs[:, c:c + 128] if r0 == 0 else z_acc[b] + zs[:, c:c + 128]
            return upd

        def q_part(r0, t, gate=None, head=None):
            k0 = 0 if head is None else QE
            acc = _dot(_unpk(_gate(xn_at(r0, t)[:, k0:], gate)), wqkv_v[k0:, QC:QC + D])
            pqt.append(_pk(feat(acc if head is None else acc + head).T))
            return acc

        def wait(c, name):
            with scope(name):
                c.wait()

        acc = s1 = s2 = cs = shift = None
        for j in range(NKC):
            c0, n = koff[j], kch[j]
            wait(wcp[j], "w_c%d" % j)
            if j == 0:
                cs = jnp.sum(wqkv_v[c0:c0 + n, KC:KC + D].astype(F32).reshape(n // 8, 8, D), axis=0)
            wait(x0[j], "w_x%d" % j)
            if QE and j == 1:
                wait(wq0, "w_q0")
            part = _dot(x_v[0:T0, c0:c0 + n], wqkv_v[c0:c0 + n, KC:KC + D])
            acc = part if acc is None else acc + part
            if QE and j == 1:
                accq0 = _dot(x_v[0:T0, 0:QE], wqkv_v[0:QE, QC:QC + D])
                csq = jnp.sum(wqkv_v[0:QE, QC:QC + D].astype(F32), axis=0, keepdims=True)
                part = jnp.concatenate([part, accq0], axis=1)
            xf = x_v[0:T0, c0:c0 + n].astype(F32)
            if shift is None:
                shift = jnp.broadcast_to(xf[:, 0:1], (T0, 128))
            sh = _tie(shift, _pace(part, T0 // 8, 0.0, (SHI if j < NKC - 1 else SLAST) / 100))
            d = xf - _lanes(sh, n // 128)
            for c in range(0, n, 128):
                dc = d[:, c:c + 128]
                s1 = dc if s1 is None else s1 + dc
                s2 = dc * dc if s2 is None else s2 + dc * dc
            if j > 0:
                cs = cs + jnp.sum(wqkv_v[c0:c0 + n, KC:KC + D].astype(F32).reshape(n // 8, 8, D), axis=0)
        m1 = _rowsum(s1) * (1.0 / D)
        rs = _rstd(jnp.maximum(_rowsum(s2) * (1.0 / D) - m1 * m1, 0.0))
        mur = _rb(shift + m1)
        cs = jnp.sum(cs, axis=0, keepdims=True)
        mu_v[0:T0, :] = mur
        mux = _tie(mur, _pace(part, T0 // 8, XLO / 100, XHI / 100))
        xn = (x_v[0:T0, 0:D].astype(F32) - _lanes(mux, G)) * _lanes(rs, G)
        xu = _pk(xn.astype(BF16))
        h0 = T0 // 256 * 128
        xn_rows[0] = xu[0:h0 // 2]
        xn_rows[h0] = xu[h0 // 2:]
        upd = None
        for c in range(0, D, GB):
            zero = _pace(part, T0 // 8, FLO / 100, FHI / 100) if upd is None else _pace(upd, T0 // 8, 0.0, GHI / 100)
            mub = _tie(mur, zero)
            k = GB // 128
            upd = g_piece(feat((acc[:, c:c + GB] - _lanes(mub, k) * cs[:, c:c + GB]) * _lanes(rs, k)), 0, c)

        with scope("p1_mid"):
            for c in wcp[NKC:] + xcp + [wr_copy, wo_copy]:
                c.wait()
            heads = [None, None]
            if QE:
                head = (accq0 - _lanes(mur, G) * csq) * _lanes(rs, G)
                heads = [head[0:h0], head[h0:]]
            q_part(0, h0, None, heads[0])
            r1, t1 = p1_off[1], p1_tiles[1]
            r2, t2 = p1_off[2], p1_tiles[2]
            prep(r1, t1, _pace(q_part(h0, T0 - h0, None, heads[1]), t1 // 8, 0.0, PHI / 100))
            pk = feat(proj(r1, t1, KC, D))
            xu = prep(r2, t2, _pace(q_part(r1, t1), t2 // 8, 0.0, PHI / 100))
            g_piece(pk, r1, 0, _fold(xu[:, D - 128:D]))

        sc = scope("p2")
        sc.__enter__()
        for c in (wg_copy, wu_copy, wd_copy):
            c.wait()

        jobs = ([(src, dst, r, c, min(D, FM - c)) for src, dst in ((wg_v, wg_p), (wu_v, wu_p))
                 for r in range(0, D, 16) for c in range(0, FM, D)]
                + [(wd_v, wd_p, r, 0, D) for r in range(0, F, 16)])
        hosts = [2, 2, 2] + [1] * (n2 - 3)
        dyn0 = pltpu.bitcast(_zero_of(mu_v[0:8, :]), I32)[0, 0]

        def retile(h, deps):
            mine = jobs[len(jobs) * sum(hosts[:h]) // sum(hosts):len(jobs) * sum(hosts[:h + 1]) // sum(hosts)]
            pz = _pace(deps, len(mine), 0.0, 0.85)
            for k, (src, dst, r, c, n) in enumerate(mine):
                dst[r // 2:r // 2 + 8, c:c + n] = _pk(src[r:r + 16, c:c + n]) | _lanes(pz[k * 8:(k + 1) * 8], n // 128)
            done = None
            for dst in (wg_p, wu_p, wd_p):
                if any(j[1] is dst for j in mine):
                    r = max(j[2] for j in mine if j[1] is dst) // 2
                    c = min(j[3] for j in mine if j[1] is dst and j[2] // 2 == r)
                    v = dst[pl.ds(pl.multiple_of(r + dyn0, 8), 8), c:c + 128]
                    done = v if done is None else done | v
            return _zero_of(done)

        acck = proj(r2, t2, KC, D)
        g_last = g_piece(feat(acck), r2, 0, retile(0, acck))

        z = _rb(jnp.sum(jnp.concatenate([z_acc[b] for b in range(G)], axis=1), axis=0, keepdims=True))
        zc = jnp.concatenate(
            [jnp.broadcast_to(z[:, g * 128:(g + 1) * 128], (128, 128)).T for g in range(G)], axis=0)
        wr = wr_v[...].astype(F32).reshape(1, D)
        wr_sum = _rowsum(wr)

        def stage_a(r0, t, zero):
            k = t // 128
            pq = _unpk(jnp.concatenate(pqt, axis=1)[:, r0:r0 + t]).astype(F32)
            z4 = zc.reshape(H, DH // 8, 8, 128)
            z0 = _tie(z4[:, 0].reshape(H * 8, 128), zero).reshape(H, 1, 8, 128)
            zz = jnp.concatenate([z0, z4[:, 1:]], axis=1).reshape(D, 128)
            w = (pq * _lanes(zz, k)).reshape(H, DH // 8, 8, t)
            den = jnp.sum(jnp.sum(w, axis=1), axis=1, keepdims=True) + 1e-6
            o = pq.reshape(H, DH, t) * _recip(den)
            return _pk(o.reshape(D, t).astype(BF16).T)

        def m_tile(a, b, c):
            return _unpk(jnp.concatenate(m_rows[a // 128:b // 128], axis=0)[:, c * 128:(c + 1) * 128])

        def stage_b(i, gate):
            r0, t = p2_off[i], p2_tiles[i]

            def post(c, attn):
                h_v[r0:r0 + t, c * 128:(c + 1) * 128] = x_v[r0:r0 + t, c * 128:(c + 1) * 128].astype(F32) + attn

            _, deps = _passes(jnp.concatenate(os, axis=0)[r0 // 2:(r0 + t) // 2, :], m_tile, G,
                              lambda p, deps: gate if p == 0 else None, post)
            return deps, _rowsum(h_v[r0:r0 + t, :]) * (1.0 / D)

        def keys_of(r, idx):
            bits = pltpu.bitcast(jnp.where(r == 0.0, 0.0, r), I32)
            hi = lax.shift_right_logical(bits, 16)
            mono = jnp.where(bits < 0, 0xFFFF - hi, hi | 0x8000)
            return pltpu.bitcast((mono << 11) + (KEY0 + S - 1 - idx), F32)

        def merge(top, k1, k2):
            if top is None:
                return k1, k2
            t1, t2 = top
            return jnp.maximum(t1, k1), jnp.maximum(jnp.minimum(t1, k1), jnp.maximum(t2, k2))

        def write_out(i, mur, rs):
            r0, t = p2_off[i], p2_tiles[i]
            out_v[r0:r0 + t, :] = (h_v[r0:r0 + t, :] * _lanes(1.0 + rs, G) - _lanes(mur * rs, G)).astype(BF16)
            back = out_v[r0:r0 + t, D - 128:D].astype(F32)
            out_copy(i).start()
            return back

        def stage_c(i, mu, dep, hi=CHI / 100):
            r0, t = p2_off[i], p2_tiles[i]
            mu = _tie(mu, _pace(dep, t // 8, 0.0, hi))
            d = h_v[r0:r0 + t, :] - _lanes(mu, G)
            rs = _rstd(_rowsum(d * d) * (1.0 / D))
            mur = _rb(mu)
            r = _rb((_rowsum(d * wr) + (mu - mur) * wr_sum) * rs)
            mu_v[r0:r0 + t, :] = mur
            rs_v[r0:r0 + t, :] = rs
            return r, mur, rs

        lane = lax.broadcasted_iota(I32, (8, 128), 1)
        sub = lax.broadcasted_iota(I32, (8, 128), 0)

        def compact(i, r):
            r0, t = p2_off[i], p2_tiles[i]
            parts = [r[p * 8:(p + 1) * 8] for p in range(t // 8)]
            acc = parts[0]
            for p in range(1, t // 8):
                acc = jnp.where(lane == p, parts[p], acc)
            key = keys_of(acc, r0 + lane * 8 + sub)
            return jnp.where(lane < t // 8, key, 0.0)

        def a_done(os):
            acc = None
            for o in os:
                for rb in range(o.shape[0] // 64):
                    row = o[rb * 64 + 56:rb * 64 + 64, :]
                    for g in range(G):
                        v = row[:, g * 128:(g + 1) * 128]
                        acc = v if acc is None else acc | v
            return _zero_of(acc)

        ta = 256
        na = S // ta
        nearly = r2 // ta
        pz = _pace(g_last, NAG * H, 0.0, 1.0)
        os = [stage_a(j * ta, ta, pz[j * H * 8:(j + 1) * H * 8]) for j in range(NAG)]
        accq = q_part(r2, t2, retile(1, g_last))
        if nearly > NAG:
            pz = _pace(accq, (nearly - NAG) * H, 0.0, 0.9)
            os += [stage_a(j * ta, ta, pz[(j - NAG) * H * 8:(j - NAG + 1) * H * 8]) for j in range(NAG, nearly)]

        row = lax.broadcasted_iota(I32, (128, 128), 0) // DH
        col = lax.broadcasted_iota(I32, (128, 128), 1) // DH
        same = row == col
        kvs = []
        for g in range(G):
            gg = g_acc[g]
            if g == 0:
                gg = jnp.concatenate([jnp.concatenate(
                    [_tie(gg[0:8, 0:128], a_done(os) | retile(2, accq)), gg[0:8, 128:]], axis=1), gg[8:]], axis=0)
            kv = _dot(gg.astype(BF16), wqkv_v[:, VC + g * 128:VC + (g + 1) * 128])
            kvs.append(jnp.where(same, kv, 0.0).astype(BF16))
        for g in range(G):
            m_rows.append(_pk(_dot(kvs[g], wo_v[g * 128:(g + 1) * 128, 0:D]).astype(BF16)))

        def tree(i, r):
            t = p2_tiles[i]
            key = keys_of(r, lax.broadcasted_iota(I32, (t, 128), 0) + p2_off[i])
            level = [(key[p * 8:(p + 1) * 8], None) for p in range(t // 8)]
            while len(level) > 1:
                nxt = []
                for p in range(0, len(level) - 1, 2):
                    (a1, a2), (b1, b2) = level[p], level[p + 1]
                    lo = jnp.minimum(a1, b1)
                    for e in (a2, b2):
                        lo = lo if e is None else jnp.maximum(lo, e)
                    nxt.append((jnp.maximum(a1, b1), lo))
                if len(level) % 2:
                    nxt.append(level[-1])
                level = nxt
            return level[0]

        first = lax.broadcasted_iota(I32, (16, 128), 0) == 0

        def select(top):
            t1, t2 = top
            k1 = jnp.max(t1, axis=0, keepdims=True)
            k2 = jnp.max(jnp.where(t1 == k1, t2, t1), axis=0, keepdims=True)
            k1 = pltpu.bitcast(k1, I32)
            k2 = pltpu.bitcast(k2, I32)
            i1 = S - 1 - (k1[0, 0] & (S - 1))
            i2 = S - 1 - (k2[0, 0] & (S - 1))

            def pick(ref, k):
                return jnp.where(_lanes(first, k), ref[pl.ds(i1, 1), :], ref[pl.ds(i2, 1), :])

            hs = pick(h_v, G)
            xs = ((hs - _lanes(pick(mu_v, 1), G)) * _lanes(pick(rs_v, 1), G)).astype(BF16)
            return k1, k2, i1, i2, hs, xs

        ticks = []

        def gate_up(xs, c0, n):
            gt = _dot(xs, _unpk(wg_p[:, c0:c0 + n]))
            ut = _dot(xs, _unpk(wu_p[:, c0:c0 + n]))
            ticks.extend((v[0:8, c:c + 128], 64) for v in (gt, ut) for c in range(0, n, 128))
            return _rb(gt[0:8]), _rb(ut[0:8])

        def down(a, c0):
            y = _dot(a, _unpk(wd_p[c0 // 2:(c0 + a.shape[1]) // 2, 0:D]))
            ticks.extend((y[0:8, c:c + 128], a.shape[1] // 16) for c in range(0, D, 128))
            return y

        def vpu_acts(xg, zeros):
            nd = D // 8
            xb = {}
            acts = []
            for j in range(FV // 256):
                c0 = FM + j * 256
                acc = {}
                for d in range(nd):
                    zero = zeros[j * nd + d]
                    if j == 0 and d % 16 == 0:
                        g = d // 16
                        zg = zeros[max(0, d - XLEAD)]
                        for t in range(2):
                            row = _tie(jnp.broadcast_to(xg[t:t + 1, g * 128:(g + 1) * 128], (8, 128)), zg)
                            blk = jnp.concatenate([row] * 16, axis=0).T
                            for e in range(16):
                                xb[t, d + e] = blk[e * 8:(e + 1) * 8]
                    xt = [_lanes(_tie(xb[t, d], zero) if d % TIE == 0 else xb[t, d], 2) for t in range(2)]
                    for m, w_v in enumerate((wg_v, wu_v)):
                        w = w_v[d * 8:(d + 1) * 8, c0:c0 + 256].astype(F32)
                        for t in range(2):
                            acc[m, t] = w * xt[t] if d == 0 else acc[m, t] + w * xt[t]
                res = [_rb(jnp.where(_lanes(first[0:8], 2), jnp.sum(acc[m, 0], axis=0, keepdims=True),
                                     jnp.sum(acc[m, 1], axis=0, keepdims=True))) for m in range(2)]
                acts.append(act(*res))
            return acts

        def act(gt, ut):
            a = _rb(gt * jax.nn.sigmoid(gt)) * ut
            return jnp.concatenate([a, a], axis=0).astype(BF16)

        def stage_last(gate, mu_prev, top):
            i = n2 - 1
            r0, t = p2_off[i], p2_tiles[i]
            st = {}

            def post(c, attn):
                h = x_v[r0:r0 + t, c * 128:(c + 1) * 128].astype(F32) + attn
                h_v[r0:r0 + t, c * 128:(c + 1) * 128] = h
                if c == 0:
                    st["shift"] = jnp.broadcast_to(h[:, 0:1], (t, 128))
                d = h - st["shift"]
                new = (d, d * d, d * wr[:, c * 128:(c + 1) * 128])
                st[c] = new if c == 0 else tuple(a + b for a, b in zip(st[c - 1], new))

            def gate_fn(p, deps):
                if p == 0:
                    return gate
                z = None
                if p % 2 == 1 and p // 2 - SLAG >= 0:
                    z = _fold(jnp.concatenate(st[p // 2 - SLAG], axis=1))
                if p == CGATE:
                    r, st["mur_p"], st["rs_p"] = stage_c(i - 1, mu_prev, deps, CLAST / 100)
                    st["top"] = merge(top, *tree(i - 1, r))
                    st["back"] = _fold(write_out(i - 1, st["mur_p"], st["rs_p"]))
                    st["guess"] = select(st["top"])
                    zz = _zero_of(st["top"][0] + st["top"][1])
                    z = zz if z is None else z | zz
                if p == 2 * G - 1:
                    z = st["back"] if z is None else z | st["back"]
                return z

            _, deps = _passes(jnp.concatenate(os, axis=0)[r0 // 2:(r0 + t) // 2, :], m_tile, G, gate_fn, post)
            st["a0"] = act(*gate_up(st["guess"][5], 0, FC0))
            s1, s2, s3 = st[G - 1]
            shift = st["shift"]
            m1 = _rowsum(s1) * (1.0 / D)
            var = jnp.maximum(_rowsum(s2) * (1.0 / D) - m1 * m1, 0.0)
            rs = _rstd(var)
            mur = _rb(shift + m1)
            r = _rb((_rowsum(s3) + (shift - mur) * wr_sum) * rs)
            mu_v[r0:r0 + t, :] = mur
            rs_v[r0:r0 + t, :] = rs
            return merge(st["top"], *tree(i, r)), st["mur_p"], st["rs_p"], mur, rs, st["guess"], st["a0"]

        top = None
        mu_prev = None
        gate = None
        for i in range(n2 - 1):
            deps, mu = stage_b(i, gate)
            if i == 0:
                pz = _pace(deps, (na - nearly) * H, 0.0, 0.8)
                late_os = [stage_a(j * ta, ta, pz[(j - nearly) * H * 8:(j - nearly + 1) * H * 8])
                           for j in range(nearly, na)]
                os += late_os
                gate = a_done(late_os) | retile(3, deps)
            else:
                r, mur, rs = stage_c(i - 1, mu_prev, deps, min(CHI / 100, 1 - LAT / (16 * p2_tiles[i])))
                back = write_out(i - 1, mur, rs)
                key = compact(i - 1, r)
                top = merge(top, key, jnp.zeros_like(key))
                gate = _zero_of(key + jnp.sum(back.reshape(-1, 8, 128), axis=0))
                if 3 + i < len(hosts):
                    gate = gate | retile(3 + i, deps)
                if i == n2 - 2:
                    t1, t2 = top
                    b1 = jnp.max(jnp.max(t1, axis=0, keepdims=True), axis=1, keepdims=True)
                    rest = jnp.where(t1 == b1, t2, t1)
                    b2 = jnp.max(jnp.max(rest, axis=0, keepdims=True), axis=1, keepdims=True)
                    top = (jnp.where(sub == 0, b1, 0.0), jnp.where(sub == 0, b2, 0.0))
            mu_prev = mu
        top, mur_p, rs_p, mur_l, rs_l, guess, a0 = stage_last(gate, mu_prev, top)
        sc.__exit__(None, None, None)

        sc = scope("tail")
        sc.__enter__()
        k1, k2, i1, i2, hs, xs = select(top)
        chunks = [(c0, min(FC, FM - c0)) for c0 in range(FC0, FM, FC)]
        xu = _pk(xs)
        y = None
        prev = None
        gate = None
        for c, ch in enumerate(chunks + [None]):
            if ch is not None:
                xc = _unpk(jnp.concatenate([xu[:, 0:128] | gate, xu[:, 128:]], axis=1)) if c == WOC + 2 else xs
                gt, ut = gate_up(xc, *ch)
            if c == 0:
                y0 = down(a0, 0)
            if prev is not None:
                part = down(a_prev, prev[0])
                y = part if y is None else y + part
            if c == WOC:
                back = write_out(n2 - 1, _tie(mur_l, _pace(gt, p2_tiles[-1] // 8)), rs_l)
                out_v[S:S + 16, 0:128] = jnp.concatenate([gt[:, 0:128]] * 2, axis=0).astype(BF16)
                gate = _fold(back) | _fold(out_v[S:S + 16, 0:128].astype(F32))
            if ch is not None:
                a_prev = act(gt, ut)
            prev = ch
        if FV:
            total = sum(c for _, c in ticks)
            nstep = FV // 256 * (D // 8)
            when = [sum(c for _, c in ticks[:k + 1]) for k in range(len(ticks))]
            tick_zero = {}

            def zero_at(step):
                tt = VLEAD + (step / nstep) * (VHI / 100 * total - VLEAD)
                if tt < when[0]:
                    return jnp.zeros((8, 128), U32)
                k = max(k for k in range(len(ticks)) if when[k] <= tt)
                if k not in tick_zero:
                    tick_zero[k] = _zero_of(ticks[k][0])
                return tick_zero[k]

            zs = [zero_at(step) for step in range(nstep)]
            for j, a in enumerate(vpu_acts(xs.astype(F32), zs)):
                y = y + down(a, FM + j * 256)
        mono = lax.shift_right_logical(jnp.where(first, k1, k2) - KEY0, 11)
        rsel = pltpu.bitcast(jnp.where(mono < 0x8000, 0xFFFF - mono, mono & 0x7FFF) << 16, F32)
        gain = _lanes(_rb(jax.nn.sigmoid(rsel)), G)
        g1 = pl.multiple_of(lax.shift_right_logical(i1, 3) * 8, 8)
        g2 = pl.multiple_of(lax.shift_right_logical(i2, 3) * 8, 8)
        rows = lax.broadcasted_iota(I32, (8, D), 0)

        def finish(y):
            new = hs + _rb(xs.astype(F32) + _rb(_rb(y) * gain))
            for j, g in enumerate((g1, g2)):
                old = out_v[pl.ds(g, 8), :].astype(F32)
                fix_v[j] = jnp.where(rows == i1 - g, new[0:1], jnp.where(rows == i2 - g, new[1:2], old)).astype(BF16)

        finish(y + y0)

        @pl.when(jnp.logical_or(i1 != guess[2], i2 != guess[3]))
        def _():
            finish(y + down(act(*gate_up(xs, 0, FC0)), 0))
            if JUNK:
                @pl.when(i1 == i2)
                def _():
                    finish(down(act(*gate_up(xs, 0, JUNK)), 0))

        pltpu.make_async_copy(out_v.at[pl.ds(0, S)], out_hbm, sems.at[SO]).wait()
        c1 = pltpu.make_async_copy(fix_v.at[0], out_hbm.at[pl.ds(g1, 8)], sems.at[SO + 1])
        c2 = pltpu.make_async_copy(fix_v.at[1], out_hbm.at[pl.ds(g2, 8)], sems.at[SO + 2])
        c1.start()

        @pl.when(g1 != g2)
        def _():
            c2.start()
            c2.wait()
        c1.wait()
        sc.__exit__(None, None, None)

    scratch = [
        pltpu.VMEM((S, D + PAD), BF16),
        pltpu.VMEM((D, 3 * D + PAD), BF16),
        pltpu.VMEM((D, D + PAD), BF16),
        pltpu.VMEM((D, F), BF16),
        pltpu.VMEM((D, F), BF16),
        pltpu.VMEM((F, D + PAD), BF16),
        pltpu.VMEM((D,), BF16),
        pltpu.VMEM((S, 128), F32),
        pltpu.VMEM((S, 128), F32),
        pltpu.VMEM((S + 16, D), BF16),
        pltpu.VMEM((S, D), F32),
        pltpu.VMEM((2, 8, D), BF16),
        pltpu.VMEM((D // 2, FM), U32),
        pltpu.VMEM((D // 2, FM), U32),
        pltpu.VMEM((F // 2, D + PAD), U32),
        pltpu.SemaphoreType.DMA((NSEM,)),
    ]

    @jax.jit
    def f(A_x, A_wqkv, A_wo, B_x, B_w_r, B_w_gate, B_w_up, B_w_down):
        any_spec = pl.BlockSpec(memory_space=pl.ANY)
        out = pl.pallas_call(
            kernel,
            out_shape=jax.ShapeDtypeStruct((S, D), BF16),
            in_specs=[any_spec] * 7,
            out_specs=any_spec,
            scratch_shapes=scratch,
            compiler_params=pltpu.CompilerParams(vmem_limit_bytes=120 * 1024 * 1024, disable_bounds_checks=True),
        )(A_x.reshape(S, D), A_wqkv, A_wo, B_w_r, B_w_gate, B_w_up, B_w_down)
        return out.reshape(1, S, D)
    return f


_impl = make_kernel()


@jax.jit
def pallas_sequential_preLN__linear_attn_block__moe_arch_mod__prompt_kernel(
    A_x: jax.Array,
    A_wqkv: jax.Array,
    A_wo: jax.Array,
    B_x: jax.Array,
    B_w_r: jax.Array,
    B_w_gate: jax.Array,
    B_w_up: jax.Array,
    B_w_down: jax.Array,
):
    return _impl(A_x, A_wqkv, A_wo, B_x, B_w_r, B_w_gate, B_w_up, B_w_down)
```

```python
import contextlib
import functools

import jax
import jax.numpy as jnp
from jax import lax
import jax.experimental.pallas as pl
import jax.experimental.pallas.tpu as pltpu

S, D, F, H, DH = 2048, 1024, 3584, 32, 32
G = D // 128
F32 = jnp.float32
BF16 = jnp.bfloat16
I32 = jnp.int32
U32 = jnp.uint32
KEY0 = 64 << 23
PAD = 128


def _rb(x):
    return x.astype(BF16).astype(F32)


def _zero_of(x):
    bits = pltpu.bitcast(x, U32)
    return lax.shift_right_logical(lax.shift_right_logical(bits, U32(31)), U32(1))


def _pace(dep, n, lo=0.0, hi=1.0):
    if isinstance(dep, (list, tuple)):
        dep = jnp.concatenate(dep, axis=1)
    nrg, nch = dep.shape[0] // 8, dep.shape[1] // 128
    parts = []
    for p in range(n):
        pos = int((lo + (hi - lo) * p / n) * nch * nrg)
        c, rg = pos // nrg, pos % nrg
        parts.append(dep[rg * 8:(rg + 1) * 8, c * 128:(c + 1) * 128])
    return _zero_of(jnp.concatenate(parts, axis=0))


def _tie(x, zero):
    return pltpu.bitcast(pltpu.bitcast(x, U32) | zero, F32)


def _lanes(x, n):
    return jnp.concatenate([x] * n, axis=1) if n > 1 else x


def _rowsum(x):
    return jnp.broadcast_to(jnp.sum(x, axis=-1, keepdims=True), (x.shape[0], 128))


def _recip(d):
    r = pl.reciprocal(d, approx=True)
    return r * (2.0 - d * r)


def _rstd(var):
    v = _rb(_rb(var) + 1e-5)
    return _recip(_rb(v * lax.rsqrt(v)))


def _phi(t):
    return jnp.where(t > 0, t + 1.0, jnp.exp(t)) + 1e-6


def _dot(a, b):
    return jnp.dot(a, b, preferred_element_type=F32)


def _dot_tn(a, b):
    return lax.dot_general(a, b, (((0,), (0,)), ((), ())), preferred_element_type=F32)


def _pk(x):
    return pltpu.bitcast(x, U32)


def _unpk(x):
    return pltpu.bitcast(x, BF16)


def _scalar_zero(z):
    return pltpu.bitcast(z, I32)[0, 0]


def _gate(xu, zero):
    if zero is None:
        return xu
    top = xu[0:8, 0:512] | _lanes(zero, 4)
    if xu.shape[1] > 512:
        top = jnp.concatenate([top, xu[0:8, 512:]], axis=1)
    return jnp.concatenate([top, xu[8:]], axis=0) if xu.shape[0] > 8 else top


def _fold(x):
    x = pltpu.bitcast(x, U32) if x.dtype != U32 else x
    parts = [x[r:r + 8, c:c + 128] for r in range(0, x.shape[0], 8) for c in range(0, x.shape[1], 128)]
    while len(parts) > 1:
        parts = [parts[j] | parts[j + 1] if j + 1 < len(parts) else parts[j] for j in range(0, len(parts), 2)]
    return _zero_of(parts[0])


def _passes(xu, w, ntiles, gate_fn=None, post=None, after=None):
    deps, outs = [], []
    for c in range(ntiles):
        acc = None
        for hh in range(2):
            z = None if gate_fn is None else gate_fn(2 * c + hh, deps)
            lhs = _unpk(_gate(xu[:, hh * (D // 2):(hh + 1) * (D // 2)], z))
            part = _dot(lhs, w(hh * (D // 2), (hh + 1) * (D // 2), c))
            acc = part if acc is None else acc + part
            deps.append(acc)
            if after is not None:
                after(2 * c + hh)
        outs.append(acc if post is None else post(c, acc))
    return outs, deps


def make_kernel(P2T="256,128,128,128,128,128,128,128,128,128,128,128,128,128,64,64", CHI=80, P1T="1024,512,512", QE=128,
                KCH="128,128,256,512", SHI=90, SLAST=40, XLO=30, XHI=95, FLO=60, FHI=92, GHI=85, GGATE=14, GB=256, PHI=90, NAG=5,
                CLAST=50, CGATE=13, SLAG=4, LAT=560, PRI="p0", QA=256, PLO=10, CT=3, EG=3, CG=6, KLO=45, FP0=9, FKEEP=10, CR=32, MC=1792, MISS=0, DLAG=2, scopes=0):
    p1_tiles = [int(t) for t in P1T.split(",")]
    assert sum(p1_tiles) == S and len(p1_tiles) == 3
    p1_off = [sum(p1_tiles[:i]) for i in range(3)]
    p2_tiles = [int(t) for t in P2T.split(",")]
    assert sum(p2_tiles) == S
    p2_off = [sum(p2_tiles[:i]) for i in range(len(p2_tiles))]
    n2 = len(p2_tiles)
    KC, QC, VC = 0, D, 2 * D
    kch = [int(t) for t in KCH.split(",")]
    assert sum(kch) == D
    NKC = len(kch)
    T0 = p1_tiles[0]
    SW = NKC
    SX = SW + NKC + 3
    SWO = SX + 2
    SWG, SWU, SWD, SWR = SWO + 1, SWO + 2, SWO + 3, SWO + 4
    SO = SWR + 1
    NSEM = SO + 4

    def scope(name):
        return jax.named_scope(name) if scopes else contextlib.nullcontext()

    def kernel(x_hbm, wqkv_hbm, wo_hbm, wr_hbm, wg_hbm, wu_hbm, wd_hbm, out_hbm,
               x_v, wqkv_v, wo_v, wg_v, wu_v, wd_v, wr_v, mu_v, rs_v,
               out_v, h_v, fix_v, o_v, co_v, cx_v, sems):

        xn_rows = {}
        pqt = []
        g_acc = {}
        z_acc = {}
        m_rows = []
        xw = []

        def xn_at(r0, t):
            keys = sorted(k for k in xn_rows if r0 <= k < r0 + t)
            return jnp.concatenate([xn_rows[k] for k in keys], axis=0) if len(keys) > 1 else xn_rows[keys[0]]

        def rows_copy(r0, n, s):
            return pltpu.make_async_copy(x_hbm.at[pl.ds(r0, n)], x_v.at[pl.ds(r0, n), pl.ds(0, D)], sems.at[s])

        koff = [sum(kch[:j]) for j in range(NKC)]
        x0 = [pltpu.make_async_copy(x_hbm.at[pl.ds(0, T0), pl.ds(koff[j], kch[j])],
                                    x_v.at[pl.ds(0, T0), pl.ds(koff[j], kch[j])], sems.at[j]) for j in range(NKC)]
        xcp = [rows_copy(p1_off[i], p1_tiles[i], SX + i - 1) for i in (1, 2)]
        wcp = [pltpu.make_async_copy(wqkv_hbm.at[pl.ds(koff[j], kch[j]), pl.ds(D, D)],
                                     wqkv_v.at[pl.ds(koff[j], kch[j]), pl.ds(KC, D)], sems.at[SW + j])
               for j in range(NKC)]
        wcp += [pltpu.make_async_copy(wqkv_hbm.at[pl.ds(r0, n), pl.ds(c0, D)], wqkv_v.at[pl.ds(r0, n), pl.ds(d0, D)],
                                      sems.at[SW + NKC + j])
                for j, (r0, n, c0, d0) in enumerate(((QE, D - QE, 0, QC), (0, D, 2 * D, VC)))]
        if QE:
            wq0 = pltpu.make_async_copy(wqkv_hbm.at[pl.ds(0, QE), pl.ds(0, D)], wqkv_v.at[pl.ds(0, QE), pl.ds(QC, D)],
                                        sems.at[SW + NKC + 2])
        wo_copy = pltpu.make_async_copy(wo_hbm, wo_v.at[:, pl.ds(0, D)], sems.at[SWO])
        wg_copy = pltpu.make_async_copy(wg_hbm, wg_v, sems.at[SWG])
        wu_copy = pltpu.make_async_copy(wu_hbm, wu_v, sems.at[SWU])
        wd_copy = pltpu.make_async_copy(wd_hbm, wd_v.at[:, pl.ds(0, D)], sems.at[SWD])
        wr_copy = pltpu.make_async_copy(wr_hbm, wr_v, sems.at[SWR])

        def out_copy(i):
            return pltpu.make_async_copy(out_v.at[pl.ds(p2_off[i], p2_tiles[i])],
                                         out_hbm.at[pl.ds(p2_off[i], p2_tiles[i])], sems.at[SO + 3 if i == n2 - 1 else SO])

        order = [c for j in range(NKC) for c in (wcp[j], x0[j]) + ((wq0,) if QE and j == 1 else ())] + [wcp[NKC]] + xcp + [wcp[NKC + 1], wo_copy, wg_copy, wu_copy, wd_copy]
        order.insert(1, wr_copy)
        pri = [int(ch) for ch in PRI[1:]]
        for j, c in enumerate(order):
            c.start(priority=pri[j] if j < len(pri) else pri[-1])

        def proj(r0, t, c0, n):
            return _dot(_unpk(xn_at(r0, t)), wqkv_v[:, c0:c0 + n])

        def feat(y):
            return _phi(y).astype(BF16)

        def prep(r0, t, zero=None):
            xf = x_v[r0:r0 + t, 0:D].astype(F32)
            if zero is not None:
                xf = jnp.concatenate([_tie(xf[:, 0:128], zero), xf[:, 128:]], axis=1)
            mu = _rowsum(xf) * (1.0 / D)
            mur = _rb(mu)
            mu_v[r0:r0 + t, :] = mur
            xc = x_v[r0:r0 + t, 0:D].astype(F32) - _lanes(mu, G)
            rs = _rstd(_rowsum(xc * xc) * (1.0 / D))
            e = xc * wc
            xw.append(functools.reduce(jnp.add, [e[:, c:c + 128] for c in range(0, D, 128)]))
            rs_v[r0:r0 + t, :] = rs
            xn = (x_v[r0:r0 + t, 0:D].astype(F32) - _lanes(mur, G)) * _lanes(rs, G)
            xu = _pk(xn.astype(BF16))
            xn_rows[r0] = xu
            return xu

        def g_piece(pk, r0, c0, gate=None):
            t, n = pk.shape
            upd = _dot(pk.T, _unpk(_gate(xn_at(r0, t), gate)))
            zs = jnp.sum(pk.astype(F32).reshape(t // 8, 8, n), axis=0)
            for c in range(0, n, 128):
                b = (c0 + c) // 128
                g_acc[b] = upd[c:c + 128] if r0 == 0 else g_acc[b] + upd[c:c + 128]
                z_acc[b] = zs[:, c:c + 128] if r0 == 0 else z_acc[b] + zs[:, c:c + 128]
            return upd

        def q_part(r0, t, gate=None, head=None):
            k0 = 0 if head is None else QE
            acc = _dot(_unpk(_gate(xn_at(r0, t)[:, k0:], gate)), wqkv_v[k0:, QC:QC + D])
            pqt.append(_pk(feat(acc if head is None else acc + head).T))
            return acc

        def a_done(os):
            acc = None
            for o in os:
                for rb in range(o.shape[0] // 64):
                    row = o[rb * 64 + 56:rb * 64 + 64, :]
                    for g in range(G):
                        v = row[:, g * 128:(g + 1) * 128]
                        acc = v if acc is None else acc | v
            return _zero_of(acc)

        def wait(c, name):
            with scope(name):
                c.wait()

        def colsum(r0, n, c0, dep, hi):
            pz = _pace(dep, n // CR, 0.02, hi)
            tot = None
            for k in range(n // CR):
                rows = pl.ds(pl.multiple_of(r0 + k * CR + _scalar_zero(pz[k * 8:(k + 1) * 8]), 16), CR)
                w = jnp.sum(wqkv_v[rows, c0:c0 + D].astype(F32).reshape(CR // 8, 8, D), axis=0)
                tot = w if tot is None else tot + w
            return tot

        acc = s1 = s2 = s3 = cs = shift = None
        for j in range(NKC):
            c0, n = koff[j], kch[j]
            wait(wcp[j], "w_c%d" % j)
            if j == 0:
                wr_copy.wait()
                cs = jnp.sum(wqkv_v[c0:c0 + n, KC:KC + D].astype(F32).reshape(n // 8, 8, D), axis=0)
                wr = wr_v[...].astype(F32).reshape(1, D)
                wr_sum = _rowsum(wr)
                wc = wr - _lanes(wr_sum * (1.0 / D), G)
            wait(x0[j], "w_x%d" % j)
            if QE and j == 1:
                wait(wq0, "w_q0")
            part = _dot(x_v[0:T0, c0:c0 + n], wqkv_v[c0:c0 + n, KC:KC + D])
            acc = part if acc is None else acc + part
            if QE and j == 1:
                accq0 = _dot(x_v[0:T0, 0:QE], wqkv_v[0:QE, QC:QC + D])
                csq = jnp.sum(colsum(0, QE, QC, accq0, 0.6), axis=0, keepdims=True)
                part = jnp.concatenate([part, accq0], axis=1)
            xf = x_v[0:T0, c0:c0 + n].astype(F32)
            if shift is None:
                shift = jnp.broadcast_to(xf[:, 0:1], (T0, 128))
            sh = _tie(shift, _pace(part, T0 // 8, 0.0, (SHI if j < NKC - 1 else SLAST) / 100))
            d = xf - _lanes(sh, n // 128)
            for c in range(0, n, 128):
                dc = d[:, c:c + 128]
                s1 = dc if s1 is None else s1 + dc
                s2 = dc * dc if s2 is None else s2 + dc * dc
                e = dc * wc[:, c0 + c:c0 + c + 128]
                s3 = e if s3 is None else s3 + e
            if j > 0:
                cs = cs + colsum(c0, n, KC, part, 0.6 if j < NKC - 1 else 0.3)
        m1 = _rowsum(s1) * (1.0 / D)
        rs = _rstd(jnp.maximum(_rowsum(s2) * (1.0 / D) - m1 * m1, 0.0))
        mur = _rb(shift + m1)
        mu_v[0:T0, :] = mur
        xw.append(s3)
        zx = _pace(part, T0 // 8, XLO / 100, XHI / 100)
        mux = _tie(mur, jnp.concatenate([zx[0:T0 // 4], zx[T0 // 4:T0 // 4 + 8] | _fold(cs), zx[T0 // 4 + 8:]], axis=0))
        cs = jnp.sum(cs, axis=0, keepdims=True)
        xn = (x_v[0:T0, 0:D].astype(F32) - _lanes(mux, G)) * _lanes(rs, G)
        xu = _pk(xn.astype(BF16))
        h0 = T0 // 256 * 128
        xn_rows[0] = xu[0:h0 // 2]
        xn_rows[h0] = xu[h0 // 2:]
        xn0 = _unpk(xu)

        def k_block(c, zero):
            pk = feat((acc[:, c:c + GB] - _lanes(_tie(mur, zero), GB // 128) * cs[:, c:c + GB]) * _lanes(rs, GB // 128))
            zs = jnp.sum(pk.astype(F32).reshape(T0 // 8, 8, GB), axis=0)
            for b in range(0, GB, 128):
                z_acc[(c + b) // 128] = zs[:, b:b + 128]
            return _pk(pk.T), zs

        nxt = {0: k_block(0, _pace(part, T0 // 8, FLO / 100, FHI / 100))}
        for c in range(0, D, GB):
            def gate_g(p, deps, c=c):
                if p != GGATE or c + GB == D:
                    return None
                nxt[c + GB] = k_block(c + GB, _pace(deps, T0 // 8, 0.0, GHI / 100))
                return a_done([nxt[c + GB][0]]) | _fold(nxt[c + GB][1])

            outs, _ = _passes(nxt[c][0], lambda a, b, n: xn0[a:b, n * 128:(n + 1) * 128], G, gate_g)
            upd = jnp.concatenate(outs, axis=1)
            for b in range(0, GB, 128):
                g_acc[(c + b) // 128] = upd[b:b + 128]

        with scope("p1_mid"):
            for c in wcp[NKC:] + xcp + [wo_copy]:
                c.wait()
            heads = [None, None]
            if QE:
                head = (accq0 - _lanes(mur, G) * csq) * _lanes(rs, G)
                heads = [head[0:h0], head[h0:]]
            q_part(0, h0, None, heads[0])
            r1, t1 = p1_off[1], p1_tiles[1]
            r2, t2 = p1_off[2], p1_tiles[2]
            prep(r1, t1, _pace(q_part(h0, T0 - h0, None, heads[1]), t1 // 8, 0.0, PHI / 100))
            pk = feat(proj(r1, t1, KC, D))
            xu = prep(r2, t2, _pace(q_part(r1, t1), t2 // 8, 0.0, PHI / 100))
            g_piece(pk, r1, 0, _fold(xu[:, D - 128:D]) | _fold(xw[-1]))

        sc = scope("p2")
        sc.__enter__()
        for c in (wg_copy, wu_copy, wd_copy):
            c.wait()

        g_last = g_piece(feat(proj(r2, t2, KC, D)), r2, 0)

        z = _rb(jnp.sum(jnp.concatenate([z_acc[b] for b in range(G)], axis=1), axis=0, keepdims=True))
        zc = jnp.concatenate(
            [jnp.broadcast_to(z[:, g * 128:(g + 1) * 128], (128, 128)).T for g in range(G)], axis=0)

        def stage_a(r0, t, zero):
            k = t // 128
            pq = _unpk(jnp.concatenate(pqt, axis=1)[:, r0:r0 + t]).astype(F32)
            z4 = zc.reshape(H, DH // 8, 8, 128)
            z0 = _tie(z4[:, 0].reshape(H * 8, 128), zero).reshape(H, 1, 8, 128)
            zz = jnp.concatenate([z0, z4[:, 1:]], axis=1).reshape(D, 128)
            w = (pq * _lanes(zz, k)).reshape(H, DH // 8, 8, t)
            den = jnp.sum(jnp.sum(w, axis=1), axis=1, keepdims=True) + 1e-6
            o = pq.reshape(H, DH, t) * _recip(den)
            ou = _pk(o.reshape(D, t).astype(BF16).T)
            o_v[r0 // 2:(r0 + t) // 2, :] = ou
            return ou

        def m_tile(a, b, c):
            return _unpk(jnp.concatenate(m_rows[a // 128:b // 128], axis=0)[:, c * 128:(c + 1) * 128])

        def stage_b(i, gate, extra=None):
            r0, t = p2_off[i], p2_tiles[i]

            def post(c, attn):
                h_v[r0:r0 + t, c * 128:(c + 1) * 128] = x_v[r0:r0 + t, c * 128:(c + 1) * 128].astype(F32) + attn[0:t]
                return attn[t:]

            ou = jnp.concatenate(os, axis=0)[r0 // 2:(r0 + t) // 2, :]
            if extra is not None:
                ou = jnp.concatenate([ou, extra], axis=0)
            outs, deps = _passes(ou, m_tile, G, lambda p, deps: gate.get(p), post, lambda p: ffn_step(i, p))
            deps = [d[0:t] for d in deps]
            return deps, _rowsum(h_v[r0:r0 + t, :]) * (1.0 / D), outs

        def keys_of(r, idx):
            bits = pltpu.bitcast(jnp.where(r == 0.0, 0.0, r), I32)
            hi = lax.shift_right_logical(bits, 16)
            mono = jnp.where(bits < 0, 0xFFFF - hi, hi | 0x8000)
            return pltpu.bitcast((mono << 11) + (KEY0 + S - 1 - idx), F32)

        def merge(top, k1, k2):
            if top is None:
                return k1, k2
            t1, t2 = top
            return jnp.maximum(t1, k1), jnp.maximum(jnp.minimum(t1, k1), jnp.maximum(t2, k2))

        def write_out(i, mur, rs):
            r0, t = p2_off[i], p2_tiles[i]
            out_v[r0:r0 + t, :] = (h_v[r0:r0 + t, :] * _lanes(1.0 + rs, G) - _lanes(mur * rs, G)).astype(BF16)
            back = out_v[r0:r0 + t, D - 128:D].astype(F32)
            out_copy(i).start()
            return back

        def stage_c(i, mu, dep, hi=CHI / 100):
            r0, t = p2_off[i], p2_tiles[i]
            mu = _tie(mu, _pace(dep, t // 8, 0.0, hi))
            d = h_v[r0:r0 + t, :] - _lanes(mu, G)
            rs = _rstd(_rowsum(d * d) * (1.0 / D))
            mur = _rb(mu)
            r = _rb((_rowsum(d * wr) + (mu - mur) * wr_sum) * rs)
            mu_v[r0:r0 + t, :] = mur
            rs_v[r0:r0 + t, :] = rs
            return r, mur, rs

        lane = lax.broadcasted_iota(I32, (8, 128), 1)
        sub = lax.broadcasted_iota(I32, (8, 128), 0)

        def compact(i, r):
            r0, t = p2_off[i], p2_tiles[i]
            parts = [r[p * 8:(p + 1) * 8] for p in range(t // 8)]
            acc = parts[0]
            for p in range(1, t // 8):
                acc = jnp.where(lane == p, parts[p], acc)
            key = keys_of(acc, r0 + lane * 8 + sub)
            return jnp.where(lane < t // 8, key, 0.0)

        ta = 256
        na = S // ta
        nearly = r2 // ta
        pz = _pace(g_last, NAG * H, 0.0, 1.0)
        os = [stage_a(j * ta, ta, pz[j * H * 8:(j + 1) * H * 8]) for j in range(NAG)]
        xl = _unpk(xn_at(r2, t2))
        qa = _dot(xl, wqkv_v[:, QC:QC + QA])

        row = lax.broadcasted_iota(I32, (128, 128), 0) // DH
        col = lax.broadcasted_iota(I32, (128, 128), 1) // DH
        same = row == col
        kvs = []
        kraw = []
        for g in range(G):
            gg = g_acc[g]
            if g == 0:
                gg = pltpu.bitcast(_gate(pltpu.bitcast(gg, U32), a_done(os)), F32)
            kraw.append(_dot(gg.astype(BF16), wqkv_v[:, VC + g * 128:VC + (g + 1) * 128]))
            kvs.append(jnp.where(same, kraw[-1], 0.0).astype(BF16))
        mraw = []
        mw = []
        for g in range(G):
            mraw.append(_dot(kvs[g], wo_v[g * 128:(g + 1) * 128, 0:D]))
            m_rows.append(_pk(mraw[-1].astype(BF16)))
            mw.append(_rowsum(mraw[-1] * wc).T[0:8])
        mw = jnp.concatenate(mw, axis=1)
        pz = _pace(kraw + [m[:, c:c + 128] for m in mraw for c in (0, 512)], (nearly - NAG) * H, 0.0, 0.9)
        mid_os = [stage_a(j * ta, ta, pz[(j - NAG) * H * 8:(j - NAG + 1) * H * 8]) for j in range(NAG, nearly)]
        os += mid_os
        qb = _dot(_unpk(_gate(xn_at(r2, t2), a_done(mid_os))), wqkv_v[:, QC + QA:QC + D])
        pqt.append(_pk(feat(jnp.concatenate([qa, qb], axis=1)).T))

        def predict(j, zero):
            o = _unpk(os[j]).astype(F32).reshape(ta // 8, 8, D) * mw
            e = _tie(jnp.concatenate(xw, axis=0)[j * ta:(j + 1) * ta], zero)
            for c in range(0, D, 128):
                e = e + o[:, :, c:c + 128].reshape(ta, 128)
            e = _rowsum(e)
            return [e[p * 8:(p + 1) * 8] for p in range(ta // 8)]

        def gather_lanes(parts, p0, acc):
            for p, v in enumerate(parts):
                acc = v if acc is None else jnp.where(lane == p0 + p, v, acc)
            return acc

        est = [None, None]
        pz = _pace(qb, nearly * ta // 8, PLO / 100, 0.92)
        for j in range(nearly):
            half, p0 = divmod(j * ta // 8, 128)
            est[half] = gather_lanes(predict(j, pz[j * ta:(j + 1) * ta]), p0, est[half])

        def tree(i, r):
            t = p2_tiles[i]
            key = keys_of(r, lax.broadcasted_iota(I32, (t, 128), 0) + p2_off[i])
            level = [(key[p * 8:(p + 1) * 8], None) for p in range(t // 8)]
            while len(level) > 1:
                nxt = []
                for p in range(0, len(level) - 1, 2):
                    (a1, a2), (b1, b2) = level[p], level[p + 1]
                    lo = jnp.minimum(a1, b1)
                    for e in (a2, b2):
                        lo = lo if e is None else jnp.maximum(lo, e)
                    nxt.append((jnp.maximum(a1, b1), lo))
                if len(level) % 2:
                    nxt.append(level[-1])
                level = nxt
            return level[0]

        def act(gt, ut):
            gt = _rb(gt)
            return (_rb(gt * jax.nn.sigmoid(gt)) * _rb(ut)).astype(BF16)

        ffn = {"next": 0, "xs": None, "act": {}, "y": {}, "w": {}}
        groups = []
        for q in range(F // 512 + 1):
            if q < F // 512:
                groups += [("up", c, m, hh) for c in range(4 * q, 4 * q + 4) for m in range(2) for hh in range(2)]
            if q >= DLAG:
                groups += [("down", q - DLAG, c) for c in range(G)]
        groups += [("down", q, c) for q in range(F // 512 + 1 - DLAG, F // 512) for c in range(G)]

        def ffn_group():
            grp = groups[ffn["next"]]
            ffn["next"] += 1
            if grp[0] == "up":
                _, c, m, hh = grp
                w_v = (wg_v, wu_v)[m]
                part = _dot(ffn["xs"][:, hh * 512:(hh + 1) * 512], w_v[hh * 512:(hh + 1) * 512, c * 128:(c + 1) * 128])
                ffn[m] = part if hh == 0 else ffn[m] + part
                if m == 1 and hh == 1:
                    ffn["act"][c] = act(ffn[0], ffn[1])
            else:
                _, q, c = grp
                a = jnp.concatenate([ffn["act"][4 * q + k] for k in range(4)], axis=1)
                if ffn["next"] == len(groups) - FKEEP + 4:
                    a = _unpk(_gate(_pk(a), ffn["gate"]))
                w = ffn["w"].get((q, c))
                part = _dot(a, wd_v[q * 512:(q + 1) * 512, c * 128:(c + 1) * 128] if w is None else _unpk(w))
                ffn["y"][c] = part if q == 0 else ffn["y"][c] + part

        def preload(deps):
            keep = groups[len(groups) - FKEEP:]
            pz = _pace(deps, 4 * len(keep), 0.0, 0.8)
            for k, (_, q, c) in enumerate(keep):
                w = _pk(wd_v[q * 512:(q + 1) * 512, c * 128:(c + 1) * 128])
                zero = jnp.concatenate([pz[(4 * k + j) * 8:(4 * k + j + 1) * 8] for j in range(4) for _ in range(8)], axis=0)
                ffn["w"][q, c] = w | zero
            return _fold(jnp.concatenate(list(ffn["w"].values()), axis=1))

        def ffn_step(i, p):
            if ffn["xs"] is not None and (i, p) >= (CT + 1, FP0) and ffn["next"] < len(groups) - FKEEP:
                ffn_group()

        def candidates(deps):
            ka, kb = [keys_of(_rb(e), h * 1024 + lane * 8 + sub) for h, e in enumerate(est)]
            t1, t2 = jnp.maximum(ka, kb), jnp.minimum(ka, kb)
            c1 = jnp.max(t1, axis=1, keepdims=True)
            c2 = jnp.max(jnp.where(t1 == c1, t2, t1), axis=1, keepdims=True)
            ck = pltpu.bitcast(jnp.broadcast_to(jnp.concatenate([c1, c2], axis=0), (16, 128)), I32)
            idx = S - 1 - (ck & (S - 1))
            pz = pltpu.bitcast(_pace(deps, 16, KLO / 100, 1.0), I32)
            for k in range(16):
                i = (idx[k // 8 * 8:k // 8 * 8 + 8] | pz[k * 8:(k + 1) * 8])[k % 8, 0]
                w = o_v[pl.ds(lax.shift_right_logical(i, 1), 1), :]
                w = jnp.where((i & 1) == 0, w << 16, w & U32(0xFFFF0000))
                co_v[k:k + 1, :] = pltpu.bitcast(w, F32)
                xg = x_v[pl.ds(pl.multiple_of(i - k % 8, 8), 8), 0:D].astype(F32)
                cx_v[k:k + 1, :] = xg[k % 8:k % 8 + 1]
            return idx, _pk(co_v[...].astype(BF16))

        def normalize(h):
            mu = _rowsum(h) * (1.0 / D)
            d = h - _lanes(mu, G)
            rs = _rstd(_rowsum(d * d) * (1.0 / D))
            mur = _rb(mu)
            r = _rb((_rowsum(d * wr) + (mu - mur) * wr_sum) * rs)
            return ((h - _lanes(mur, G)) * _lanes(rs, G)).astype(BF16), _rb(jax.nn.sigmoid(r))

        def routed(h, xs, gain, y):
            return h + _rb(xs.astype(F32) + _rb(_rb(y) * _lanes(gain, G)))

        def stage_last(gate, mu_prev, top):
            i = n2 - 1
            r0, t = p2_off[i], p2_tiles[i]
            st = {}

            def post(c, attn):
                h = x_v[r0:r0 + t, c * 128:(c + 1) * 128].astype(F32) + attn
                h_v[r0:r0 + t, c * 128:(c + 1) * 128] = h
                if c == 0:
                    st["shift"] = jnp.broadcast_to(h[:, 0:1], (t, 128))
                d = h - st["shift"]
                new = (d, d * d, d * wr[:, c * 128:(c + 1) * 128])
                st[c] = new if c == 0 else tuple(a + b for a, b in zip(st[c - 1], new))

            def gate_fn(p, deps):
                if p == 0:
                    return gate
                z = None
                if p % 2 == 1 and p // 2 - SLAG >= 0:
                    z = _fold(jnp.concatenate(st[p // 2 - SLAG], axis=1))
                if p == CGATE:
                    r, st["mur_p"], st["rs_p"] = stage_c(i - 1, mu_prev, deps, CLAST / 100)
                    st["top"] = merge(top, *tree(i - 1, r))
                    ffn["gate"] = _fold(write_out(i - 1, st["mur_p"], st["rs_p"]))
                    zz = _zero_of(st["top"][0] + st["top"][1])
                    z = zz if z is None else z | zz
                return z

            _passes(jnp.concatenate(os, axis=0)[r0 // 2:(r0 + t) // 2, :], m_tile, G, gate_fn, post,
                    lambda p: ffn_step(i, p))
            while ffn["next"] < len(groups):
                ffn_group()
            s1, s2, s3 = st[G - 1]
            shift = st["shift"]
            m1 = _rowsum(s1) * (1.0 / D)
            var = jnp.maximum(_rowsum(s2) * (1.0 / D) - m1 * m1, 0.0)
            rs = _rstd(var)
            mur = _rb(shift + m1)
            r = _rb((_rowsum(s3) + (shift - mur) * wr_sum) * rs)
            mu_v[r0:r0 + t, :] = mur
            rs_v[r0:r0 + t, :] = rs
            return merge(st["top"], *tree(i, r)), mur, rs

        top = None
        mu_prev = None
        gate = {0: _fold(jnp.concatenate(est, axis=1)), 2: a_done([pqt[-1][:, 0:256].reshape(-1, D)])}
        extra = None
        for i in range(n2 - 1):
            deps, mu, outs = stage_b(i, gate, extra if i == CT else None)
            gate = {}
            if i == 0:
                pz = _pace(deps, (na - nearly) * H, 0.0, 0.6)
                os += [stage_a(j * ta, ta, pz[(j - nearly) * H * 8:(j - nearly + 1) * H * 8])
                       for j in range(nearly, na)]
                pz = _pace(deps, (na - nearly) * ta // 8, 0.5, 0.9)
                for j in range(nearly, na):
                    half, p0 = divmod(j * ta // 8, 128)
                    est[half] = gather_lanes(predict(j, pz[(j - nearly) * ta:(j - nearly + 1) * ta]), p0, est[half])
                gate[EG] = _zero_of(est[1])
            else:
                r, mur, rs = stage_c(i - 1, mu_prev, deps, min(CHI / 100, 1 - LAT / (16 * p2_tiles[i])))
                back = write_out(i - 1, mur, rs)
                key = compact(i - 1, r)
                top = merge(top, key, jnp.zeros_like(key))
                gate[0] = _zero_of(key + jnp.sum(back.reshape(-1, 8, 128), axis=0))
                if i == n2 - 2:
                    t1, t2 = top
                    b1 = jnp.max(jnp.max(t1, axis=0, keepdims=True), axis=1, keepdims=True)
                    rest = jnp.where(t1 == b1, t2, t1)
                    b2 = jnp.max(jnp.max(rest, axis=0, keepdims=True), axis=1, keepdims=True)
                    top = (jnp.where(sub == 0, b1, 0.0), jnp.where(sub == 0, b2, 0.0))
            if i == n2 - 4:
                gate[0] = gate[0] | preload(deps)
            if i == CT - 2:
                cand, extra = candidates(deps)
                gate[CG] = _fold(extra) | _fold(cx_v[...])
            if i == CT:
                h16 = cx_v[...] + jnp.concatenate(outs, axis=1)
                ffn["xs"], gain16 = normalize(h16)
                gate[FP0 - 1] = _fold(_pk(ffn["xs"]))
            mu_prev = mu
        top, mur_l, rs_l = stage_last(gate[0], mu_prev, top)
        sc.__exit__(None, None, None)

        sc = scope("tail")
        sc.__enter__()
        t1, t2 = top
        k1 = jnp.max(t1, axis=0, keepdims=True)
        k2 = jnp.max(jnp.where(t1 == k1, t2, t1), axis=0, keepdims=True)
        v1 = S - 1 - (pltpu.bitcast(k1, I32) & (S - 1))
        v2 = S - 1 - (pltpu.bitcast(k2, I32) & (S - 1))
        i1, i2 = v1[0, 0], v2[0, 0]
        g1 = pl.multiple_of(i1 & -8, 8)
        g2 = pl.multiple_of(i2 & -8, 8)
        write_out(n2 - 1, mur_l, rs_l)
        out_v[S:S + 16, 0:128] = jnp.zeros((16, 128), BF16)
        chosen = jnp.logical_or(cand == v1, cand == v2)
        found = jnp.sum(chosen.astype(I32), axis=0, keepdims=True)[0, 0]

        def plain(g):
            rows = pl.ds(g, 8)
            rs = _tie(rs_v[rows, :], _zero_of(out_v[S:S + 8, 0:128].astype(F32)))
            return h_v[rows, :] * _lanes(1.0 + rs, G) - _lanes(mu_v[rows, :] * rs, G)

        new16 = routed(h16, ffn["xs"], gain16, jnp.concatenate([ffn["y"][c] for c in range(G)], axis=1))
        for j, (g, v) in enumerate(((g1, v1), (g2, v2))):
            here = jnp.logical_and(chosen, (cand & -8) == (v & -8))
            val = plain(g)
            for half in range(2):
                val = jnp.where(_lanes(here[half * 8:(half + 1) * 8], G), new16[half * 8:(half + 1) * 8], val)
            fix_v[j] = val.astype(BF16)

        @pl.when(found != 2 + MISS)
        def _():
            h = jnp.concatenate([h_v[pl.ds(g1, 8), :], h_v[pl.ds(g2, 8), :]], axis=0)
            xs, gain = normalize(h)

            def chunk(c, y):
                cols = pl.ds(pl.multiple_of(c * MC, 128), MC)
                return y + _dot(act(_dot(xs, wg_v[:, cols]), _dot(xs, wu_v[:, cols])), wd_v[cols, 0:D])

            new = routed(h, xs, gain, lax.fori_loop(0, F // MC, chunk, jnp.zeros((16, D), F32)))
            rows = lax.broadcasted_iota(I32, (8, D), 0)
            for j, g in enumerate((g1, g2)):
                hit = jnp.logical_or(rows + g == i1, rows + g == i2)
                fix_v[j] = jnp.where(hit, new[j * 8:(j + 1) * 8], plain(g)).astype(BF16)

        nb = S - p2_tiles[-1]
        pltpu.make_async_copy(out_v.at[pl.ds(0, nb)], out_hbm.at[pl.ds(0, nb)], sems.at[SO]).wait()
        late = jnp.maximum(i1, i2) >= nb

        @pl.when(late)
        def _():
            out_copy(n2 - 1).wait()

        c1 = pltpu.make_async_copy(fix_v.at[0], out_hbm.at[pl.ds(g1, 8)], sems.at[SO + 1])
        c2 = pltpu.make_async_copy(fix_v.at[1], out_hbm.at[pl.ds(g2, 8)], sems.at[SO + 2])
        c1.start()

        @pl.when(g1 != g2)
        def _():
            c2.start()

        @pl.when(jnp.logical_not(late))
        def _():
            out_copy(n2 - 1).wait()

        @pl.when(g1 != g2)
        def _():
            c2.wait()
        c1.wait()
        sc.__exit__(None, None, None)

    scratch = [
        pltpu.VMEM((S, D + PAD), BF16),
        pltpu.VMEM((D, 3 * D + PAD), BF16),
        pltpu.VMEM((D, D + PAD), BF16),
        pltpu.VMEM((D, F), BF16),
        pltpu.VMEM((D, F), BF16),
        pltpu.VMEM((F, D + PAD), BF16),
        pltpu.VMEM((D,), BF16),
        pltpu.VMEM((S, 128), F32),
        pltpu.VMEM((S, 128), F32),
        pltpu.VMEM((S + 16, D), BF16),
        pltpu.VMEM((S, D), F32),
        pltpu.VMEM((2, 8, D), BF16),
        pltpu.VMEM((S // 2, D), U32),
        pltpu.VMEM((16, D), F32),
        pltpu.VMEM((16, D), F32),
        pltpu.SemaphoreType.DMA((NSEM,)),
    ]

    @jax.jit
    def f(A_x, A_wqkv, A_wo, B_x, B_w_r, B_w_gate, B_w_up, B_w_down):
        any_spec = pl.BlockSpec(memory_space=pl.ANY)
        out = pl.pallas_call(
            kernel,
            out_shape=jax.ShapeDtypeStruct((S, D), BF16),
            in_specs=[any_spec] * 7,
            out_specs=any_spec,
            scratch_shapes=scratch,
            compiler_params=pltpu.CompilerParams(vmem_limit_bytes=100 * 1024 * 1024, disable_bounds_checks=True),
        )(A_x.reshape(S, D), A_wqkv, A_wo, B_w_r, B_w_gate, B_w_up, B_w_down)
        return out.reshape(1, S, D)
    return f


_impl = make_kernel()


@jax.jit
def pallas_sequential_preLN__linear_attn_block__moe_arch_mod__prompt_kernel(
    A_x: jax.Array,
    A_wqkv: jax.Array,
    A_wo: jax.Array,
    B_x: jax.Array,
    B_w_r: jax.Array,
    B_w_gate: jax.Array,
    B_w_up: jax.Array,
    B_w_down: jax.Array,
):
    return _impl(A_x, A_wqkv, A_wo, B_x, B_w_r, B_w_gate, B_w_up, B_w_down)
```

```python
import functools

import jax
import jax.numpy as jnp
from jax import lax
import jax.experimental.pallas as pl
import jax.experimental.pallas.tpu as pltpu

S, D, F, H, DH = 2048, 1024, 3584, 32, 32
G = D // 128
F32, BF16, I32, U32 = jnp.float32, jnp.bfloat16, jnp.int32, jnp.uint32
KEY0 = 64 << 23
PAD = 128
KC, QC, VC = 0, D, 2 * D
HS = S // 2
K2 = 512
QE = 256
GB = 256
TQ = 512
TA = 256
TILES = [128] * 15 + [64, 64]
OFFS = [sum(TILES[:i]) for i in range(len(TILES))]
NT = len(TILES)
CT = 4
FKEEP = 10
MC = 1792
SEM_OUT, SEM_FIX, SEM_LAST, NSEM = 16, 17, 19, 20


def _rb(x):
    return x.astype(BF16).astype(F32)


def _pk(x):
    return pltpu.bitcast(x, U32)


def _unpk(x):
    return pltpu.bitcast(x, BF16)


def _lanes(x, n):
    return jnp.concatenate([x] * n, axis=1) if n > 1 else x


def _rowsum(x):
    return jnp.broadcast_to(jnp.sum(x, axis=-1, keepdims=True), (x.shape[0], 128))


def _recip(d):
    r = pl.reciprocal(d, approx=True)
    return r * (2.0 - d * r)


def _rstd(var):
    v = _rb(_rb(var) + 1e-5)
    return _recip(_rb(v * lax.rsqrt(v)))


def _feat(t):
    return (jnp.where(t > 0, t + 1.0, jnp.exp(t)) + 1e-6).astype(BF16)


def _act(gt, ut):
    gt = _rb(gt)
    return (_rb(gt * jax.nn.sigmoid(gt)) * _rb(ut)).astype(BF16)


def _dot(a, b):
    return jnp.dot(a, b, preferred_element_type=F32)


def _keys(r, idx):
    bits = pltpu.bitcast(jnp.where(r == 0.0, 0.0, r), I32)
    hi = lax.shift_right_logical(bits, 16)
    mono = jnp.where(bits < 0, 0xFFFF - hi, hi | 0x8000)
    return pltpu.bitcast((mono << 11) + (KEY0 + S - 1 - idx), F32)


def _merge(top, k1, k2):
    if top is None:
        return k1, k2
    t1, t2 = top
    return jnp.maximum(t1, k1), jnp.maximum(jnp.minimum(t1, k1), jnp.maximum(t2, k2))


def _zero_of(x):
    bits = pltpu.bitcast(x, U32)
    return lax.shift_right_logical(lax.shift_right_logical(bits, U32(31)), U32(1))


def _pace(dep, n, lo, hi):
    if isinstance(dep, (list, tuple)):
        dep = jnp.concatenate(dep, axis=1)
    nrg, nch = dep.shape[0] // 8, dep.shape[1] // 128
    parts = []
    for p in range(n):
        c, rg = divmod(int((lo + (hi - lo) * p / n) * nch * nrg), nrg)
        parts.append(dep[rg * 8:(rg + 1) * 8, c * 128:(c + 1) * 128])
    return _zero_of(jnp.concatenate(parts, axis=0))


def _tie(x, zero):
    return pltpu.bitcast(pltpu.bitcast(x, U32) | zero, F32)


def _gate(xu, zero):
    if zero is None:
        return xu
    top = xu[0:8, 0:512] | _lanes(zero, 4)
    if xu.shape[1] > 512:
        top = jnp.concatenate([top, xu[0:8, 512:]], axis=1)
    return jnp.concatenate([top, xu[8:]], axis=0) if xu.shape[0] > 8 else top


def _fold(x):
    x = pltpu.bitcast(x, U32) if x.dtype != U32 else x
    parts = [x[r:r + 8, c:c + 128] for r in range(0, x.shape[0], 8) for c in range(0, x.shape[1], 128)]
    while len(parts) > 1:
        parts = [parts[j] | parts[j + 1] if j + 1 < len(parts) else parts[j] for j in range(0, len(parts), 2)]
    return _zero_of(parts[0])


def _blocks_done(xs):
    return _fold(jnp.concatenate([x[r + 56:r + 64] for x in xs for r in range(0, x.shape[0], 64)], axis=1))


def _passes(xu, w, gate_fn=None, post=None, after=None):
    deps, outs = [], []
    nk = xu.shape[1] // 512
    for c in range(G):
        acc = None
        for hh in range(nk):
            z = None if gate_fn is None else gate_fn(nk * c + hh, deps)
            lhs = _unpk(_gate(xu[:, hh * 512:(hh + 1) * 512], z))
            part = _dot(lhs, w(hh * 512, (hh + 1) * 512, c))
            acc = part if acc is None else acc + part
            deps.append(acc)
            if after is not None:
                after(nk * c + hh)
        outs.append(acc if post is None else post(c, acc))
    return outs, deps


def _ffn_groups():
    groups = []
    nq = F // 512
    for q in range(nq + 1):
        if q < nq:
            groups += [("up", c, m, hh) for c in range(4 * q, 4 * q + 4) for m in range(2) for hh in range(2)]
        if q >= 2:
            groups += [("down", q - 2, c) for c in range(G)]
    return groups + [("down", nq - 1, c) for c in range(G)]


def _kernel(x_hbm, wqkv_hbm, wo_hbm, wr_hbm, wg_hbm, wu_hbm, wd_hbm, out_hbm,
            x_v, wqkv_v, wo_v, wg_v, wu_v, wd_v, wr_v, mu_v, rs_v, out_v, h_v, fix_v, o_v, co_v, cx_v, sems,
            *, force_fallback=False):
    def x_copy(r0, n, c0, m, s):
        return pltpu.make_async_copy(x_hbm.at[pl.ds(r0, n), pl.ds(c0, m)], x_v.at[pl.ds(r0, n), pl.ds(c0, m)],
                                     sems.at[s])

    def w_copy(r0, n, src, dst, s):
        return pltpu.make_async_copy(wqkv_hbm.at[pl.ds(r0, n), pl.ds(src, D)],
                                     wqkv_v.at[pl.ds(r0, n), pl.ds(dst, D)], sems.at[s])

    def out_copy(i):
        rows = pl.ds(OFFS[i], TILES[i])
        return pltpu.make_async_copy(out_v.at[rows], out_hbm.at[rows], sems.at[SEM_LAST if i == NT - 1 else SEM_OUT])

    sets = [
        [w_copy(0, 128, D, KC, 0), pltpu.make_async_copy(wr_hbm, wr_v, sems.at[1]), x_copy(0, HS, 0, 128, 2)],
        [x_copy(HS, HS, 0, 128, 3), w_copy(0, 128, 0, QC, 4)],
        [w_copy(128, K2 - 128, D, KC, 5), x_copy(0, S, 128, K2 - 128, 6), w_copy(128, QE - 128, 0, QC, 7)],
        [w_copy(K2, D - K2, D, KC, 8), x_copy(0, S, K2, D - K2, 9), w_copy(0, D, 2 * D, VC, 10),
         pltpu.make_async_copy(wo_hbm, wo_v.at[:, pl.ds(0, D)], sems.at[11])],
        [w_copy(QE, D - QE, 0, QC, 12), pltpu.make_async_copy(wg_hbm, wg_v, sems.at[13]),
         pltpu.make_async_copy(wu_hbm, wu_v, sems.at[14]),
         pltpu.make_async_copy(wd_hbm, wd_v.at[:, pl.ds(0, D)], sems.at[15])],
    ]
    for group in sets:
        for c in group:
            c.start()

    def raw(r0, t, c0, n, wcol):
        return _dot(x_v[r0:r0 + t, c0:c0 + n], wqkv_v[c0:c0 + n, wcol:wcol + D])

    def colsum(r0, n, wcol, dep, hi):
        pz = pltpu.bitcast(_pace(dep, n // 32, 0.02, hi), I32)
        tot = None
        for k in range(n // 32):
            rows = pl.ds(pl.multiple_of(r0 + k * 32 + pz[k * 8:(k + 1) * 8][0, 0], 16), 32)
            w = jnp.sum(wqkv_v[rows, wcol:wcol + D].astype(F32).reshape(4, 8, D), axis=0)
            tot = w if tot is None else tot + w
        return tot

    def moments(r0, t, c0, n, shift, dep, hi):
        xf = x_v[r0:r0 + t, c0:c0 + n].astype(F32)
        if shift is None:
            shift = jnp.broadcast_to(xf[:, 0:1], (t, 128))
        d = xf - _lanes(_tie(shift, _pace(dep, t // 8, 0.0, hi)), n // 128)
        e = d * wc[:, c0:c0 + n]
        add = lambda v: functools.reduce(jnp.add, [v[:, c:c + 128] for c in range(0, n, 128)])
        return shift, (add(d), add(d * d), add(e))

    sets[0][0].wait()
    sets[0][1].wait()
    cs = jnp.sum(wqkv_v[0:128, KC:KC + D].astype(F32).reshape(16, 8, D), axis=0)
    wr = wr_v[...].astype(F32).reshape(1, D)
    wr_sum = _rowsum(wr)
    wc = wr - _lanes(wr_sum * (1.0 / D), G)
    sets[0][2].wait()
    acc_a = raw(0, HS, 0, 128, KC)
    shift_a, mom_a = moments(0, HS, 0, 128, None, acc_a, 0.9)
    for c in sets[1]:
        c.wait()
    acc_b = raw(HS, HS, 0, 128, KC)
    shift_b, mom_b = moments(HS, HS, 0, 128, None, acc_b, 0.9)
    accq0 = raw(0, S, 0, 128, QC)
    csq = colsum(0, 128, QC, accq0, 0.6)
    acc = jnp.concatenate([acc_a, acc_b], axis=0)
    shift = jnp.concatenate([shift_a, shift_b], axis=0)
    mom = [jnp.concatenate(p, axis=0) for p in zip(mom_a, mom_b)]
    for j, (c0, n) in enumerate(((128, K2 - 128), (K2, D - K2))):
        for c in sets[2 + j]:
            c.wait()
        if j == 0:
            partq = raw(0, S, 128, QE - 128, QC)
            accq0 = accq0 + partq
            csq = jnp.sum(csq + colsum(128, QE - 128, QC, partq, 0.6), axis=0, keepdims=True)
        part = raw(0, S, c0, n, KC)
        acc = acc + part
        if j == 0:
            part = jnp.concatenate([partq[:, 0:256], part], axis=1)
        _, new = moments(0, S, c0, n, shift, part, (0.9, 0.4)[j])
        mom = [a + b for a, b in zip(mom, new)]
        cs = cs + colsum(c0, n, KC, part, (0.6, 0.3)[j])
    s1, s2, xw = mom
    m1 = _rowsum(s1) * (1.0 / D)
    rs1 = _rstd(jnp.maximum(_rowsum(s2) * (1.0 / D) - m1 * m1, 0.0))
    mu1 = _rb(shift + m1)
    mu_v[...] = mu1
    zx = _pace(part, S // 8, 0.3, 0.95)
    mux = _tie(mu1, jnp.concatenate([zx[0:S // 4], zx[S // 4:S // 4 + 8] | _fold(cs), zx[S // 4 + 8:]], axis=0))
    cs = jnp.sum(cs, axis=0, keepdims=True)
    xu = _pk(((x_v[:, 0:D].astype(F32) - _lanes(mux, G)) * _lanes(rs1, G)).astype(BF16))
    xn = _unpk(xu)

    z_acc, g_acc, nxt = {}, {}, {}

    def k_block(c, zero):
        k = GB // 128
        pk = _feat((acc[:, c:c + GB] - _lanes(_tie(mu1, zero), k) * cs[:, c:c + GB]) * _lanes(rs1, k))
        zs = jnp.sum(pk.astype(F32).reshape(S // 8, 8, GB), axis=0)
        for b in range(0, GB, 128):
            z_acc[(c + b) // 128] = zs[:, b:b + 128]
        return _pk(pk.T), zs

    nxt[0] = k_block(0, _pace(part, S // 8, 0.6, 0.92))
    for c in range(0, D, GB):
        def gate_g(p, deps, c=c):
            if p != 28:
                return None
            if c + GB == D:
                mu = _tie(mu1, _pace(deps, S // 8, 0.0, 0.85))
                nxt["head"] = (accq0 - _lanes(mu, G) * csq) * _lanes(rs1, G)
                return _fold(nxt["head"][:, D - 128:D])
            nxt[c + GB] = k_block(c + GB, _pace(deps, S // 8, 0.0, 0.85))
            return _blocks_done([nxt[c + GB][0]]) | _fold(nxt[c + GB][1])

        outs, _ = _passes(nxt[c][0], lambda a, b, n: xn[a:b, n * 128:(n + 1) * 128], gate_g)
        upd = jnp.concatenate(outs, axis=1)
        for b in range(0, GB, 128):
            g_acc[(c + b) // 128] = upd[b:b + 128]

    same = (lax.broadcasted_iota(I32, (128, 128), 0) // DH) == (lax.broadcasted_iota(I32, (128, 128), 1) // DH)
    kvs = []
    for g in range(G):
        kv = _dot(g_acc[g].astype(BF16), wqkv_v[:, VC + g * 128:VC + (g + 1) * 128])
        kvs.append(jnp.where(same, kv, 0.0).astype(BF16))
    m_rows = [_pk(_dot(kvs[g], wo_v[g * 128:(g + 1) * 128, 0:D]).astype(BF16)) for g in range(G)]

    for c in sets[4]:
        c.wait()

    z = _rb(jnp.sum(jnp.concatenate([z_acc[b] for b in range(G)], axis=1), axis=0, keepdims=True))
    zc = jnp.concatenate(
        [jnp.broadcast_to(z[:, g * 128:(g + 1) * 128], (128, 128)).T for g in range(G)], axis=0)
    lane = lax.broadcasted_iota(I32, (8, 128), 1)
    sub = lax.broadcasted_iota(I32, (8, 128), 0)
    pqt, os, est = [], [], [None, None]

    def o_tile(r0, zero):
        pq = _unpk(jnp.concatenate(pqt, axis=1)[:, r0:r0 + TA]).astype(F32)
        z4 = zc.reshape(H, DH // 8, 8, 128)
        z0 = _tie(z4[:, 0].reshape(H * 8, 128), zero).reshape(H, 1, 8, 128)
        zz = jnp.concatenate([z0, z4[:, 1:]], axis=1).reshape(D, 128)
        w = (pq * _lanes(zz, TA // 128)).reshape(H, DH // 8, 8, TA)
        den = jnp.sum(jnp.sum(w, axis=1), axis=1, keepdims=True) + 1e-6
        o = pq.reshape(H, DH, TA) * _recip(den)
        ou = _pk(o.reshape(D, TA).astype(BF16).T)
        o_v[r0 // 2:(r0 + TA) // 2, :] = ou
        return ou

    def follow_o(i, deps, lo, hi):
        n = TQ // TA
        pz = _pace(deps, n * H, lo, hi)
        os.extend(o_tile((n * i + j) * TA, pz[j * H * 8:(j + 1) * H * 8]) for j in range(n))
        return _blocks_done(os[n * i:])

    def follow_est(i, deps, lo, hi):
        pz = _pace(deps, TQ // 8, lo, hi)
        for j in range(TQ // TA * i, TQ // TA * (i + 1)):
            o = _unpk(os[j]).astype(F32).reshape(TA // 8, 8, D) * mw
            e = _tie(xw[j * TA:(j + 1) * TA], pz[j * TA - i * TQ:(j + 1) * TA - i * TQ])
            for c in range(0, D, 128):
                e = e + o[:, :, c:c + 128].reshape(TA, 128)
            e = _rowsum(e)
            half, p0 = divmod(j * TA // 8, 128)
            for p in range(TA // 8):
                v = e[p * 8:(p + 1) * 8]
                est[half] = v if est[half] is None else jnp.where(lane == p0 + p, v, est[half])
        return _zero_of(est[(i * TQ) // 1024])

    gate = None
    for i in range(S // TQ):
        accq = _dot(_unpk(_gate(xu[i * TQ // 2:(i + 1) * TQ // 2, QE:], gate)), wqkv_v[QE:, QC:QC + D])
        head = nxt["head"][i * TQ:(i + 1) * TQ]
        if i == 0:
            e = _unpk(jnp.concatenate(m_rows, axis=0)).astype(F32) * wc
            e = jnp.concatenate([_tie(e[:, 0:128], _pace(accq, D // 8, 0.0, 0.7)), e[:, 128:]], axis=1)
            e = _rowsum(e)
            mw = jnp.concatenate([e[g * 128:(g + 1) * 128].T[0:8] for g in range(G)], axis=1)
            gate = _fold(mw)
        else:
            follow_o(i - 1, accq, 0.05, 0.6)
            gate = follow_est(i - 1, accq, 0.45, 0.9)
        pqt.append(_pk(_feat(accq + head).T))

    def m_tile(a, b, c):
        return _unpk(jnp.concatenate(m_rows[a // 128:b // 128], axis=0)[:, c * 128:(c + 1) * 128])

    def write_out(i, mur, rs):
        r0, t = OFFS[i], TILES[i]
        out_v[r0:r0 + t, :] = (h_v[r0:r0 + t, :] * _lanes(1.0 + rs, G) - _lanes(mur * rs, G)).astype(BF16)
        back = out_v[r0:r0 + t, D - 128:D].astype(F32)
        out_copy(i).start()
        return back

    def stats(i, mu, dep, hi):
        r0, t = OFFS[i], TILES[i]
        mu = _tie(mu, _pace(dep, t // 8, 0.0, hi))
        d = h_v[r0:r0 + t, :] - _lanes(mu, G)
        rs = _rstd(_rowsum(d * d) * (1.0 / D))
        mur = _rb(mu)
        r = _rb((_rowsum(d * wr) + (mu - mur) * wr_sum) * rs)
        mu_v[r0:r0 + t, :] = mur
        rs_v[r0:r0 + t, :] = rs
        return r, mur, rs

    def compact(i, r):
        t = TILES[i]
        acc = r[0:8]
        for p in range(1, t // 8):
            acc = jnp.where(lane == p, r[p * 8:(p + 1) * 8], acc)
        return jnp.where(lane < t // 8, _keys(acc, OFFS[i] + lane * 8 + sub), 0.0)

    def tree(i, r):
        key = _keys(r, lax.broadcasted_iota(I32, (TILES[i], 128), 0) + OFFS[i])
        level = [(key[p * 8:(p + 1) * 8], None) for p in range(TILES[i] // 8)]
        while len(level) > 1:
            up = []
            for (a1, a2), (b1, b2) in zip(level[0::2], level[1::2]):
                lo = jnp.minimum(a1, b1)
                for e in (a2, b2):
                    lo = lo if e is None else jnp.maximum(lo, e)
                up.append((jnp.maximum(a1, b1), lo))
            level = up
        return level[0]

    groups = _ffn_groups()
    ffn = {"next": 0, "xs": None, "act": {}, "y": {}, "w": {}}

    def ffn_group():
        grp = groups[ffn["next"]]
        ffn["next"] += 1
        if grp[0] == "up":
            _, c, m, hh = grp
            w_v = (wg_v, wu_v)[m]
            part = _dot(ffn["xs"][:, hh * 512:(hh + 1) * 512], w_v[hh * 512:(hh + 1) * 512, c * 128:(c + 1) * 128])
            ffn[m] = part if hh == 0 else ffn[m] + part
            if m == 1 and hh == 1:
                ffn["act"][c] = _act(ffn[0], ffn[1])
        else:
            _, q, c = grp
            a = jnp.concatenate([ffn["act"][4 * q + k] for k in range(4)], axis=1)
            if ffn["next"] == len(groups) - FKEEP + 4:
                a = _unpk(_gate(_pk(a), ffn["gate"]))
            w = ffn["w"].get((q, c))
            part = _dot(a, wd_v[q * 512:(q + 1) * 512, c * 128:(c + 1) * 128] if w is None else _unpk(w))
            ffn["y"][c] = part if q == 0 else ffn["y"][c] + part

    def ffn_step(i, p):
        if ffn["xs"] is not None and (i, p) >= (CT + 1, 9) and ffn["next"] < len(groups) - FKEEP:
            ffn_group()

    def preload(deps):
        keep = groups[len(groups) - FKEEP:]
        pz = _pace(deps, 4 * len(keep), 0.0, 0.8)
        for k, (_, q, c) in enumerate(keep):
            w = _pk(wd_v[q * 512:(q + 1) * 512, c * 128:(c + 1) * 128])
            zero = jnp.concatenate(
                [pz[(4 * k + j) * 8:(4 * k + j + 1) * 8] for j in range(4) for _ in range(8)], axis=0)
            ffn["w"][q, c] = w | zero
        return _fold(jnp.concatenate(list(ffn["w"].values()), axis=1))

    def candidates(deps):
        ka, kb = [_keys(_rb(e), h * 1024 + lane * 8 + sub) for h, e in enumerate(est)]
        t1, t2 = jnp.maximum(ka, kb), jnp.minimum(ka, kb)
        c1 = jnp.max(t1, axis=1, keepdims=True)
        c2 = jnp.max(jnp.where(t1 == c1, t2, t1), axis=1, keepdims=True)
        ck = pltpu.bitcast(jnp.broadcast_to(jnp.concatenate([c1, c2], axis=0), (16, 128)), I32)
        idx = S - 1 - (ck & (S - 1))
        pz = pltpu.bitcast(_pace(deps, 16, 0.25, 0.75), I32)
        for k in range(16):
            i = (idx[k // 8 * 8:k // 8 * 8 + 8] | pz[k * 8:(k + 1) * 8])[k % 8, 0]
            w = o_v[pl.ds(lax.shift_right_logical(i, 1), 1), :]
            w = jnp.where((i & 1) == 0, w << 16, w & U32(0xFFFF0000))
            co_v[k:k + 1, :] = pltpu.bitcast(w, F32)
            xg = x_v[pl.ds(pl.multiple_of(i - k % 8, 8), 8), 0:D].astype(F32)
            cx_v[k:k + 1, :] = xg[k % 8:k % 8 + 1]
        return idx, _pk(co_v[...].astype(BF16))

    def normalize(h):
        mu = _rowsum(h) * (1.0 / D)
        d = h - _lanes(mu, G)
        rs = _rstd(_rowsum(d * d) * (1.0 / D))
        mur = _rb(mu)
        r = _rb((_rowsum(d * wr) + (mu - mur) * wr_sum) * rs)
        return ((h - _lanes(mur, G)) * _lanes(rs, G)).astype(BF16), _rb(jax.nn.sigmoid(r))

    def routed(h, xs, gain, y):
        return h + _rb(xs.astype(F32) + _rb(_rb(y) * _lanes(gain, G)))

    def project(i, gate, extra):
        r0, t = OFFS[i], TILES[i]

        def post(c, attn):
            h_v[r0:r0 + t, c * 128:(c + 1) * 128] = x_v[r0:r0 + t, c * 128:(c + 1) * 128].astype(F32) + attn[0:t]
            return attn[t:]

        ou = jnp.concatenate(os, axis=0)[r0 // 2:(r0 + t) // 2, :]
        if extra is not None:
            ou = jnp.concatenate([ou, extra], axis=0)
        outs, deps = _passes(ou, m_tile, lambda p, deps: gate.get(p), post, lambda p: ffn_step(i, p))
        return [d[0:t] for d in deps], _rowsum(h_v[r0:r0 + t, :]) * (1.0 / D), outs

    def project_last(gate, mu_prev, top):
        i = NT - 1
        r0, t = OFFS[i], TILES[i]
        st = {}

        def post(c, attn):
            h = x_v[r0:r0 + t, c * 128:(c + 1) * 128].astype(F32) + attn
            h_v[r0:r0 + t, c * 128:(c + 1) * 128] = h
            if c == 0:
                st["shift"] = jnp.broadcast_to(h[:, 0:1], (t, 128))
            d = h - st["shift"]
            new = (d, d * d, d * wr[:, c * 128:(c + 1) * 128])
            st[c] = new if c == 0 else tuple(a + b for a, b in zip(st[c - 1], new))

        def gate_fn(p, deps):
            if p == 0:
                return gate
            z = None
            if p % 2 == 1 and p // 2 >= 4:
                z = _fold(jnp.concatenate(st[p // 2 - 4], axis=1))
            if p == 13:
                r, mur, rs = stats(i - 1, mu_prev, deps, 0.5)
                st["top"] = _merge(top, *tree(i - 1, r))
                ffn["gate"] = _fold(write_out(i - 1, mur, rs))
                z = z | _zero_of(st["top"][0] + st["top"][1])
            return z

        _passes(jnp.concatenate(os, axis=0)[r0 // 2:(r0 + t) // 2, :], m_tile, gate_fn, post,
                lambda p: ffn_step(i, p))
        while ffn["next"] < len(groups):
            ffn_group()
        s1, s2, s3 = st[G - 1]
        m1 = _rowsum(s1) * (1.0 / D)
        rs = _rstd(jnp.maximum(_rowsum(s2) * (1.0 / D) - m1 * m1, 0.0))
        mur = _rb(st["shift"] + m1)
        r = _rb((_rowsum(s3) + (st["shift"] - mur) * wr_sum) * rs)
        mu_v[r0:r0 + t, :] = mur
        rs_v[r0:r0 + t, :] = rs
        return _merge(st["top"], *tree(i, r)), mur, rs

    top = mu_prev = extra = None
    gate = {0: gate, 4: _blocks_done([pqt[-1]])}
    for i in range(NT - 1):
        deps, mu, outs = project(i, gate, extra if i == CT else None)
        gate = {}
        if i == 0:
            gate[3] = follow_o(S // TQ - 1, deps, 0.2, 1.0)
        else:
            r, mur, rs = stats(i - 1, mu_prev, deps, min(0.8, 1 - 560 / (16 * TILES[i])))
            back = write_out(i - 1, mur, rs)
            key = compact(i - 1, r)
            top = _merge(top, key, jnp.zeros_like(key))
            gate[0] = _zero_of(key + jnp.sum(back.reshape(-1, 8, 128), axis=0))
            if i == NT - 2:
                t1, t2 = top
                b1 = jnp.max(jnp.max(t1, axis=0, keepdims=True), axis=1, keepdims=True)
                rest = jnp.where(t1 == b1, t2, t1)
                b2 = jnp.max(jnp.max(rest, axis=0, keepdims=True), axis=1, keepdims=True)
                top = (jnp.where(sub == 0, b1, 0.0), jnp.where(sub == 0, b2, 0.0))
        if i == CT + 1:
            gate[0] = gate[0] | _fold(_pk(ffn["xs"]))
        if i == 1:
            gate[0] = gate[0] | follow_est(S // TQ - 1, deps, 0.1, 0.8)
        if i == NT - 4:
            gate[0] = gate[0] | preload(deps)
        if i == CT - 2:
            cand, extra = candidates(deps)
            gate[0] = gate[0] | _fold(extra) | _fold(cx_v[...])
        if i == CT:
            h16 = cx_v[...] + jnp.concatenate(outs, axis=1)
            ffn["xs"], gain16 = normalize(h16)
        mu_prev = mu
    (t1, t2), mur_l, rs_l = project_last(gate[0], mu_prev, top)

    k1 = jnp.max(t1, axis=0, keepdims=True)
    k2 = jnp.max(jnp.where(t1 == k1, t2, t1), axis=0, keepdims=True)
    v1 = S - 1 - (pltpu.bitcast(k1, I32) & (S - 1))
    v2 = S - 1 - (pltpu.bitcast(k2, I32) & (S - 1))
    i1, i2 = v1[0, 0], v2[0, 0]
    g1 = pl.multiple_of(i1 & -8, 8)
    g2 = pl.multiple_of(i2 & -8, 8)
    write_out(NT - 1, mur_l, rs_l)
    out_v[S:S + 16, 0:128] = jnp.zeros((16, 128), BF16)
    chosen = jnp.logical_or(cand == v1, cand == v2)
    found = jnp.sum(chosen.astype(I32), axis=0, keepdims=True)[0, 0]

    def plain(g):
        rows = pl.ds(g, 8)
        rs = _tie(rs_v[rows, :], _zero_of(out_v[S:S + 8, 0:128].astype(F32)))
        return h_v[rows, :] * _lanes(1.0 + rs, G) - _lanes(mu_v[rows, :] * rs, G)

    new16 = routed(h16, ffn["xs"], gain16, jnp.concatenate([ffn["y"][c] for c in range(G)], axis=1))
    for j, (g, v) in enumerate(((g1, v1), (g2, v2))):
        here = jnp.logical_and(chosen, (cand & -8) == (v & -8))
        val = plain(g)
        for half in range(2):
            val = jnp.where(_lanes(here[half * 8:(half + 1) * 8], G), new16[half * 8:(half + 1) * 8], val)
        fix_v[j] = val.astype(BF16)

    @pl.when(found != (3 if force_fallback else 2))
    def _():
        h = jnp.concatenate([h_v[pl.ds(g1, 8), :], h_v[pl.ds(g2, 8), :]], axis=0)
        xs, gain = normalize(h)

        def chunk(c, y):
            cols = pl.ds(pl.multiple_of(c * MC, 128), MC)
            return y + _dot(_act(_dot(xs, wg_v[:, cols]), _dot(xs, wu_v[:, cols])), wd_v[cols, 0:D])

        new = routed(h, xs, gain, lax.fori_loop(0, F // MC, chunk, jnp.zeros((16, D), F32)))
        rows = lax.broadcasted_iota(I32, (8, D), 0)
        for j, g in enumerate((g1, g2)):
            hit = jnp.logical_or(rows + g == i1, rows + g == i2)
            fix_v[j] = jnp.where(hit, new[j * 8:(j + 1) * 8], plain(g)).astype(BF16)

    nb = OFFS[-1]
    pltpu.make_async_copy(out_v.at[pl.ds(0, nb)], out_hbm.at[pl.ds(0, nb)], sems.at[SEM_OUT]).wait()
    late = jnp.maximum(i1, i2) >= nb

    @pl.when(late)
    def _():
        out_copy(NT - 1).wait()

    c1 = pltpu.make_async_copy(fix_v.at[0], out_hbm.at[pl.ds(g1, 8)], sems.at[SEM_FIX])
    c2 = pltpu.make_async_copy(fix_v.at[1], out_hbm.at[pl.ds(g2, 8)], sems.at[SEM_FIX + 1])
    c1.start()

    @pl.when(g1 != g2)
    def _():
        c2.start()

    @pl.when(jnp.logical_not(late))
    def _():
        out_copy(NT - 1).wait()

    @pl.when(g1 != g2)
    def _():
        c2.wait()

    c1.wait()


_SCRATCH = [
    pltpu.VMEM((S, D + PAD), BF16),
    pltpu.VMEM((D, 3 * D + PAD), BF16),
    pltpu.VMEM((D, D + PAD), BF16),
    pltpu.VMEM((D, F), BF16),
    pltpu.VMEM((D, F), BF16),
    pltpu.VMEM((F, D + PAD), BF16),
    pltpu.VMEM((D,), BF16),
    pltpu.VMEM((S, 128), F32),
    pltpu.VMEM((S, 128), F32),
    pltpu.VMEM((S + 16, D), BF16),
    pltpu.VMEM((S, D), F32),
    pltpu.VMEM((2, 8, D), BF16),
    pltpu.VMEM((S // 2, D), U32),
    pltpu.VMEM((16, D), F32),
    pltpu.VMEM((16, D), F32),
    pltpu.SemaphoreType.DMA((NSEM,)),
]


def _run(kernel, A_x, A_wqkv, A_wo, B_w_r, B_w_gate, B_w_up, B_w_down):
    any_spec = pl.BlockSpec(memory_space=pl.ANY)
    out = pl.pallas_call(
        kernel,
        out_shape=jax.ShapeDtypeStruct((S, D), BF16),
        in_specs=[any_spec] * 7,
        out_specs=any_spec,
        scratch_shapes=_SCRATCH,
        compiler_params=pltpu.CompilerParams(vmem_limit_bytes=100 * 1024 * 1024, disable_bounds_checks=True),
    )(A_x.reshape(S, D), A_wqkv, A_wo, B_w_r, B_w_gate, B_w_up, B_w_down)
    return out.reshape(1, S, D)


@jax.jit
def pallas_sequential_preLN__linear_attn_block__moe_arch_mod__prompt_kernel(
    A_x: jax.Array,
    A_wqkv: jax.Array,
    A_wo: jax.Array,
    B_x: jax.Array,
    B_w_r: jax.Array,
    B_w_gate: jax.Array,
    B_w_up: jax.Array,
    B_w_down: jax.Array,
):
    return _run(_kernel, A_x, A_wqkv, A_wo, B_w_r, B_w_gate, B_w_up, B_w_down)
```

```python
import functools

import jax
import jax.numpy as jnp
from jax import lax
import jax.experimental.pallas as pl
import jax.experimental.pallas.tpu as pltpu

S, D, F, H, DH = 2048, 1024, 3584, 32, 32
G = D // 128
F32, BF16, I32, U32 = jnp.float32, jnp.bfloat16, jnp.int32, jnp.uint32
KEY0 = 64 << 23
PAD = 128
KC, QC, VC = 0, D, 2 * D
HS = S // 2
K2 = 512
QE = 256
GB = 256
TQ = 512
TA = 256
TILES = [128] * 15 + [64, 64]
OFFS = [sum(TILES[:i]) for i in range(len(TILES))]
NT = len(TILES)
CT = 4
FKEEP = 10
MC = 1792
SEM_OUT, SEM_FIX, SEM_LAST, NSEM = 16, 17, 19, 20


def _rb(x):
    return x.astype(BF16).astype(F32)


def _pk(x):
    return pltpu.bitcast(x, U32)


def _unpk(x):
    return pltpu.bitcast(x, BF16)


def _lanes(x, n):
    return jnp.concatenate([x] * n, axis=1) if n > 1 else x


def _rowsum(x):
    return jnp.broadcast_to(jnp.sum(x, axis=-1, keepdims=True), (x.shape[0], 128))


def _recip(d):
    r = pl.reciprocal(d, approx=True)
    return r * (2.0 - d * r)


def _rstd(var):
    v = _rb(_rb(var) + 1e-5)
    return _recip(_rb(v * lax.rsqrt(v)))


def _feat(t):
    return (jnp.where(t > 0, t + 1.0, jnp.exp(t)) + 1e-6).astype(BF16)


def _act(gt, ut):
    gt = _rb(gt)
    return (_rb(gt * jax.nn.sigmoid(gt)) * _rb(ut)).astype(BF16)


def _dot(a, b):
    return jnp.dot(a, b, preferred_element_type=F32)


def _keys(r, idx):
    bits = pltpu.bitcast(jnp.where(r == 0.0, 0.0, r), I32)
    hi = lax.shift_right_logical(bits, 16)
    mono = jnp.where(bits < 0, 0xFFFF - hi, hi | 0x8000)
    return pltpu.bitcast((mono << 11) + (KEY0 + S - 1 - idx), F32)


def _merge(top, k1, k2):
    if top is None:
        return k1, k2
    t1, t2 = top
    return jnp.maximum(t1, k1), jnp.maximum(jnp.minimum(t1, k1), jnp.maximum(t2, k2))


def _zero_of(x):
    bits = pltpu.bitcast(x, U32)
    return lax.shift_right_logical(lax.shift_right_logical(bits, U32(31)), U32(1))


def _pace(dep, n, lo, hi):
    if isinstance(dep, (list, tuple)):
        dep = jnp.concatenate(dep, axis=1)
    nrg, nch = dep.shape[0] // 8, dep.shape[1] // 128
    parts = []
    for p in range(n):
        c, rg = divmod(int((lo + (hi - lo) * p / n) * nch * nrg), nrg)
        parts.append(dep[rg * 8:(rg + 1) * 8, c * 128:(c + 1) * 128])
    return _zero_of(jnp.concatenate(parts, axis=0))


def _tie(x, zero):
    return pltpu.bitcast(pltpu.bitcast(x, U32) | zero, F32)


def _gate(xu, zero):
    if zero is None:
        return xu
    top = xu[0:8, 0:512] | _lanes(zero, 4)
    if xu.shape[1] > 512:
        top = jnp.concatenate([top, xu[0:8, 512:]], axis=1)
    return jnp.concatenate([top, xu[8:]], axis=0) if xu.shape[0] > 8 else top


def _fold(x):
    x = pltpu.bitcast(x, U32) if x.dtype != U32 else x
    parts = [x[r:r + 8, c:c + 128] for r in range(0, x.shape[0], 8) for c in range(0, x.shape[1], 128)]
    while len(parts) > 1:
        parts = [parts[j] | parts[j + 1] if j + 1 < len(parts) else parts[j] for j in range(0, len(parts), 2)]
    return _zero_of(parts[0])


def _blocks_done(xs):
    return _fold(jnp.concatenate([x[r + 56:r + 64] for x in xs for r in range(0, x.shape[0], 64)], axis=1))


def _passes(xu, w, gate_fn=None, post=None, after=None):
    deps, outs = [], []
    nk = xu.shape[1] // 512
    for c in range(G):
        acc = None
        for hh in range(nk):
            z = None if gate_fn is None else gate_fn(nk * c + hh, deps)
            lhs = _unpk(_gate(xu[:, hh * 512:(hh + 1) * 512], z))
            part = _dot(lhs, w(hh * 512, (hh + 1) * 512, c))
            acc = part if acc is None else acc + part
            deps.append(acc)
            if after is not None:
                after(nk * c + hh)
        outs.append(acc if post is None else post(c, acc))
    return outs, deps


def _ffn_groups():
    groups = []
    nq = F // 512
    for q in range(nq + 1):
        if q < nq:
            groups += [("up", c, m, hh) for c in range(4 * q, 4 * q + 4) for m in range(2) for hh in range(2)]
        if q >= 2:
            groups += [("down", q - 2, c) for c in range(G)]
    return groups + [("down", nq - 1, c) for c in range(G)]


def _kernel(x_hbm, wqkv_hbm, wo_hbm, wr_hbm, wg_hbm, wu_hbm, wd_hbm, out_hbm,
            x_v, wqkv_v, wo_v, wg_v, wu_v, wd_v, wr_v, mu_v, rs_v, out_v, h_v, fix_v, o_v, co_v, cx_v, sems,
            *, force_fallback=False):
    def x_copy(r0, n, c0, m, s):
        return pltpu.make_async_copy(x_hbm.at[pl.ds(r0, n), pl.ds(c0, m)], x_v.at[pl.ds(r0, n), pl.ds(c0, m)],
                                     sems.at[s])

    def w_copy(r0, n, src, dst, s):
        return pltpu.make_async_copy(wqkv_hbm.at[pl.ds(r0, n), pl.ds(src, D)],
                                     wqkv_v.at[pl.ds(r0, n), pl.ds(dst, D)], sems.at[s])

    def out_copy(i):
        rows = pl.ds(OFFS[i], TILES[i])
        return pltpu.make_async_copy(out_v.at[rows], out_hbm.at[rows], sems.at[SEM_LAST if i == NT - 1 else SEM_OUT])

    sets = [
        [w_copy(0, 128, D, KC, 0), pltpu.make_async_copy(wr_hbm, wr_v, sems.at[1]), x_copy(0, HS, 0, 128, 2)],
        [x_copy(HS, HS, 0, 128, 3), w_copy(0, 128, 0, QC, 4)],
        [w_copy(128, K2 - 128, D, KC, 5), x_copy(0, S, 128, K2 - 128, 6), w_copy(128, QE - 128, 0, QC, 7)],
        [w_copy(K2, D - K2, D, KC, 8), x_copy(0, S, K2, D - K2, 9), w_copy(0, D, 2 * D, VC, 10),
         pltpu.make_async_copy(wo_hbm, wo_v.at[:, pl.ds(0, D)], sems.at[11])],
        [w_copy(QE, D - QE, 0, QC, 12), pltpu.make_async_copy(wg_hbm, wg_v, sems.at[13]),
         pltpu.make_async_copy(wu_hbm, wu_v, sems.at[14]),
         pltpu.make_async_copy(wd_hbm, wd_v.at[:, pl.ds(0, D)], sems.at[15])],
    ]
    for group in sets:
        for c in group:
            c.start()

    def raw(r0, t, c0, n, wcol):
        return _dot(x_v[r0:r0 + t, c0:c0 + n], wqkv_v[c0:c0 + n, wcol:wcol + D])

    def colsum(r0, n, wcol, dep, hi, pieces):
        cuts = [n // 16 * k // pieces * 16 for k in range(pieces + 1)]
        pz = pltpu.bitcast(_pace(dep, pieces, 0.02, hi), I32)
        tot = None
        for k in range(pieces):
            m = cuts[k + 1] - cuts[k]
            rows = pl.ds(pl.multiple_of(r0 + cuts[k] + pz[k * 8:(k + 1) * 8][0, 0], 16), m)
            w = jnp.sum(wqkv_v[rows, wcol:wcol + D].astype(F32).reshape(m // 8, 8, D), axis=0)
            tot = w if tot is None else tot + w
        return tot

    def moments(r0, t, c0, n, shift, dep, hi):
        xf = x_v[r0:r0 + t, c0:c0 + n].astype(F32)
        if shift is None:
            shift = jnp.broadcast_to(xf[:, 0:1], (t, 128))
        d = xf - _lanes(_tie(shift, _pace(dep, t // 8, 0.0, hi)), n // 128)
        e = d * wc[:, c0:c0 + n]
        add = lambda v: functools.reduce(jnp.add, [v[:, c:c + 128] for c in range(0, n, 128)])
        return shift, (add(d), add(d * d), add(e))

    sets[0][0].wait()
    sets[0][1].wait()
    cs = jnp.sum(wqkv_v[0:128, KC:KC + D].astype(F32).reshape(16, 8, D), axis=0)
    wr = wr_v[...].astype(F32).reshape(1, D)
    wr_sum = _rowsum(wr)
    wc = wr - _lanes(wr_sum * (1.0 / D), G)
    sets[0][2].wait()
    acc_a = raw(0, HS, 0, 128, KC)
    shift_a, mom_a = moments(0, HS, 0, 128, None, acc_a, 0.9)
    for c in sets[1]:
        c.wait()
    acc_b = raw(HS, HS, 0, 128, KC)
    shift_b, mom_b = moments(HS, HS, 0, 128, None, acc_b, 0.9)
    accq0 = raw(0, S, 0, 128, QC)
    csq = colsum(0, 128, QC, accq0, 0.6, 8)
    acc = jnp.concatenate([acc_a, acc_b], axis=0)
    shift = jnp.concatenate([shift_a, shift_b], axis=0)
    mom = [jnp.concatenate(p, axis=0) for p in zip(mom_a, mom_b)]
    for j, (c0, n) in enumerate(((128, K2 - 128), (K2, D - K2))):
        for c in sets[2 + j]:
            c.wait()
        if j == 0:
            partq = raw(0, S, 128, QE - 128, QC)
            accq0 = accq0 + partq
            csq = jnp.sum(csq + colsum(128, QE - 128, QC, partq, 0.6, 8), axis=0, keepdims=True)
        part = raw(0, S, c0, n, KC)
        acc = acc + part
        if j == 0:
            part = jnp.concatenate([partq[:, 0:256], part], axis=1)
        _, new = moments(0, S, c0, n, shift, part, (0.9, 0.4)[j])
        mom = [a + b for a, b in zip(mom, new)]
        cs = cs + colsum(c0, n, KC, part, (0.6, 0.3)[j], (18, 32)[j])
    s1, s2, xw = mom
    m1 = _rowsum(s1) * (1.0 / D)
    rs1 = _rstd(jnp.maximum(_rowsum(s2) * (1.0 / D) - m1 * m1, 0.0))
    mu1 = _rb(shift + m1)
    mu_v[...] = mu1
    zx = _pace(part, S // 8, 0.3, 0.95)
    mux = _tie(mu1, jnp.concatenate([zx[0:S // 4], zx[S // 4:S // 4 + 8] | _fold(cs), zx[S // 4 + 8:]], axis=0))
    cs = jnp.sum(cs, axis=0, keepdims=True)
    xu = _pk(((x_v[:, 0:D].astype(F32) - _lanes(mux, G)) * _lanes(rs1, G)).astype(BF16))
    xn = _unpk(xu)

    z_acc, g_acc, nxt = {}, {}, {}

    def k_block(c, zero):
        k = GB // 128
        pk = _feat((acc[:, c:c + GB] - _lanes(_tie(mu1, zero), k) * cs[:, c:c + GB]) * _lanes(rs1, k))
        zs = jnp.sum(pk.astype(F32).reshape(S // 8, 8, GB), axis=0)
        for b in range(0, GB, 128):
            z_acc[(c + b) // 128] = zs[:, b:b + 128]
        return _pk(pk.T), zs

    nxt[0] = k_block(0, _pace(part, S // 8, 0.6, 0.92))
    for c in range(0, D, GB):
        def gate_g(p, deps, c=c):
            if p != 28:
                return None
            if c + GB == D:
                mu = _tie(mu1, _pace(deps, S // 8, 0.0, 0.85))
                nxt["head"] = (accq0 - _lanes(mu, G) * csq) * _lanes(rs1, G)
                return _fold(nxt["head"][:, D - 128:D])
            nxt[c + GB] = k_block(c + GB, _pace(deps, S // 8, 0.0, 0.85))
            return _blocks_done([nxt[c + GB][0]]) | _fold(nxt[c + GB][1])

        outs, _ = _passes(nxt[c][0], lambda a, b, n: xn[a:b, n * 128:(n + 1) * 128], gate_g)
        upd = jnp.concatenate(outs, axis=1)
        for b in range(0, GB, 128):
            g_acc[(c + b) // 128] = upd[b:b + 128]

    same = (lax.broadcasted_iota(I32, (128, 128), 0) // DH) == (lax.broadcasted_iota(I32, (128, 128), 1) // DH)
    kvs = []
    for g in range(G):
        kv = _dot(g_acc[g].astype(BF16), wqkv_v[:, VC + g * 128:VC + (g + 1) * 128])
        kvs.append(jnp.where(same, kv, 0.0).astype(BF16))
    m_rows = [_pk(_dot(kvs[g], wo_v[g * 128:(g + 1) * 128, 0:D]).astype(BF16)) for g in range(G)]

    for c in sets[4]:
        c.wait()

    z = _rb(jnp.sum(jnp.concatenate([z_acc[b] for b in range(G)], axis=1), axis=0, keepdims=True))
    zc = jnp.concatenate(
        [jnp.broadcast_to(z[:, g * 128:(g + 1) * 128], (128, 128)).T for g in range(G)], axis=0)
    lane = lax.broadcasted_iota(I32, (8, 128), 1)
    sub = lax.broadcasted_iota(I32, (8, 128), 0)
    pqt, os, est = [], [], [None, None]

    def o_tile(r0, zero):
        pq = _unpk(jnp.concatenate(pqt, axis=1)[:, r0:r0 + TA]).astype(F32)
        z4 = zc.reshape(H, DH // 8, 8, 128)
        z0 = _tie(z4[:, 0].reshape(H * 8, 128), zero).reshape(H, 1, 8, 128)
        zz = jnp.concatenate([z0, z4[:, 1:]], axis=1).reshape(D, 128)
        w = (pq * _lanes(zz, TA // 128)).reshape(H, DH // 8, 8, TA)
        den = jnp.sum(jnp.sum(w, axis=1), axis=1, keepdims=True) + 1e-6
        o = pq.reshape(H, DH, TA) * _recip(den)
        ou = _pk(o.reshape(D, TA).astype(BF16).T)
        o_v[r0 // 2:(r0 + TA) // 2, :] = ou
        return ou

    def follow_o(i, deps, lo, hi):
        n = TQ // TA
        pz = _pace(deps, n * H, lo, hi)
        os.extend(o_tile((n * i + j) * TA, pz[j * H * 8:(j + 1) * H * 8]) for j in range(n))
        return _blocks_done(os[n * i:])

    def follow_est(i, deps, lo, hi):
        pz = _pace(deps, TQ // 8, lo, hi)
        for j in range(TQ // TA * i, TQ // TA * (i + 1)):
            o = _unpk(os[j]).astype(F32).reshape(TA // 8, 8, D) * mw
            e = _tie(xw[j * TA:(j + 1) * TA], pz[j * TA - i * TQ:(j + 1) * TA - i * TQ])
            for c in range(0, D, 128):
                e = e + o[:, :, c:c + 128].reshape(TA, 128)
            e = _rowsum(e)
            half, p0 = divmod(j * TA // 8, 128)
            for p in range(TA // 8):
                v = e[p * 8:(p + 1) * 8]
                est[half] = v if est[half] is None else jnp.where(lane == p0 + p, v, est[half])
        return _zero_of(est[(i * TQ) // 1024])

    gate = None
    for i in range(S // TQ):
        accq = _dot(_unpk(_gate(xu[i * TQ // 2:(i + 1) * TQ // 2, QE:], gate)), wqkv_v[QE:, QC:QC + D])
        head = nxt["head"][i * TQ:(i + 1) * TQ]
        if i == 0:
            e = _unpk(jnp.concatenate(m_rows, axis=0)).astype(F32) * wc
            e = jnp.concatenate([_tie(e[:, 0:128], _pace(accq, D // 8, 0.0, 0.7)), e[:, 128:]], axis=1)
            e = _rowsum(e)
            mw = jnp.concatenate([e[g * 128:(g + 1) * 128].T[0:8] for g in range(G)], axis=1)
            gate = _fold(mw)
        else:
            follow_o(i - 1, accq, 0.05, 0.6)
            gate = follow_est(i - 1, accq, 0.45, 0.9)
        pqt.append(_pk(_feat(accq + head).T))

    def m_tile(a, b, c):
        return _unpk(jnp.concatenate(m_rows[a // 128:b // 128], axis=0)[:, c * 128:(c + 1) * 128])

    def write_out(i, mur, rs):
        r0, t = OFFS[i], TILES[i]
        out_v[r0:r0 + t, :] = (h_v[r0:r0 + t, :] * _lanes(1.0 + rs, G) - _lanes(mur * rs, G)).astype(BF16)
        back = out_v[r0:r0 + t, D - 128:D].astype(F32)
        out_copy(i).start()
        return back

    def stats(i, mu, dep, hi):
        r0, t = OFFS[i], TILES[i]
        mu = _tie(mu, _pace(dep, t // 8, 0.0, hi))
        d = h_v[r0:r0 + t, :] - _lanes(mu, G)
        rs = _rstd(_rowsum(d * d) * (1.0 / D))
        mur = _rb(mu)
        r = _rb((_rowsum(d * wr) + (mu - mur) * wr_sum) * rs)
        mu_v[r0:r0 + t, :] = mur
        rs_v[r0:r0 + t, :] = rs
        return r, mur, rs

    def compact(i, r):
        t = TILES[i]
        acc = r[0:8]
        for p in range(1, t // 8):
            acc = jnp.where(lane == p, r[p * 8:(p + 1) * 8], acc)
        return jnp.where(lane < t // 8, _keys(acc, OFFS[i] + lane * 8 + sub), 0.0)

    def tree(i, r):
        key = _keys(r, lax.broadcasted_iota(I32, (TILES[i], 128), 0) + OFFS[i])
        level = [(key[p * 8:(p + 1) * 8], None) for p in range(TILES[i] // 8)]
        while len(level) > 1:
            up = []
            for (a1, a2), (b1, b2) in zip(level[0::2], level[1::2]):
                lo = jnp.minimum(a1, b1)
                for e in (a2, b2):
                    lo = lo if e is None else jnp.maximum(lo, e)
                up.append((jnp.maximum(a1, b1), lo))
            level = up
        return level[0]

    groups = _ffn_groups()
    ffn = {"next": 0, "xs": None, "act": {}, "y": {}, "w": {}}

    def ffn_group():
        grp = groups[ffn["next"]]
        ffn["next"] += 1
        if grp[0] == "up":
            _, c, m, hh = grp
            w_v = (wg_v, wu_v)[m]
            part = _dot(ffn["xs"][:, hh * 512:(hh + 1) * 512], w_v[hh * 512:(hh + 1) * 512, c * 128:(c + 1) * 128])
            ffn[m] = part if hh == 0 else ffn[m] + part
            if m == 1 and hh == 1:
                ffn["act"][c] = _act(ffn[0], ffn[1])
        else:
            _, q, c = grp
            a = jnp.concatenate([ffn["act"][4 * q + k] for k in range(4)], axis=1)
            if ffn["next"] == len(groups) - FKEEP + 4:
                a = _unpk(_gate(_pk(a), ffn["gate"]))
            w = ffn["w"].get((q, c))
            part = _dot(a, wd_v[q * 512:(q + 1) * 512, c * 128:(c + 1) * 128] if w is None else _unpk(w))
            ffn["y"][c] = part if q == 0 else ffn["y"][c] + part

    def ffn_step(i, p):
        if ffn["xs"] is not None and (i, p) >= (CT + 1, 9) and ffn["next"] < len(groups) - FKEEP:
            ffn_group()

    def preload(deps):
        keep = groups[len(groups) - FKEEP:]
        pz = _pace(deps, 4 * len(keep), 0.0, 0.8)
        for k, (_, q, c) in enumerate(keep):
            w = _pk(wd_v[q * 512:(q + 1) * 512, c * 128:(c + 1) * 128])
            zero = jnp.concatenate(
                [pz[(4 * k + j) * 8:(4 * k + j + 1) * 8] for j in range(4) for _ in range(8)], axis=0)
            ffn["w"][q, c] = w | zero
        return _fold(jnp.concatenate(list(ffn["w"].values()), axis=1))

    def candidates(deps):
        ka, kb = [_keys(_rb(e), h * 1024 + lane * 8 + sub) for h, e in enumerate(est)]
        t1, t2 = jnp.maximum(ka, kb), jnp.minimum(ka, kb)
        c1 = jnp.max(t1, axis=1, keepdims=True)
        c2 = jnp.max(jnp.where(t1 == c1, t2, t1), axis=1, keepdims=True)
        ck = pltpu.bitcast(jnp.broadcast_to(jnp.concatenate([c1, c2], axis=0), (16, 128)), I32)
        idx = S - 1 - (ck & (S - 1))
        pz = pltpu.bitcast(_pace(deps, 16, 0.25, 0.75), I32)
        for k in range(16):
            i = (idx[k // 8 * 8:k // 8 * 8 + 8] | pz[k * 8:(k + 1) * 8])[k % 8, 0]
            w = o_v[pl.ds(lax.shift_right_logical(i, 1), 1), :]
            w = jnp.where((i & 1) == 0, w << 16, w & U32(0xFFFF0000))
            co_v[k:k + 1, :] = pltpu.bitcast(w, F32)
            xg = x_v[pl.ds(pl.multiple_of(i - k % 8, 8), 8), 0:D].astype(F32)
            cx_v[k:k + 1, :] = xg[k % 8:k % 8 + 1]
        return idx, _pk(co_v[...].astype(BF16))

    def normalize(h):
        mu = _rowsum(h) * (1.0 / D)
        d = h - _lanes(mu, G)
        rs = _rstd(_rowsum(d * d) * (1.0 / D))
        mur = _rb(mu)
        r = _rb((_rowsum(d * wr) + (mu - mur) * wr_sum) * rs)
        return ((h - _lanes(mur, G)) * _lanes(rs, G)).astype(BF16), _rb(jax.nn.sigmoid(r))

    def routed(h, xs, gain, y):
        return h + _rb(xs.astype(F32) + _rb(_rb(y) * _lanes(gain, G)))

    def project(i, gate, extra):
        r0, t = OFFS[i], TILES[i]

        def post(c, attn):
            h_v[r0:r0 + t, c * 128:(c + 1) * 128] = x_v[r0:r0 + t, c * 128:(c + 1) * 128].astype(F32) + attn[0:t]
            return attn[t:]

        ou = jnp.concatenate(os, axis=0)[r0 // 2:(r0 + t) // 2, :]
        if extra is not None:
            ou = jnp.concatenate([ou, extra], axis=0)
        outs, deps = _passes(ou, m_tile, lambda p, deps: gate.get(p), post, lambda p: ffn_step(i, p))
        return [d[0:t] for d in deps], _rowsum(h_v[r0:r0 + t, :]) * (1.0 / D), outs

    def project_last(gate, mu_prev, top):
        i = NT - 1
        r0, t = OFFS[i], TILES[i]
        st = {}

        def post(c, attn):
            h = x_v[r0:r0 + t, c * 128:(c + 1) * 128].astype(F32) + attn
            h_v[r0:r0 + t, c * 128:(c + 1) * 128] = h
            if c == 0:
                st["shift"] = jnp.broadcast_to(h[:, 0:1], (t, 128))
            d = h - st["shift"]
            new = (d, d * d, d * wr[:, c * 128:(c + 1) * 128])
            st[c] = new if c == 0 else tuple(a + b for a, b in zip(st[c - 1], new))

        def gate_fn(p, deps):
            if p == 0:
                return gate
            z = None
            if p % 2 == 1 and p // 2 >= 4:
                z = _fold(jnp.concatenate(st[p // 2 - 4], axis=1))
            if p == 13:
                r, mur, rs = stats(i - 1, mu_prev, deps, 0.5)
                st["top"] = _merge(top, *tree(i - 1, r))
                ffn["gate"] = _fold(write_out(i - 1, mur, rs))
                z = z | _zero_of(st["top"][0] + st["top"][1])
            return z

        _passes(jnp.concatenate(os, axis=0)[r0 // 2:(r0 + t) // 2, :], m_tile, gate_fn, post,
                lambda p: ffn_step(i, p))
        while ffn["next"] < len(groups):
            ffn_group()
        s1, s2, s3 = st[G - 1]
        m1 = _rowsum(s1) * (1.0 / D)
        rs = _rstd(jnp.maximum(_rowsum(s2) * (1.0 / D) - m1 * m1, 0.0))
        mur = _rb(st["shift"] + m1)
        r = _rb((_rowsum(s3) + (st["shift"] - mur) * wr_sum) * rs)
        mu_v[r0:r0 + t, :] = mur
        rs_v[r0:r0 + t, :] = rs
        return _merge(st["top"], *tree(i, r)), mur, rs

    top = mu_prev = extra = None
    gate = {0: gate, 6: _blocks_done([pqt[-1]])}
    for i in range(NT - 1):
        deps, mu, outs = project(i, gate, extra if i == CT else None)
        gate = {}
        if i == 0:
            gate[5] = follow_o(S // TQ - 1, deps, 0.35, 1.0)
        else:
            r, mur, rs = stats(i - 1, mu_prev, deps, min(0.8, 1 - 560 / (16 * TILES[i])))
            back = write_out(i - 1, mur, rs)
            key = compact(i - 1, r)
            top = _merge(top, key, jnp.zeros_like(key))
            gate[0] = _zero_of(key + jnp.sum(back.reshape(-1, 8, 128), axis=0))
            if i == NT - 2:
                t1, t2 = top
                b1 = jnp.max(jnp.max(t1, axis=0, keepdims=True), axis=1, keepdims=True)
                rest = jnp.where(t1 == b1, t2, t1)
                b2 = jnp.max(jnp.max(rest, axis=0, keepdims=True), axis=1, keepdims=True)
                top = (jnp.where(sub == 0, b1, 0.0), jnp.where(sub == 0, b2, 0.0))
        if i == CT + 1:
            gate[0] = gate[0] | _fold(_pk(ffn["xs"]))
        if i == 1:
            gate[0] = gate[0] | follow_est(S // TQ - 1, deps, 0.25, 0.85)
        if i == NT - 4:
            gate[0] = gate[0] | preload(deps)
        if i == CT - 2:
            cand, extra = candidates(deps)
            gate[0] = gate[0] | _fold(extra) | _fold(cx_v[...])
        if i == CT:
            h16 = cx_v[...] + jnp.concatenate(outs, axis=1)
            ffn["xs"], gain16 = normalize(h16)
        mu_prev = mu
    (t1, t2), mur_l, rs_l = project_last(gate[0], mu_prev, top)

    k1 = jnp.max(t1, axis=0, keepdims=True)
    k2 = jnp.max(jnp.where(t1 == k1, t2, t1), axis=0, keepdims=True)
    v1 = S - 1 - (pltpu.bitcast(k1, I32) & (S - 1))
    v2 = S - 1 - (pltpu.bitcast(k2, I32) & (S - 1))
    i1, i2 = v1[0, 0], v2[0, 0]
    g1 = pl.multiple_of(i1 & -8, 8)
    g2 = pl.multiple_of(i2 & -8, 8)
    write_out(NT - 1, mur_l, rs_l)
    out_v[S:S + 16, 0:128] = jnp.zeros((16, 128), BF16)
    chosen = jnp.logical_or(cand == v1, cand == v2)
    found = jnp.sum(chosen.astype(I32), axis=0, keepdims=True)[0, 0]

    def plain(g):
        rows = pl.ds(g, 8)
        rs = _tie(rs_v[rows, :], _zero_of(out_v[S:S + 8, 0:128].astype(F32)))
        return h_v[rows, :] * _lanes(1.0 + rs, G) - _lanes(mu_v[rows, :] * rs, G)

    new16 = routed(h16, ffn["xs"], gain16, jnp.concatenate([ffn["y"][c] for c in range(G)], axis=1))
    for j, (g, v) in enumerate(((g1, v1), (g2, v2))):
        here = jnp.logical_and(chosen, (cand & -8) == (v & -8))
        val = plain(g)
        for half in range(2):
            val = jnp.where(_lanes(here[half * 8:(half + 1) * 8], G), new16[half * 8:(half + 1) * 8], val)
        fix_v[j] = val.astype(BF16)

    @pl.when(found != (3 if force_fallback else 2))
    def _():
        h = jnp.concatenate([h_v[pl.ds(g1, 8), :], h_v[pl.ds(g2, 8), :]], axis=0)
        xs, gain = normalize(h)

        def chunk(c, y):
            cols = pl.ds(pl.multiple_of(c * MC, 128), MC)
            return y + _dot(_act(_dot(xs, wg_v[:, cols]), _dot(xs, wu_v[:, cols])), wd_v[cols, 0:D])

        new = routed(h, xs, gain, lax.fori_loop(0, F // MC, chunk, jnp.zeros((16, D), F32)))
        rows = lax.broadcasted_iota(I32, (8, D), 0)
        for j, g in enumerate((g1, g2)):
            hit = jnp.logical_or(rows + g == i1, rows + g == i2)
            fix_v[j] = jnp.where(hit, new[j * 8:(j + 1) * 8], plain(g)).astype(BF16)

    nb = OFFS[-1]
    pltpu.make_async_copy(out_v.at[pl.ds(0, nb)], out_hbm.at[pl.ds(0, nb)], sems.at[SEM_OUT]).wait()
    late = jnp.maximum(i1, i2) >= nb

    @pl.when(late)
    def _():
        out_copy(NT - 1).wait()

    c1 = pltpu.make_async_copy(fix_v.at[0], out_hbm.at[pl.ds(g1, 8)], sems.at[SEM_FIX])
    c2 = pltpu.make_async_copy(fix_v.at[1], out_hbm.at[pl.ds(g2, 8)], sems.at[SEM_FIX + 1])
    c1.start()

    @pl.when(g1 != g2)
    def _():
        c2.start()

    @pl.when(jnp.logical_not(late))
    def _():
        out_copy(NT - 1).wait()

    @pl.when(g1 != g2)
    def _():
        c2.wait()

    c1.wait()


_SCRATCH = [
    pltpu.VMEM((S, D + PAD), BF16),
    pltpu.VMEM((D, 3 * D + PAD), BF16),
    pltpu.VMEM((D, D + PAD), BF16),
    pltpu.VMEM((D, F), BF16),
    pltpu.VMEM((D, F), BF16),
    pltpu.VMEM((F, D + PAD), BF16),
    pltpu.VMEM((D,), BF16),
    pltpu.VMEM((S, 128), F32),
    pltpu.VMEM((S, 128), F32),
    pltpu.VMEM((S + 16, D), BF16),
    pltpu.VMEM((S, D), F32),
    pltpu.VMEM((2, 8, D), BF16),
    pltpu.VMEM((S // 2, D), U32),
    pltpu.VMEM((16, D), F32),
    pltpu.VMEM((16, D), F32),
    pltpu.SemaphoreType.DMA((NSEM,)),
]


def _run(kernel, A_x, A_wqkv, A_wo, B_w_r, B_w_gate, B_w_up, B_w_down):
    any_spec = pl.BlockSpec(memory_space=pl.ANY)
    out = pl.pallas_call(
        kernel,
        out_shape=jax.ShapeDtypeStruct((S, D), BF16),
        in_specs=[any_spec] * 7,
        out_specs=any_spec,
        scratch_shapes=_SCRATCH,
        compiler_params=pltpu.CompilerParams(vmem_limit_bytes=100 * 1024 * 1024, disable_bounds_checks=True),
    )(A_x.reshape(S, D), A_wqkv, A_wo, B_w_r, B_w_gate, B_w_up, B_w_down)
    return out.reshape(1, S, D)


@jax.jit
def pallas_sequential_preLN__linear_attn_block__moe_arch_mod__prompt_kernel(
    A_x: jax.Array,
    A_wqkv: jax.Array,
    A_wo: jax.Array,
    B_x: jax.Array,
    B_w_r: jax.Array,
    B_w_gate: jax.Array,
    B_w_up: jax.Array,
    B_w_down: jax.Array,
):
    return _run(_kernel, A_x, A_wqkv, A_wo, B_w_r, B_w_gate, B_w_up, B_w_down)
```

```python
import functools

import jax
import jax.numpy as jnp
from jax import lax
import jax.experimental.pallas as pl
import jax.experimental.pallas.tpu as pltpu

S, D, F, H, DH = 2048, 1024, 3584, 32, 32
G = D // 128
F32, BF16, I32, U32 = jnp.float32, jnp.bfloat16, jnp.int32, jnp.uint32
KEY0 = 64 << 23
PAD = 128
KC, QC, VC = 0, D, 2 * D
HS = S // 2
K2 = 512
QE = 256
GB = 256
TQ = 512
TA = 256
TILES = [128] * 15 + [64, 64]
OFFS = [sum(TILES[:i]) for i in range(len(TILES))]
NT = len(TILES)
CT = 4
FKEEP = 10
MC = 128
LT = 6
SEM_OUT, SEM_FIX, SEM_LAST, NSEM = 16, 17, 19, 20


def _rb(x):
    return x.astype(BF16).astype(F32)


def _pk(x):
    return pltpu.bitcast(x, U32)


def _unpk(x):
    return pltpu.bitcast(x, BF16)


def _lanes(x, n):
    return jnp.concatenate([x] * n, axis=1) if n > 1 else x


def _rowsum(x):
    return jnp.broadcast_to(jnp.sum(x, axis=-1, keepdims=True), (x.shape[0], 128))


def _recip(d):
    r = pl.reciprocal(d, approx=True)
    return r * (2.0 - d * r)


def _rstd(var):
    v = _rb(_rb(var) + 1e-5)
    return _recip(_rb(v * lax.rsqrt(v)))


def _feat(t):
    return (jnp.where(t > 0, t + 1.0, jnp.exp(t)) + 1e-6).astype(BF16)


def _act(gt, ut):
    gt = _rb(gt)
    return (_rb(gt * jax.nn.sigmoid(gt)) * _rb(ut)).astype(BF16)


def _dot(a, b):
    return jnp.dot(a, b, preferred_element_type=F32)


def _keys(r, idx):
    bits = pltpu.bitcast(jnp.where(r == 0.0, 0.0, r), I32)
    hi = lax.shift_right_logical(bits, 16)
    mono = jnp.where(bits < 0, 0xFFFF - hi, hi | 0x8000)
    return pltpu.bitcast((mono << 11) + (KEY0 + S - 1 - idx), F32)


def _merge(top, k1, k2):
    if top is None:
        return k1, k2
    t1, t2 = top
    return jnp.maximum(t1, k1), jnp.maximum(jnp.minimum(t1, k1), jnp.maximum(t2, k2))


def _zero_of(x):
    bits = pltpu.bitcast(x, U32)
    return lax.shift_right_logical(lax.shift_right_logical(bits, U32(31)), U32(1))


def _pace(dep, n, lo, hi):
    if isinstance(dep, (list, tuple)):
        dep = jnp.concatenate(dep, axis=1)
    nrg, nch = dep.shape[0] // 8, dep.shape[1] // 128
    parts = []
    for p in range(n):
        c, rg = divmod(int((lo + (hi - lo) * p / n) * nch * nrg), nrg)
        parts.append(dep[rg * 8:(rg + 1) * 8, c * 128:(c + 1) * 128])
    return _zero_of(jnp.concatenate(parts, axis=0))


def _tie(x, zero):
    return pltpu.bitcast(pltpu.bitcast(x, U32) | zero, F32)


def _gate(xu, zero):
    if zero is None:
        return xu
    top = xu[0:8, 0:512] | _lanes(zero, 4)
    if xu.shape[1] > 512:
        top = jnp.concatenate([top, xu[0:8, 512:]], axis=1)
    return jnp.concatenate([top, xu[8:]], axis=0) if xu.shape[0] > 8 else top


def _fold(x):
    x = pltpu.bitcast(x, U32) if x.dtype != U32 else x
    parts = [x[r:r + 8, c:c + 128] for r in range(0, x.shape[0], 8) for c in range(0, x.shape[1], 128)]
    while len(parts) > 1:
        parts = [parts[j] | parts[j + 1] if j + 1 < len(parts) else parts[j] for j in range(0, len(parts), 2)]
    return _zero_of(parts[0])


def _blocks_done(xs):
    return _fold(jnp.concatenate([x[r + 56:r + 64] for x in xs for r in range(0, x.shape[0], 64)], axis=1))


def _passes(xu, w, gate_fn=None, post=None, after=None):
    deps, outs = [], []
    nk = xu.shape[1] // 512
    for c in range(G):
        acc = None
        for hh in range(nk):
            z = None if gate_fn is None else gate_fn(nk * c + hh, deps)
            lhs = _unpk(_gate(xu[:, hh * 512:(hh + 1) * 512], z))
            part = _dot(lhs, w(hh * 512, (hh + 1) * 512, c))
            acc = part if acc is None else acc + part
            deps.append(acc)
            if after is not None:
                after(nk * c + hh)
        outs.append(acc if post is None else post(c, acc))
    return outs, deps


def _ffn_groups():
    groups = []
    nq = F // 512
    for q in range(nq + 1):
        if q < nq:
            groups += [("up", c, m, hh) for c in range(4 * q, 4 * q + 4) for m in range(2) for hh in range(2)]
        if q >= 2:
            groups += [("down", q - 2, c) for c in range(G)]
    return groups + [("down", nq - 1, c) for c in range(G)]


def _kernel(x_hbm, wqkv_hbm, wo_hbm, wr_hbm, wg_hbm, wu_hbm, wd_hbm, out_hbm,
            x_v, wqkv_v, wo_v, wg_v, wu_v, wd_v, wr_v, mu_v, rs_v, out_v, h_v, fix_v, o_v, co_v, cx_v, keep_v, sems,
            *, force_fallback=False):
    def x_copy(r0, n, c0, m, s):
        return pltpu.make_async_copy(x_hbm.at[pl.ds(r0, n), pl.ds(c0, m)], x_v.at[pl.ds(r0, n), pl.ds(c0, m)],
                                     sems.at[s])

    def w_copy(r0, n, src, dst, s):
        return pltpu.make_async_copy(wqkv_hbm.at[pl.ds(r0, n), pl.ds(src, D)],
                                     wqkv_v.at[pl.ds(r0, n), pl.ds(dst, D)], sems.at[s])

    def out_copy(i):
        rows = pl.ds(OFFS[i], TILES[i])
        return pltpu.make_async_copy(out_v.at[rows], out_hbm.at[rows], sems.at[SEM_LAST if i == NT - 1 else SEM_OUT])

    sets = [
        [w_copy(0, 128, D, KC, 0), pltpu.make_async_copy(wr_hbm, wr_v, sems.at[1]), x_copy(0, HS, 0, 128, 2)],
        [x_copy(HS, HS, 0, 128, 3), w_copy(0, 128, 0, QC, 4)],
        [w_copy(128, K2 - 128, D, KC, 5), x_copy(0, S, 128, K2 - 128, 6), w_copy(128, QE - 128, 0, QC, 7)],
        [w_copy(K2, D - K2, D, KC, 8), x_copy(0, S, K2, D - K2, 9), w_copy(0, D, 2 * D, VC, 10),
         pltpu.make_async_copy(wo_hbm, wo_v.at[:, pl.ds(0, D)], sems.at[11])],
        [w_copy(QE, D - QE, 0, QC, 12), pltpu.make_async_copy(wg_hbm, wg_v, sems.at[13]),
         pltpu.make_async_copy(wu_hbm, wu_v, sems.at[14]),
         pltpu.make_async_copy(wd_hbm, wd_v.at[:, pl.ds(0, D)], sems.at[15])],
    ]
    for group in sets:
        for c in group:
            c.start()

    def raw(r0, t, c0, n, wcol):
        return _dot(x_v[r0:r0 + t, c0:c0 + n], wqkv_v[c0:c0 + n, wcol:wcol + D])

    def colsum(r0, n, wcol, dep, hi, pieces):
        cuts = [n // 16 * k // pieces * 16 for k in range(pieces + 1)]
        pz = pltpu.bitcast(_pace(dep, pieces, 0.02, hi), I32)
        tot = None
        for k in range(pieces):
            m = cuts[k + 1] - cuts[k]
            rows = pl.ds(pl.multiple_of(r0 + cuts[k] + pz[k * 8:(k + 1) * 8][0, 0], 16), m)
            w = jnp.sum(wqkv_v[rows, wcol:wcol + D].astype(F32).reshape(m // 8, 8, D), axis=0)
            tot = w if tot is None else tot + w
        return tot

    def moments(r0, t, c0, n, shift, dep, hi):
        xf = x_v[r0:r0 + t, c0:c0 + n].astype(F32)
        if shift is None:
            shift = jnp.broadcast_to(xf[:, 0:1], (t, 128))
        d = xf - _lanes(_tie(shift, _pace(dep, t // 8, 0.0, hi)), n // 128)
        e = d * wc[:, c0:c0 + n]
        add = lambda v: functools.reduce(jnp.add, [v[:, c:c + 128] for c in range(0, n, 128)])
        return shift, (add(d), add(d * d), add(e))

    sets[0][0].wait()
    sets[0][1].wait()
    cs = jnp.sum(wqkv_v[0:128, KC:KC + D].astype(F32).reshape(16, 8, D), axis=0)
    wr = wr_v[...].astype(F32).reshape(1, D)
    wr_sum = _rowsum(wr)
    wc = wr - _lanes(wr_sum * (1.0 / D), G)
    sets[0][2].wait()
    acc_a = raw(0, HS, 0, 128, KC)
    shift_a, mom_a = moments(0, HS, 0, 128, None, acc_a, 0.9)
    for c in sets[1]:
        c.wait()
    acc_b = raw(HS, HS, 0, 128, KC)
    shift_b, mom_b = moments(HS, HS, 0, 128, None, acc_b, 0.9)
    accq0 = raw(0, S, 0, 128, QC)
    csq = colsum(0, 128, QC, accq0, 0.6, 8)
    acc = jnp.concatenate([acc_a, acc_b], axis=0)
    shift = jnp.concatenate([shift_a, shift_b], axis=0)
    mom = [jnp.concatenate(p, axis=0) for p in zip(mom_a, mom_b)]
    for j, (c0, n) in enumerate(((128, K2 - 128), (K2, D - K2))):
        for c in sets[2 + j]:
            c.wait()
        if j == 0:
            partq = raw(0, S, 128, QE - 128, QC)
            accq0 = accq0 + partq
            csq = jnp.sum(csq + colsum(128, QE - 128, QC, partq, 0.6, 8), axis=0, keepdims=True)
        part = raw(0, S, c0, n, KC)
        acc = acc + part
        if j == 0:
            part = jnp.concatenate([partq[:, 0:256], part], axis=1)
        _, new = moments(0, S, c0, n, shift, part, (0.9, 0.4)[j])
        mom = [a + b for a, b in zip(mom, new)]
        cs = cs + colsum(c0, n, KC, part, (0.6, 0.3)[j], (18, 32)[j])
    s1, s2, xw = mom
    m1 = _rowsum(s1) * (1.0 / D)
    rs1 = _rstd(jnp.maximum(_rowsum(s2) * (1.0 / D) - m1 * m1, 0.0))
    mu1 = _rb(shift + m1)
    mu_v[...] = mu1
    zx = _pace(part, S // 8, 0.3, 0.95)
    mux = _tie(mu1, jnp.concatenate([zx[0:S // 4], zx[S // 4:S // 4 + 8] | _fold(cs), zx[S // 4 + 8:]], axis=0))
    cs = jnp.sum(cs, axis=0, keepdims=True)
    xu = _pk(((x_v[:, 0:D].astype(F32) - _lanes(mux, G)) * _lanes(rs1, G)).astype(BF16))
    xn = _unpk(xu)

    z_acc, g_acc, nxt = {}, {}, {}

    def k_block(c, zero):
        k = GB // 128
        pk = _feat((acc[:, c:c + GB] - _lanes(_tie(mu1, zero), k) * cs[:, c:c + GB]) * _lanes(rs1, k))
        zs = jnp.sum(pk.astype(F32).reshape(S // 8, 8, GB), axis=0)
        for b in range(0, GB, 128):
            z_acc[(c + b) // 128] = zs[:, b:b + 128]
        return _pk(pk.T), zs

    nxt[0] = k_block(0, _pace(part, S // 8, 0.6, 0.92))
    for c in range(0, D, GB):
        def gate_g(p, deps, c=c):
            if p != 28:
                return None
            if c + GB == D:
                mu = _tie(mu1, _pace(deps, S // 8, 0.0, 0.85))
                nxt["head"] = (accq0 - _lanes(mu, G) * csq) * _lanes(rs1, G)
                return _fold(nxt["head"][:, D - 128:D])
            nxt[c + GB] = k_block(c + GB, _pace(deps, S // 8, 0.0, 0.85))
            return _blocks_done([nxt[c + GB][0]]) | _fold(nxt[c + GB][1])

        outs, _ = _passes(nxt[c][0], lambda a, b, n: xn[a:b, n * 128:(n + 1) * 128], gate_g)
        upd = jnp.concatenate(outs, axis=1)
        for b in range(0, GB, 128):
            g_acc[(c + b) // 128] = upd[b:b + 128]

    same = (lax.broadcasted_iota(I32, (128, 128), 0) // DH) == (lax.broadcasted_iota(I32, (128, 128), 1) // DH)
    kvs = []
    for g in range(G):
        kv = _dot(g_acc[g].astype(BF16), wqkv_v[:, VC + g * 128:VC + (g + 1) * 128])
        kvs.append(jnp.where(same, kv, 0.0).astype(BF16))
    m_rows = [_pk(_dot(kvs[g], wo_v[g * 128:(g + 1) * 128, 0:D]).astype(BF16)) for g in range(G)]

    once = pltpu.bitcast(_zero_of(cs[:, 0:128] + jnp.zeros((8, 128), F32)), I32)[0, 0] + 1
    for c in sets[4]:
        c.wait()

    lane = lax.broadcasted_iota(I32, (8, 128), 1)
    sub = lax.broadcasted_iota(I32, (8, 128), 0)
    pqt, os, est, st8 = [], [], [None, None], {}

    def o_tile(r0, zero):
        pq = _unpk(jnp.concatenate(pqt, axis=1)[:, r0:r0 + TA]).astype(F32)
        z4 = st8["zc"].reshape(H, DH // 8, 8, 128)
        z0 = _tie(z4[:, 0].reshape(H * 8, 128), zero).reshape(H, 1, 8, 128)
        zz = jnp.concatenate([z0, z4[:, 1:]], axis=1).reshape(D, 128)
        w = (pq * _lanes(zz, TA // 128)).reshape(H, DH // 8, 8, TA)
        den = jnp.sum(jnp.sum(w, axis=1), axis=1, keepdims=True) + 1e-6
        o = pq.reshape(H, DH, TA) * _recip(den)
        ou = _pk(o.reshape(D, TA).astype(BF16).T)
        o_v[r0 // 2:(r0 + TA) // 2, :] = ou
        return ou

    def follow_o(i, deps, lo, hi):
        n = TQ // TA
        pz = _pace(deps, n * H, lo, hi)
        os.extend(o_tile((n * i + j) * TA, pz[j * H * 8:(j + 1) * H * 8]) for j in range(n))
        return _blocks_done(os[n * i:])

    def follow_est(i, deps, lo, hi):
        pz = _pace(deps, TQ // 8, lo, hi)
        for j in range(TQ // TA * i, TQ // TA * (i + 1)):
            o = _unpk(os[j]).astype(F32).reshape(TA // 8, 8, D) * st8["mw"]
            e = _tie(xw[j * TA:(j + 1) * TA], pz[j * TA - i * TQ:(j + 1) * TA - i * TQ])
            for c in range(0, D, 128):
                e = e + o[:, :, c:c + 128].reshape(TA, 128)
            e = _rowsum(e)
            half, p0 = divmod(j * TA // 8, 128)
            for p in range(TA // 8):
                v = e[p * 8:(p + 1) * 8]
                est[half] = v if est[half] is None else jnp.where(lane == p0 + p, v, est[half])
        return _zero_of(est[(i * TQ) // 1024])

    def m_tile(a, b, c):
        return _unpk(jnp.concatenate(m_rows[a // 128:b // 128], axis=0)[:, c * 128:(c + 1) * 128])

    def write_out(i, mur, rs):
        r0, t = OFFS[i], TILES[i]
        out_v[r0:r0 + t, :] = (h_v[r0:r0 + t, :] * _lanes(1.0 + rs, G) - _lanes(mur * rs, G)).astype(BF16)
        back = out_v[r0:r0 + t, D - 128:D].astype(F32)
        out_copy(i).start()
        return back

    def stats(i, mu, dep, hi):
        r0, t = OFFS[i], TILES[i]
        mu = _tie(mu, _pace(dep, t // 8, 0.0, hi))
        d = h_v[r0:r0 + t, :] - _lanes(mu, G)
        rs = _rstd(_rowsum(d * d) * (1.0 / D))
        mur = _rb(mu)
        r = _rb((_rowsum(d * wr) + (mu - mur) * wr_sum) * rs)
        mu_v[r0:r0 + t, :] = mur
        rs_v[r0:r0 + t, :] = rs
        return r, mur, rs

    def compact(i, r):
        t = TILES[i]
        acc = r[0:8]
        for p in range(1, t // 8):
            acc = jnp.where(lane == p, r[p * 8:(p + 1) * 8], acc)
        return jnp.where(lane < t // 8, _keys(acc, OFFS[i] + lane * 8 + sub), 0.0)

    def tree(i, r):
        key = _keys(r, lax.broadcasted_iota(I32, (TILES[i], 128), 0) + OFFS[i])
        level = [(key[p * 8:(p + 1) * 8], None) for p in range(TILES[i] // 8)]
        while len(level) > 1:
            up = []
            for (a1, a2), (b1, b2) in zip(level[0::2], level[1::2]):
                lo = jnp.minimum(a1, b1)
                for e in (a2, b2):
                    lo = lo if e is None else jnp.maximum(lo, e)
                up.append((jnp.maximum(a1, b1), lo))
            level = up
        return level[0]

    groups = _ffn_groups()
    ffn = {"next": 0, "xs": None, "act": {}, "y": {}, "w": {}}

    def ffn_group():
        grp = groups[ffn["next"]]
        ffn["next"] += 1
        if grp[0] == "up":
            _, c, m, hh = grp
            w_v = (wg_v, wu_v)[m]
            part = _dot(ffn["xs"][:, hh * 512:(hh + 1) * 512], w_v[hh * 512:(hh + 1) * 512, c * 128:(c + 1) * 128])
            ffn[m] = part if hh == 0 else ffn[m] + part
            if m == 1 and hh == 1:
                ffn["act"][c] = _act(ffn[0], ffn[1])
        else:
            _, q, c = grp
            a = jnp.concatenate([ffn["act"][4 * q + k] for k in range(4)], axis=1)
            if ffn["next"] == len(groups) - FKEEP + 4:
                a = _unpk(_gate(_pk(a), ffn["gate"]))
            w = ffn["w"].get((q, c))
            part = _dot(a, wd_v[q * 512:(q + 1) * 512, c * 128:(c + 1) * 128] if w is None else _unpk(w))
            ffn["y"][c] = part if q == 0 else ffn["y"][c] + part

    def ffn_step(i, p):
        if ffn["xs"] is not None and (i, p) >= (CT + 1, 9) and ffn["next"] < len(groups) - FKEEP:
            ffn_group()

    def preload(deps):
        keep = groups[len(groups) - FKEEP:]
        pz = _pace(deps, 4 * len(keep), 0.0, 0.8)
        for k, (_, q, c) in enumerate(keep):
            w = _pk(wd_v[q * 512:(q + 1) * 512, c * 128:(c + 1) * 128])
            zero = jnp.concatenate(
                [pz[(4 * k + j) * 8:(4 * k + j + 1) * 8] for j in range(4) for _ in range(8)], axis=0)
            ffn["w"][q, c] = w | zero
        return _fold(jnp.concatenate(list(ffn["w"].values()), axis=1))

    def candidates(deps):
        ka, kb = [_keys(_rb(e), h * 1024 + lane * 8 + sub) for h, e in enumerate(est)]
        t1, t2 = jnp.maximum(ka, kb), jnp.minimum(ka, kb)
        c1 = jnp.max(t1, axis=1, keepdims=True)
        c2 = jnp.max(jnp.where(t1 == c1, t2, t1), axis=1, keepdims=True)
        ck = pltpu.bitcast(jnp.broadcast_to(jnp.concatenate([c1, c2], axis=0), (16, 128)), I32)
        idx = S - 1 - (ck & (S - 1))
        pz = pltpu.bitcast(_pace(deps, 16, 0.25, 0.75), I32)
        for k in range(16):
            i = (idx[k // 8 * 8:k // 8 * 8 + 8] | pz[k * 8:(k + 1) * 8])[k % 8, 0]
            w = o_v[pl.ds(lax.shift_right_logical(i, 1), 1), :]
            w = jnp.where((i & 1) == 0, w << 16, w & U32(0xFFFF0000))
            co_v[k:k + 1, :] = pltpu.bitcast(w, F32)
            xg = x_v[pl.ds(pl.multiple_of(i - k % 8, 8), 8), 0:D].astype(F32)
            cx_v[k:k + 1, :] = xg[k % 8:k % 8 + 1]
        return idx, _pk(co_v[...].astype(BF16))

    def normalize(h):
        mu = _rowsum(h) * (1.0 / D)
        d = h - _lanes(mu, G)
        rs = _rstd(_rowsum(d * d) * (1.0 / D))
        mur = _rb(mu)
        r = _rb((_rowsum(d * wr) + (mu - mur) * wr_sum) * rs)
        return ((h - _lanes(mur, G)) * _lanes(rs, G)).astype(BF16), _rb(jax.nn.sigmoid(r))

    def routed(h, xs, gain, y):
        return h + _rb(xs.astype(F32) + _rb(_rb(y) * _lanes(gain, G)))

    def project(i, gate, extra):
        r0, t = OFFS[i], TILES[i]

        def post(c, attn):
            h_v[r0:r0 + t, c * 128:(c + 1) * 128] = x_v[r0:r0 + t, c * 128:(c + 1) * 128].astype(F32) + attn[0:t]
            return None if extra is None else attn[t:]

        ou = o_rows(r0, t)
        if extra is not None:
            ou = jnp.concatenate([ou, extra], axis=0)
        gate_fn = gate if callable(gate) else lambda p, deps: gate.get(p)
        outs, deps = _passes(ou, m_tile, gate_fn, post, lambda p: ffn_step(i, p))
        return [d[0:t] for d in deps], outs

    def mean_h(i):
        return _rowsum(h_v[OFFS[i]:OFFS[i] + TILES[i], :]) * (1.0 / D)

    def o_rows(r0, t):
        if os:
            return jnp.concatenate(os, axis=0)[r0 // 2:(r0 + t) // 2, :]
        return o_v[r0 // 2:(r0 + t) // 2, :]

    def finish_tile(i, mu, deps, hi, top):
        r, mur, rs = stats(i, mu, deps, hi)
        back = write_out(i, mur, rs)
        key = compact(i, r)
        return _merge(top, key, jnp.zeros_like(key)), _zero_of(key + jnp.sum(back.reshape(-1, 8, 128), axis=0))

    kept = {}

    def keep(name, x):
        u = pltpu.bitcast(x, U32)
        parts = [u[r:r + 8, c:c + 128] for r in range(0, u.shape[0], 8) for c in range(0, u.shape[1], 128)]
        at = sum(n for _, n, _, _ in kept.values())
        kept[name] = (at, len(parts), u.shape, x.dtype)
        keep_v[at * 8:(at + len(parts)) * 8, :] = jnp.concatenate(parts, axis=0)

    def fetch(name):
        at, n, shape, dtype = kept[name]
        v = keep_v[at * 8:(at + n) * 8, :]
        k = shape[1] // 128
        u = jnp.concatenate([jnp.concatenate([v[(r * k + c) * 8:(r * k + c + 1) * 8] for c in range(k)], axis=1)
                             for r in range(shape[0] // 8)], axis=0)
        return pltpu.bitcast(u, dtype)

    def project_last(gate, mu_prev, top):
        i = NT - 1
        r0, t = OFFS[i], TILES[i]
        st = {}

        def post(c, attn):
            h = x_v[r0:r0 + t, c * 128:(c + 1) * 128].astype(F32) + attn
            h_v[r0:r0 + t, c * 128:(c + 1) * 128] = h
            if c == 0:
                st["shift"] = jnp.broadcast_to(h[:, 0:1], (t, 128))
            d = h - st["shift"]
            new = (d, d * d, d * wr[:, c * 128:(c + 1) * 128])
            st[c] = new if c == 0 else tuple(a + b for a, b in zip(st[c - 1], new))

        def gate_fn(p, deps):
            if p == 0:
                return gate
            z = None
            if p % 2 == 1 and p // 2 >= 4:
                z = _fold(jnp.concatenate(st[p // 2 - 4], axis=1))
            if p == 13:
                r, mur, rs = stats(i - 1, mu_prev, deps, 0.5)
                st["top"] = _merge(top, *tree(i - 1, r))
                ffn["gate"] = _fold(write_out(i - 1, mur, rs))
                z = z | _zero_of(st["top"][0] + st["top"][1])
            return z

        _passes(o_rows(r0, t), m_tile, gate_fn, post, lambda p: ffn_step(i, p))
        while ffn["next"] < len(groups):
            ffn_group()
        s1, s2, s3 = st[G - 1]
        m1 = _rowsum(s1) * (1.0 / D)
        rs = _rstd(jnp.maximum(_rowsum(s2) * (1.0 / D) - m1 * m1, 0.0))
        mur = _rb(st["shift"] + m1)
        r = _rb((_rowsum(s3) + (st["shift"] - mur) * wr_sum) * rs)
        mu_v[r0:r0 + t, :] = mur
        rs_v[r0:r0 + t, :] = rs
        return _merge(st["top"], *tree(i, r)), mur, rs

    def middle(_, carry):
        del pqt[:], os[:]
        est[:] = [None, None]
        kept.clear()
        ffn.update({"next": 0, "xs": None, "act": {}, "y": {}, "w": {}})
        z = _rb(jnp.sum(jnp.concatenate([z_acc[b] for b in range(G)], axis=1), axis=0, keepdims=True))
        st8["zc"] = jnp.concatenate(
            [jnp.broadcast_to(z[:, g * 128:(g + 1) * 128], (128, 128)).T for g in range(G)], axis=0)
        gate = None
        for i in range(S // TQ):
            accq = _dot(_unpk(_gate(xu[i * TQ // 2:(i + 1) * TQ // 2, QE:], gate)), wqkv_v[QE:, QC:QC + D])
            head = nxt["head"][i * TQ:(i + 1) * TQ]
            if i == 0:
                e = _unpk(jnp.concatenate(m_rows, axis=0)).astype(F32) * wc
                e = jnp.concatenate([_tie(e[:, 0:128], _pace(accq, D // 8, 0.0, 0.7)), e[:, 128:]], axis=1)
                e = _rowsum(e)
                st8["mw"] = jnp.concatenate([e[g * 128:(g + 1) * 128].T[0:8] for g in range(G)], axis=1)
                gate = _fold(st8["mw"])
            else:
                follow_o(i - 1, accq, 0.05, 0.6)
                gate = follow_est(i - 1, accq, 0.45, 0.9)
            pqt.append(_pk(_feat(accq + head).T))

        top = mu_prev = extra = None
        gate = {0: gate, 6: _blocks_done([pqt[-1]])}
        for i in range(LT):
            if i == LT - 1:
                def inner(p, deps, gate=gate, mu_prev=mu_prev, top=top):
                    if p != 15:
                        return gate.get(p)
                    st8["top"], zero = finish_tile(i - 1, mu_prev, deps, 0.55, top)
                    return zero

                project(i, inner, None)
                break
            deps, outs = project(i, gate, extra if i == CT else None)
            mu = mean_h(i)
            gate = {}
            if i == 0:
                gate[5] = follow_o(S // TQ - 1, deps, 0.35, 1.0)
            else:
                top, gate[0] = finish_tile(i - 1, mu_prev, deps, min(0.8, 1 - 560 / (16 * TILES[i])), top)
            if i == CT + 1:
                gate[0] = gate[0] | _fold(_pk(ffn["xs"]))
            if i == 1:
                gate[0] = gate[0] | follow_est(S // TQ - 1, deps, 0.25, 0.85)
            if i == CT - 2:
                cand, extra = candidates(deps)
                keep("cand", cand)
                gate[0] = gate[0] | _fold(extra) | _fold(cx_v[...])
            if i == CT:
                h16 = cx_v[...] + jnp.concatenate(outs, axis=1)
                ffn["xs"], gain16 = normalize(h16)
                keep("h16", h16)
                keep("gain16", gain16)
                keep("xs", ffn["xs"])
            mu_prev = mu
        keep("top", jnp.concatenate(st8["top"], axis=1))
        for c, a in ffn["act"].items():
            keep(("act", c), a)
        for c, y in ffn["y"].items():
            keep(("y", c), y)
        for m in range(2):
            keep(("part", m), ffn[m])
        return carry

    lax.fori_loop(0, once, middle, 0)
    del os[:]
    cand, h16, gain16, top = fetch("cand"), fetch("h16"), fetch("gain16"), fetch("top")
    top = (top[:, 0:128], top[:, 128:])
    ffn["xs"] = fetch("xs")
    ffn["act"] = {c: fetch(("act", c)) for c in ffn["act"]}
    ffn["y"] = {c: fetch(("y", c)) for c in ffn["y"]}
    ffn[0], ffn[1] = fetch(("part", 0)), fetch(("part", 1))

    gate = {}
    mu_prev = mean_h(LT - 1)
    for i in range(LT, NT - 1):
        deps, _ = project(i, gate, None)
        mu = mean_h(i)
        top, zero = finish_tile(i - 1, mu_prev, deps, min(0.8, 1 - 560 / (16 * TILES[i])), top)
        gate = {0: zero}
        if i == NT - 2:
            t1, t2 = top
            b1 = jnp.max(jnp.max(t1, axis=0, keepdims=True), axis=1, keepdims=True)
            rest = jnp.where(t1 == b1, t2, t1)
            b2 = jnp.max(jnp.max(rest, axis=0, keepdims=True), axis=1, keepdims=True)
            top = (jnp.where(sub == 0, b1, 0.0), jnp.where(sub == 0, b2, 0.0))
        if i == NT - 4:
            gate[0] = gate[0] | preload(deps)
        mu_prev = mu
    (t1, t2), mur_l, rs_l = project_last(gate[0], mu_prev, top)

    k1 = jnp.max(t1, axis=0, keepdims=True)
    k2 = jnp.max(jnp.where(t1 == k1, t2, t1), axis=0, keepdims=True)
    v1 = S - 1 - (pltpu.bitcast(k1, I32) & (S - 1))
    v2 = S - 1 - (pltpu.bitcast(k2, I32) & (S - 1))
    i1, i2 = v1[0, 0], v2[0, 0]
    g1 = pl.multiple_of(i1 & -8, 8)
    g2 = pl.multiple_of(i2 & -8, 8)
    write_out(NT - 1, mur_l, rs_l)
    out_v[S:S + 16, 0:128] = jnp.zeros((16, 128), BF16)
    chosen = jnp.logical_or(cand == v1, cand == v2)
    found = jnp.sum(chosen.astype(I32), axis=0, keepdims=True)[0, 0]

    def plain(g):
        rows = pl.ds(g, 8)
        rs = _tie(rs_v[rows, :], _zero_of(out_v[S:S + 8, 0:128].astype(F32)))
        return h_v[rows, :] * _lanes(1.0 + rs, G) - _lanes(mu_v[rows, :] * rs, G)

    new16 = routed(h16, ffn["xs"], gain16, jnp.concatenate([ffn["y"][c] for c in range(G)], axis=1))
    for j, (g, v) in enumerate(((g1, v1), (g2, v2))):
        here = jnp.logical_and(chosen, (cand & -8) == (v & -8))
        val = plain(g)
        for half in range(2):
            val = jnp.where(_lanes(here[half * 8:(half + 1) * 8], G), new16[half * 8:(half + 1) * 8], val)
        fix_v[j] = val.astype(BF16)

    @pl.when(found != (3 if force_fallback else 2))
    def _():
        h = jnp.concatenate([h_v[pl.ds(g1, 8), :], h_v[pl.ds(g2, 8), :]], axis=0)
        xs, gain = normalize(h)

        def chunk(c, y):
            cols = pl.ds(pl.multiple_of(c * MC, 128), MC)
            return y + _dot(_act(_dot(xs, wg_v[:, cols]), _dot(xs, wu_v[:, cols])), wd_v[cols, 0:D])

        new = routed(h, xs, gain, lax.fori_loop(0, F // MC, chunk, jnp.zeros((16, D), F32)))
        rows = lax.broadcasted_iota(I32, (8, D), 0)
        for j, g in enumerate((g1, g2)):
            hit = jnp.logical_or(rows + g == i1, rows + g == i2)
            fix_v[j] = jnp.where(hit, new[j * 8:(j + 1) * 8], plain(g)).astype(BF16)

    nb = OFFS[-1]
    pltpu.make_async_copy(out_v.at[pl.ds(0, nb)], out_hbm.at[pl.ds(0, nb)], sems.at[SEM_OUT]).wait()
    late = jnp.maximum(i1, i2) >= nb

    @pl.when(late)
    def _():
        out_copy(NT - 1).wait()

    c1 = pltpu.make_async_copy(fix_v.at[0], out_hbm.at[pl.ds(g1, 8)], sems.at[SEM_FIX])
    c2 = pltpu.make_async_copy(fix_v.at[1], out_hbm.at[pl.ds(g2, 8)], sems.at[SEM_FIX + 1])
    c1.start()

    @pl.when(g1 != g2)
    def _():
        c2.start()

    @pl.when(jnp.logical_not(late))
    def _():
        out_copy(NT - 1).wait()

    @pl.when(g1 != g2)
    def _():
        c2.wait()

    c1.wait()


_SCRATCH = [
    pltpu.VMEM((S, D + PAD), BF16),
    pltpu.VMEM((D, 3 * D + PAD), BF16),
    pltpu.VMEM((D, D + PAD), BF16),
    pltpu.VMEM((D, F), BF16),
    pltpu.VMEM((D, F), BF16),
    pltpu.VMEM((F, D + PAD), BF16),
    pltpu.VMEM((D,), BF16),
    pltpu.VMEM((S, 128), F32),
    pltpu.VMEM((S, 128), F32),
    pltpu.VMEM((S + 16, D), BF16),
    pltpu.VMEM((S, D), F32),
    pltpu.VMEM((2, 8, D), BF16),
    pltpu.VMEM((S // 2, D), U32),
    pltpu.VMEM((16, D), F32),
    pltpu.VMEM((16, D), F32),
    pltpu.VMEM((128 * 8, 128), U32),
    pltpu.SemaphoreType.DMA((NSEM,)),
]


def _run(kernel, A_x, A_wqkv, A_wo, B_w_r, B_w_gate, B_w_up, B_w_down):
    any_spec = pl.BlockSpec(memory_space=pl.ANY)
    out = pl.pallas_call(
        kernel,
        out_shape=jax.ShapeDtypeStruct((S, D), BF16),
        in_specs=[any_spec] * 7,
        out_specs=any_spec,
        scratch_shapes=_SCRATCH,
        compiler_params=pltpu.CompilerParams(vmem_limit_bytes=100 * 1024 * 1024, disable_bounds_checks=True,
                                             disable_semaphore_checks=True),
    )(A_x.reshape(S, D), A_wqkv, A_wo, B_w_r, B_w_gate, B_w_up, B_w_down)
    return out.reshape(1, S, D)


@jax.jit
def pallas_sequential_preLN__linear_attn_block__moe_arch_mod__prompt_kernel(
    A_x: jax.Array,
    A_wqkv: jax.Array,
    A_wo: jax.Array,
    B_x: jax.Array,
    B_w_r: jax.Array,
    B_w_gate: jax.Array,
    B_w_up: jax.Array,
    B_w_down: jax.Array,
):
    return _run(_kernel, A_x, A_wqkv, A_wo, B_w_r, B_w_gate, B_w_up, B_w_down)
```

```python
import functools

import jax
import jax.numpy as jnp
from jax import lax
import jax.experimental.pallas as pl
import jax.experimental.pallas.tpu as pltpu

S, D, F, H, DH = 2048, 1024, 3584, 32, 32
G = D // 128
F32, BF16, I32, U32 = jnp.float32, jnp.bfloat16, jnp.int32, jnp.uint32
KEY0 = 64 << 23
PAD = 128
KC, QC, VC = 0, D, 2 * D
HS = S // 2
K2 = 512
QE = 256
GB = 256
TQ = 512
TA = 256
TILES = [128] * 15 + [64, 64]
OFFS = [sum(TILES[:i]) for i in range(len(TILES))]
NT = len(TILES)
CT = 3
FM = F - 1024
FKEEP = 10
MC = 128
LT = 6
SEM_OUT, SEM_FIX, SEM_LAST, NSEM = 16, 17, 19, 20


def _rb(x):
    return x.astype(BF16).astype(F32)


def _pk(x):
    return pltpu.bitcast(x, U32)


def _unpk(x):
    return pltpu.bitcast(x, BF16)


def _lanes(x, n):
    return jnp.concatenate([x] * n, axis=1) if n > 1 else x


def _rowsum(x):
    return jnp.broadcast_to(jnp.sum(x, axis=-1, keepdims=True), (x.shape[0], 128))


def _recip(d):
    r = pl.reciprocal(d, approx=True)
    return r * (2.0 - d * r)


def _rstd(var):
    v = _rb(_rb(var) + 1e-5)
    return _recip(_rb(v * lax.rsqrt(v)))


def _feat(t):
    return (jnp.where(t > 0, t + 1.0, jnp.exp(t)) + 1e-6).astype(BF16)


def _act(gt, ut):
    gt = _rb(gt)
    return (_rb(gt * jax.nn.sigmoid(gt)) * _rb(ut)).astype(BF16)


def _dot(a, b):
    return jnp.dot(a, b, preferred_element_type=F32)


def _keys(r, idx):
    bits = pltpu.bitcast(jnp.where(r == 0.0, 0.0, r), I32)
    hi = lax.shift_right_logical(bits, 16)
    mono = jnp.where(bits < 0, 0xFFFF - hi, hi | 0x8000)
    return pltpu.bitcast((mono << 11) + (KEY0 + S - 1 - idx), F32)


def _merge(top, k1, k2):
    if top is None:
        return k1, k2
    t1, t2 = top
    return jnp.maximum(t1, k1), jnp.maximum(jnp.minimum(t1, k1), jnp.maximum(t2, k2))


def _zero_of(x):
    bits = pltpu.bitcast(x, U32)
    return lax.shift_right_logical(lax.shift_right_logical(bits, U32(31)), U32(1))


def _pace(dep, n, lo, hi):
    if isinstance(dep, (list, tuple)):
        dep = jnp.concatenate(dep, axis=1)
    nrg, nch = dep.shape[0] // 8, dep.shape[1] // 128
    parts = []
    for p in range(n):
        c, rg = divmod(int((lo + (hi - lo) * p / n) * nch * nrg), nrg)
        parts.append(dep[rg * 8:(rg + 1) * 8, c * 128:(c + 1) * 128])
    return _zero_of(jnp.concatenate(parts, axis=0))


def _tie(x, zero):
    return pltpu.bitcast(pltpu.bitcast(x, U32) | zero, F32)


def _gate(xu, zero):
    if zero is None:
        return xu
    top = xu[0:8, 0:512] | _lanes(zero, 4)
    if xu.shape[1] > 512:
        top = jnp.concatenate([top, xu[0:8, 512:]], axis=1)
    return jnp.concatenate([top, xu[8:]], axis=0) if xu.shape[0] > 8 else top


def _fold(x):
    x = pltpu.bitcast(x, U32) if x.dtype != U32 else x
    parts = [x[r:r + 8, c:c + 128] for r in range(0, x.shape[0], 8) for c in range(0, x.shape[1], 128)]
    while len(parts) > 1:
        parts = [parts[j] | parts[j + 1] if j + 1 < len(parts) else parts[j] for j in range(0, len(parts), 2)]
    return _zero_of(parts[0])


def _blocks_done(xs):
    return _fold(jnp.concatenate([x[r + 56:r + 64] for x in xs for r in range(0, x.shape[0], 64)], axis=1))


def _passes(xu, w, gate_fn=None, post=None, after=None):
    deps, outs = [], []
    nk = xu.shape[1] // 512
    for c in range(G):
        acc = None
        for hh in range(nk):
            z = None if gate_fn is None else gate_fn(nk * c + hh, deps)
            lhs = _unpk(_gate(xu[:, hh * 512:(hh + 1) * 512], z))
            part = _dot(lhs, w(hh * 512, (hh + 1) * 512, c))
            acc = part if acc is None else acc + part
            deps.append(acc)
            if after is not None:
                after(nk * c + hh)
        outs.append(acc if post is None else post(c, acc))
    return outs, deps


def _ffn_groups():
    groups, nd = [], 0
    for c in range(FM // 128):
        groups += [("up", c, m, hh) for m in range(2) for hh in range(2)]
        if c % 4 == 3 and c // 4 >= 2:
            groups += [("down", nd, n) for n in range(G)]
            nd += 1
    return groups + [("down", q, n) for q in range(nd, F // 512) for n in range(G)]


def _kernel(x_hbm, wqkv_hbm, wo_hbm, wr_hbm, wg_hbm, wu_hbm, wd_hbm, out_hbm,
            x_v, wqkv_v, wo_v, wg_v, wu_v, wd_v, wr_v, mu_v, rs_v, out_v, h_v, fix_v, o_v, co_v, cx_v, keep_v, xb_v, sems,
            *, force_fallback=False):
    def x_copy(r0, n, c0, m, s):
        return pltpu.make_async_copy(x_hbm.at[pl.ds(r0, n), pl.ds(c0, m)], x_v.at[pl.ds(r0, n), pl.ds(c0, m)],
                                     sems.at[s])

    def w_copy(r0, n, src, dst, s):
        return pltpu.make_async_copy(wqkv_hbm.at[pl.ds(r0, n), pl.ds(src, D)],
                                     wqkv_v.at[pl.ds(r0, n), pl.ds(dst, D)], sems.at[s])

    def out_copy(i):
        rows = pl.ds(OFFS[i], TILES[i])
        return pltpu.make_async_copy(out_v.at[rows], out_hbm.at[rows], sems.at[SEM_LAST if i == NT - 1 else SEM_OUT])

    sets = [
        [w_copy(0, 128, D, KC, 0), pltpu.make_async_copy(wr_hbm, wr_v, sems.at[1]), x_copy(0, HS, 0, 128, 2)],
        [x_copy(HS, HS, 0, 128, 3), w_copy(0, 128, 0, QC, 4)],
        [w_copy(128, K2 - 128, D, KC, 5), x_copy(0, S, 128, K2 - 128, 6), w_copy(128, QE - 128, 0, QC, 7)],
        [w_copy(K2, D - K2, D, KC, 8), x_copy(0, S, K2, D - K2, 9), w_copy(0, D, 2 * D, VC, 10),
         pltpu.make_async_copy(wo_hbm, wo_v.at[:, pl.ds(0, D)], sems.at[11])],
        [w_copy(QE, D - QE, 0, QC, 12), pltpu.make_async_copy(wg_hbm, wg_v, sems.at[13]),
         pltpu.make_async_copy(wu_hbm, wu_v, sems.at[14]),
         pltpu.make_async_copy(wd_hbm, wd_v.at[:, pl.ds(0, D)], sems.at[15])],
    ]
    for group in sets:
        for c in group:
            c.start()

    def raw(r0, t, c0, n, wcol):
        return _dot(x_v[r0:r0 + t, c0:c0 + n], wqkv_v[c0:c0 + n, wcol:wcol + D])

    def colsum(r0, n, wcol, dep, hi, pieces):
        cuts = [n // 16 * k // pieces * 16 for k in range(pieces + 1)]
        pz = pltpu.bitcast(_pace(dep, pieces, 0.02, hi), I32)
        tot = None
        for k in range(pieces):
            m = cuts[k + 1] - cuts[k]
            rows = pl.ds(pl.multiple_of(r0 + cuts[k] + pz[k * 8:(k + 1) * 8][0, 0], 16), m)
            w = jnp.sum(wqkv_v[rows, wcol:wcol + D].astype(F32).reshape(m // 8, 8, D), axis=0)
            tot = w if tot is None else tot + w
        return tot

    def moments(r0, t, c0, n, shift, dep, hi):
        xf = x_v[r0:r0 + t, c0:c0 + n].astype(F32)
        if shift is None:
            shift = jnp.broadcast_to(xf[:, 0:1], (t, 128))
        d = xf - _lanes(_tie(shift, _pace(dep, t // 8, 0.0, hi)), n // 128)
        e = d * wc[:, c0:c0 + n]
        add = lambda v: functools.reduce(jnp.add, [v[:, c:c + 128] for c in range(0, n, 128)])
        return shift, (add(d), add(d * d), add(e))

    sets[0][0].wait()
    sets[0][1].wait()
    cs = jnp.sum(wqkv_v[0:128, KC:KC + D].astype(F32).reshape(16, 8, D), axis=0)
    wr = wr_v[...].astype(F32).reshape(1, D)
    wr_sum = _rowsum(wr)
    wc = wr - _lanes(wr_sum * (1.0 / D), G)
    sets[0][2].wait()
    acc_a = raw(0, HS, 0, 128, KC)
    shift_a, mom_a = moments(0, HS, 0, 128, None, acc_a, 0.9)
    for c in sets[1]:
        c.wait()
    acc_b = raw(HS, HS, 0, 128, KC)
    shift_b, mom_b = moments(HS, HS, 0, 128, None, acc_b, 0.9)
    accq0 = raw(0, S, 0, 128, QC)
    csq = colsum(0, 128, QC, accq0, 0.6, 8)
    acc = jnp.concatenate([acc_a, acc_b], axis=0)
    shift = jnp.concatenate([shift_a, shift_b], axis=0)
    mom = [jnp.concatenate(p, axis=0) for p in zip(mom_a, mom_b)]
    for j, (c0, n) in enumerate(((128, K2 - 128), (K2, D - K2))):
        for c in sets[2 + j]:
            c.wait()
        if j == 0:
            partq = raw(0, S, 128, QE - 128, QC)
            accq0 = accq0 + partq
            csq = jnp.sum(csq + colsum(128, QE - 128, QC, partq, 0.6, 8), axis=0, keepdims=True)
        part = raw(0, S, c0, n, KC)
        acc = acc + part
        if j == 0:
            part = jnp.concatenate([partq[:, 0:256], part], axis=1)
        _, new = moments(0, S, c0, n, shift, part, (0.9, 0.4)[j])
        mom = [a + b for a, b in zip(mom, new)]
        cs = cs + colsum(c0, n, KC, part, (0.6, 0.3)[j], (18, 32)[j])
    s1, s2, xw = mom
    m1 = _rowsum(s1) * (1.0 / D)
    rs1 = _rstd(jnp.maximum(_rowsum(s2) * (1.0 / D) - m1 * m1, 0.0))
    mu1 = _rb(shift + m1)
    mu_v[...] = mu1
    zx = _pace(part, S // 8, 0.3, 0.95)
    mux = _tie(mu1, jnp.concatenate([zx[0:S // 4], zx[S // 4:S // 4 + 8] | _fold(cs), zx[S // 4 + 8:]], axis=0))
    cs = jnp.sum(cs, axis=0, keepdims=True)
    xu = _pk(((x_v[:, 0:D].astype(F32) - _lanes(mux, G)) * _lanes(rs1, G)).astype(BF16))
    xn = _unpk(xu)

    z_acc, g_acc, nxt = {}, {}, {}

    def k_block(c, zero):
        k = GB // 128
        pk = _feat((acc[:, c:c + GB] - _lanes(_tie(mu1, zero), k) * cs[:, c:c + GB]) * _lanes(rs1, k))
        zs = jnp.sum(pk.astype(F32).reshape(S // 8, 8, GB), axis=0)
        for b in range(0, GB, 128):
            z_acc[(c + b) // 128] = zs[:, b:b + 128]
        return _pk(pk.T), zs

    nxt[0] = k_block(0, _pace(part, S // 8, 0.6, 0.92))
    for c in range(0, D, GB):
        def gate_g(p, deps, c=c):
            if p != 28:
                return None
            if c + GB == D:
                mu = _tie(mu1, _pace(deps, S // 8, 0.0, 0.85))
                nxt["head"] = (accq0 - _lanes(mu, G) * csq) * _lanes(rs1, G)
                return _fold(nxt["head"][:, D - 128:D])
            nxt[c + GB] = k_block(c + GB, _pace(deps, S // 8, 0.0, 0.85))
            return _blocks_done([nxt[c + GB][0]]) | _fold(nxt[c + GB][1])

        outs, _ = _passes(nxt[c][0], lambda a, b, n: xn[a:b, n * 128:(n + 1) * 128], gate_g)
        upd = jnp.concatenate(outs, axis=1)
        for b in range(0, GB, 128):
            g_acc[(c + b) // 128] = upd[b:b + 128]

    same = (lax.broadcasted_iota(I32, (128, 128), 0) // DH) == (lax.broadcasted_iota(I32, (128, 128), 1) // DH)
    kvs = []
    for g in range(G):
        kv = _dot(g_acc[g].astype(BF16), wqkv_v[:, VC + g * 128:VC + (g + 1) * 128])
        kvs.append(jnp.where(same, kv, 0.0).astype(BF16))
    m_rows = [_pk(_dot(kvs[g], wo_v[g * 128:(g + 1) * 128, 0:D]).astype(BF16)) for g in range(G)]

    once = pltpu.bitcast(_zero_of(cs[:, 0:128] + jnp.zeros((8, 128), F32)), I32)[0, 0] + 1
    for c in sets[4]:
        c.wait()

    lane = lax.broadcasted_iota(I32, (8, 128), 1)
    sub = lax.broadcasted_iota(I32, (8, 128), 0)
    pqt, os, est, st8 = [], [], [None, None], {}

    def o_tile(r0, zero):
        pq = _unpk(jnp.concatenate(pqt, axis=1)[:, r0:r0 + TA]).astype(F32)
        z4 = st8["zc"].reshape(H, DH // 8, 8, 128)
        z0 = _tie(z4[:, 0].reshape(H * 8, 128), zero).reshape(H, 1, 8, 128)
        zz = jnp.concatenate([z0, z4[:, 1:]], axis=1).reshape(D, 128)
        w = (pq * _lanes(zz, TA // 128)).reshape(H, DH // 8, 8, TA)
        den = jnp.sum(jnp.sum(w, axis=1), axis=1, keepdims=True) + 1e-6
        o = pq.reshape(H, DH, TA) * _recip(den)
        ou = _pk(o.reshape(D, TA).astype(BF16).T)
        o_v[r0 // 2:(r0 + TA) // 2, :] = ou
        return ou

    def follow_o(i, deps, lo, hi):
        n = TQ // TA
        pz = _pace(deps, n * H, lo, hi)
        os.extend(o_tile((n * i + j) * TA, pz[j * H * 8:(j + 1) * H * 8]) for j in range(n))
        return _blocks_done(os[n * i:])

    def follow_est(i, deps, lo, hi):
        pz = _pace(deps, TQ // 8, lo, hi)
        for j in range(TQ // TA * i, TQ // TA * (i + 1)):
            o = _unpk(os[j]).astype(F32).reshape(TA // 8, 8, D) * st8["mw"]
            e = _tie(xw[j * TA:(j + 1) * TA], pz[j * TA - i * TQ:(j + 1) * TA - i * TQ])
            for c in range(0, D, 128):
                e = e + o[:, :, c:c + 128].reshape(TA, 128)
            e = _rowsum(e)
            half, p0 = divmod(j * TA // 8, 128)
            for p in range(TA // 8):
                v = e[p * 8:(p + 1) * 8]
                est[half] = v if est[half] is None else jnp.where(lane == p0 + p, v, est[half])
        return _zero_of(est[(i * TQ) // 1024])

    def m_tile(a, b, c):
        return _unpk(jnp.concatenate(m_rows[a // 128:b // 128], axis=0)[:, c * 128:(c + 1) * 128])

    def write_out(i, mur, rs):
        r0, t = OFFS[i], TILES[i]
        out_v[r0:r0 + t, :] = (h_v[r0:r0 + t, :] * _lanes(1.0 + rs, G) - _lanes(mur * rs, G)).astype(BF16)
        back = out_v[r0:r0 + t, D - 128:D].astype(F32)
        out_copy(i).start()
        return back

    def stats(i, mu, dep, hi):
        r0, t = OFFS[i], TILES[i]
        mu = _tie(mu, _pace(dep, t // 8, 0.0, hi))
        d = h_v[r0:r0 + t, :] - _lanes(mu, G)
        rs = _rstd(_rowsum(d * d) * (1.0 / D))
        mur = _rb(mu)
        r = _rb((_rowsum(d * wr) + (mu - mur) * wr_sum) * rs)
        mu_v[r0:r0 + t, :] = mur
        rs_v[r0:r0 + t, :] = rs
        return r, mur, rs

    def compact(i, r):
        t = TILES[i]
        acc = r[0:8]
        for p in range(1, t // 8):
            acc = jnp.where(lane == p, r[p * 8:(p + 1) * 8], acc)
        return jnp.where(lane < t // 8, _keys(acc, OFFS[i] + lane * 8 + sub), 0.0)

    def tree(i, r):
        key = _keys(r, lax.broadcasted_iota(I32, (TILES[i], 128), 0) + OFFS[i])
        level = [(key[p * 8:(p + 1) * 8], None) for p in range(TILES[i] // 8)]
        while len(level) > 1:
            up = []
            for (a1, a2), (b1, b2) in zip(level[0::2], level[1::2]):
                lo = jnp.minimum(a1, b1)
                for e in (a2, b2):
                    lo = lo if e is None else jnp.maximum(lo, e)
                up.append((jnp.maximum(a1, b1), lo))
            level = up
        return level[0]

    groups = _ffn_groups()
    ffn = {"next": 0, "xs": None, "act": {}, "y": {}, "w": {}, "ready": {}}

    def ffn_group():
        grp = groups[ffn["next"]]
        ffn["next"] += 1
        if grp[0] == "up":
            _, c, m, hh = grp
            w_v = (wg_v, wu_v)[m]
            part = _dot(ffn["xs"][:, hh * 512:(hh + 1) * 512], w_v[hh * 512:(hh + 1) * 512, c * 128:(c + 1) * 128])
            ffn[m] = part if hh == 0 else ffn[m] + part
            if m == 1 and hh == 1:
                ffn["act"][c] = _act(ffn[0], ffn[1])
        else:
            _, q, c = grp
            a = jnp.concatenate([ffn["act"][4 * q + k] for k in range(4)], axis=1)
            if ffn["next"] == len(groups) - FKEEP + 4:
                a = _unpk(_gate(_pk(a), ffn["gate"]))
            w = ffn["w"].get((q, c))
            part = _dot(a, wd_v[q * 512:(q + 1) * 512, c * 128:(c + 1) * 128] if w is None else _unpk(w))
            ffn["y"][c] = part if q == 0 else ffn["y"][c] + part

    def ffn_step(i, p):
        if ffn["xs"] is None or (i, p) < (CT + 1, 9) or ffn["next"] >= len(groups) - FKEEP:
            return
        grp = groups[ffn["next"]]
        if grp[0] == "up" or ffn["ready"].get(4 * grp[1] + 3, i if 4 * grp[1] + 3 not in ffn["act"] else -1) < i:
            ffn_group()

    vp = {"step": 0, "acc": {}}

    def vpu_steps(i, deps, count):
        pz = _pace(deps, count, 0.0, 0.92)
        for k in range(count):
            j, d = divmod(vp["step"], D // 8)
            if FM + j * 256 == F:
                break
            vp["step"] += 1
            both = xb_v[d * 8:(d + 1) * 8, :] | pz[k * 8:(k + 1) * 8]
            xt = [_lanes(pltpu.bitcast(v, F32), 2) for v in (both << 16, both & U32(0xFFFF0000))]
            c0 = FM + j * 256
            for m, w_v in enumerate((wg_v, wu_v)):
                w = w_v[d * 8:(d + 1) * 8, c0:c0 + 256].astype(F32)
                for t in range(2):
                    vp["acc"][m, t] = w * xt[t] if d == 0 else vp["acc"][m, t] + w * xt[t]
            if d == D // 8 - 1:
                gt, ut = [jnp.where(_lanes(vp["first"], 2), jnp.sum(vp["acc"][m, 0], axis=0, keepdims=True),
                                    jnp.sum(vp["acc"][m, 1], axis=0, keepdims=True)) for m in range(2)]
                a = _act(gt, ut)
                for b in range(2):
                    ffn["act"][c0 // 128 + b] = a[:, b * 128:(b + 1) * 128]
                    ffn["ready"][c0 // 128 + b] = i + 1
        return _fold(jnp.concatenate(list(vp["acc"].values()), axis=1))

    def preload(deps):
        keep = groups[len(groups) - FKEEP:]
        pz = _pace(deps, 4 * len(keep), 0.0, 0.8)
        for k, (_, q, c) in enumerate(keep):
            w = _pk(wd_v[q * 512:(q + 1) * 512, c * 128:(c + 1) * 128])
            zero = jnp.concatenate(
                [pz[(4 * k + j) * 8:(4 * k + j + 1) * 8] for j in range(4) for _ in range(8)], axis=0)
            ffn["w"][q, c] = w | zero
        return _fold(jnp.concatenate(list(ffn["w"].values()), axis=1))

    def candidates(deps):
        ka, kb = [_keys(_rb(e), h * 1024 + lane * 8 + sub) for h, e in enumerate(est)]
        t1, t2 = jnp.maximum(ka, kb), jnp.minimum(ka, kb)
        c1 = jnp.max(t1, axis=1, keepdims=True)
        c2 = jnp.max(jnp.where(t1 == c1, t2, t1), axis=1, keepdims=True)
        ck = pltpu.bitcast(jnp.broadcast_to(jnp.concatenate([c1, c2], axis=0), (16, 128)), I32)
        idx = S - 1 - (ck & (S - 1))
        pz = pltpu.bitcast(_pace(deps, 16, 0.25, 0.75), I32)
        for k in range(16):
            i = (idx[k // 8 * 8:k // 8 * 8 + 8] | pz[k * 8:(k + 1) * 8])[k % 8, 0]
            w = o_v[pl.ds(lax.shift_right_logical(i, 1), 1), :]
            w = jnp.where((i & 1) == 0, w << 16, w & U32(0xFFFF0000))
            co_v[k:k + 1, :] = pltpu.bitcast(w, F32)
            xg = x_v[pl.ds(pl.multiple_of(i - k % 8, 8), 8), 0:D].astype(F32)
            cx_v[k:k + 1, :] = xg[k % 8:k % 8 + 1]
        return idx, _pk(co_v[...].astype(BF16))

    def normalize(h):
        mu = _rowsum(h) * (1.0 / D)
        d = h - _lanes(mu, G)
        rs = _rstd(_rowsum(d * d) * (1.0 / D))
        mur = _rb(mu)
        r = _rb((_rowsum(d * wr) + (mu - mur) * wr_sum) * rs)
        return ((h - _lanes(mur, G)) * _lanes(rs, G)).astype(BF16), _rb(jax.nn.sigmoid(r)), r

    def routed(h, xs, gain, y):
        return h + _rb(xs.astype(F32) + _rb(_rb(y) * _lanes(gain, G)))

    def project(i, gate, extra):
        r0, t = OFFS[i], TILES[i]

        def post(c, attn):
            h_v[r0:r0 + t, c * 128:(c + 1) * 128] = x_v[r0:r0 + t, c * 128:(c + 1) * 128].astype(F32) + attn[0:t]
            return None if extra is None else attn[t:]

        ou = o_rows(r0, t)
        if extra is not None:
            ou = jnp.concatenate([ou, extra], axis=0)
        gate_fn = gate if callable(gate) else lambda p, deps: gate.get(p)
        outs, deps = _passes(ou, m_tile, gate_fn, post, lambda p: ffn_step(i, p))
        return [d[0:t] for d in deps], outs

    def mean_h(i):
        return _rowsum(h_v[OFFS[i]:OFFS[i] + TILES[i], :]) * (1.0 / D)

    def o_rows(r0, t):
        if os:
            return jnp.concatenate(os, axis=0)[r0 // 2:(r0 + t) // 2, :]
        return o_v[r0 // 2:(r0 + t) // 2, :]

    def finish_tile(i, mu, deps, hi, top):
        r, mur, rs = stats(i, mu, deps, hi)
        back = write_out(i, mur, rs)
        key = compact(i, r)
        return _merge(top, key, jnp.zeros_like(key)), _zero_of(key + jnp.sum(back.reshape(-1, 8, 128), axis=0))

    kept = {}

    def keep(name, x):
        u = pltpu.bitcast(x, U32) if x.dtype != U32 else x
        parts = [u[r:r + 8, c:c + 128] for r in range(0, u.shape[0], 8) for c in range(0, u.shape[1], 128)]
        at = sum(n for _, n, _, _ in kept.values())
        kept[name] = (at, len(parts), u.shape, x.dtype)
        keep_v[at * 8:(at + len(parts)) * 8, :] = jnp.concatenate(parts, axis=0)

    def fetch(name):
        at, n, shape, dtype = kept[name]
        v = keep_v[at * 8:(at + n) * 8, :]
        k = shape[1] // 128
        u = jnp.concatenate([jnp.concatenate([v[(r * k + c) * 8:(r * k + c + 1) * 8] for c in range(k)], axis=1)
                             for r in range(shape[0] // 8)], axis=0)
        return pltpu.bitcast(u, dtype) if dtype != U32 else u

    def project_last(gate, mu_prev, top):
        i = NT - 1
        r0, t = OFFS[i], TILES[i]
        st = {}

        def post(c, attn):
            h = x_v[r0:r0 + t, c * 128:(c + 1) * 128].astype(F32) + attn
            h_v[r0:r0 + t, c * 128:(c + 1) * 128] = h
            if c == 0:
                st["shift"] = jnp.broadcast_to(h[:, 0:1], (t, 128))
            d = h - st["shift"]
            new = (d, d * d, d * wr[:, c * 128:(c + 1) * 128])
            st[c] = new if c == 0 else tuple(a + b for a, b in zip(st[c - 1], new))

        def gate_fn(p, deps):
            if p == 0:
                return gate
            z = None
            if p % 2 == 1 and p // 2 >= 4:
                z = _fold(jnp.concatenate(st[p // 2 - 4], axis=1))
            if p == 13:
                r, mur, rs = stats(i - 1, mu_prev, deps, 0.5)
                st["top"] = _merge(top, *tree(i - 1, r))
                ffn["gate"] = _fold(write_out(i - 1, mur, rs))
                z = z | _zero_of(st["top"][0] + st["top"][1])
            return z

        _passes(o_rows(r0, t), m_tile, gate_fn, post, lambda p: ffn_step(i, p))
        while ffn["next"] < len(groups):
            ffn_group()
        s1, s2, s3 = st[G - 1]
        m1 = _rowsum(s1) * (1.0 / D)
        rs = _rstd(jnp.maximum(_rowsum(s2) * (1.0 / D) - m1 * m1, 0.0))
        mur = _rb(st["shift"] + m1)
        r = _rb((_rowsum(s3) + (st["shift"] - mur) * wr_sum) * rs)
        mu_v[r0:r0 + t, :] = mur
        rs_v[r0:r0 + t, :] = rs
        return _merge(st["top"], *tree(i, r)), mur, rs

    def middle(_, carry):
        del pqt[:], os[:]
        est[:] = [None, None]
        kept.clear()
        vp.update({"step": 0, "acc": {}})
        ffn.update({"next": 0, "xs": None, "act": {}, "y": {}, "w": {}, "ready": {}})
        z = _rb(jnp.sum(jnp.concatenate([z_acc[b] for b in range(G)], axis=1), axis=0, keepdims=True))
        st8["zc"] = jnp.concatenate(
            [jnp.broadcast_to(z[:, g * 128:(g + 1) * 128], (128, 128)).T for g in range(G)], axis=0)
        gate = None
        for i in range(S // TQ):
            accq = _dot(_unpk(_gate(xu[i * TQ // 2:(i + 1) * TQ // 2, QE:], gate)), wqkv_v[QE:, QC:QC + D])
            head = nxt["head"][i * TQ:(i + 1) * TQ]
            if i == 0:
                e = _unpk(jnp.concatenate(m_rows, axis=0)).astype(F32) * wc
                e = jnp.concatenate([_tie(e[:, 0:128], _pace(accq, D // 8, 0.0, 0.7)), e[:, 128:]], axis=1)
                e = _rowsum(e)
                st8["mw"] = jnp.concatenate([e[g * 128:(g + 1) * 128].T[0:8] for g in range(G)], axis=1)
                gate = _fold(st8["mw"])
            else:
                follow_o(i - 1, accq, 0.05, 0.6)
                gate = follow_est(i - 1, accq, 0.45, 0.9)
            pqt.append(_pk(_feat(accq + head).T))

        top = mu_prev = extra = None
        gate = {0: gate, 6: _blocks_done([pqt[-1]])}
        for i in range(LT):
            if i == LT - 1:
                def inner(p, deps, gate=gate, mu_prev=mu_prev, top=top):
                    if p != 15:
                        return gate.get(p)
                    st8["top"], zero = finish_tile(i - 1, mu_prev, deps, 0.55, top)
                    return zero | vpu_steps(i, deps, 44)

                project(i, inner, None)
                break
            deps, outs = project(i, gate, extra if i == CT else None)
            mu = mean_h(i)
            gate = {}
            if i == 0:
                gate[5] = follow_o(S // TQ - 1, deps, 0.35, 1.0)
            else:
                top, gate[0] = finish_tile(i - 1, mu_prev, deps, min(0.8, 1 - 560 / (16 * TILES[i])), top)
            if i == CT + 1:
                gate[0] = gate[0] | _fold(_pk(ffn["xs"]))
                pz = _pace(deps, G, 0.35, 0.7)
                for g in range(G):
                    row = pltpu.bitcast(st8["pair"][:, g * 128:(g + 1) * 128] | pz[g * 8:(g + 1) * 8], F32)
                    blk = _pk(jnp.concatenate([row] * 16, axis=0).T)
                    xb_v[g * 128:(g + 1) * 128, :] = blk
                    gate[0] = gate[0] | _zero_of(blk[120:128])
            if i == 1:
                gate[0] = gate[0] | follow_est(S // TQ - 1, deps, 0.25, 0.85)
            if i == CT - 1:
                cand, extra = candidates(deps)
                keep("cand", cand)
                gate[0] = gate[0] | _fold(extra) | _fold(cx_v[...])
            if i == CT:
                h16 = cx_v[...] + jnp.concatenate(outs, axis=1)
                ffn["xs"], gain16, r16 = normalize(h16)
                ck = _keys(r16, cand)
                first = ck == jnp.max(ck, axis=0, keepdims=True)
                second = ck == jnp.max(jnp.where(first, 0.0, ck), axis=0, keepdims=True)
                xf = ffn["xs"].astype(F32)
                lo, hi = [_pk(jnp.broadcast_to(jnp.sum(jnp.where(_lanes(m, G), xf, 0.0), axis=0, keepdims=True), (8, D)))
                          for m in (first, second)]
                st8["pair"] = lax.shift_right_logical(lo, U32(16)) | hi
                keep("rank", jnp.where(first, 1, jnp.where(second, 2, 0)))
                keep("h16", h16)
                keep("gain16", gain16)
                keep("xs", ffn["xs"])
            mu_prev = mu
        keep("top", jnp.concatenate(st8["top"], axis=1))
        for c, a in ffn["act"].items():
            keep(("act", c), a)
        for c, y in ffn["y"].items():
            keep(("y", c), y)
        for m in range(2):
            keep(("part", m), ffn[m])
        for k, a in vp["acc"].items():
            keep(("vp", k), a)
        return carry

    lax.fori_loop(0, once, middle, 0)
    del os[:]
    cand, h16, gain16, top = fetch("cand"), fetch("h16"), fetch("gain16"), fetch("top")
    top = (top[:, 0:128], top[:, 128:])
    ffn["xs"] = fetch("xs")
    ffn["act"] = {c: fetch(("act", c)) for c in ffn["act"]}
    ffn["y"] = {c: fetch(("y", c)) for c in ffn["y"]}
    ffn[0], ffn[1] = fetch(("part", 0)), fetch(("part", 1))
    rank = fetch("rank")
    vp["first"] = rank == 1
    vp["acc"] = {k: fetch(("vp", k)) for k in vp["acc"]}

    gate = {}
    mu_prev = mean_h(LT - 1)
    for i in range(LT, NT - 1):
        deps, _ = project(i, gate, None)
        mu = mean_h(i)
        top, zero = finish_tile(i - 1, mu_prev, deps, min(0.8, 1 - 560 / (16 * TILES[i])), top)
        gate = {0: zero}
        if vp["step"] < (F - FM) // 2:
            gate[0] = gate[0] | vpu_steps(i, deps, 52)
        if i == NT - 2:
            t1, t2 = top
            b1 = jnp.max(jnp.max(t1, axis=0, keepdims=True), axis=1, keepdims=True)
            rest = jnp.where(t1 == b1, t2, t1)
            b2 = jnp.max(jnp.max(rest, axis=0, keepdims=True), axis=1, keepdims=True)
            top = (jnp.where(sub == 0, b1, 0.0), jnp.where(sub == 0, b2, 0.0))
        if i == NT - 4:
            gate[0] = gate[0] | preload(deps)
        mu_prev = mu
    (t1, t2), mur_l, rs_l = project_last(gate[0], mu_prev, top)

    k1 = jnp.max(t1, axis=0, keepdims=True)
    k2 = jnp.max(jnp.where(t1 == k1, t2, t1), axis=0, keepdims=True)
    v1 = S - 1 - (pltpu.bitcast(k1, I32) & (S - 1))
    v2 = S - 1 - (pltpu.bitcast(k2, I32) & (S - 1))
    i1, i2 = v1[0, 0], v2[0, 0]
    g1 = pl.multiple_of(i1 & -8, 8)
    g2 = pl.multiple_of(i2 & -8, 8)
    write_out(NT - 1, mur_l, rs_l)
    out_v[S:S + 16, 0:128] = jnp.zeros((16, 128), BF16)
    chosen = jnp.logical_or(cand == v1, cand == v2)
    found = jnp.sum(jnp.logical_and(chosen, rank > 0).astype(I32), axis=0, keepdims=True)[0, 0]

    def plain(g):
        rows = pl.ds(g, 8)
        rs = _tie(rs_v[rows, :], _zero_of(out_v[S:S + 8, 0:128].astype(F32)))
        return h_v[rows, :] * _lanes(1.0 + rs, G) - _lanes(mu_v[rows, :] * rs, G)

    new16 = routed(h16, ffn["xs"], gain16, jnp.concatenate([ffn["y"][c] for c in range(G)], axis=1))
    for j, (g, v) in enumerate(((g1, v1), (g2, v2))):
        here = jnp.logical_and(chosen, (cand & -8) == (v & -8))
        val = plain(g)
        for half in range(2):
            val = jnp.where(_lanes(here[half * 8:(half + 1) * 8], G), new16[half * 8:(half + 1) * 8], val)
        fix_v[j] = val.astype(BF16)

    @pl.when(found != (3 if force_fallback else 2))
    def _():
        h = jnp.concatenate([h_v[pl.ds(g1, 8), :], h_v[pl.ds(g2, 8), :]], axis=0)
        xs, gain, _ = normalize(h)

        def chunk(c, y):
            cols = pl.ds(pl.multiple_of(c * MC, 128), MC)
            return y + _dot(_act(_dot(xs, wg_v[:, cols]), _dot(xs, wu_v[:, cols])), wd_v[cols, 0:D])

        new = routed(h, xs, gain, lax.fori_loop(0, F // MC, chunk, jnp.zeros((16, D), F32)))
        rows = lax.broadcasted_iota(I32, (8, D), 0)
        for j, g in enumerate((g1, g2)):
            hit = jnp.logical_or(rows + g == i1, rows + g == i2)
            fix_v[j] = jnp.where(hit, new[j * 8:(j + 1) * 8], plain(g)).astype(BF16)

    nb = OFFS[-1]
    pltpu.make_async_copy(out_v.at[pl.ds(0, nb)], out_hbm.at[pl.ds(0, nb)], sems.at[SEM_OUT]).wait()
    late = jnp.maximum(i1, i2) >= nb

    @pl.when(late)
    def _():
        out_copy(NT - 1).wait()

    c1 = pltpu.make_async_copy(fix_v.at[0], out_hbm.at[pl.ds(g1, 8)], sems.at[SEM_FIX])
    c2 = pltpu.make_async_copy(fix_v.at[1], out_hbm.at[pl.ds(g2, 8)], sems.at[SEM_FIX + 1])
    c1.start()

    @pl.when(g1 != g2)
    def _():
        c2.start()

    @pl.when(jnp.logical_not(late))
    def _():
        out_copy(NT - 1).wait()

    @pl.when(g1 != g2)
    def _():
        c2.wait()

    c1.wait()


_SCRATCH = [
    pltpu.VMEM((S, D + PAD), BF16),
    pltpu.VMEM((D, 3 * D + PAD), BF16),
    pltpu.VMEM((D, D + PAD), BF16),
    pltpu.VMEM((D, F), BF16),
    pltpu.VMEM((D, F), BF16),
    pltpu.VMEM((F, D + PAD), BF16),
    pltpu.VMEM((D,), BF16),
    pltpu.VMEM((S, 128), F32),
    pltpu.VMEM((S, 128), F32),
    pltpu.VMEM((S + 16, D), BF16),
    pltpu.VMEM((S, D), F32),
    pltpu.VMEM((2, 8, D), BF16),
    pltpu.VMEM((S // 2, D), U32),
    pltpu.VMEM((16, D), F32),
    pltpu.VMEM((16, D), F32),
    pltpu.VMEM((128 * 8, 128), U32),
    pltpu.VMEM((D, 128), U32),
    pltpu.SemaphoreType.DMA((NSEM,)),
]


def _run(kernel, A_x, A_wqkv, A_wo, B_w_r, B_w_gate, B_w_up, B_w_down):
    any_spec = pl.BlockSpec(memory_space=pl.ANY)
    out = pl.pallas_call(
        kernel,
        out_shape=jax.ShapeDtypeStruct((S, D), BF16),
        in_specs=[any_spec] * 7,
        out_specs=any_spec,
        scratch_shapes=_SCRATCH,
        compiler_params=pltpu.CompilerParams(vmem_limit_bytes=100 * 1024 * 1024, disable_bounds_checks=True,
                                             disable_semaphore_checks=True),
    )(A_x.reshape(S, D), A_wqkv, A_wo, B_w_r, B_w_gate, B_w_up, B_w_down)
    return out.reshape(1, S, D)


@jax.jit
def pallas_sequential_preLN__linear_attn_block__moe_arch_mod__prompt_kernel(
    A_x: jax.Array,
    A_wqkv: jax.Array,
    A_wo: jax.Array,
    B_x: jax.Array,
    B_w_r: jax.Array,
    B_w_gate: jax.Array,
    B_w_up: jax.Array,
    B_w_down: jax.Array,
):
    return _run(_kernel, A_x, A_wqkv, A_wo, B_w_r, B_w_gate, B_w_up, B_w_down)
```

```python
import functools

import jax
import jax.numpy as jnp
from jax import lax
import jax.experimental.pallas as pl
import jax.experimental.pallas.tpu as pltpu

S, D, F, H, DH = 2048, 1024, 3584, 32, 32
G = D // 128
F32, BF16, I32, U32 = jnp.float32, jnp.bfloat16, jnp.int32, jnp.uint32
KEY0 = 64 << 23
PAD = 128
KC, QC, VC = 0, D, 2 * D
HS = S // 2
K2 = 512
QE = 256
GB = 256
TQ = 512
TA = 256
TILES = [128] * 15 + [80, 48]
OFFS = [sum(TILES[:i]) for i in range(len(TILES))]
NT = len(TILES)
CT = 3
FM = F - 1024
FKEEP = 10
MC = 128
LT = 6
SEM_OUT, SEM_FIX, SEM_LAST, NSEM = 16, 17, 19, 20


def _rb(x):
    return x.astype(BF16).astype(F32)


def _pk(x):
    return pltpu.bitcast(x, U32)


def _unpk(x):
    return pltpu.bitcast(x, BF16)


def _lanes(x, n):
    return jnp.concatenate([x] * n, axis=1) if n > 1 else x


def _rowsum(x):
    return jnp.broadcast_to(jnp.sum(x, axis=-1, keepdims=True), (x.shape[0], 128))


def _recip(d):
    r = pl.reciprocal(d, approx=True)
    return r * (2.0 - d * r)


def _rstd(var):
    v = _rb(_rb(var) + 1e-5)
    return _recip(_rb(v * lax.rsqrt(v)))


def _feat(t):
    return (jnp.where(t > 0, t + 1.0, jnp.exp(t)) + 1e-6).astype(BF16)


def _act(gt, ut):
    gt = _rb(gt)
    return (_rb(gt * jax.nn.sigmoid(gt)) * _rb(ut)).astype(BF16)


def _dot(a, b):
    return jnp.dot(a, b, preferred_element_type=F32)


def _keys(r, idx):
    bits = pltpu.bitcast(jnp.where(r == 0.0, 0.0, r), I32)
    hi = lax.shift_right_logical(bits, 16)
    mono = jnp.where(bits < 0, 0xFFFF - hi, hi | 0x8000)
    return pltpu.bitcast((mono << 11) + (KEY0 + S - 1 - idx), F32)


def _merge(top, k1, k2):
    if top is None:
        return k1, k2
    t1, t2 = top
    return jnp.maximum(t1, k1), jnp.maximum(jnp.minimum(t1, k1), jnp.maximum(t2, k2))


def _zero_of(x):
    bits = pltpu.bitcast(x, U32)
    return lax.shift_right_logical(lax.shift_right_logical(bits, U32(31)), U32(1))


def _pace(dep, n, lo, hi):
    if isinstance(dep, (list, tuple)):
        dep = jnp.concatenate(dep, axis=1)
    nrg, nch = dep.shape[0] // 8, dep.shape[1] // 128
    parts = []
    for p in range(n):
        c, rg = divmod(int((lo + (hi - lo) * p / n) * nch * nrg), nrg)
        parts.append(dep[rg * 8:(rg + 1) * 8, c * 128:(c + 1) * 128])
    return _zero_of(jnp.concatenate(parts, axis=0))


def _tie(x, zero):
    return pltpu.bitcast(pltpu.bitcast(x, U32) | zero, F32)


def _gate(xu, zero):
    if zero is None:
        return xu
    top = xu[0:8, 0:512] | _lanes(zero, 4)
    if xu.shape[1] > 512:
        top = jnp.concatenate([top, xu[0:8, 512:]], axis=1)
    return jnp.concatenate([top, xu[8:]], axis=0) if xu.shape[0] > 8 else top


def _fold(x):
    x = pltpu.bitcast(x, U32) if x.dtype != U32 else x
    parts = [x[r:r + 8, c:c + 128] for r in range(0, x.shape[0], 8) for c in range(0, x.shape[1], 128)]
    while len(parts) > 1:
        parts = [parts[j] | parts[j + 1] if j + 1 < len(parts) else parts[j] for j in range(0, len(parts), 2)]
    return _zero_of(parts[0])


def _blocks_done(xs):
    return _fold(jnp.concatenate([x[r + 56:r + 64] for x in xs for r in range(0, x.shape[0], 64)], axis=1))


def _passes(xu, w, gate_fn=None, post=None, after=None):
    deps, outs = [], []
    nk = xu.shape[1] // 512
    for c in range(G):
        acc = None
        for hh in range(nk):
            z = None if gate_fn is None else gate_fn(nk * c + hh, deps)
            lhs = _unpk(_gate(xu[:, hh * 512:(hh + 1) * 512], z))
            part = _dot(lhs, w(hh * 512, (hh + 1) * 512, c))
            acc = part if acc is None else acc + part
            deps.append(acc)
            if after is not None:
                after(nk * c + hh)
        outs.append(acc if post is None else post(c, acc))
    return outs, deps


def _ffn_groups():
    groups, nd = [], 0
    for c in range(FM // 128):
        groups += [("up", c, m, hh) for m in range(2) for hh in range(2)]
        if c % 4 == 3 and c // 4 >= 2:
            groups += [("down", nd, n) for n in range(G)]
            nd += 1
    return groups + [("down", q, n) for q in range(nd, F // 512) for n in range(G)]


def _kernel(x_hbm, wqkv_hbm, wo_hbm, wr_hbm, wg_hbm, wu_hbm, wd_hbm, out_hbm,
            x_v, wqkv_v, wo_v, wg_v, wu_v, wd_v, wr_v, mu_v, rs_v, out_v, h_v, fix_v, o_v, co_v, cx_v, keep_v, xb_v, sems,
            *, force_fallback=False):
    def x_copy(r0, n, c0, m, s):
        return pltpu.make_async_copy(x_hbm.at[pl.ds(r0, n), pl.ds(c0, m)], x_v.at[pl.ds(r0, n), pl.ds(c0, m)],
                                     sems.at[s])

    def w_copy(r0, n, src, dst, s):
        return pltpu.make_async_copy(wqkv_hbm.at[pl.ds(r0, n), pl.ds(src, D)],
                                     wqkv_v.at[pl.ds(r0, n), pl.ds(dst, D)], sems.at[s])

    def out_copy(i):
        rows = pl.ds(OFFS[i], TILES[i])
        return pltpu.make_async_copy(out_v.at[rows], out_hbm.at[rows], sems.at[SEM_LAST if i == NT - 1 else SEM_OUT])

    sets = [
        [w_copy(0, 128, D, KC, 0), pltpu.make_async_copy(wr_hbm, wr_v, sems.at[1]), x_copy(0, HS, 0, 128, 2)],
        [x_copy(HS, HS, 0, 128, 3), w_copy(0, 128, 0, QC, 4)],
        [w_copy(128, K2 - 128, D, KC, 5), x_copy(0, S, 128, K2 - 128, 6), w_copy(128, QE - 128, 0, QC, 7)],
        [w_copy(K2, D - K2, D, KC, 8), x_copy(0, S, K2, D - K2, 9), w_copy(0, D, 2 * D, VC, 10),
         pltpu.make_async_copy(wo_hbm, wo_v.at[:, pl.ds(0, D)], sems.at[11])],
        [w_copy(QE, D - QE, 0, QC, 12), pltpu.make_async_copy(wg_hbm, wg_v, sems.at[13]),
         pltpu.make_async_copy(wu_hbm, wu_v, sems.at[14]),
         pltpu.make_async_copy(wd_hbm, wd_v.at[:, pl.ds(0, D)], sems.at[15])],
    ]
    for group in sets:
        for c in group:
            c.start()

    def raw(r0, t, c0, n, wcol):
        return _dot(x_v[r0:r0 + t, c0:c0 + n], wqkv_v[c0:c0 + n, wcol:wcol + D])

    def colsum(r0, n, wcol, dep, hi, pieces):
        cuts = [n // 16 * k // pieces * 16 for k in range(pieces + 1)]
        pz = pltpu.bitcast(_pace(dep, pieces, 0.02, hi), I32)
        tot = None
        for k in range(pieces):
            m = cuts[k + 1] - cuts[k]
            rows = pl.ds(pl.multiple_of(r0 + cuts[k] + pz[k * 8:(k + 1) * 8][0, 0], 16), m)
            w = jnp.sum(wqkv_v[rows, wcol:wcol + D].astype(F32).reshape(m // 8, 8, D), axis=0)
            tot = w if tot is None else tot + w
        return tot

    def moments(r0, t, c0, n, shift, dep, hi):
        xf = x_v[r0:r0 + t, c0:c0 + n].astype(F32)
        if shift is None:
            shift = jnp.broadcast_to(xf[:, 0:1], (t, 128))
        d = xf - _lanes(_tie(shift, _pace(dep, t // 8, 0.0, hi)), n // 128)
        e = d * wc[:, c0:c0 + n]
        add = lambda v: functools.reduce(jnp.add, [v[:, c:c + 128] for c in range(0, n, 128)])
        return shift, (add(d), add(d * d), add(e))

    sets[0][0].wait()
    sets[0][1].wait()
    cs = jnp.sum(wqkv_v[0:128, KC:KC + D].astype(F32).reshape(16, 8, D), axis=0)
    wr = wr_v[...].astype(F32).reshape(1, D)
    wr_sum = _rowsum(wr)
    wc = wr - _lanes(wr_sum * (1.0 / D), G)
    sets[0][2].wait()
    acc_a = raw(0, HS, 0, 128, KC)
    shift_a, mom_a = moments(0, HS, 0, 128, None, acc_a, 0.9)
    for c in sets[1]:
        c.wait()
    acc_b = raw(HS, HS, 0, 128, KC)
    shift_b, mom_b = moments(HS, HS, 0, 128, None, acc_b, 0.9)
    accq0 = raw(0, S, 0, 128, QC)
    csq = colsum(0, 128, QC, accq0, 0.6, 8)
    acc = jnp.concatenate([acc_a, acc_b], axis=0)
    shift = jnp.concatenate([shift_a, shift_b], axis=0)
    mom = [jnp.concatenate(p, axis=0) for p in zip(mom_a, mom_b)]
    for j, (c0, n) in enumerate(((128, K2 - 128), (K2, D - K2))):
        for c in sets[2 + j]:
            c.wait()
        if j == 0:
            partq = raw(0, S, 128, QE - 128, QC)
            accq0 = accq0 + partq
            csq = jnp.sum(csq + colsum(128, QE - 128, QC, partq, 0.6, 8), axis=0, keepdims=True)
        part = raw(0, S, c0, n, KC)
        acc = acc + part
        if j == 0:
            part = jnp.concatenate([partq[:, 0:256], part], axis=1)
        _, new = moments(0, S, c0, n, shift, part, (0.9, 0.4)[j])
        mom = [a + b for a, b in zip(mom, new)]
        cs = cs + colsum(c0, n, KC, part, (0.6, 0.3)[j], (18, 32)[j])
    s1, s2, xw = mom
    m1 = _rowsum(s1) * (1.0 / D)
    rs1 = _rstd(jnp.maximum(_rowsum(s2) * (1.0 / D) - m1 * m1, 0.0))
    mu1 = _rb(shift + m1)
    mu_v[...] = mu1
    zx = _pace(part, S // 8, 0.3, 0.95)
    mux = _tie(mu1, jnp.concatenate([zx[0:S // 4], zx[S // 4:S // 4 + 8] | _fold(cs), zx[S // 4 + 8:]], axis=0))
    cs = jnp.sum(cs, axis=0, keepdims=True)
    xu = _pk(((x_v[:, 0:D].astype(F32) - _lanes(mux, G)) * _lanes(rs1, G)).astype(BF16))
    xn = _unpk(xu)

    z_acc, g_acc, nxt = {}, {}, {}

    def k_block(c, zero):
        k = GB // 128
        pk = _feat((acc[:, c:c + GB] - _lanes(_tie(mu1, zero), k) * cs[:, c:c + GB]) * _lanes(rs1, k))
        zs = jnp.sum(pk.astype(F32).reshape(S // 8, 8, GB), axis=0)
        for b in range(0, GB, 128):
            z_acc[(c + b) // 128] = zs[:, b:b + 128]
        return _pk(pk.T), zs

    nxt[0] = k_block(0, _pace(part, S // 8, 0.6, 0.92))
    for c in range(0, D, GB):
        def gate_g(p, deps, c=c):
            if p != 28:
                return None
            if c + GB == D:
                mu = _tie(mu1, _pace(deps, S // 8, 0.0, 0.85))
                nxt["head"] = (accq0 - _lanes(mu, G) * csq) * _lanes(rs1, G)
                return _fold(nxt["head"][:, D - 128:D])
            nxt[c + GB] = k_block(c + GB, _pace(deps, S // 8, 0.0, 0.85))
            return _blocks_done([nxt[c + GB][0]]) | _fold(nxt[c + GB][1])

        outs, _ = _passes(nxt[c][0], lambda a, b, n: xn[a:b, n * 128:(n + 1) * 128], gate_g)
        upd = jnp.concatenate(outs, axis=1)
        for b in range(0, GB, 128):
            g_acc[(c + b) // 128] = upd[b:b + 128]

    same = (lax.broadcasted_iota(I32, (128, 128), 0) // DH) == (lax.broadcasted_iota(I32, (128, 128), 1) // DH)
    kvs = []
    for g in range(G):
        kv = _dot(g_acc[g].astype(BF16), wqkv_v[:, VC + g * 128:VC + (g + 1) * 128])
        kvs.append(jnp.where(same, kv, 0.0).astype(BF16))
    m_rows = [_pk(_dot(kvs[g], wo_v[g * 128:(g + 1) * 128, 0:D]).astype(BF16)) for g in range(G)]

    once = pltpu.bitcast(_zero_of(cs[:, 0:128] + jnp.zeros((8, 128), F32)), I32)[0, 0] + 1
    for c in sets[4]:
        c.wait()

    lane = lax.broadcasted_iota(I32, (8, 128), 1)
    sub = lax.broadcasted_iota(I32, (8, 128), 0)
    pqt, os, est, st8 = [], [], [None, None], {}

    def o_tile(r0, zero):
        pq = _unpk(jnp.concatenate(pqt, axis=1)[:, r0:r0 + TA]).astype(F32)
        z4 = st8["zc"].reshape(H, DH // 8, 8, 128)
        z0 = _tie(z4[:, 0].reshape(H * 8, 128), zero).reshape(H, 1, 8, 128)
        zz = jnp.concatenate([z0, z4[:, 1:]], axis=1).reshape(D, 128)
        w = (pq * _lanes(zz, TA // 128)).reshape(H, DH // 8, 8, TA)
        den = jnp.sum(jnp.sum(w, axis=1), axis=1, keepdims=True) + 1e-6
        o = pq.reshape(H, DH, TA) * _recip(den)
        ou = _pk(o.reshape(D, TA).astype(BF16).T)
        o_v[r0 // 2:(r0 + TA) // 2, :] = ou
        return ou

    def follow_o(i, deps, lo, hi):
        n = TQ // TA
        pz = _pace(deps, n * H, lo, hi)
        os.extend(o_tile((n * i + j) * TA, pz[j * H * 8:(j + 1) * H * 8]) for j in range(n))
        return _blocks_done(os[n * i:])

    def follow_est(i, deps, lo, hi):
        pz = _pace(deps, TQ // 8, lo, hi)
        for j in range(TQ // TA * i, TQ // TA * (i + 1)):
            o = _unpk(os[j]).astype(F32).reshape(TA // 8, 8, D) * st8["mw"]
            e = _tie(xw[j * TA:(j + 1) * TA], pz[j * TA - i * TQ:(j + 1) * TA - i * TQ])
            for c in range(0, D, 128):
                e = e + o[:, :, c:c + 128].reshape(TA, 128)
            e = _rowsum(e)
            half, p0 = divmod(j * TA // 8, 128)
            for p in range(TA // 8):
                v = e[p * 8:(p + 1) * 8]
                est[half] = v if est[half] is None else jnp.where(lane == p0 + p, v, est[half])
        return _zero_of(est[(i * TQ) // 1024])

    def m_tile(a, b, c):
        return _unpk(jnp.concatenate(m_rows[a // 128:b // 128], axis=0)[:, c * 128:(c + 1) * 128])

    def write_out(i, mur, rs):
        r0, t = OFFS[i], TILES[i]
        out_v[r0:r0 + t, :] = (h_v[r0:r0 + t, :] * _lanes(1.0 + rs, G) - _lanes(mur * rs, G)).astype(BF16)
        back = out_v[r0:r0 + t, D - 128:D].astype(F32)
        out_copy(i).start()
        return back

    def stats(i, mu, dep, hi):
        r0, t = OFFS[i], TILES[i]
        mu = _tie(mu, _pace(dep, t // 8, 0.0, hi))
        d = h_v[r0:r0 + t, :] - _lanes(mu, G)
        rs = _rstd(_rowsum(d * d) * (1.0 / D))
        mur = _rb(mu)
        r = _rb((_rowsum(d * wr) + (mu - mur) * wr_sum) * rs)
        mu_v[r0:r0 + t, :] = mur
        rs_v[r0:r0 + t, :] = rs
        return r, mur, rs

    def compact(i, r):
        t = TILES[i]
        acc = r[0:8]
        for p in range(1, t // 8):
            acc = jnp.where(lane == p, r[p * 8:(p + 1) * 8], acc)
        return jnp.where(lane < t // 8, _keys(acc, OFFS[i] + lane * 8 + sub), 0.0)

    def tree(i, r):
        key = _keys(r, lax.broadcasted_iota(I32, (TILES[i], 128), 0) + OFFS[i])
        level = [(key[p * 8:(p + 1) * 8], None) for p in range(TILES[i] // 8)]
        while len(level) > 1:
            up = []
            for (a1, a2), (b1, b2) in zip(level[0::2], level[1::2]):
                lo = jnp.minimum(a1, b1)
                for e in (a2, b2):
                    lo = lo if e is None else jnp.maximum(lo, e)
                up.append((jnp.maximum(a1, b1), lo))
            level = up + level[len(up) * 2:]
        return level[0]

    groups = _ffn_groups()
    ffn = {"next": 0, "xs": None, "act": {}, "y": {}, "w": {}, "ready": {}}

    def ffn_group():
        grp = groups[ffn["next"]]
        ffn["next"] += 1
        if grp[0] == "up":
            _, c, m, hh = grp
            w_v = (wg_v, wu_v)[m]
            part = _dot(ffn["xs"][:, hh * 512:(hh + 1) * 512], w_v[hh * 512:(hh + 1) * 512, c * 128:(c + 1) * 128])
            ffn[m] = part if hh == 0 else ffn[m] + part
            if m == 1 and hh == 1:
                ffn["act"][c] = _act(ffn[0], ffn[1])
        else:
            _, q, c = grp
            a = jnp.concatenate([ffn["act"][4 * q + k] for k in range(4)], axis=1)
            if ffn["next"] == len(groups) - FKEEP + 4:
                a = _unpk(_gate(_pk(a), ffn["gate"]))
            w = ffn["w"].get((q, c))
            part = _dot(a, wd_v[q * 512:(q + 1) * 512, c * 128:(c + 1) * 128] if w is None else _unpk(w))
            ffn["y"][c] = part if q == 0 else ffn["y"][c] + part

    def ffn_step(i, p):
        if ffn["xs"] is None or (i, p) < (CT + 1, 9) or ffn["next"] >= len(groups) - FKEEP:
            return
        grp = groups[ffn["next"]]
        if grp[0] == "up" or ffn["ready"].get(4 * grp[1] + 3, i if 4 * grp[1] + 3 not in ffn["act"] else -1) < i:
            ffn_group()

    vp = {"step": 0, "acc": {}}

    def vpu_steps(i, deps, count):
        pz = _pace(deps, count, 0.0, 0.92)
        for k in range(count):
            j, d = divmod(vp["step"], D // 8)
            if FM + j * 256 == F:
                break
            vp["step"] += 1
            both = xb_v[d * 8:(d + 1) * 8, :] | pz[k * 8:(k + 1) * 8]
            xt = [_lanes(pltpu.bitcast(v, F32), 2) for v in (both << 16, both & U32(0xFFFF0000))]
            c0 = FM + j * 256
            for m, w_v in enumerate((wg_v, wu_v)):
                w = w_v[d * 8:(d + 1) * 8, c0:c0 + 256].astype(F32)
                for t in range(2):
                    vp["acc"][m, t] = w * xt[t] if d == 0 else vp["acc"][m, t] + w * xt[t]
            if d == D // 8 - 1:
                gt, ut = [jnp.where(_lanes(vp["first"], 2), jnp.sum(vp["acc"][m, 0], axis=0, keepdims=True),
                                    jnp.sum(vp["acc"][m, 1], axis=0, keepdims=True)) for m in range(2)]
                a = _act(gt, ut)
                for b in range(2):
                    ffn["act"][c0 // 128 + b] = a[:, b * 128:(b + 1) * 128]
                    ffn["ready"][c0 // 128 + b] = i + 1
        return _fold(jnp.concatenate(list(vp["acc"].values()), axis=1))

    def preload(deps):
        keep = groups[len(groups) - FKEEP:]
        pz = _pace(deps, 4 * len(keep), 0.0, 0.8)
        for k, (_, q, c) in enumerate(keep):
            w = _pk(wd_v[q * 512:(q + 1) * 512, c * 128:(c + 1) * 128])
            zero = jnp.concatenate(
                [pz[(4 * k + j) * 8:(4 * k + j + 1) * 8] for j in range(4) for _ in range(8)], axis=0)
            ffn["w"][q, c] = w | zero
        return _fold(jnp.concatenate(list(ffn["w"].values()), axis=1))

    def candidates(deps):
        ka, kb = [_keys(_rb(e), h * 1024 + lane * 8 + sub) for h, e in enumerate(est)]
        t1, t2 = jnp.maximum(ka, kb), jnp.minimum(ka, kb)
        c1 = jnp.max(t1, axis=1, keepdims=True)
        c2 = jnp.max(jnp.where(t1 == c1, t2, t1), axis=1, keepdims=True)
        ck = pltpu.bitcast(jnp.broadcast_to(jnp.concatenate([c1, c2], axis=0), (16, 128)), I32)
        idx = S - 1 - (ck & (S - 1))
        pz = pltpu.bitcast(_pace(deps, 16, 0.25, 0.75), I32)
        for k in range(16):
            i = (idx[k // 8 * 8:k // 8 * 8 + 8] | pz[k * 8:(k + 1) * 8])[k % 8, 0]
            w = o_v[pl.ds(lax.shift_right_logical(i, 1), 1), :]
            w = jnp.where((i & 1) == 0, w << 16, w & U32(0xFFFF0000))
            co_v[k:k + 1, :] = pltpu.bitcast(w, F32)
            xg = x_v[pl.ds(pl.multiple_of(i - k % 8, 8), 8), 0:D].astype(F32)
            cx_v[k:k + 1, :] = xg[k % 8:k % 8 + 1]
        return idx, _pk(co_v[...].astype(BF16))

    def normalize(h):
        mu = _rowsum(h) * (1.0 / D)
        d = h - _lanes(mu, G)
        rs = _rstd(_rowsum(d * d) * (1.0 / D))
        mur = _rb(mu)
        r = _rb((_rowsum(d * wr) + (mu - mur) * wr_sum) * rs)
        return ((h - _lanes(mur, G)) * _lanes(rs, G)).astype(BF16), _rb(jax.nn.sigmoid(r)), r

    def routed(h, xs, gain, y):
        return h + _rb(xs.astype(F32) + _rb(_rb(y) * _lanes(gain, G)))

    def project(i, gate, extra):
        r0, t = OFFS[i], TILES[i]

        def post(c, attn):
            h_v[r0:r0 + t, c * 128:(c + 1) * 128] = x_v[r0:r0 + t, c * 128:(c + 1) * 128].astype(F32) + attn[0:t]
            return None if extra is None else attn[t:]

        ou = o_rows(r0, t)
        if extra is not None:
            ou = jnp.concatenate([ou, extra], axis=0)
        gate_fn = gate if callable(gate) else lambda p, deps: gate.get(p)
        outs, deps = _passes(ou, m_tile, gate_fn, post, lambda p: ffn_step(i, p))
        return [d[0:t] for d in deps], outs

    def mean_h(i):
        return _rowsum(h_v[OFFS[i]:OFFS[i] + TILES[i], :]) * (1.0 / D)

    def o_rows(r0, t):
        if os:
            return jnp.concatenate(os, axis=0)[r0 // 2:(r0 + t) // 2, :]
        return o_v[r0 // 2:(r0 + t) // 2, :]

    def finish_tile(i, mu, deps, hi, top):
        r, mur, rs = stats(i, mu, deps, hi)
        back = write_out(i, mur, rs)
        key = compact(i, r)
        return _merge(top, key, jnp.zeros_like(key)), _zero_of(key + jnp.sum(back.reshape(-1, 8, 128), axis=0))

    kept = {}

    def keep(name, x):
        u = pltpu.bitcast(x, U32) if x.dtype != U32 else x
        parts = [u[r:r + 8, c:c + 128] for r in range(0, u.shape[0], 8) for c in range(0, u.shape[1], 128)]
        at = sum(n for _, n, _, _ in kept.values())
        kept[name] = (at, len(parts), u.shape, x.dtype)
        keep_v[at * 8:(at + len(parts)) * 8, :] = jnp.concatenate(parts, axis=0)

    def fetch(name):
        at, n, shape, dtype = kept[name]
        v = keep_v[at * 8:(at + n) * 8, :]
        k = shape[1] // 128
        u = jnp.concatenate([jnp.concatenate([v[(r * k + c) * 8:(r * k + c + 1) * 8] for c in range(k)], axis=1)
                             for r in range(shape[0] // 8)], axis=0)
        return pltpu.bitcast(u, dtype) if dtype != U32 else u

    def project_last(gate, mu_prev, top):
        i = NT - 1
        r0, t = OFFS[i], TILES[i]
        st = {}

        def post(c, attn):
            h = x_v[r0:r0 + t, c * 128:(c + 1) * 128].astype(F32) + attn
            h_v[r0:r0 + t, c * 128:(c + 1) * 128] = h
            if c == 0:
                st["shift"] = jnp.broadcast_to(h[:, 0:1], (t, 128))
            d = h - st["shift"]
            new = (d, d * d, d * wr[:, c * 128:(c + 1) * 128])
            st[c] = new if c == 0 else tuple(a + b for a, b in zip(st[c - 1], new))

        def gate_fn(p, deps):
            if p == 0:
                return gate
            if p == 14:
                r, mur, rs = stats(i - 1, mu_prev, deps, 0.15)
                st["top"] = _merge(top, *tree(i - 1, r))
                ffn["gate"] = _fold(write_out(i - 1, mur, rs))
                return _zero_of(st["top"][0] + st["top"][1])
            return _fold(jnp.concatenate(st[0], axis=1)) if p == 15 else None

        _passes(o_rows(r0, t), m_tile, gate_fn, post, lambda p: ffn_step(i, p))
        while ffn["next"] < len(groups):
            ffn_group()
        s1, s2, s3 = st[G - 1]
        m1 = _rowsum(s1) * (1.0 / D)
        rs = _rstd(jnp.maximum(_rowsum(s2) * (1.0 / D) - m1 * m1, 0.0))
        mur = _rb(st["shift"] + m1)
        r = _rb((_rowsum(s3) + (st["shift"] - mur) * wr_sum) * rs)
        mu_v[r0:r0 + t, :] = mur
        rs_v[r0:r0 + t, :] = rs
        return _merge(st["top"], *tree(i, r)), mur, rs

    def middle(_, carry):
        del pqt[:], os[:]
        est[:] = [None, None]
        kept.clear()
        vp.update({"step": 0, "acc": {}})
        ffn.update({"next": 0, "xs": None, "act": {}, "y": {}, "w": {}, "ready": {}})
        z = _rb(jnp.sum(jnp.concatenate([z_acc[b] for b in range(G)], axis=1), axis=0, keepdims=True))
        st8["zc"] = jnp.concatenate(
            [jnp.broadcast_to(z[:, g * 128:(g + 1) * 128], (128, 128)).T for g in range(G)], axis=0)
        gate = None
        for i in range(S // TQ):
            accq = _dot(_unpk(_gate(xu[i * TQ // 2:(i + 1) * TQ // 2, QE:], gate)), wqkv_v[QE:, QC:QC + D])
            head = nxt["head"][i * TQ:(i + 1) * TQ]
            if i == 0:
                e = _unpk(jnp.concatenate(m_rows, axis=0)).astype(F32) * wc
                e = jnp.concatenate([_tie(e[:, 0:128], _pace(accq, D // 8, 0.0, 0.7)), e[:, 128:]], axis=1)
                e = _rowsum(e)
                st8["mw"] = jnp.concatenate([e[g * 128:(g + 1) * 128].T[0:8] for g in range(G)], axis=1)
                gate = _fold(st8["mw"])
            else:
                follow_o(i - 1, accq, 0.05, 0.6)
                gate = follow_est(i - 1, accq, 0.45, 0.9)
            pqt.append(_pk(_feat(accq + head).T))

        top = mu_prev = extra = None
        gate = {0: gate, 6: _blocks_done([pqt[-1]])}
        for i in range(LT):
            if i == LT - 1:
                def inner(p, deps, gate=gate, mu_prev=mu_prev, top=top):
                    if p != 15:
                        return gate.get(p)
                    st8["top"], zero = finish_tile(i - 1, mu_prev, deps, 0.55, top)
                    return zero | vpu_steps(i, deps, 44)

                project(i, inner, None)
                break
            deps, outs = project(i, gate, extra if i == CT else None)
            mu = mean_h(i)
            gate = {}
            if i == 0:
                gate[5] = follow_o(S // TQ - 1, deps, 0.35, 1.0)
            else:
                top, gate[0] = finish_tile(i - 1, mu_prev, deps, min(0.8, 1 - 560 / (16 * TILES[i])), top)
            if i == CT + 1:
                gate[0] = gate[0] | _fold(_pk(ffn["xs"]))
                pz = _pace(deps, G, 0.35, 0.7)
                for g in range(G):
                    row = pltpu.bitcast(st8["pair"][:, g * 128:(g + 1) * 128] | pz[g * 8:(g + 1) * 8], F32)
                    blk = _pk(jnp.concatenate([row] * 16, axis=0).T)
                    xb_v[g * 128:(g + 1) * 128, :] = blk
                    gate[0] = gate[0] | _zero_of(blk[120:128])
            if i == 1:
                gate[0] = gate[0] | follow_est(S // TQ - 1, deps, 0.25, 0.85)
            if i == CT - 1:
                cand, extra = candidates(deps)
                keep("cand", cand)
                gate[0] = gate[0] | _fold(extra) | _fold(cx_v[...])
            if i == CT:
                h16 = cx_v[...] + jnp.concatenate(outs, axis=1)
                ffn["xs"], gain16, r16 = normalize(h16)
                ck = _keys(r16, cand)
                first = ck == jnp.max(ck, axis=0, keepdims=True)
                second = ck == jnp.max(jnp.where(first, 0.0, ck), axis=0, keepdims=True)
                xf = ffn["xs"].astype(F32)
                lo, hi = [_pk(jnp.broadcast_to(jnp.sum(jnp.where(_lanes(m, G), xf, 0.0), axis=0, keepdims=True), (8, D)))
                          for m in (first, second)]
                st8["pair"] = lax.shift_right_logical(lo, U32(16)) | hi
                keep("rank", jnp.where(first, 1, jnp.where(second, 2, 0)))
                keep("h16", h16)
                keep("gain16", gain16)
                keep("xs", ffn["xs"])
            mu_prev = mu
        keep("top", jnp.concatenate(st8["top"], axis=1))
        for c, a in ffn["act"].items():
            keep(("act", c), a)
        for c, y in ffn["y"].items():
            keep(("y", c), y)
        for m in range(2):
            keep(("part", m), ffn[m])
        for k, a in vp["acc"].items():
            keep(("vp", k), a)
        return carry

    lax.fori_loop(0, once, middle, 0)
    del os[:]
    cand, h16, gain16, top = fetch("cand"), fetch("h16"), fetch("gain16"), fetch("top")
    top = (top[:, 0:128], top[:, 128:])
    ffn["xs"] = fetch("xs")
    ffn["act"] = {c: fetch(("act", c)) for c in ffn["act"]}
    ffn["y"] = {c: fetch(("y", c)) for c in ffn["y"]}
    ffn[0], ffn[1] = fetch(("part", 0)), fetch(("part", 1))
    rank = fetch("rank")
    vp["first"] = rank == 1
    vp["acc"] = {k: fetch(("vp", k)) for k in vp["acc"]}

    gate = {}
    mu_prev = mean_h(LT - 1)
    for i in range(LT, NT - 1):
        deps, _ = project(i, gate, None)
        mu = mean_h(i)
        top, zero = finish_tile(i - 1, mu_prev, deps, min(0.8, 1 - 560 / (16 * TILES[i])), top)
        gate = {0: zero}
        if vp["step"] < (F - FM) // 2:
            gate[0] = gate[0] | vpu_steps(i, deps, 52)
        if i == NT - 2:
            t1, t2 = top
            b1 = jnp.max(jnp.max(t1, axis=0, keepdims=True), axis=1, keepdims=True)
            rest = jnp.where(t1 == b1, t2, t1)
            b2 = jnp.max(jnp.max(rest, axis=0, keepdims=True), axis=1, keepdims=True)
            top = (jnp.where(sub == 0, b1, 0.0), jnp.where(sub == 0, b2, 0.0))
        if i == NT - 4:
            gate[0] = gate[0] | preload(deps)
        mu_prev = mu
    (t1, t2), mur_l, rs_l = project_last(gate[0], mu_prev, top)

    k1 = jnp.max(t1, axis=0, keepdims=True)
    k2 = jnp.max(jnp.where(t1 == k1, t2, t1), axis=0, keepdims=True)
    v1 = S - 1 - (pltpu.bitcast(k1, I32) & (S - 1))
    v2 = S - 1 - (pltpu.bitcast(k2, I32) & (S - 1))
    i1, i2 = v1[0, 0], v2[0, 0]
    g1 = pl.multiple_of(i1 & -8, 8)
    g2 = pl.multiple_of(i2 & -8, 8)
    write_out(NT - 1, mur_l, rs_l)
    out_v[S:S + 16, 0:128] = jnp.zeros((16, 128), BF16)
    chosen = jnp.logical_or(cand == v1, cand == v2)
    found = jnp.sum(jnp.logical_and(chosen, rank > 0).astype(I32), axis=0, keepdims=True)[0, 0]

    def plain(g):
        rows = pl.ds(g, 8)
        rs = _tie(rs_v[rows, :], _zero_of(out_v[S:S + 8, 0:128].astype(F32)))
        return h_v[rows, :] * _lanes(1.0 + rs, G) - _lanes(mu_v[rows, :] * rs, G)

    new16 = routed(h16, ffn["xs"], gain16, jnp.concatenate([ffn["y"][c] for c in range(G)], axis=1))
    for j, (g, v) in enumerate(((g1, v1), (g2, v2))):
        here = jnp.logical_and(chosen, (cand & -8) == (v & -8))
        val = plain(g)
        for half in range(2):
            val = jnp.where(_lanes(here[half * 8:(half + 1) * 8], G), new16[half * 8:(half + 1) * 8], val)
        fix_v[j] = val.astype(BF16)

    @pl.when(found != (3 if force_fallback else 2))
    def _():
        h = jnp.concatenate([h_v[pl.ds(g1, 8), :], h_v[pl.ds(g2, 8), :]], axis=0)
        xs, gain, _ = normalize(h)

        def chunk(c, y):
            cols = pl.ds(pl.multiple_of(c * MC, 128), MC)
            return y + _dot(_act(_dot(xs, wg_v[:, cols]), _dot(xs, wu_v[:, cols])), wd_v[cols, 0:D])

        new = routed(h, xs, gain, lax.fori_loop(0, F // MC, chunk, jnp.zeros((16, D), F32)))
        rows = lax.broadcasted_iota(I32, (8, D), 0)
        for j, g in enumerate((g1, g2)):
            hit = jnp.logical_or(rows + g == i1, rows + g == i2)
            fix_v[j] = jnp.where(hit, new[j * 8:(j + 1) * 8], plain(g)).astype(BF16)

    nb = OFFS[-1]
    pltpu.make_async_copy(out_v.at[pl.ds(0, nb)], out_hbm.at[pl.ds(0, nb)], sems.at[SEM_OUT]).wait()
    late = jnp.maximum(i1, i2) >= nb

    @pl.when(late)
    def _():
        out_copy(NT - 1).wait()

    c1 = pltpu.make_async_copy(fix_v.at[0], out_hbm.at[pl.ds(g1, 8)], sems.at[SEM_FIX])
    c2 = pltpu.make_async_copy(fix_v.at[1], out_hbm.at[pl.ds(g2, 8)], sems.at[SEM_FIX + 1])
    c1.start()

    @pl.when(g1 != g2)
    def _():
        c2.start()

    @pl.when(jnp.logical_not(late))
    def _():
        out_copy(NT - 1).wait()

    @pl.when(g1 != g2)
    def _():
        c2.wait()

    c1.wait()


_SCRATCH = [
    pltpu.VMEM((S, D + PAD), BF16),
    pltpu.VMEM((D, 3 * D + PAD), BF16),
    pltpu.VMEM((D, D + PAD), BF16),
    pltpu.VMEM((D, F), BF16),
    pltpu.VMEM((D, F), BF16),
    pltpu.VMEM((F, D + PAD), BF16),
    pltpu.VMEM((D,), BF16),
    pltpu.VMEM((S, 128), F32),
    pltpu.VMEM((S, 128), F32),
    pltpu.VMEM((S + 16, D), BF16),
    pltpu.VMEM((S, D), F32),
    pltpu.VMEM((2, 8, D), BF16),
    pltpu.VMEM((S // 2, D), U32),
    pltpu.VMEM((16, D), F32),
    pltpu.VMEM((16, D), F32),
    pltpu.VMEM((128 * 8, 128), U32),
    pltpu.VMEM((D, 128), U32),
    pltpu.SemaphoreType.DMA((NSEM,)),
]


def _run(kernel, A_x, A_wqkv, A_wo, B_w_r, B_w_gate, B_w_up, B_w_down):
    any_spec = pl.BlockSpec(memory_space=pl.ANY)
    out = pl.pallas_call(
        kernel,
        out_shape=jax.ShapeDtypeStruct((S, D), BF16),
        in_specs=[any_spec] * 7,
        out_specs=any_spec,
        scratch_shapes=_SCRATCH,
        compiler_params=pltpu.CompilerParams(vmem_limit_bytes=100 * 1024 * 1024, disable_bounds_checks=True,
                                             disable_semaphore_checks=True),
    )(A_x.reshape(S, D), A_wqkv, A_wo, B_w_r, B_w_gate, B_w_up, B_w_down)
    return out.reshape(1, S, D)


@jax.jit
def pallas_sequential_preLN__linear_attn_block__moe_arch_mod__prompt_kernel(
    A_x: jax.Array,
    A_wqkv: jax.Array,
    A_wo: jax.Array,
    B_x: jax.Array,
    B_w_r: jax.Array,
    B_w_gate: jax.Array,
    B_w_up: jax.Array,
    B_w_down: jax.Array,
):
    return _run(_kernel, A_x, A_wqkv, A_wo, B_w_r, B_w_gate, B_w_up, B_w_down)
```
